```python
import jax
import jax.numpy as jnp

def _softmax(x, axis=-1):
    return jax.nn.softmax(x, axis=axis)
def _gelu(x):
    return jax.nn.gelu(x, approximate=True)
def _silu(x):
    return jax.nn.silu(x)
def _sigmoid(x):
    return jax.nn.sigmoid(x)
def _layernorm(x, axis=-1, eps=1e-5):
    m = jnp.mean(x, axis=axis, keepdims=True)
    v = jnp.var(x, axis=axis, keepdims=True)
    return (x - m) / jnp.sqrt(v + eps)
def _scatter_add(tgt, idx, src, axis=0):
    return tgt.at[idx].add(src)
def _segment_sum(src, seg, n):
    return jax.ops.segment_sum(src, seg, n)
class _Rng:
    def __init__(self, key):
        self._k = key
    def _next(self):
        self._k, sub = jax.random.split(self._k)
        return sub
    def normal(self, shape):
        return jax.random.normal(self._next(), shape, dtype=jnp.bfloat16)
    def randint(self, lo, hi, shape):
        return jax.random.randint(self._next(), shape, lo, hi, dtype=jnp.int32)
    def uniform(self, shape, lo=0.0, hi=1.0):
        return jax.random.uniform(self._next(), shape, jnp.bfloat16, lo, hi)
    def permutation(self, n):
        return jax.random.permutation(self._next(), n)


kernel_name = 'standalone__seq2seq_rnn_t_joint__speech'

def setup_inputs():
    _rng = _Rng(jax.random.key(int.from_bytes(__import__("os").urandom(4), "little")))
    _w = (lambda a: (lambda t: t.astype(jnp.bfloat16) if jnp.issubdtype(t.dtype, jnp.floating) else t)(jnp.asarray(a)))
    B, T, D, K = 2, 16000, 256, 31
    U = 8
    sc = (1.0 / (K * D)) ** 0.5
    sd = (1.0 / D) ** 0.5
    return {
        "x": _w((lambda *s: _rng.normal(s) * 0.05)(B, T, D) * 0.5),
        "w1": _w((lambda *s: _rng.normal(s) * 0.05)(K, D, D) * sc),
        "w2": _w((lambda *s: _rng.normal(s) * 0.05)(K, D, D) * sc),
        "g": _w((lambda *s: _rng.normal(s) * 0.05)(B, U, D) * 0.5),
        "w_f": _w((lambda *s: _rng.normal(s) * 0.05)(D, D) * sd),
        "w_g": _w((lambda *s: _rng.normal(s) * 0.05)(D, D) * sd),
        "w_o": _w((lambda *s: _rng.normal(s) * 0.05)(D, D) * sd),
    }

def reference(x, w1, w2, g, w_f, w_g, w_o):
    B, T, D = x.shape
    K = w1.shape[0]
    pad = K // 2
    xp = jnp.pad(x, ((0,0),(pad,pad),(0,0)))
    h = jnp.zeros_like(x)
    for i in range(K):
        h = h + jnp.einsum("btc,cd->btd", xp[:, i:i+T, :], w1[i])
    h = _gelu(h)[:, ::2, :]
    T1 = h.shape[1]
    hp = jnp.pad(h, ((0,0),(pad,pad),(0,0)))
    f = jnp.zeros_like(h)
    for i in range(K):
        f = f + jnp.einsum("btc,cd->btd", hp[:, i:i+T1, :], w2[i])
    f = _gelu(f)[:, ::2, :]
    fe = jnp.einsum("btd,de->bte", f, w_f)
    ge = jnp.einsum("bud,de->bue", g, w_g)
    j = jnp.tanh(fe[:, :, None, :] + ge[:, None, :, :])
    return jnp.einsum("btud,dv->btuv", j, w_o)
```

```python
import functools
import math

import jax
import jax.numpy as jnp
import numpy as np
from jax import lax
from jax.experimental import pallas as pl
from jax.experimental.pallas import tpu as pltpu

f32, u32, bf16, i32 = jnp.float32, jnp.uint32, jnp.bfloat16, jnp.int32

N = 64
S = 48
SEG = 8


class V:
    __slots__ = ("a", "s")

    def __init__(self, a, s=1):
        self.a = a
        self.s = s

    def __neg__(self):
        return V(self.a, -self.s)

    def __add__(self, o):
        if self.s == o.s:
            return V(self.a + o.a, self.s)
        if self.s > 0:
            return V(self.a - o.a, 1)
        return V(o.a - self.a, 1)

    def __sub__(self, o):
        return self + (-o)

    def scale(self, c):
        if c == 1.0:
            return self
        if c == -1.0:
            return -self
        return V(self.a * np.float32(abs(c)), self.s * (1 if c > 0 else -1))

    def signed(self, s):
        return self.a if self.s * s > 0 else -self.a


class C:
    __slots__ = ("r", "i")

    def __init__(self, r, i):
        self.r = r
        self.i = i

    def __add__(self, o):
        return C(self.r + o.r, self.i + o.i)

    def __sub__(self, o):
        return C(self.r - o.r, self.i - o.i)

    def __neg__(self):
        return C(-self.r, -self.i)

    def mul_w(self, num, den):
        num %= den
        if num == 0:
            return self
        if 4 * num == den:
            return C(-self.i, self.r)
        if 2 * num == den:
            return -self
        if 4 * num == 3 * den:
            return C(self.i, -self.r)
        if (8 * num) % den == 0:
            o = (8 * num) // den
            h = math.sqrt(0.5)
            sc = 1 if o in (1, 7) else -1
            ss = 1 if o in (1, 3) else -1
            r, m = self.r, self.i
            re = (r if sc > 0 else -r) - (m if ss > 0 else -m)
            im = (r if ss > 0 else -r) + (m if sc > 0 else -m)
            return C(re.scale(h), im.scale(h))
        c = math.cos(2 * math.pi * num / den)
        s = math.sin(2 * math.pi * num / den)
        return C(self.r.scale(c) - self.i.scale(s), self.r.scale(s) + self.i.scale(c))


def _add(a, b):
    if a is None:
        return b
    if b is None:
        return a
    return a + b


def _sub(a, b):
    if b is None:
        return a
    if a is None:
        return -b
    return a - b


def fft8(x, sgn, need=tuple(range(8))):
    def rot(a, num, den):
        return None if a is None else a.mul_w(sgn * num, den)

    need = set(need)
    a0, a1 = _add(x[0], x[4]), _sub(x[0], x[4])
    a2, a3 = _add(x[2], x[6]), rot(_sub(x[2], x[6]), 1, 4)
    a4, a5 = _add(x[1], x[5]), _sub(x[1], x[5])
    a6, a7 = _add(x[3], x[7]), rot(_sub(x[3], x[7]), 1, 4)
    out = {}
    if need & {0, 4}:
        b0, b4 = _add(a0, a2), _add(a4, a6)
        if 0 in need:
            out[0] = _add(b0, b4)
        if 4 in need:
            out[4] = _sub(b0, b4)
    if need & {2, 6}:
        b2, b6 = _sub(a0, a2), rot(_sub(a4, a6), 1, 4)
        if 2 in need:
            out[2] = _add(b2, b6)
        if 6 in need:
            out[6] = _sub(b2, b6)
    if need & {1, 5}:
        b1, b5 = _add(a1, a3), rot(_add(a5, a7), 1, 8)
        if 1 in need:
            out[1] = _add(b1, b5)
        if 5 in need:
            out[5] = _sub(b1, b5)
    if need & {3, 7}:
        b3, b7 = _sub(a1, a3), rot(_sub(a5, a7), 3, 8)
        if 3 in need:
            out[3] = _add(b3, b7)
        if 7 in need:
            out[7] = _sub(b3, b7)
    return out


class _Sym:
    def __add__(self, o):
        return self

    __sub__ = __mul__ = __add__

    def __neg__(self):
        return self


def _fft64_signs(sgn, present=tuple(range(64)), in_sign=None):
    d = _Sym()
    in_sign = in_sign or {}
    x = [C(V(d, in_sign.get((n, 0), 1)), V(d, in_sign.get((n, 1), 1))) if n in present else None
         for n in range(64)]
    t = {}
    for n2 in range(8):
        a = fft8([x[8 * n1 + n2] for n1 in range(8)], sgn)
        for k1 in range(8):
            t[k1, n2] = a[k1].mul_w(sgn * n2 * k1, 64)
    s1 = {key: (v.r.s, v.i.s) for key, v in t.items()}
    s2 = {}
    for k1 in range(8):
        b = fft8([t[k1, n2] for n2 in range(8)], sgn)
        for k2 in range(8):
            s2[k1 + 8 * k2] = b[k2]
    return s1, s2


def _unit(k, j):
    return (k - 1) * 3 + j


UNIT0, UNIT32 = 93, 94
NUNITS = 95


def _lhs_forms(m, z):
    if m in (0, 32):
        u = UNIT0 if m == 0 else UNIT32
        return [(u, 0, z.r), (u, 1, z.i)]
    if m < 32:
        return [(_unit(m, 0), 0, z.r + z.i), (_unit(m, 1), 0, z.r), (_unit(m, 2), 0, z.i)]
    k = 64 - m
    return [(_unit(k, 0), 1, z.r - z.i), (_unit(k, 1), 1, z.r), (_unit(k, 2), 1, z.i)]


def _lhs_signs():
    _, s2 = _fft64_signs(-1)
    sg = {}
    for m in range(64):
        for u, h, v in _lhs_forms(m, s2[m]):
            sg[u, h] = v.s
    return sg


LHS_SIGN = _lhs_signs()


def _y_signs():
    return {(m, 1): -1 for m in range(33, 64)}


def _unpack(w):
    lo = pltpu.unpack_elementwise(w, index=0, packed_dtype=bf16, unpacked_dtype=f32)
    hi = pltpu.unpack_elementwise(w, index=1, packed_dtype=bf16, unpacked_dtype=f32)
    return lo, hi


def _pack(lo, hi):
    return pltpu.pack_elementwise([lo, hi], packed_dtype=bf16)


_GC1 = 2.0 * math.sqrt(2.0 / math.pi)
_GC2 = 8.0 * 0.044715 * math.sqrt(2.0 / math.pi)


def _gelu_half(v):
    a = v.a
    p = (a * a) * np.float32(_GC2) + np.float32(_GC1)
    t = jnp.tanh(p * a)
    return a * t + a if v.s > 0 else a * t - a


def _lanes(t):
    return pl.ds(128 * t, 128)


def weight_transform(w_ref, u_ref, t_ref, rg):
    rows = pl.ds(pl.multiple_of(rg * 16, 16), 16)
    urow = pl.ds(pl.multiple_of(rg * 8, 8), 8)
    urow_b = pl.ds(pl.multiple_of(rg * 8 + 128, 8), 8)
    taps = [[[None, None] for _ in range(31)] for _ in range(2)]
    for i in range(31):
        for dt in range(2):
            lo, hi = _unpack(pltpu.bitcast(w_ref[i, rows, _lanes(dt)], u32))
            taps[0][i][dt] = lo
            taps[1][i][dt] = hi
    sigma = 1.0 / 256.0
    tau = 1.0 / 128.0

    def wa(p, d, dt):
        return None if d == 0 else V(taps[p][2 * d - 1][dt])

    def wb(p, d, dt):
        return V(taps[p][2 * d][dt])

    def store(u, half, nt, v0, v1):
        s = LHS_SIGN[u, half]
        val = _pack(v0.signed(s), v1.signed(s))
        u_ref[u, urow_b if half else urow, _lanes(nt)] = val

    res = {}
    for p in range(2):
        for dt in range(2):
            for name, f in (("a", wa), ("b", wb)):
                ev = od = None
                for d in range(16):
                    if d % 2 == 0:
                        ev = _add(ev, f(p, d, dt))
                    else:
                        od = _add(od, f(p, d, dt))
                res[p, dt, name, 0] = _add(ev, od).scale(tau)
                res[p, dt, name, 32] = _sub(ev, od).scale(tau)
    for m, u in ((0, UNIT0), (32, UNIT32)):
        for dt in range(2):
            store(u, 0, dt, res[0, dt, "a", m], res[1, dt, "a", m])
            store(u, 1, dt, res[0, dt, "b", m], res[1, dt, "b", m])

    for pm in (1, -1):
        sgn1 = {}
        for p in range(2):
            z = []
            for d in range(16):
                if pm > 0:
                    re = _sub(wa(p, d, 0), wb(p, d, 1))
                    im = _add(wb(p, d, 0), wa(p, d, 1))
                else:
                    re = _add(wa(p, d, 0), wb(p, d, 1))
                    im = _sub(wb(p, d, 0), wa(p, d, 1))
                z.append(C(re.scale(sigma), im.scale(sigma)))
            for n2 in range(8):
                a = fft8([z[n2], z[8 + n2]] + [None] * 6, 1)
                for k1 in range(8):
                    t = a[k1].mul_w(n2 * k1, 64)
                    t_ref[p, (k1 * 8 + n2) * 2] = t.r.a
                    t_ref[p, (k1 * 8 + n2) * 2 + 1] = t.i.a
                    sgn1[k1, n2] = (t.r.s, t.i.s)
        for k1 in range(8):
            need = [k2 for k2 in range(8) if (k1 + 8 * k2) not in (0, 32)]
            outs = []
            for p in range(2):
                xs = [C(V(t_ref[p, (k1 * 8 + n2) * 2], sgn1[k1, n2][0]),
                        V(t_ref[p, (k1 * 8 + n2) * 2 + 1], sgn1[k1, n2][1])) for n2 in range(8)]
                outs.append(fft8(xs, 1, need))
            for k2 in need:
                m = k1 + 8 * k2
                f0, f1 = outs[0][k2], outs[1][k2]
                if m < 32:
                    nt = 0 if pm > 0 else 1
                    store(_unit(m, 0), 1, nt, f0.r, f1.r)
                    store(_unit(m, 1), 1, nt, f0.i - f0.r, f1.i - f1.r)
                    store(_unit(m, 2), 1, nt, -(f0.r + f0.i), -(f1.r + f1.i))
                else:
                    k = 64 - m
                    nt = 1 if pm > 0 else 0
                    store(_unit(k, 0), 0, nt, f0.r, f1.r)
                    store(_unit(k, 1), 0, nt, -(f0.r + f0.i), -(f1.r + f1.i))
                    store(_unit(k, 2), 0, nt, f0.r - f0.i, f1.r - f1.i)


def fwd_group(load, t_ref, x_ref, g):
    rows = pl.ds(pl.multiple_of(g * 8, 8), 8)
    for ct in range(2):
        sg = {}
        for h in range(2):
            for n2 in range(8):
                xs = []
                for n1 in range(8):
                    lo, hi = _unpack(load(h, 8 * n1 + n2, ct))
                    xs.append(C(V(lo), V(hi)))
                a = fft8(xs, -1)
                for k1 in range(8):
                    t = a[k1].mul_w(-n2 * k1, 64)
                    t_ref[h, (k1 * 8 + n2) * 2] = t.r.a
                    t_ref[h, (k1 * 8 + n2) * 2 + 1] = t.i.a
                    sg[k1, n2] = (t.r.s, t.i.s)
                yield
        for k1 in range(8):
            outs = []
            for h in range(2):
                xs = [C(V(t_ref[h, (k1 * 8 + n2) * 2], sg[k1, n2][0]),
                        V(t_ref[h, (k1 * 8 + n2) * 2 + 1], sg[k1, n2][1])) for n2 in range(8)]
                outs.append(fft8(xs, -1))
            for k2 in range(8):
                m = k1 + 8 * k2
                f0 = _lhs_forms(m, outs[0][k2])
                f1 = _lhs_forms(m, outs[1][k2])
                for (u, half, v0), (_, _, v1) in zip(f0, f1):
                    assert v0.s == v1.s == LHS_SIGN[u, half]
                    x_ref[u, rows, _lanes(2 * half + ct)] = _pack(v0.a, v1.a)
            yield


def _mm(x_ref, u_ref, j, mrows):
    a = pltpu.bitcast(x_ref[j, pl.ds(0, mrows // 2), :], bf16)
    w = pltpu.bitcast(u_ref[j], bf16)
    return jnp.dot(a, w, preferred_element_type=f32)


def pair_matmul(x_ref, u_ref, y_ref, k, mrows):
    j = (k - 1) * 3
    k1 = _mm(x_ref, u_ref, j, mrows)
    k2 = _mm(x_ref, u_ref, j + 1, mrows)
    k3 = _mm(x_ref, u_ref, j + 2, mrows)
    yr = k1 - k3
    yi = k1 + k2
    rows = pl.ds(0, mrows)
    y_ref[2 * k, rows, :] = yr[:, :128]
    y_ref[2 * k + 1, rows, :] = yi[:, :128]
    y_ref[2 * (64 - k), rows, :] = yr[:, 128:]
    y_ref[2 * (64 - k) + 1, rows, :] = yi[:, 128:]


def real_matmul(x_ref, u_ref, y_ref, m, mrows):
    y = _mm(x_ref, u_ref, UNIT0 if m == 0 else UNIT32, mrows)
    rows = pl.ds(0, mrows)
    y_ref[2 * m, rows, :] = y[:, :128]
    y_ref[2 * m + 1, rows, :] = y[:, 128:]


def inv_pass1(y_ref, t_ref, g, h):
    rows = pl.ds(pl.multiple_of(g * 16 + 8 * h, 8), 8)
    ysg = _y_signs()
    sg = {}
    for n2 in range(8):
        xs = []
        for n1 in range(8):
            m = 8 * n1 + n2
            xs.append(C(V(y_ref[2 * m, rows, :], ysg.get((m, 0), 1)),
                        V(y_ref[2 * m + 1, rows, :], ysg.get((m, 1), 1))))
        a = fft8(xs, 1)
        for k1 in range(8):
            t = a[k1].mul_w(n2 * k1, 64)
            t_ref[h, (k1 * 8 + n2) * 2] = t.r.a
            t_ref[h, (k1 * 8 + n2) * 2 + 1] = t.i.a
            sg[k1, n2] = (t.r.s, t.i.s)
        yield
    return sg


def _inv_signs():
    s1, _ = _fft64_signs(1, in_sign=_y_signs())
    return s1


INV_S1 = _inv_signs()


def inv_pass2(t_ref, h, k1):
    xs = [C(V(t_ref[h, (k1 * 8 + n2) * 2], INV_S1[k1, n2][0]),
            V(t_ref[h, (k1 * 8 + n2) * 2 + 1], INV_S1[k1, n2][1])) for n2 in range(8)]
    b = fft8(xs, 1, range(S // 8))
    return {k2: (_gelu_half(b[k2].r), _gelu_half(b[k2].i)) for k2 in range(S // 8)}


def inv_group_conv1(y_ref, t_ref, zh_ref, g, tau0):
    for h in range(2):
        for _ in inv_pass1(y_ref, t_ref, g, h):
            yield
    for h in range(2):
        for k1 in range(0, 8, 2):
            ev = inv_pass2(t_ref, h, k1)
            od = inv_pass2(t_ref, h, k1 + 1)
            for k2 in range(S // 8):
                for dt in range(2):
                    zh_ref[tau0 + (k1 // 2 + 4 * k2), h, :, _lanes(dt)] = _pack(ev[k2][dt], od[k2][dt])
            yield


def inv_group_conv2(y_ref, t_ref, f_ref, g, tau0):
    for h in range(2):
        for _ in inv_pass1(y_ref, t_ref, g, h):
            yield
    for k1 in range(8):
        oa = inv_pass2(t_ref, 0, k1)
        ob = inv_pass2(t_ref, 1, k1)
        for k2 in range(S // 8):
            for dt in range(2):
                f_ref[tau0 + (k1 + 8 * k2), :, _lanes(dt)] = _pack(oa[k2][dt], ob[k2][dt])
        yield


def _run(gen):
    for _ in gen:
        pass


def _make_kernel(T):
    T1, T2 = T // 2, T // 4
    L1 = (T1 + 16) // SEG
    L2 = L1 // 2
    assert L1 * SEG == T1 + 16 and L1 % 2 == 0
    NB1 = -(-L1 // S)
    NB2 = -(-L2 // S)
    XPAD = 8
    XB = T1 + 16
    XROWS = XPAD + 2 * XB + 64
    ZH = (NB2 - 1) * S + N
    G1 = 7
    assert NB1 % G1 == 0
    MMAX = max(G1, NB2) * 16
    TB = 56
    NCH = -(-L2 // TB)

    def kernel(x_hbm, w1_hbm, w2_hbm, g_ref, wf_ref, wg_ref, wo_ref, o_hbm,
               xs0, xs1, w_ref, u_ref, x_ref, y_ref, t_ref, zh_ref, f_ref, fe_ref, ge_ref, st_ref,
               sem_w, sem_x, sem_o):
        xs = (xs0, xs1)
        xh = x_hbm.bitcast(u32)
        cp_w1 = pltpu.make_async_copy(w1_hbm, w_ref.at[0], sem_w.at[0])
        cp_w2 = pltpu.make_async_copy(w2_hbm, w_ref.at[1], sem_w.at[1])
        cp_w1.start()
        cp_x = []
        for b in range(2):
            for ct in range(2):
                cp = pltpu.make_async_copy(xh.at[b, :, _lanes(ct)],
                                           xs[ct].at[pl.ds(XPAD + b * XB, T1), :],
                                           sem_x.at[2 * b + ct])
                cp.start()
                cp_x.append(cp)
        cp_w2.start()

        z8 = jnp.zeros((8, 128), u32)
        for ct in range(2):
            xs[ct][pl.ds(0, 8), :] = z8
            for r in range(XPAD + T1, XPAD + XB, 8):
                xs[ct][pl.ds(r, 8), :] = z8
            for r in range(XPAD + XB + T1, XROWS, 8):
                xs[ct][pl.ds(r, 8), :] = z8

        def zero_zh(i, c):
            for h in range(2):
                zh_ref[i, h] = jnp.zeros((8, 256), u32)
            return c
        lax.fori_loop(0, ZH, zero_zh, 0)

        def transform(slot):
            def body(rg, c):
                weight_transform(w_ref.at[slot], u_ref, t_ref, rg)
                return c
            lax.fori_loop(0, 16, body, 0)

        def matmuls(mrows):
            def body(i, c):
                for q in range(3):
                    pair_matmul(x_ref, u_ref, y_ref, 1 + 3 * i + q, mrows)
                return c
            lax.fori_loop(0, 10, body, 0)
            pair_matmul(x_ref, u_ref, y_ref, 31, mrows)
            real_matmul(x_ref, u_ref, y_ref, 0, mrows)
            real_matmul(x_ref, u_ref, y_ref, 32, mrows)

        cp_w1.wait()
        transform(0)
        for cp in cp_x:
            cp.wait()

        def conv1_chunk(c, carry):
            def fwd_body(g, cc):
                blk = c * G1 + g
                base = blk * S

                def load(h, n, ct):
                    return xs[ct][pl.ds(base + n + h * L1, 8, stride=2 * L1), :]
                _run(fwd_group(load, t_ref, x_ref, g))
                return cc
            lax.fori_loop(0, G1, fwd_body, 0)
            matmuls(G1 * 16)

            def inv_body(g, cc):
                blk = c * G1 + g
                _run(inv_group_conv1(y_ref, t_ref, zh_ref, g, 8 + blk * (S // 2)))
                return cc
            lax.fori_loop(0, G1, inv_body, 0)
            return carry
        lax.fori_loop(0, NB1 // G1, conv1_chunk, 0)

        row = lax.broadcasted_iota(i32, (8, 256), 0)
        last_valid = T2 - (SEG - 1) * L2
        for h in range(2):
            for t in range(last_valid, NB1 * S // 2):
                zh_ref[8 + t, h] = jnp.where(row == SEG - 1, jnp.uint32(0), zh_ref[8 + t, h])
            for j in range(8):
                v = pltpu.roll(zh_ref[8 + L2 - 8 + j, h], 1, axis=0)
                zh_ref[j, h] = jnp.where(row == 0, jnp.uint32(0), v)
            for j in range(8):
                v = pltpu.roll(zh_ref[8 + j, h], SEG - 1, axis=0)
                zh_ref[8 + L2 + j, h] = jnp.where(row == SEG - 1, jnp.uint32(0), v)

        cp_w2.wait()
        transform(1)

        def fwd2_body(g, cc):
            def load(h, n, ct):
                return zh_ref[g * S + n, h, :, _lanes(ct)]
            _run(fwd_group(load, t_ref, x_ref, g))
            return cc
        lax.fori_loop(0, NB2, fwd2_body, 0)
        matmuls(NB2 * 16)

        def inv2_body(g, cc):
            _run(inv_group_conv2(y_ref, t_ref, f_ref, g, g * S))
            return cc
        lax.fori_loop(0, NB2, inv2_body, 0)

        gg = g_ref[...].reshape(16, 256)
        ge_ref[...] = jnp.dot(gg, wg_ref[...], preferred_element_type=f32)

        def out_copy(slot, b, e, t0, nvalid):
            r0 = (b * T2 + e * L2) * 8 + t0 * 8
            return pltpu.make_async_copy(st_ref.at[slot, pl.ds(0, nvalid * 8), :],
                                         o_hbm.at[pl.ds(r0, nvalid * 8), :],
                                         sem_o.at[slot])

        def width(e, ch):
            lim = L2 if e < SEG - 1 else last_valid
            return min(TB, lim - ch * TB)

        def joint_chunk(ch, full):
            t0 = ch * TB
            fl = pltpu.bitcast(f_ref[pl.ds(t0, TB)].reshape(TB * 8, 256), bf16)
            fe_ref[...] = jnp.dot(fl, wf_ref[...], preferred_element_type=f32)
            for b in range(2):
                ge = ge_ref[pl.ds(8 * b, 8), :]
                for e in range(SEG):
                    r = 4 * (e & 3) + 2 * b + (e >> 2)
                    slot = e & 1
                    js = []
                    for t in range(TB):
                        fr = jnp.broadcast_to(fe_ref[pl.ds(16 * t + r, 1), :], (8, 256))
                        js.append(jnp.tanh(fr + ge))
                    jl = jnp.concatenate(js, axis=0).astype(bf16)
                    y = jnp.dot(jl, wo_ref[...], preferred_element_type=f32)
                    nv = TB if full else width(e, NCH - 1)
                    pb, pe = (b, e - 2) if e >= 2 else ((0, e + SEG - 2) if b == 1 else (None, None))
                    if pb is not None:
                        pnv = TB if full else width(pe, NCH - 1)
                        out_copy(slot, pb, pe, t0, pnv).wait()
                    st_ref[slot] = y.astype(bf16)
                    out_copy(slot, b, e, t0, nv).start()
            for e in (SEG - 2, SEG - 1):
                nv = TB if full else width(e, NCH - 1)
                out_copy(e & 1, 1, e, t0, nv).wait()

        def joint_body(ch, c):
            joint_chunk(ch, True)
            return c
        lax.fori_loop(0, NCH - 1, joint_body, 0)
        joint_chunk(NCH - 1, False)

    scratch = [
        pltpu.VMEM((XROWS, 128), u32), pltpu.VMEM((XROWS, 128), u32),
        pltpu.VMEM((2, 31, 256, 256), bf16),
        pltpu.VMEM((NUNITS, 256, 256), u32),
        pltpu.VMEM((NUNITS, MMAX // 2, 512), u32),
        pltpu.VMEM((128, MMAX, 128), f32),
        pltpu.VMEM((2, 128, 8, 128), f32),
        pltpu.VMEM((ZH, 2, 8, 256), u32),
        pltpu.VMEM((max(NB2 * S, NCH * TB), 8, 256), u32),
        pltpu.VMEM((TB * 16, 256), f32),
        pltpu.VMEM((16, 256), f32),
        pltpu.VMEM((2, TB * 8, 256), bf16),
        pltpu.SemaphoreType.DMA((2,)),
        pltpu.SemaphoreType.DMA((4,)),
        pltpu.SemaphoreType.DMA((2,)),
    ]
    return kernel, scratch


def _call(x, w1, w2, g, w_f, w_g, w_o, interpret=False):
    B, T, D = x.shape
    kernel, scratch = _make_kernel(T)
    T2 = T // 4
    any_spec = pl.BlockSpec(memory_space=pl.ANY)
    vmem = pl.BlockSpec(memory_space=pltpu.VMEM)
    out = pl.pallas_call(
        kernel,
        out_shape=jax.ShapeDtypeStruct((B * T2 * 8, D), bf16),
        in_specs=[any_spec, any_spec, any_spec, vmem, vmem, vmem, vmem],
        out_specs=any_spec,
        scratch_shapes=scratch,
        compiler_params=pltpu.CompilerParams(vmem_limit_bytes=126 * 2**20),
        interpret=interpret,
        name="conv_stem_rnnt_joint",
    )(x, w1, w2, g, w_f, w_g, w_o)
    return out.reshape(B, T2, 8, D)


@jax.jit
def pallas_standalone__seq2seq_rnn_t_joint__speech_kernel(x, w1, w2, g, w_f, w_g, w_o):
    return _call(x, w1, w2, g, w_f, w_g, w_o)
```

```python
import functools
import math

import jax
import jax.numpy as jnp
import numpy as np
from jax import lax
from jax.experimental import pallas as pl
from jax.experimental.pallas import tpu as pltpu

f32, u32, bf16, i32 = jnp.float32, jnp.uint32, jnp.bfloat16, jnp.int32

PROFILE_SCOPES = False


class _NoScope:
    def __enter__(self):
        return self

    def __exit__(self, *a):
        return False


def scope(name):
    return jax.named_scope(name) if PROFILE_SCOPES else _NoScope()

N = 64
S = 48
SEG = 8


class V:
    __slots__ = ("a", "s")

    def __init__(self, a, s=1):
        self.a = a
        self.s = s

    def __neg__(self):
        return V(self.a, -self.s)

    def __add__(self, o):
        if self.s == o.s:
            return V(self.a + o.a, self.s)
        if self.s > 0:
            return V(self.a - o.a, 1)
        return V(o.a - self.a, 1)

    def __sub__(self, o):
        return self + (-o)

    def scale(self, c):
        if c == 1.0:
            return self
        if c == -1.0:
            return -self
        return V(self.a * np.float32(abs(c)), self.s * (1 if c > 0 else -1))

    def signed(self, s):
        return self.a if self.s * s > 0 else -self.a


class C:
    __slots__ = ("r", "i")

    def __init__(self, r, i):
        self.r = r
        self.i = i

    def __add__(self, o):
        return C(self.r + o.r, self.i + o.i)

    def __sub__(self, o):
        return C(self.r - o.r, self.i - o.i)

    def __neg__(self):
        return C(-self.r, -self.i)

    def mul_w(self, num, den):
        num %= den
        if num == 0:
            return self
        if 4 * num == den:
            return C(-self.i, self.r)
        if 2 * num == den:
            return -self
        if 4 * num == 3 * den:
            return C(self.i, -self.r)
        if (8 * num) % den == 0:
            o = (8 * num) // den
            h = math.sqrt(0.5)
            sc = 1 if o in (1, 7) else -1
            ss = 1 if o in (1, 3) else -1
            r, m = self.r, self.i
            re = (r if sc > 0 else -r) - (m if ss > 0 else -m)
            im = (r if ss > 0 else -r) + (m if sc > 0 else -m)
            return C(re.scale(h), im.scale(h))
        c = math.cos(2 * math.pi * num / den)
        s = math.sin(2 * math.pi * num / den)
        return C(self.r.scale(c) - self.i.scale(s), self.r.scale(s) + self.i.scale(c))


def _add(a, b):
    if a is None:
        return b
    if b is None:
        return a
    return a + b


def _sub(a, b):
    if b is None:
        return a
    if a is None:
        return -b
    return a - b


def fft8(x, sgn, need=tuple(range(8))):
    def rot(a, num, den):
        return None if a is None else a.mul_w(sgn * num, den)

    need = set(need)
    a0, a1 = _add(x[0], x[4]), _sub(x[0], x[4])
    a2, a3 = _add(x[2], x[6]), rot(_sub(x[2], x[6]), 1, 4)
    a4, a5 = _add(x[1], x[5]), _sub(x[1], x[5])
    a6, a7 = _add(x[3], x[7]), rot(_sub(x[3], x[7]), 1, 4)
    out = {}
    if need & {0, 4}:
        b0, b4 = _add(a0, a2), _add(a4, a6)
        if 0 in need:
            out[0] = _add(b0, b4)
        if 4 in need:
            out[4] = _sub(b0, b4)
    if need & {2, 6}:
        b2, b6 = _sub(a0, a2), rot(_sub(a4, a6), 1, 4)
        if 2 in need:
            out[2] = _add(b2, b6)
        if 6 in need:
            out[6] = _sub(b2, b6)
    if need & {1, 5}:
        b1, b5 = _add(a1, a3), rot(_add(a5, a7), 1, 8)
        if 1 in need:
            out[1] = _add(b1, b5)
        if 5 in need:
            out[5] = _sub(b1, b5)
    if need & {3, 7}:
        b3, b7 = _sub(a1, a3), rot(_sub(a5, a7), 3, 8)
        if 3 in need:
            out[3] = _add(b3, b7)
        if 7 in need:
            out[7] = _sub(b3, b7)
    return out


class _Sym:
    def __add__(self, o):
        return self

    __sub__ = __mul__ = __add__

    def __neg__(self):
        return self


def _fft64_signs(sgn, present=tuple(range(64)), in_sign=None):
    d = _Sym()
    in_sign = in_sign or {}
    x = [C(V(d, in_sign.get((n, 0), 1)), V(d, in_sign.get((n, 1), 1))) if n in present else None
         for n in range(64)]
    t = {}
    for n2 in range(8):
        a = fft8([x[8 * n1 + n2] for n1 in range(8)], sgn)
        for k1 in range(8):
            t[k1, n2] = a[k1].mul_w(sgn * n2 * k1, 64)
    s1 = {key: (v.r.s, v.i.s) for key, v in t.items()}
    s2 = {}
    for k1 in range(8):
        b = fft8([t[k1, n2] for n2 in range(8)], sgn)
        for k2 in range(8):
            s2[k1 + 8 * k2] = b[k2]
    return s1, s2


def _unit(k, j):
    return (k - 1) * 3 + j


UNIT0, UNIT32 = 93, 94
NUNITS = 95


def _lhs_forms(m, z):
    if m in (0, 32):
        u = UNIT0 if m == 0 else UNIT32
        return [(u, 0, z.r), (u, 1, z.i)]
    if m < 32:
        return [(_unit(m, 0), 0, z.r + z.i), (_unit(m, 1), 0, z.r), (_unit(m, 2), 0, z.i)]
    k = 64 - m
    return [(_unit(k, 0), 1, z.r - z.i), (_unit(k, 1), 1, z.r), (_unit(k, 2), 1, z.i)]


def _lhs_signs():
    _, s2 = _fft64_signs(-1)
    sg = {}
    for m in range(64):
        for u, h, v in _lhs_forms(m, s2[m]):
            sg[u, h] = v.s
    return sg


LHS_SIGN = _lhs_signs()


def _y_signs():
    return {(m, 1): -1 for m in range(33, 64)}


def _unpack(w):
    lo = pltpu.unpack_elementwise(w, index=0, packed_dtype=bf16, unpacked_dtype=f32)
    hi = pltpu.unpack_elementwise(w, index=1, packed_dtype=bf16, unpacked_dtype=f32)
    return lo, hi


def _pack(lo, hi):
    return pltpu.pack_elementwise([lo, hi], packed_dtype=bf16)


_GC1 = 2.0 * math.sqrt(2.0 / math.pi)
_GC2 = 8.0 * 0.044715 * math.sqrt(2.0 / math.pi)


def _gelu_half(v):
    a = v.a
    p = (a * a) * np.float32(_GC2) + np.float32(_GC1)
    t = jnp.tanh(p * a)
    return a * t + a if v.s > 0 else a * t - a


def _lanes(t):
    return pl.ds(128 * t, 128)


class Pacer:
    def __init__(self, never, zero=None):
        self.never = never
        self.tok = None
        self.tok2 = None
        self.last = None
        self.outs = []
        self.zero = zero
        self.pending = []
        self.unit = 0

    def gate(self, a):
        vals = [v for q, v in self.pending if q <= self.unit]
        self.pending = [(q, v) for q, v in self.pending if q > self.unit]
        self.unit += 1
        if not vals:
            return a
        m, k = a.shape
        tiles = [[a[8 * r:8 * r + 8, 128 * c:128 * c + 128] for c in range(k // 128)] for r in range(m // 8)]
        flat = [(r, c) for r in range(m // 8) for c in range(k // 128)]
        for i, v in enumerate(vals):
            r, c = flat[i % len(flat)]
            tiles[r][c] = self.tie(tiles[r][c], v)
        return jnp.concatenate([jnp.concatenate(row, axis=1) for row in tiles], axis=0)

    def here(self, x):
        tok, self.tok = self.tok, None
        tok2, self.tok2 = self.tok2, None
        return self.tie(self.tie(x, tok), tok2)

    def mark(self, x, nth=None):
        self.last = x
        if self.never is not None and nth is not None and nth % DUE_EVERY == DUE_EVERY - 1:
            self.outs.append(x)
        return x

    def due(self, x):
        if self.never is not None:
            self.outs.append(x)
        return x

    def tie(self, x, tok):
        if tok is None:
            return x
        if tok.dtype != x.dtype:
            tok = pltpu.bitcast(tok, x.dtype)
        return jnp.where(self.never, tok, x)


def weight_transform(w_ref, u_ref, t_ref, rg):
    rows = pl.ds(pl.multiple_of(rg * 16, 16), 16)
    urow = pl.ds(pl.multiple_of(rg * 8, 8), 8)
    urow_b = pl.ds(pl.multiple_of(rg * 8 + 128, 8), 8)
    taps = [[[None, None] for _ in range(31)] for _ in range(2)]
    for i in range(31):
        for dt in range(2):
            lo, hi = _unpack(pltpu.bitcast(w_ref[i, rows, _lanes(dt)], u32))
            taps[0][i][dt] = lo
            taps[1][i][dt] = hi
    sigma = 1.0 / 256.0
    tau = 1.0 / 128.0

    def wa(p, d, dt):
        return None if d == 0 else V(taps[p][2 * d - 1][dt])

    def wb(p, d, dt):
        return V(taps[p][2 * d][dt])

    def store(u, half, nt, v0, v1):
        s = LHS_SIGN[u, half]
        val = _pack(v0.signed(s), v1.signed(s))
        u_ref[u, urow_b if half else urow, _lanes(nt)] = val

    res = {}
    for p in range(2):
        for dt in range(2):
            for name, f in (("a", wa), ("b", wb)):
                ev = od = None
                for d in range(16):
                    if d % 2 == 0:
                        ev = _add(ev, f(p, d, dt))
                    else:
                        od = _add(od, f(p, d, dt))
                res[p, dt, name, 0] = _add(ev, od).scale(tau)
                res[p, dt, name, 32] = _sub(ev, od).scale(tau)
    for m, u in ((0, UNIT0), (32, UNIT32)):
        for dt in range(2):
            store(u, 0, dt, res[0, dt, "a", m], res[1, dt, "a", m])
            store(u, 1, dt, res[0, dt, "b", m], res[1, dt, "b", m])

    for pm in (1, -1):
        sgn1 = {}
        for p in range(2):
            z = []
            for d in range(16):
                if pm > 0:
                    re = _sub(wa(p, d, 0), wb(p, d, 1))
                    im = _add(wb(p, d, 0), wa(p, d, 1))
                else:
                    re = _add(wa(p, d, 0), wb(p, d, 1))
                    im = _sub(wb(p, d, 0), wa(p, d, 1))
                z.append(C(re.scale(sigma), im.scale(sigma)))
            for n2 in range(8):
                a = fft8([z[n2], z[8 + n2]] + [None] * 6, 1)
                for k1 in range(8):
                    t = a[k1].mul_w(n2 * k1, 64)
                    t_ref[p, (k1 * 8 + n2) * 2] = t.r.a
                    t_ref[p, (k1 * 8 + n2) * 2 + 1] = t.i.a
                    sgn1[k1, n2] = (t.r.s, t.i.s)
        for k1 in range(8):
            need = [k2 for k2 in range(8) if (k1 + 8 * k2) not in (0, 32)]
            outs = []
            for p in range(2):
                xs = [C(V(t_ref[p, (k1 * 8 + n2) * 2], sgn1[k1, n2][0]),
                        V(t_ref[p, (k1 * 8 + n2) * 2 + 1], sgn1[k1, n2][1])) for n2 in range(8)]
                outs.append(fft8(xs, 1, need))
            for k2 in need:
                m = k1 + 8 * k2
                f0, f1 = outs[0][k2], outs[1][k2]
                if m < 32:
                    nt = 0 if pm > 0 else 1
                    store(_unit(m, 0), 1, nt, f0.r, f1.r)
                    store(_unit(m, 1), 1, nt, f0.i - f0.r, f1.i - f1.r)
                    store(_unit(m, 2), 1, nt, -(f0.r + f0.i), -(f1.r + f1.i))
                else:
                    k = 64 - m
                    nt = 1 if pm > 0 else 0
                    store(_unit(k, 0), 0, nt, f0.r, f1.r)
                    store(_unit(k, 1), 0, nt, -(f0.r + f0.i), -(f1.r + f1.i))
                    store(_unit(k, 2), 0, nt, f0.r - f0.i, f1.r - f1.i)


class View:
    def __init__(self, pool, base):
        self.pool = pool
        self.base = base

    def __getitem__(self, idx):
        h, i = idx
        return pltpu.bitcast(self.pool[self.base + h * 128 + i], f32)

    def __setitem__(self, idx, val):
        h, i = idx
        self.pool[self.base + h * 128 + i] = pltpu.bitcast(val, u32)


class XView:
    def __init__(self, pool, base, mg):
        self.pool, self.base, self.mg = pool, base, mg

    def index(self, u, g, c):
        return self.base + (u * self.mg + g) * 4 + c

    def store(self, u, g, c, val):
        self.pool[self.index(u, g, c)] = val

    def load(self, u, zero=None):
        rows = []
        for g in range(self.mg):
            row = []
            for c in range(4):
                idx = self.index(u, g, c)
                if zero is not None and g == 0 and c == 0:
                    idx = idx + zero
                row.append(self.pool[idx])
            rows.append(jnp.concatenate(row, axis=1))
        return jnp.concatenate(rows, axis=0)


COST_F1, COST_F2, COST_I1, COST_I2 = 105, 152, 91, 260
FWD_S1, _ = _fft64_signs(-1)
INV_S1, _ = _fft64_signs(1, in_sign=_y_signs())
CLASSES = ((1, 7), (2, 6), (3, 5), (4, 0))


def _class_units(cls):
    ks = [k for k in range(1, 32) if k % 8 in cls or (-k) % 8 in cls]
    ks.sort(key=lambda k: (0 if k % 8 == cls[0] else 1, k))
    out = [("pair", k) for k in ks]
    if 0 in cls:
        out += [("real", 0), ("real", 32)]
    return out


def fwd_p1(load, t_ref, h, n2, ct, pc):
    xs = []
    for n1 in range(8):
        w = load(h, 8 * n1 + n2, ct)
        if n1 == 0:
            w = pc.here(w)
        lo, hi = _unpack(w)
        xs.append(C(V(lo), V(hi)))
    a = fft8(xs, -1)
    for k1 in range(8):
        t = a[k1].mul_w(-n2 * k1, 64)
        assert (t.r.s, t.i.s) == FWD_S1[k1, n2]
        t_ref[h, (k1 * 8 + n2) * 2] = t.r.a
        t_ref[h, (k1 * 8 + n2) * 2 + 1] = t.i.a
    return COST_F1


def fwd_p2(t_ref, x_ref, g, ct, k1, pc):
    outs = []
    for h in range(2):
        xs = [C(V(t_ref[h, (k1 * 8 + n2) * 2], FWD_S1[k1, n2][0]),
                V(t_ref[h, (k1 * 8 + n2) * 2 + 1], FWD_S1[k1, n2][1])) for n2 in range(8)]
        if h == 0:
            xs[0].r.a = pc.here(xs[0].r.a)
        outs.append(fft8(xs, -1))
    for k2 in range(8):
        m = k1 + 8 * k2
        f0 = _lhs_forms(m, outs[0][k2])
        f1 = _lhs_forms(m, outs[1][k2])
        for i, ((u, half, v0), (_, _, v1)) in enumerate(zip(f0, f1)):
            assert v0.s == v1.s == LHS_SIGN[u, half]
            x_ref.store(u, g, 2 * half + ct, _pack(v0.a, v1.a))
    return COST_F2


def inv_p1(y_ref, t_ref, g, h, n2, pc):
    rows = pl.ds(g * 16 + 8 * h, 8)
    ysg = _y_signs()
    xs = []
    for n1 in range(8):
        m = 8 * n1 + n2
        xs.append(C(V(y_ref[2 * m, rows, :], ysg.get((m, 0), 1)),
                    V(y_ref[2 * m + 1, rows, :], ysg.get((m, 1), 1))))
    xs[0].r.a = pc.here(xs[0].r.a)
    a = fft8(xs, 1)
    for k1 in range(8):
        t = a[k1].mul_w(n2 * k1, 64)
        assert (t.r.s, t.i.s) == INV_S1[k1, n2]
        t_ref[h, (k1 * 8 + n2) * 2] = t.r.a
        t_ref[h, (k1 * 8 + n2) * 2 + 1] = t.i.a
    return COST_I1


def _inv_out(t_ref, h, k1, pc):
    xs = [C(V(t_ref[h, (k1 * 8 + n2) * 2], INV_S1[k1, n2][0]),
            V(t_ref[h, (k1 * 8 + n2) * 2 + 1], INV_S1[k1, n2][1])) for n2 in range(8)]
    xs[0].r.a = pc.here(xs[0].r.a)
    b = fft8(xs, 1, range(S // 8))
    return {k2: (_gelu_half(b[k2].r), _gelu_half(b[k2].i)) for k2 in range(S // 8)}


def inv_p2_conv1(t_ref, zh_ref, tau0, q, pc):
    h, k1 = q // 4, 2 * (q % 4)
    ev = _inv_out(t_ref, h, k1, pc)
    od = _inv_out(t_ref, h, k1 + 1, pc)
    for k2 in range(S // 8):
        for dt in range(2):
            zh_ref[tau0 + (k1 // 2 + 4 * k2), h, :, _lanes(dt)] = pc.due(_pack(ev[k2][dt], od[k2][dt]))
    return COST_I2


def inv_p2_conv2(t_ref, f_ref, tau0, k1, pc):
    oa = _inv_out(t_ref, 0, k1, pc)
    ob = _inv_out(t_ref, 1, k1, pc)
    for k2 in range(S // 8):
        for dt in range(2):
            f_ref[tau0 + (k1 + 8 * k2), :, _lanes(dt)] = pc.due(_pack(oa[k2][dt], ob[k2][dt]))
    return COST_I2


def _mm(x_ref, u_ref, j, pc=None):
    a = x_ref.load(j, None if pc is None else pc.zero)
    if pc is not None:
        a = pc.gate(a)
    a = pltpu.bitcast(a, bf16)
    w = pltpu.bitcast(u_ref[j], bf16)
    return jnp.dot(a, w, preferred_element_type=f32)


def _tokens(y):
    m = y.shape[0]
    return [y[8 * r:8 * r + 8, 128 * n:128 * n + 128] for n in range(2) for r in range(m // 8)]


def matmul_stream(x_ref, u_ref, y_ref, pc=None):
    for cls in CLASSES:
        for kind, k in _class_units(cls):
            if kind == "pair":
                j = (k - 1) * 3
                k1 = _mm(x_ref, u_ref, j, pc)
                yield _tokens(k1)
                k2 = _mm(x_ref, u_ref, j + 1, pc)
                yi = k1 + k2
                y_ref[2 * k + 1] = yi[:, :128]
                y_ref[2 * (64 - k) + 1] = yi[:, 128:]
                yield _tokens(k2)
                k3 = _mm(x_ref, u_ref, j + 2, pc)
                yr = k1 - k3
                y_ref[2 * k] = yr[:, :128]
                y_ref[2 * (64 - k)] = yr[:, 128:]
                yield _tokens(k3)
            else:
                y = _mm(x_ref, u_ref, UNIT0 if k == 0 else UNIT32, pc)
                y_ref[2 * k] = y[:, :128]
                y_ref[2 * k + 1] = y[:, 128:]
                yield _tokens(y)


def run_step(mm, pieces, costs, pc, ntok, lead, lag=None, due=None):
    total = float(sum(costs))
    lag = LAG if lag is None else lag
    tokens = []
    marks = []
    c = 0.0
    for piece, cost in zip(pieces, costs):
        pc.tok = None
        pc.tok2 = marks[-lag] if lag and len(marks) >= lag else None
        if c >= lead:
            want = min(int((c - lead) / (total - lead) * ntok), ntok - 1)
            ahead = min(want + AHEAD * (ntok // NUNITS), ntok - 1)
            while ahead >= len(tokens):
                tokens += next(mm)
            pc.tok = tokens[want]
        pc.outs = []
        piece()
        marks.append(pc.last)
        for i, v in enumerate(pc.outs):
            q = pc.unit + (DUE if due is None else due) + i // 4
            if q < NUNITS:
                pc.pending.append((q, v))
        c += cost
    pc.tok = pc.tok2 = None
    for _ in mm:
        pass


def _make_kernel(T):
    T1, T2 = T // 2, T // 4
    L1 = (T1 + 16) // SEG
    L2 = L1 // 2
    assert L1 * SEG == T1 + 16 and L1 % 2 == 0
    NB1 = -(-L1 // S)
    NB2 = -(-L2 // S)
    XPAD = 8
    XB = T1 + 16
    XROWS = XPAD + 2 * XB + 64
    MG = 3
    M = 16 * MG
    NC1 = -(-NB1 // MG)
    NC2 = -(-NB2 // MG)
    ZH = (NB2 - 1) * S + N
    ZDUMP = ZH
    TB = 56
    NCH = -(-L2 // TB)
    FROWS = max(NB2 * S, NCH * TB)
    FDUMP = FROWS
    last_valid = T2 - (SEG - 1) * L2
    XPART = (0, 304, 592)

    def x_rows(e, part):
        def start(e, part):
            if e >= SEG:
                return T1
            return max(L1 * e + XPART[part] - (8 if part == 0 else 0), 0) // 8 * 8
        if part + 1 < len(XPART):
            return start(e, part), start(e, part + 1)
        return start(e, part), start(e + 1, 0)

    def kernel(x_hbm, w1_hbm, w2_hbm, g_ref, wf_ref, wg_ref, wo_ref, o_hbm,
               xs0, xs1, w_ref, u_ref, pool, y_ref, zh_ref, f_ref, fe_ref, ge_ref,
               st_ref, sem_w, sem_x, sem_o):
        xs = (xs0, xs1)
        x_ref = XView(pool, 0, MG)
        tf = [[View(pool, NUNITS * MG * 4 + (g * 2 + ct) * 256) for ct in range(2)] for g in range(MG)]
        ti = [View(pool, NUNITS * MG * 4 + MG * 512 + g * 256) for g in range(MG)]
        xh = x_hbm.bitcast(u32)

        def w1_copy(q):
            rows = pl.ds(64 * q, 64)
            return pltpu.make_async_copy(w1_hbm.at[:, rows, :], w_ref.at[0, :, rows, :], sem_w.at[q])

        w2_copy = pltpu.make_async_copy(w2_hbm, w_ref.at[1], sem_w.at[4])

        def x_copies(part):
            cps = []
            for b in range(2):
                for e in range(SEG):
                    lo, hi = x_rows(e, part)
                    for ct in range(2):
                        cps.append(pltpu.make_async_copy(
                            xh.at[b, pl.ds(lo, hi - lo), _lanes(ct)],
                            xs[ct].at[pl.ds(XPAD + b * XB + lo, hi - lo), :],
                            sem_x.at[part]))
            return cps

        w1_copy(0).start()
        w1_copy(1).start()

        z8 = jnp.zeros((8, 128), u32)
        for ct in range(2):
            xs[ct][pl.ds(0, 8), :] = z8
            for r in range(XPAD + T1, XPAD + XB, 8):
                xs[ct][pl.ds(r, 8), :] = z8
            for r in range(XPAD + XB + T1, XROWS, 8):
                xs[ct][pl.ds(r, 8), :] = z8

        def zero_zh(i, c):
            for h in range(2):
                zh_ref[ZH - 1 - i, h] = jnp.zeros((8, 256), u32)
            return c
        lax.fori_loop(0, ZH - 8 - L2, zero_zh, 0)

        def zero_y(i, c):
            y_ref[i] = jnp.zeros((M, 128), f32)
            return c
        lax.fori_loop(0, 128, zero_y, 0)

        def zero_t(i, c):
            for h in range(2):
                for g in range(MG):
                    pool[NUNITS * MG * 4 + MG * 512 + g * 256 + h * 128 + i] = jnp.zeros((8, 128), u32)
            return c
        lax.fori_loop(0, 128, zero_t, 0)

        gg = g_ref[...].reshape(16, 256)
        ge_all = jnp.dot(gg, wg_ref[...], preferred_element_type=f32)
        ge_ref[...] = ge_all

        def transform(slot, hook=None):
            def body(rg, c):
                if hook is not None:
                    hook(rg)
                weight_transform(w_ref.at[slot], u_ref, tf[0][0], rg)
                return c
            lax.fori_loop(0, 16, body, 0)

        def w1_hook(rg):
            for q in range(4):
                @pl.when(rg == 4 * q)
                def _(q=q):
                    w1_copy(q).wait()
                    if q + 2 < 4:
                        w1_copy(q + 2).start()
                    if q >= 1:
                        for cp in x_copies(q - 1):
                            cp.start()

        def conv(nchunk, nblk, make_load, inv_p2, out_index, wait_input=None):
            def loads(c):
                return [make_load(jnp.minimum(c * MG + g, nblk - 1)) for g in range(MG)]

            def P(fn, *a):
                return functools.partial(fn, *a)

            def f1(ld, pc):
                return [(P(fwd_p1, ld[g], tf[g][ct], h, n2, ct, pc), COST_F1)
                        for g in range(MG) for ct in range(2) for h in range(2) for n2 in range(8)]

            def f2(cls, pc):
                return [(P(fwd_p2, tf[g][ct], x_ref, g, ct, k1, pc), COST_F2)
                        for g in range(MG) for ct in range(2) for k1 in cls]

            def i1(cls, pc):
                return [(P(inv_p1, y_ref, ti[g], g, h, n2, pc), COST_I1)
                        for g in range(MG) for h in range(2) for n2 in cls]

            def i2(c, pc):
                return [(P(inv_p2, ti[g], out_index(c, g), q, pc), COST_I2)
                        for g in range(MG) for q in range(8)]

            idle = Pacer(None)
            if wait_input is not None:
                wait_input(0)
            with scope("pro"):
                for piece, _ in f1(loads(0), idle):
                    piece()
                for cls in CLASSES[:3]:
                    for piece, _ in f2(cls, idle):
                        piece()

            def step(c, cc):
                if wait_input is not None:
                    wait_input(c + 1)
                pc = Pacer(c < 0, lax.shift_right_arithmetic(c, 20))
                nxt = f1(loads(jnp.minimum(c + 1, nchunk - 1)), pc)
                half = len(nxt) // 2
                seq = (i1(CLASSES[3], pc) + f2(CLASSES[3], pc) + i2(c - 1, pc)
                       + nxt[:half] + i1(CLASSES[0], pc) + nxt[half:]
                       + f2(CLASSES[0], pc) + i1(CLASSES[1], pc) + f2(CLASSES[1], pc)
                       + i1(CLASSES[2], pc) + f2(CLASSES[2], pc))
                run_step(matmul_stream(x_ref, u_ref, y_ref, pc), [q[0] for q in seq], [q[1] for q in seq],
                         pc, NUNITS * (M // 4), LEAD)
                return cc
            with scope("steps"):
                lax.fori_loop(0, nchunk, step, 0)

            with scope("epi"):
                for piece, _ in i1(CLASSES[3], idle) + i2(nchunk - 1, idle):
                    piece()

        with scope("wt1"):
            transform(0, w1_hook)

        def wait_x0(c):
            if isinstance(c, int):
                for cp in x_copies(0):
                    cp.wait()
                return
            for part, first in ((1, 2), (2, 4)):
                @pl.when(c == first)
                def _(part=part):
                    for cp in x_copies(part):
                        cp.wait()

            @pl.when(c == 2)
            def _():
                w2_copy.start()

        def load1(blk):
            base = blk * S

            def load(h, n, ct):
                return xs[ct][pl.ds(base + n + h * L1, 8, stride=2 * L1), :]
            return load

        def inv1(tb, tau0, q, pc):
            return inv_p2_conv1(tb, zh_ref, tau0, q, pc)

        def out1(c, g):
            if isinstance(c, int):
                return 8 + (c * MG + g) * (S // 2)
            return jnp.where(c >= 0, 8 + (c * MG + g) * (S // 2), ZDUMP + g * (S // 2))

        conv(NC1, NB1, load1, inv1, out1, wait_x0)

        row = lax.broadcasted_iota(i32, (8, 256), 0)
        for h in range(2):
            for t in range(last_valid, NB1 * S // 2):
                zh_ref[8 + t, h] = jnp.where(row == SEG - 1, jnp.uint32(0), zh_ref[8 + t, h])
            for j in range(8):
                v = pltpu.roll(zh_ref[8 + L2 - 8 + j, h], 1, axis=0)
                zh_ref[j, h] = jnp.where(row == 0, jnp.uint32(0), v)
            for j in range(8):
                v = pltpu.roll(zh_ref[8 + j, h], SEG - 1, axis=0)
                zh_ref[8 + L2 + j, h] = jnp.where(row == SEG - 1, jnp.uint32(0), v)

        w2_copy.wait()
        with scope("wt2"):
            transform(1)

        def load2(blk):
            def load(h, n, ct):
                return zh_ref[blk * S + n, h, :, _lanes(ct)]
            return load

        def inv2(tb, tau0, q, pc):
            return inv_p2_conv2(tb, f_ref, tau0, q, pc)

        def out2(c, g):
            if isinstance(c, int):
                return min(c * MG + g, NB2 - 1) * S
            return jnp.where(c >= 0, jnp.minimum(c * MG + g, NB2 - 1) * S, FDUMP + g * S)

        conv(NC2, NB2, load2, inv2, out2)

        never = jnp.max(jnp.abs(ge_all)) < 0.0
        order = [(b, e) for b in range(2) for e in range(SEG)]

        def out_copy(half, q, t0, nvalid):
            b, e = order[q]
            r0 = (b * T2 + e * L2) * 8 + t0 * 8
            return pltpu.make_async_copy(st_ref.at[half, q, pl.ds(0, nvalid * 8), :],
                                         o_hbm.at[pl.ds(r0, nvalid * 8), :],
                                         sem_o.at[half])

        def width(e):
            lim = L2 if e < SEG - 1 else last_valid
            return lim - (NCH - 1) * TB

        def joint_chunk(ch, half, full, never):
            pc = Pacer(never)
            t0 = ch * TB
            fl = pltpu.bitcast(f_ref[pl.ds(t0, TB)].reshape(TB * 8, 256), bf16)
            fe = jnp.dot(fl, wf_ref[...], preferred_element_type=f32)
            fe_ref[...] = fe
            prev = [fe[8 * r:8 * r + 8, 128 * n:128 * n + 128] for n in range(2) for r in range(2 * TB)]
            prev = prev[len(prev) // 2:]
            for q, (b, e) in enumerate(order):
                ge = ge_ref[pl.ds(8 * b, 8), :]
                r = 4 * (e & 3) + 2 * b + (e >> 2)
                js = []
                for t in range(TB):
                    row = jnp.broadcast_to(fe_ref[pl.ds(16 * t + r, 1), :], (8, 256))
                    tok = prev[(t * len(prev)) // TB]
                    gt = jnp.concatenate([pc.tie(ge[:, :128], tok), pc.tie(ge[:, 128:], tok)], axis=1)
                    js.append(jnp.tanh(row + gt))
                jl = jnp.concatenate(js, axis=0).astype(bf16)
                y = jnp.dot(jl, wo_ref[...], preferred_element_type=f32)
                prev = [y[8 * rr:8 * rr + 8, 128 * n:128 * n + 128] for n in range(2) for rr in range(TB)]
                st_ref[half, q] = y.astype(bf16)
                out_copy(half, q, t0, TB if full else width(e)).start()

        def wait_chunk(half, full):
            for q, (b, e) in enumerate(order):
                out_copy(half, q, 0, TB if full else width(e)).wait()

        def joint_body(ch, c):
            half = ch % 2

            @pl.when(ch >= 2)
            def _():
                wait_chunk(half, True)
            joint_chunk(ch, half, True, ch < 0)
            return c
        with scope("joint"):
            lax.fori_loop(0, NCH - 1, joint_body, 0)
            last_half = (NCH - 1) % 2
            wait_chunk(last_half, True)
            joint_chunk(NCH - 1, last_half, False, never)
            wait_chunk(1 - last_half, True)
            wait_chunk(last_half, False)

    scratch = [
        pltpu.VMEM((XROWS, 128), u32), pltpu.VMEM((XROWS, 128), u32),
        pltpu.VMEM((2, 31, 256, 256), bf16),
        pltpu.VMEM((NUNITS, 256, 256), u32),
        pltpu.VMEM((NUNITS * MG * 4 + MG * 512 + MG * 256, 8, 128), u32),
        pltpu.VMEM((128, M, 128), f32),
        pltpu.VMEM((ZH + MG * S // 2, 2, 8, 256), u32),
        pltpu.VMEM((FROWS + MG * S, 8, 256), u32),
        pltpu.VMEM((TB * 16, 256), f32),
        pltpu.VMEM((16, 256), f32),
        pltpu.VMEM((2, 2 * SEG, TB * 8, 256), bf16),
        pltpu.SemaphoreType.DMA((5,)),
        pltpu.SemaphoreType.DMA((3,)),
        pltpu.SemaphoreType.DMA((2,)),
    ]
    return kernel, scratch


LEAD = 0
LAG = 0
AHEAD = 3
DUE = 2
DUE_EVERY = 1000


def _call(x, w1, w2, g, w_f, w_g, w_o, interpret=False):
    B, T, D = x.shape
    kernel, scratch = _make_kernel(T)
    T2 = T // 4
    any_spec = pl.BlockSpec(memory_space=pl.ANY)
    vmem = pl.BlockSpec(memory_space=pltpu.VMEM)
    out = pl.pallas_call(
        kernel,
        out_shape=jax.ShapeDtypeStruct((B * T2 * 8, D), bf16),
        in_specs=[any_spec, any_spec, any_spec, vmem, vmem, vmem, vmem],
        out_specs=any_spec,
        scratch_shapes=scratch,
        compiler_params=pltpu.CompilerParams(vmem_limit_bytes=126 * 2**20),
        interpret=interpret,
        name="conv_stem_rnnt_joint",
    )(x, w1, w2, g, w_f, w_g, w_o)
    return out.reshape(B, T2, 8, D)


@jax.jit
def pallas_standalone__seq2seq_rnn_t_joint__speech_kernel(x, w1, w2, g, w_f, w_g, w_o):
    return _call(x, w1, w2, g, w_f, w_g, w_o)
```

```python
import functools
import math

import jax
import jax.numpy as jnp
import numpy as np
from jax import lax
from jax.experimental import pallas as pl
from jax.experimental.pallas import tpu as pltpu

f32, u32, bf16, i32 = jnp.float32, jnp.uint32, jnp.bfloat16, jnp.int32

PROFILE_SCOPES = False


class _NoScope:
    def __enter__(self):
        return self

    def __exit__(self, *a):
        return False


def scope(name):
    return jax.named_scope(name) if PROFILE_SCOPES else _NoScope()

N = 64
S = 48
SEG = 8


class V:
    __slots__ = ("a", "s")

    def __init__(self, a, s=1):
        self.a = a
        self.s = s

    def __neg__(self):
        return V(self.a, -self.s)

    def __add__(self, o):
        if self.s == o.s:
            return V(self.a + o.a, self.s)
        if self.s > 0:
            return V(self.a - o.a, 1)
        return V(o.a - self.a, 1)

    def __sub__(self, o):
        return self + (-o)

    def scale(self, c):
        if c == 1.0:
            return self
        if c == -1.0:
            return -self
        return V(self.a * np.float32(abs(c)), self.s * (1 if c > 0 else -1))

    def times(self, c):
        return self.a * np.float32(self.s * c)

    def signed(self, s):
        return self.a if self.s * s > 0 else -self.a


class C:
    __slots__ = ("r", "i")

    def __init__(self, r, i):
        self.r = r
        self.i = i

    def __add__(self, o):
        return C(self.r + o.r, self.i + o.i)

    def __sub__(self, o):
        return C(self.r - o.r, self.i - o.i)

    def __neg__(self):
        return C(-self.r, -self.i)

    def mul_w(self, num, den):
        num %= den
        if num == 0:
            return self
        if 4 * num == den:
            return C(-self.i, self.r)
        if 2 * num == den:
            return -self
        if 4 * num == 3 * den:
            return C(self.i, -self.r)
        if (8 * num) % den == 0:
            o = (8 * num) // den
            h = math.sqrt(0.5)
            sc = 1 if o in (1, 7) else -1
            ss = 1 if o in (1, 3) else -1
            r, m = self.r, self.i
            re = (r if sc > 0 else -r) - (m if ss > 0 else -m)
            im = (r if ss > 0 else -r) + (m if sc > 0 else -m)
            return C(re.scale(h), im.scale(h))
        c = math.cos(2 * math.pi * num / den)
        s = math.sin(2 * math.pi * num / den)
        return C(self.r.scale(c) - self.i.scale(s), self.r.scale(s) + self.i.scale(c))


def _add(a, b):
    if a is None:
        return b
    if b is None:
        return a
    return a + b


def _sub(a, b):
    if b is None:
        return a
    if a is None:
        return -b
    return a - b


def fft8(x, sgn, need=tuple(range(8))):
    def rot(a, num, den):
        return None if a is None else a.mul_w(sgn * num, den)

    need = set(need)
    a0, a1 = _add(x[0], x[4]), _sub(x[0], x[4])
    a2, a3 = _add(x[2], x[6]), rot(_sub(x[2], x[6]), 1, 4)
    a4, a5 = _add(x[1], x[5]), _sub(x[1], x[5])
    a6, a7 = _add(x[3], x[7]), rot(_sub(x[3], x[7]), 1, 4)
    out = {}
    if need & {0, 4}:
        b0, b4 = _add(a0, a2), _add(a4, a6)
        if 0 in need:
            out[0] = _add(b0, b4)
        if 4 in need:
            out[4] = _sub(b0, b4)
    if need & {2, 6}:
        b2, b6 = _sub(a0, a2), rot(_sub(a4, a6), 1, 4)
        if 2 in need:
            out[2] = _add(b2, b6)
        if 6 in need:
            out[6] = _sub(b2, b6)
    if need & {1, 5}:
        b1, b5 = _add(a1, a3), rot(_add(a5, a7), 1, 8)
        if 1 in need:
            out[1] = _add(b1, b5)
        if 5 in need:
            out[5] = _sub(b1, b5)
    if need & {3, 7}:
        b3, b7 = _sub(a1, a3), rot(_sub(a5, a7), 3, 8)
        if 3 in need:
            out[3] = _add(b3, b7)
        if 7 in need:
            out[7] = _sub(b3, b7)
    return out


class _Sym:
    def __add__(self, o):
        return self

    __sub__ = __mul__ = __add__

    def __neg__(self):
        return self


def _fft64_signs(sgn, present=tuple(range(64)), in_sign=None):
    d = _Sym()
    in_sign = in_sign or {}
    x = [C(V(d, in_sign.get((n, 0), 1)), V(d, in_sign.get((n, 1), 1))) if n in present else None
         for n in range(64)]
    t = {}
    for n2 in range(8):
        a = fft8([x[8 * n1 + n2] for n1 in range(8)], sgn)
        for k1 in range(8):
            t[k1, n2] = a[k1].mul_w(sgn * n2 * k1, 64)
    s1 = {key: (v.r.s, v.i.s) for key, v in t.items()}
    s2 = {}
    for k1 in range(8):
        b = fft8([t[k1, n2] for n2 in range(8)], sgn)
        for k2 in range(8):
            s2[k1 + 8 * k2] = b[k2]
    return s1, s2


def _unit(k, j):
    return (k - 1) * 3 + j


UNIT0, UNIT32 = 93, 94
NUNITS = 95


def _lhs_forms(m, z):
    if m in (0, 32):
        u = UNIT0 if m == 0 else UNIT32
        return [(u, 0, z.r), (u, 1, z.i)]
    if m < 32:
        return [(_unit(m, 0), 0, z.r + z.i), (_unit(m, 1), 0, z.r), (_unit(m, 2), 0, z.i)]
    k = 64 - m
    return [(_unit(k, 0), 1, z.r - z.i), (_unit(k, 1), 1, z.r), (_unit(k, 2), 1, z.i)]


def _lhs_signs():
    _, s2 = _fft64_signs(-1)
    sg = {}
    for m in range(64):
        for u, h, v in _lhs_forms(m, s2[m]):
            sg[u, h] = v.s
    return sg


LHS_SIGN = _lhs_signs()


def _weight_forms(m, pm):
    if m < 32:
        nt = 0 if pm > 0 else 1
        return [(_unit(m, 0), 1, nt, (1, 0)), (_unit(m, 1), 1, nt, (-1, 1)), (_unit(m, 2), 1, nt, (-1, -1))]
    k = 64 - m
    nt = 1 if pm > 0 else 0
    return [(_unit(k, 0), 0, nt, (1, 0)), (_unit(k, 1), 0, nt, (-1, -1)), (_unit(k, 2), 0, nt, (1, -1))]


def _weight_plan():
    s1, s2 = _fft64_signs(1, present=range(16))
    forms = {}
    for pm in (1, -1):
        for m in range(1, 64):
            if m == 32:
                continue
            for u, half, nt, (cr, ci) in _weight_forms(m, pm):
                forms[u, half, nt] = (cr * s2[m].r.s, ci * s2[m].i.s)
    col = {}
    for u in range(93):
        for nt in range(2):
            def negs(sig):
                n = 0
                for half in range(2):
                    cr, ci = forms[u, half, nt]
                    w = sig * LHS_SIGN[u, half]
                    n += (w * cr <= 0 and w * ci <= 0)
                return n
            col[u, nt] = 1 if negs(1) <= negs(-1) else -1
    for u in (UNIT0, UNIT32):
        col[u, 0] = col[u, 1] = 1
    return s1, s2, col


WT_S1, WT_S2, COL_SIGN = _weight_plan()


def _recombine(k1, k2, k3, k):
    out = {}
    for nt in range(2):
        yr = k1[nt] - k3[nt]
        yi = k1[nt] + k2[nt]
        if nt == 0:
            out[k, 0], out[k, 1] = yr, yi
        else:
            out[64 - k, 0], out[64 - k, 1] = yr, -yi
    return out


def _y_signs():
    d = _Sym()
    sg = {}
    for k in range(1, 32):
        ks = [[V(d, COL_SIGN[_unit(k, j), nt]) for nt in range(2)] for j in range(3)]
        for key, v in _recombine(ks[0], ks[1], ks[2], k).items():
            sg[key] = v.s
    for m, u in ((0, UNIT0), (32, UNIT32)):
        sg[m, 0], sg[m, 1] = COL_SIGN[u, 0], COL_SIGN[u, 1]
    return sg


Y_SIGN = _y_signs()


def _unpack(w):
    lo = pltpu.unpack_elementwise(w, index=0, packed_dtype=bf16, unpacked_dtype=f32)
    hi = pltpu.unpack_elementwise(w, index=1, packed_dtype=bf16, unpacked_dtype=f32)
    return lo, hi


def _pack(lo, hi):
    return pltpu.pack_elementwise([lo, hi], packed_dtype=bf16)


_GC1 = 2.0 * math.sqrt(2.0 / math.pi)
_GC2 = 8.0 * 0.044715 * math.sqrt(2.0 / math.pi)


def _gelu_half(v):
    a = v.a
    p = (a * a) * np.float32(_GC2) + np.float32(_GC1)
    t = jnp.tanh(p * a)
    return a * t + a if v.s > 0 else a * t - a


def _lanes(t):
    return pl.ds(128 * t, 128)


class Pacer:
    def __init__(self, never, zero=None):
        self.never = never
        self.tok = None
        self.tok2 = None
        self.last = None
        self.outs = []
        self.zero = zero
        self.pending = []
        self.unit = 0

    def gate(self, a):
        vals = [v for q, v in self.pending if q <= self.unit]
        self.pending = [(q, v) for q, v in self.pending if q > self.unit]
        self.unit += 1
        if not vals:
            return a
        m, k = a.shape
        tiles = [[a[8 * r:8 * r + 8, 128 * c:128 * c + 128] for c in range(k // 128)] for r in range(m // 8)]
        flat = [(r, c) for r in range(m // 8) for c in range(k // 128)]
        for i, v in enumerate(vals):
            r, c = flat[i % len(flat)]
            tiles[r][c] = self.tie(tiles[r][c], v)
        return jnp.concatenate([jnp.concatenate(row, axis=1) for row in tiles], axis=0)

    def here(self, x):
        tok, self.tok = self.tok, None
        tok2, self.tok2 = self.tok2, None
        return self.tie(self.tie(x, tok), tok2)

    def mark(self, x, nth=None):
        self.last = x
        if self.never is not None and nth is not None and nth % DUE_EVERY == DUE_EVERY - 1:
            self.outs.append(x)
        return x

    def due(self, x):
        if self.never is not None:
            self.outs.append(x)
        return x

    def tie(self, x, tok):
        if tok is None:
            return x
        if tok.dtype != x.dtype:
            tok = pltpu.bitcast(tok, x.dtype)
        return jnp.where(self.never, tok, x)


def _combo(f, cr, ci, want):
    if ci == 0:
        return f.r.signed(want * cr)
    v = (f.r if cr > 0 else -f.r) + (f.i if ci > 0 else -f.i)
    if v.s * want > 0:
        return v.a
    if f.r.s * cr != f.i.s * ci:
        return ((-f.r) if cr > 0 else f.r).__add__((-f.i) if ci > 0 else f.i).a
    return -v.a


def weight_transform(w_ref, u_ref, t_ref, z_ref, rg):
    rows = pl.ds(pl.multiple_of(rg * 8, 8), 8)
    urow = (rows, pl.ds(pl.multiple_of(rg * 8 + 128, 8), 8))
    sigma = 1.0 / 256.0
    tau = 1.0 / 128.0

    def store(u, half, nt, a0, a1):
        u_ref[u, urow[half], _lanes(nt)] = _pack(a0, a1)

    acc = {}
    for d in range(16):
        wa = [[None, None], [None, None]]
        wb = [[None, None], [None, None]]
        for dt in range(2):
            if d > 0:
                lo, hi = _unpack(w_ref[2 * d - 1, rows, _lanes(dt)])
                wa[0][dt], wa[1][dt] = V(lo), V(hi)
            lo, hi = _unpack(w_ref[2 * d, rows, _lanes(dt)])
            wb[0][dt], wb[1][dt] = V(lo), V(hi)
        for p in range(2):
            for dt in range(2):
                for name, val in (("a", wa[p][dt]), ("b", wb[p][dt])):
                    key = (p, dt, name, d % 2)
                    acc[key] = _add(acc.get(key), val)
            zp = (_sub(wa[p][0], wb[p][1]), _add(wb[p][0], wa[p][1]))
            zm = (_add(wa[p][0], wb[p][1]), _sub(wb[p][0], wa[p][1]))
            for j, z in enumerate((zp, zm)):
                for comp in range(2):
                    z_ref[j, (p * 16 + d) * 2 + comp] = z[comp].times(sigma)
    for m, u in ((0, UNIT0), (32, UNIT32)):
        for dt in range(2):
            for half, name in enumerate(("a", "b")):
                vals = []
                for p in range(2):
                    ev, od = acc[p, dt, name, 0], acc[p, dt, name, 1]
                    v = _add(ev, od) if m == 0 else _sub(ev, od)
                    vals.append(v.times(tau * LHS_SIGN[u, half] * COL_SIGN[u, dt]))
                store(u, half, dt, vals[0], vals[1])

    for j, pm in enumerate((1, -1)):
        for p in range(2):
            for n2 in range(8):
                z = [C(V(z_ref[j, (p * 16 + d) * 2]), V(z_ref[j, (p * 16 + d) * 2 + 1])) for d in (n2, n2 + 8)]
                a = fft8(z + [None] * 6, 1)
                for k1 in range(8):
                    t = a[k1].mul_w(n2 * k1, 64)
                    assert (t.r.s, t.i.s) == WT_S1[k1, n2]
                    t_ref[p, (k1 * 8 + n2) * 2] = t.r.a
                    t_ref[p, (k1 * 8 + n2) * 2 + 1] = t.i.a
        for k1 in range(8):
            need = [k2 for k2 in range(8) if (k1 + 8 * k2) not in (0, 32)]
            outs = []
            for p in range(2):
                xs = [C(V(t_ref[p, (k1 * 8 + n2) * 2], WT_S1[k1, n2][0]),
                        V(t_ref[p, (k1 * 8 + n2) * 2 + 1], WT_S1[k1, n2][1])) for n2 in range(8)]
                outs.append(fft8(xs, 1, need))
            for k2 in need:
                m = k1 + 8 * k2
                for u, half, nt, (cr, ci) in _weight_forms(m, pm):
                    want = LHS_SIGN[u, half] * COL_SIGN[u, nt]
                    store(u, half, nt, _combo(outs[0][k2], cr, ci, want), _combo(outs[1][k2], cr, ci, want))


class View:
    def __init__(self, pool, base):
        self.pool = pool
        self.base = base

    def __getitem__(self, idx):
        h, i = idx
        return pltpu.bitcast(self.pool[self.base + h * 128 + i], f32)

    def __setitem__(self, idx, val):
        h, i = idx
        self.pool[self.base + h * 128 + i] = pltpu.bitcast(val, u32)


class XView:
    def __init__(self, pool, base, mg):
        self.pool, self.base, self.mg = pool, base, mg

    def index(self, u, g, c):
        return self.base + (u * self.mg + g) * 4 + c

    def store(self, u, g, c, val):
        self.pool[self.index(u, g, c)] = val

    def load(self, u, zero=None):
        rows = []
        for g in range(self.mg):
            row = []
            for c in range(4):
                idx = self.index(u, g, c)
                if zero is not None and g == 0 and c == 0:
                    idx = idx + zero
                row.append(self.pool[idx])
            rows.append(jnp.concatenate(row, axis=1))
        return jnp.concatenate(rows, axis=0)


COST_F1, COST_F2, COST_I1, COST_I2, COST_ACT = 105, 152, 91, 52, 78
FWD_S1, _ = _fft64_signs(-1)
INV_S1, _INV_OUT = _fft64_signs(1, in_sign=Y_SIGN)
INV_S2 = {m: (v.r.s, v.i.s) for m, v in _INV_OUT.items()}
CLASSES = ((1, 7), (2, 6), (3, 5), (4, 0))


def _class_units(cls):
    ks = [k for k in range(1, 32) if k % 8 in cls or (-k) % 8 in cls]
    ks.sort(key=lambda k: (0 if k % 8 == cls[0] else 1, k))
    out = [("pair", k) for k in ks]
    if 0 in cls:
        out += [("real", 0), ("real", 32)]
    return out


def fwd_p1(load, t_ref, h, n2, ct, pc):
    xs = []
    for n1 in range(8):
        w = load(h, 8 * n1 + n2, ct)
        if n1 == 0:
            w = pc.here(w)
        lo, hi = _unpack(w)
        xs.append(C(V(lo), V(hi)))
    a = fft8(xs, -1)
    for k1 in range(8):
        t = a[k1].mul_w(-n2 * k1, 64)
        assert (t.r.s, t.i.s) == FWD_S1[k1, n2]
        t_ref[h, (k1 * 8 + n2) * 2] = t.r.a
        t_ref[h, (k1 * 8 + n2) * 2 + 1] = t.i.a
    return COST_F1


def fwd_p2(t_ref, x_ref, g, ct, k1, pc):
    outs = []
    for h in range(2):
        xs = [C(V(t_ref[h, (k1 * 8 + n2) * 2], FWD_S1[k1, n2][0]),
                V(t_ref[h, (k1 * 8 + n2) * 2 + 1], FWD_S1[k1, n2][1])) for n2 in range(8)]
        if h == 0:
            xs[0].r.a = pc.here(xs[0].r.a)
        outs.append(fft8(xs, -1))
    for k2 in range(8):
        m = k1 + 8 * k2
        f0 = _lhs_forms(m, outs[0][k2])
        f1 = _lhs_forms(m, outs[1][k2])
        for i, ((u, half, v0), (_, _, v1)) in enumerate(zip(f0, f1)):
            assert v0.s == v1.s == LHS_SIGN[u, half]
            x_ref.store(u, g, 2 * half + ct, _pack(v0.a, v1.a))
    return COST_F2


def inv_p1(y_ref, t_ref, g, h, n2, pc):
    rows = pl.ds(g * 16 + 8 * h, 8)
    ysg = Y_SIGN
    xs = []
    for n1 in range(8):
        m = 8 * n1 + n2
        xs.append(C(V(y_ref[2 * m, rows, :], ysg.get((m, 0), 1)),
                    V(y_ref[2 * m + 1, rows, :], ysg.get((m, 1), 1))))
    xs[0].r.a = pc.here(xs[0].r.a)
    a = fft8(xs, 1)
    for k1 in range(8):
        t = a[k1].mul_w(n2 * k1, 64)
        assert (t.r.s, t.i.s) == INV_S1[k1, n2]
        t_ref[h, (k1 * 8 + n2) * 2] = t.r.a
        t_ref[h, (k1 * 8 + n2) * 2 + 1] = t.i.a
    return COST_I1


def inv_p2(t_ref, r_ref, h, k1, pc):
    xs = [C(V(t_ref[h, (k1 * 8 + n2) * 2], INV_S1[k1, n2][0]),
            V(t_ref[h, (k1 * 8 + n2) * 2 + 1], INV_S1[k1, n2][1])) for n2 in range(8)]
    xs[0].r.a = pc.here(xs[0].r.a)
    b = fft8(xs, 1, range(S // 8))
    for k2 in range(S // 8):
        assert (b[k2].r.s, b[k2].i.s) == INV_S2[k1 + 8 * k2]
        r_ref[h, (k1 * 6 + k2) * 2] = b[k2].r.a
        r_ref[h, (k1 * 6 + k2) * 2 + 1] = b[k2].i.a
    return COST_I2


def _act(r_ref, h, k1, k2, dt, first, pc):
    a = r_ref[h, (k1 * 6 + k2) * 2 + dt]
    if first:
        a = pc.here(a)
    return _gelu_half(V(a, INV_S2[k1 + 8 * k2][dt]))


def act_conv1(r_ref, zh_ref, tau0, q, pc):
    h, k1, part = q // 8, 2 * ((q % 8) // 2), q % 2
    first = True
    for k2 in range(3 * part, 3 * part + 3):
        for dt in range(2):
            ev = _act(r_ref, h, k1, k2, dt, first, pc)
            od = _act(r_ref, h, k1 + 1, k2, dt, False, pc)
            first = False
            zh_ref[tau0 + (k1 // 2 + 4 * k2), h, :, _lanes(dt)] = pc.due(_pack(ev, od))
    return COST_ACT


def act_conv2(r_ref, f_ref, tau0, q, pc):
    k1, part = q // 2, q % 2
    first = True
    for k2 in range(3 * part, 3 * part + 3):
        for dt in range(2):
            oa = _act(r_ref, 0, k1, k2, dt, first, pc)
            ob = _act(r_ref, 1, k1, k2, dt, False, pc)
            first = False
            f_ref[tau0 + (k1 + 8 * k2), :, _lanes(dt)] = pc.due(_pack(oa, ob))
    return COST_ACT


def inverse_tail(t_ref, r_ref, act, pc, pairs_in_time):
    P = functools.partial
    out = []
    if pairs_in_time:
        for h in range(2):
            for kp in range(4):
                out += [(P(inv_p2, t_ref, r_ref, h, 2 * kp + j, pc), COST_I2) for j in range(2)]
                out += [(P(act, h * 8 + kp * 2 + j, pc), COST_ACT) for j in range(2)]
    else:
        for k1 in range(8):
            out += [(P(inv_p2, t_ref, r_ref, h, k1, pc), COST_I2) for h in range(2)]
            out += [(P(act, k1 * 2 + j, pc), COST_ACT) for j in range(2)]
    return out


def _mm(x_ref, u_ref, j, pc=None):
    opaque = pc is not None and pc.unit % OPQ_EVERY == 0
    a = x_ref.load(j, pc.zero if opaque else None)
    if pc is not None:
        a = pc.gate(a)
    a = pltpu.bitcast(a, bf16)
    w = pltpu.bitcast(u_ref[j], bf16)
    return jnp.dot(a, w, preferred_element_type=f32)


def _tokens(y):
    m = y.shape[0]
    return [y[8 * r:8 * r + 8, 128 * n:128 * n + 128] for n in range(2) for r in range(m // 8)]


def matmul_stream(x_ref, u_ref, y_ref, pc=None):
    def tiles(y, u):
        return [V(y[:, :128], COL_SIGN[u, 0]), V(y[:, 128:], COL_SIGN[u, 1])]

    for cls in CLASSES:
        for kind, k in _class_units(cls):
            if kind == "pair":
                j = (k - 1) * 3
                y1 = _mm(x_ref, u_ref, j, pc)
                k1 = tiles(y1, j)
                yield _tokens(y1)
                y2 = _mm(x_ref, u_ref, j + 1, pc)
                k2 = tiles(y2, j + 1)
                for nt, m in ((0, k), (1, 64 - k)):
                    yi = k1[nt] + k2[nt]
                    assert (yi.s if nt == 0 else -yi.s) == Y_SIGN[m, 1]
                    y_ref[2 * m + 1] = yi.a
                yield _tokens(y2)
                y3 = _mm(x_ref, u_ref, j + 2, pc)
                k3 = tiles(y3, j + 2)
                for nt, m in ((0, k), (1, 64 - k)):
                    yr = k1[nt] - k3[nt]
                    assert yr.s == Y_SIGN[m, 0]
                    y_ref[2 * m] = yr.a
                yield _tokens(y3)
            else:
                y = _mm(x_ref, u_ref, UNIT0 if k == 0 else UNIT32, pc)
                y_ref[2 * k] = y[:, :128]
                y_ref[2 * k + 1] = y[:, 128:]
                yield _tokens(y)


def run_step(mm, pieces, costs, pc, ntok, lead, lag=None, due=None):
    total = float(sum(costs))
    lag = LAG if lag is None else lag
    tokens = []
    marks = []
    c = 0.0
    for piece, cost in zip(pieces, costs):
        pc.tok = None
        pc.tok2 = marks[-lag] if lag and len(marks) >= lag else None
        if c >= lead:
            want = min(int((c - lead) / (total - lead) * ntok), ntok - 1)
            ahead = min(want + AHEAD * (ntok // NUNITS), ntok - 1)
            while ahead >= len(tokens):
                tokens += next(mm)
            pc.tok = tokens[want]
        pc.outs = []
        piece()
        marks.append(pc.last)
        for i, v in enumerate(pc.outs):
            q = pc.unit + (DUE if due is None else due) + i // 4
            if q < NUNITS:
                pc.pending.append((q, v))
        c += cost
    pc.tok = pc.tok2 = None
    for _ in mm:
        pass


def _make_kernel(T):
    T1, T2 = T // 2, T // 4
    L1 = (T1 + 16) // SEG
    L2 = L1 // 2
    assert L1 * SEG == T1 + 16 and L1 % 2 == 0
    NB1 = -(-L1 // S)
    NB2 = -(-L2 // S)
    XPAD = 8
    XB = T1 + 16
    XROWS = XPAD + 2 * XB + 64
    MG = 3
    M = 16 * MG
    NC1 = -(-NB1 // MG)
    NC2 = -(-NB2 // MG)
    ZH = (NB2 - 1) * S + N
    ZDUMP = ZH
    TB = 56
    NCH = -(-L2 // TB)
    FROWS = max(NB2 * S, NCH * TB)
    FDUMP = FROWS
    last_valid = T2 - (SEG - 1) * L2
    XPART = (0, 304, 592)

    def x_rows(e, part):
        def start(e, part):
            if e >= SEG:
                return T1
            return max(L1 * e + XPART[part] - (8 if part == 0 else 0), 0) // 8 * 8
        if part + 1 < len(XPART):
            return start(e, part), start(e, part + 1)
        return start(e, part), start(e + 1, 0)

    def kernel(x_hbm, w1_hbm, w2_hbm, g_ref, wf_ref, wg_ref, wo_ref, o_hbm,
               xs0, xs1, w_ref, u_ref, pool, y_ref, zh_ref, f_ref, fe_ref, ge_ref,
               st_ref, sem_w, sem_x, sem_o):
        xs = (xs0, xs1)
        x_ref = XView(pool, 0, MG)
        tf = [[View(pool, NUNITS * MG * 4 + (g * 2 + ct) * 256) for ct in range(2)] for g in range(MG)]
        ti = [View(pool, NUNITS * MG * 4 + MG * 512 + g * 256) for g in range(MG)]
        tr = [View(pool, NUNITS * MG * 4 + MG * 768 + g * 256) for g in range(MG)]
        xh = x_hbm.bitcast(u32)
        w1w = w1_hbm.bitcast(u32)
        w2w = w2_hbm.bitcast(u32)

        def w1_copy(q):
            rows = pl.ds(32 * q, 32)
            return pltpu.make_async_copy(w1w.at[:, rows, :], w_ref.at[0, :, rows, :], sem_w.at[q])

        w2_copy = pltpu.make_async_copy(w2w, w_ref.at[1], sem_w.at[4])

        def x_copies(part):
            cps = []
            for b in range(2):
                for e in range(SEG):
                    lo, hi = x_rows(e, part)
                    for ct in range(2):
                        cps.append(pltpu.make_async_copy(
                            xh.at[b, pl.ds(lo, hi - lo), _lanes(ct)],
                            xs[ct].at[pl.ds(XPAD + b * XB + lo, hi - lo), :],
                            sem_x.at[part]))
            return cps

        w1_copy(0).start()
        w1_copy(1).start()

        z8 = jnp.zeros((8, 128), u32)
        for ct in range(2):
            xs[ct][pl.ds(0, 8), :] = z8
            for r in range(XPAD + T1, XPAD + XB, 8):
                xs[ct][pl.ds(r, 8), :] = z8
            for r in range(XPAD + XB + T1, XROWS, 8):
                xs[ct][pl.ds(r, 8), :] = z8

        def zero_zh(i, c):
            for h in range(2):
                zh_ref[ZH - 1 - i, h] = jnp.zeros((8, 256), u32)
            return c
        lax.fori_loop(0, ZH - 8 - L2, zero_zh, 0)

        def zero_y(i, c):
            y_ref[i] = jnp.zeros((M, 128), f32)
            return c
        lax.fori_loop(0, 128, zero_y, 0)

        def zero_t(i, c):
            for h in range(2):
                for g in range(MG):
                    pool[NUNITS * MG * 4 + MG * 512 + g * 256 + h * 128 + i] = jnp.zeros((8, 128), u32)
            return c
        lax.fori_loop(0, 128, zero_t, 0)

        gg = g_ref[...].reshape(16, 256)
        ge_all = jnp.dot(gg, wg_ref[...], preferred_element_type=f32)
        ge_ref[...] = ge_all

        def transform(slot, hook=None):
            def body(rg, c):
                if hook is not None:
                    hook(rg)
                weight_transform(w_ref.at[slot], u_ref, tf[0][0], tf[0][1], rg)
                return c
            lax.fori_loop(0, 16, body, 0)

        def w1_hook(rg):
            for q in range(4):
                @pl.when(rg == 4 * q)
                def _(q=q):
                    w1_copy(q).wait()
                    if q + 2 < 4:
                        w1_copy(q + 2).start()
                    if q >= 1:
                        for cp in x_copies(q - 1):
                            cp.start()

        def conv(nchunk, nblk, make_load, act, pairs_in_time, out_index, wait_input=None):
            def loads(c):
                return [make_load(jnp.minimum(c * MG + g, nblk - 1)) for g in range(MG)]

            def P(fn, *a):
                return functools.partial(fn, *a)

            def f1(ld, pc):
                return [(P(fwd_p1, ld[g], tf[g][ct], h, n2, ct, pc), COST_F1)
                        for g in range(MG) for ct in range(2) for h in range(2) for n2 in range(8)]

            def f2(cls, pc):
                return [(P(fwd_p2, tf[g][ct], x_ref, g, ct, k1, pc), COST_F2)
                        for g in range(MG) for ct in range(2) for k1 in cls]

            def i1(cls, pc):
                return [(P(inv_p1, y_ref, ti[g], g, h, n2, pc), COST_I1)
                        for g in range(MG) for h in range(2) for n2 in cls]

            def i2(c, pc):
                out = []
                for g in range(MG):
                    out += inverse_tail(ti[g], tr[g], P(act, tr[g], out_index(c, g)), pc, pairs_in_time)
                return out

            idle = Pacer(None)
            if wait_input is not None:
                wait_input(0)
            with scope("pro"):
                for piece, _ in f1(loads(0), idle):
                    piece()
                for cls in CLASSES[:3]:
                    for piece, _ in f2(cls, idle):
                        piece()

            def step(c, cc):
                if wait_input is not None:
                    wait_input(c + 1)
                pc = Pacer(c < 0, lax.shift_right_arithmetic(c, 20))
                nxt = f1(loads(jnp.minimum(c + 1, nchunk - 1)), pc)
                half = len(nxt) // 2
                seq = (i1(CLASSES[3], pc) + f2(CLASSES[3], pc) + i2(c - 1, pc)
                       + nxt[:half] + i1(CLASSES[0], pc) + nxt[half:]
                       + f2(CLASSES[0], pc) + i1(CLASSES[1], pc) + f2(CLASSES[1], pc)
                       + i1(CLASSES[2], pc) + f2(CLASSES[2], pc))
                run_step(matmul_stream(x_ref, u_ref, y_ref, pc), [q[0] for q in seq], [q[1] for q in seq],
                         pc, NUNITS * (M // 4), LEAD)
                return cc
            with scope("steps"):
                lax.fori_loop(0, nchunk, step, 0)

            with scope("epi"):
                for piece, _ in i1(CLASSES[3], idle) + i2(nchunk - 1, idle):
                    piece()

        with scope("wt1"):
            transform(0, w1_hook)

        def wait_x0(c):
            if isinstance(c, int):
                for cp in x_copies(0):
                    cp.wait()
                return
            for part, first in ((1, 2), (2, 4)):
                @pl.when(c == first)
                def _(part=part):
                    for cp in x_copies(part):
                        cp.wait()

            @pl.when(c == 2)
            def _():
                w2_copy.start()

        def load1(blk):
            base = blk * S

            def load(h, n, ct):
                return xs[ct][pl.ds(base + n + h * L1, 8, stride=2 * L1), :]
            return load

        def act1(rb, tau0, q, pc):
            return act_conv1(rb, zh_ref, tau0, q, pc)

        def out1(c, g):
            if isinstance(c, int):
                return 8 + (c * MG + g) * (S // 2)
            return jnp.where(c >= 0, 8 + (c * MG + g) * (S // 2), ZDUMP + g * (S // 2))

        conv(NC1, NB1, load1, act1, True, out1, wait_x0)

        row = lax.broadcasted_iota(i32, (8, 256), 0)
        for h in range(2):
            for t in range(last_valid, NB1 * S // 2):
                zh_ref[8 + t, h] = jnp.where(row == SEG - 1, jnp.uint32(0), zh_ref[8 + t, h])
            for j in range(8):
                v = pltpu.roll(zh_ref[8 + L2 - 8 + j, h], 1, axis=0)
                zh_ref[j, h] = jnp.where(row == 0, jnp.uint32(0), v)
            for j in range(8):
                v = pltpu.roll(zh_ref[8 + j, h], SEG - 1, axis=0)
                zh_ref[8 + L2 + j, h] = jnp.where(row == SEG - 1, jnp.uint32(0), v)

        w2_copy.wait()
        with scope("wt2"):
            transform(1)

        def load2(blk):
            def load(h, n, ct):
                return zh_ref[blk * S + n, h, :, _lanes(ct)]
            return load

        def act2(rb, tau0, q, pc):
            return act_conv2(rb, f_ref, tau0, q, pc)

        def out2(c, g):
            if isinstance(c, int):
                return min(c * MG + g, NB2 - 1) * S
            return jnp.where(c >= 0, jnp.minimum(c * MG + g, NB2 - 1) * S, FDUMP + g * S)

        conv(NC2, NB2, load2, act2, False, out2)

        never = jnp.max(jnp.abs(ge_all)) < 0.0
        order = [(b, e) for b in range(2) for e in range(SEG)]

        def out_copy(half, q, t0, nvalid):
            b, e = order[q]
            r0 = (b * T2 + e * L2) * 8 + t0 * 8
            return pltpu.make_async_copy(st_ref.at[half, q, pl.ds(0, nvalid * 8), :],
                                         o_hbm.at[pl.ds(r0, nvalid * 8), :],
                                         sem_o.at[half])

        def width(e):
            lim = L2 if e < SEG - 1 else last_valid
            return lim - (NCH - 1) * TB

        def joint_chunk(ch, half, full, never):
            pc = Pacer(never)
            t0 = ch * TB
            fl = pltpu.bitcast(f_ref[pl.ds(t0, TB)].reshape(TB * 8, 256), bf16)
            fe = jnp.dot(fl, wf_ref[...], preferred_element_type=f32)
            fe_ref[...] = fe
            prev = [fe[8 * r:8 * r + 8, 128 * n:128 * n + 128] for n in range(2) for r in range(2 * TB)]
            prev = prev[len(prev) // 2:]
            for q, (b, e) in enumerate(order):
                ge = ge_ref[pl.ds(8 * b, 8), :]
                r = 4 * (e & 3) + 2 * b + (e >> 2)
                js = []
                for t in range(TB):
                    row = jnp.broadcast_to(fe_ref[pl.ds(16 * t + r, 1), :], (8, 256))
                    tok = prev[(t * len(prev)) // TB]
                    gt = jnp.concatenate([pc.tie(ge[:, :128], tok), pc.tie(ge[:, 128:], tok)], axis=1)
                    js.append(jnp.tanh(row + gt))
                jl = jnp.concatenate(js, axis=0).astype(bf16)
                y = jnp.dot(jl, wo_ref[...], preferred_element_type=f32)
                prev = [y[8 * rr:8 * rr + 8, 128 * n:128 * n + 128] for n in range(2) for rr in range(TB)]
                st_ref[half, q] = y.astype(bf16)
                out_copy(half, q, t0, TB if full else width(e)).start()

        def wait_chunk(half, full):
            for q, (b, e) in enumerate(order):
                out_copy(half, q, 0, TB if full else width(e)).wait()

        def joint_body(ch, c):
            half = ch % 2

            @pl.when(ch >= 2)
            def _():
                wait_chunk(half, True)
            joint_chunk(ch, half, True, ch < 0)
            return c
        with scope("joint"):
            lax.fori_loop(0, NCH - 1, joint_body, 0)
            last_half = (NCH - 1) % 2
            wait_chunk(last_half, True)
            joint_chunk(NCH - 1, last_half, False, never)
            wait_chunk(1 - last_half, True)
            wait_chunk(last_half, False)

    scratch = [
        pltpu.VMEM((XROWS, 128), u32), pltpu.VMEM((XROWS, 128), u32),
        pltpu.VMEM((2, 31, 128, 256), u32),
        pltpu.VMEM((NUNITS, 256, 256), u32),
        pltpu.VMEM((NUNITS * MG * 4 + MG * 1024, 8, 128), u32),
        pltpu.VMEM((128, M, 128), f32),
        pltpu.VMEM((ZH + MG * S // 2, 2, 8, 256), u32),
        pltpu.VMEM((FROWS + MG * S, 8, 256), u32),
        pltpu.VMEM((TB * 16, 256), f32),
        pltpu.VMEM((16, 256), f32),
        pltpu.VMEM((2, 2 * SEG, TB * 8, 256), bf16),
        pltpu.SemaphoreType.DMA((5,)),
        pltpu.SemaphoreType.DMA((3,)),
        pltpu.SemaphoreType.DMA((2,)),
    ]
    return kernel, scratch


LEAD = 0
LAG = 0
AHEAD = 3
OPQ_EVERY = 1
DUE = 2
DUE_EVERY = 1000


def _call(x, w1, w2, g, w_f, w_g, w_o, interpret=False):
    B, T, D = x.shape
    kernel, scratch = _make_kernel(T)
    T2 = T // 4
    any_spec = pl.BlockSpec(memory_space=pl.ANY)
    vmem = pl.BlockSpec(memory_space=pltpu.VMEM)
    out = pl.pallas_call(
        kernel,
        out_shape=jax.ShapeDtypeStruct((B * T2 * 8, D), bf16),
        in_specs=[any_spec, any_spec, any_spec, vmem, vmem, vmem, vmem],
        out_specs=any_spec,
        scratch_shapes=scratch,
        compiler_params=pltpu.CompilerParams(vmem_limit_bytes=126 * 2**20),
        interpret=interpret,
        name="conv_stem_rnnt_joint",
    )(x, w1, w2, g, w_f, w_g, w_o)
    return out.reshape(B, T2, 8, D)


@jax.jit
def pallas_standalone__seq2seq_rnn_t_joint__speech_kernel(x, w1, w2, g, w_f, w_g, w_o):
    return _call(x, w1, w2, g, w_f, w_g, w_o)
```

```python
import functools
import math

import jax
import jax.numpy as jnp
import numpy as np
from jax import lax
from jax.experimental import pallas as pl
from jax.experimental.pallas import tpu as pltpu

f32, u32, bf16, i32 = jnp.float32, jnp.uint32, jnp.bfloat16, jnp.int32

PROFILE_SCOPES = False


class _NoScope:
    def __enter__(self):
        return self

    def __exit__(self, *a):
        return False


def scope(name):
    return jax.named_scope(name) if PROFILE_SCOPES else _NoScope()

N = 64
S = 48
SEG = 8


class V:
    __slots__ = ("a", "s")

    def __init__(self, a, s=1):
        self.a = a
        self.s = s

    def __neg__(self):
        return V(self.a, -self.s)

    def __add__(self, o):
        if self.s == o.s:
            return V(self.a + o.a, self.s)
        if self.s > 0:
            return V(self.a - o.a, 1)
        return V(o.a - self.a, 1)

    def __sub__(self, o):
        return self + (-o)

    def scale(self, c):
        if c == 1.0:
            return self
        if c == -1.0:
            return -self
        return V(self.a * np.float32(abs(c)), self.s * (1 if c > 0 else -1))

    def times(self, c):
        return self.a * np.float32(self.s * c)

    def signed(self, s):
        return self.a if self.s * s > 0 else -self.a


class C:
    __slots__ = ("r", "i")

    def __init__(self, r, i):
        self.r = r
        self.i = i

    def __add__(self, o):
        return C(self.r + o.r, self.i + o.i)

    def __sub__(self, o):
        return C(self.r - o.r, self.i - o.i)

    def __neg__(self):
        return C(-self.r, -self.i)

    def mul_w(self, num, den):
        num %= den
        if num == 0:
            return self
        if 4 * num == den:
            return C(-self.i, self.r)
        if 2 * num == den:
            return -self
        if 4 * num == 3 * den:
            return C(self.i, -self.r)
        if (8 * num) % den == 0:
            o = (8 * num) // den
            h = math.sqrt(0.5)
            sc = 1 if o in (1, 7) else -1
            ss = 1 if o in (1, 3) else -1
            r, m = self.r, self.i
            re = (r if sc > 0 else -r) - (m if ss > 0 else -m)
            im = (r if ss > 0 else -r) + (m if sc > 0 else -m)
            return C(re.scale(h), im.scale(h))
        c = math.cos(2 * math.pi * num / den)
        s = math.sin(2 * math.pi * num / den)
        return C(self.r.scale(c) - self.i.scale(s), self.r.scale(s) + self.i.scale(c))


def _add(a, b):
    if a is None:
        return b
    if b is None:
        return a
    return a + b


def _sub(a, b):
    if b is None:
        return a
    if a is None:
        return -b
    return a - b


def fft8(x, sgn, need=tuple(range(8))):
    def rot(a, num, den):
        return None if a is None else a.mul_w(sgn * num, den)

    need = set(need)
    a0, a1 = _add(x[0], x[4]), _sub(x[0], x[4])
    a2, a3 = _add(x[2], x[6]), rot(_sub(x[2], x[6]), 1, 4)
    a4, a5 = _add(x[1], x[5]), _sub(x[1], x[5])
    a6, a7 = _add(x[3], x[7]), rot(_sub(x[3], x[7]), 1, 4)
    out = {}
    if need & {0, 4}:
        b0, b4 = _add(a0, a2), _add(a4, a6)
        if 0 in need:
            out[0] = _add(b0, b4)
        if 4 in need:
            out[4] = _sub(b0, b4)
    if need & {2, 6}:
        b2, b6 = _sub(a0, a2), rot(_sub(a4, a6), 1, 4)
        if 2 in need:
            out[2] = _add(b2, b6)
        if 6 in need:
            out[6] = _sub(b2, b6)
    if need & {1, 5}:
        b1, b5 = _add(a1, a3), rot(_add(a5, a7), 1, 8)
        if 1 in need:
            out[1] = _add(b1, b5)
        if 5 in need:
            out[5] = _sub(b1, b5)
    if need & {3, 7}:
        b3, b7 = _sub(a1, a3), rot(_sub(a5, a7), 3, 8)
        if 3 in need:
            out[3] = _add(b3, b7)
        if 7 in need:
            out[7] = _sub(b3, b7)
    return out


class _Sym:
    def __add__(self, o):
        return self

    __sub__ = __mul__ = __add__

    def __neg__(self):
        return self


def _fft64_signs(sgn, present=tuple(range(64)), in_sign=None):
    d = _Sym()
    in_sign = in_sign or {}
    x = [C(V(d, in_sign.get((n, 0), 1)), V(d, in_sign.get((n, 1), 1))) if n in present else None
         for n in range(64)]
    t = {}
    for n2 in range(8):
        a = fft8([x[8 * n1 + n2] for n1 in range(8)], sgn)
        for k1 in range(8):
            t[k1, n2] = a[k1].mul_w(sgn * n2 * k1, 64)
    s1 = {key: (v.r.s, v.i.s) for key, v in t.items()}
    s2 = {}
    for k1 in range(8):
        b = fft8([t[k1, n2] for n2 in range(8)], sgn)
        for k2 in range(8):
            s2[k1 + 8 * k2] = b[k2]
    return s1, s2


def _unit(k, j):
    return (k - 1) * 3 + j


UNIT0, UNIT32 = 93, 94
NUNITS = 95


def _lhs_forms(m, z):
    if m in (0, 32):
        u = UNIT0 if m == 0 else UNIT32
        return [(u, 0, z.r), (u, 1, z.i)]
    if m < 32:
        return [(_unit(m, 0), 0, z.r + z.i), (_unit(m, 1), 0, z.r), (_unit(m, 2), 0, z.i)]
    k = 64 - m
    return [(_unit(k, 0), 1, z.r - z.i), (_unit(k, 1), 1, z.r), (_unit(k, 2), 1, z.i)]


def _lhs_signs():
    _, s2 = _fft64_signs(-1)
    sg = {}
    for m in range(64):
        for u, h, v in _lhs_forms(m, s2[m]):
            sg[u, h] = v.s
    return sg


LHS_SIGN = _lhs_signs()


def _weight_forms(m, pm):
    if m < 32:
        nt = 0 if pm > 0 else 1
        return [(_unit(m, 0), 1, nt, (1, 0)), (_unit(m, 1), 1, nt, (-1, 1)), (_unit(m, 2), 1, nt, (-1, -1))]
    k = 64 - m
    nt = 1 if pm > 0 else 0
    return [(_unit(k, 0), 0, nt, (1, 0)), (_unit(k, 1), 0, nt, (-1, -1)), (_unit(k, 2), 0, nt, (1, -1))]


def _weight_plan():
    s1, s2 = _fft64_signs(1, present=range(16))
    forms = {}
    for pm in (1, -1):
        for m in range(1, 64):
            if m == 32:
                continue
            for u, half, nt, (cr, ci) in _weight_forms(m, pm):
                forms[u, half, nt] = (cr * s2[m].r.s, ci * s2[m].i.s)
    col = {}
    for u in range(93):
        for nt in range(2):
            def negs(sig):
                n = 0
                for half in range(2):
                    cr, ci = forms[u, half, nt]
                    w = sig * LHS_SIGN[u, half]
                    n += (w * cr <= 0 and w * ci <= 0)
                return n
            col[u, nt] = 1 if negs(1) <= negs(-1) else -1
    for u in (UNIT0, UNIT32):
        col[u, 0] = col[u, 1] = 1
    return s1, s2, col


WT_S1, WT_S2, COL_SIGN = _weight_plan()


def _recombine(k1, k2, k3, k):
    out = {}
    for nt in range(2):
        yr = k1[nt] - k3[nt]
        yi = k1[nt] + k2[nt]
        if nt == 0:
            out[k, 0], out[k, 1] = yr, yi
        else:
            out[64 - k, 0], out[64 - k, 1] = yr, -yi
    return out


def _y_signs():
    d = _Sym()
    sg = {}
    for k in range(1, 32):
        ks = [[V(d, COL_SIGN[_unit(k, j), nt]) for nt in range(2)] for j in range(3)]
        for key, v in _recombine(ks[0], ks[1], ks[2], k).items():
            sg[key] = v.s
    for m, u in ((0, UNIT0), (32, UNIT32)):
        sg[m, 0], sg[m, 1] = COL_SIGN[u, 0], COL_SIGN[u, 1]
    return sg


Y_SIGN = _y_signs()


def _unpack(w):
    lo = pltpu.unpack_elementwise(w, index=0, packed_dtype=bf16, unpacked_dtype=f32)
    hi = pltpu.unpack_elementwise(w, index=1, packed_dtype=bf16, unpacked_dtype=f32)
    return lo, hi


def _pack(lo, hi):
    return pltpu.pack_elementwise([lo, hi], packed_dtype=bf16)


_GC1 = 2.0 * math.sqrt(2.0 / math.pi)
_GC2 = 8.0 * 0.044715 * math.sqrt(2.0 / math.pi)


def _gelu_half(v):
    a = v.a
    p = (a * a) * np.float32(_GC2) + np.float32(_GC1)
    t = jnp.tanh(p * a)
    return a * t + a if v.s > 0 else a * t - a


def _lanes(t):
    return pl.ds(128 * t, 128)


class Pacer:
    def __init__(self, never, zero=None):
        self.never = never
        self.tok = None
        self.tok2 = None
        self.last = None
        self.outs = []
        self.zero = zero
        self.pending = []
        self.unit = 0

    def gate(self, a):
        vals = [v for q, v in self.pending if q <= self.unit]
        self.pending = [(q, v) for q, v in self.pending if q > self.unit]
        self.unit += 1
        if not vals:
            return a
        m, k = a.shape
        tiles = [[a[8 * r:8 * r + 8, 128 * c:128 * c + 128] for c in range(k // 128)] for r in range(m // 8)]
        flat = [(r, c) for r in range(m // 8) for c in range(k // 128)]
        for i, v in enumerate(vals):
            r, c = flat[i % len(flat)]
            tiles[r][c] = self.tie(tiles[r][c], v)
        return jnp.concatenate([jnp.concatenate(row, axis=1) for row in tiles], axis=0)

    def here(self, x):
        tok, self.tok = self.tok, None
        tok2, self.tok2 = self.tok2, None
        return self.tie(self.tie(x, tok), tok2)

    def mark(self, x, nth=None):
        self.last = x
        if self.never is not None and nth is not None and nth % DUE_EVERY == DUE_EVERY - 1:
            self.outs.append(x)
        return x

    def due(self, x):
        if self.never is not None:
            self.outs.append(x)
        return x

    def tie(self, x, tok):
        if tok is None:
            return x
        if tok.dtype != x.dtype:
            tok = pltpu.bitcast(tok, x.dtype)
        return jnp.where(self.never, tok, x)


def _combo(f, cr, ci, want):
    if ci == 0:
        return f.r.signed(want * cr)
    v = (f.r if cr > 0 else -f.r) + (f.i if ci > 0 else -f.i)
    if v.s * want > 0:
        return v.a
    if f.r.s * cr != f.i.s * ci:
        return ((-f.r) if cr > 0 else f.r).__add__((-f.i) if ci > 0 else f.i).a
    return -v.a


def weight_transform(w_ref, u_ref, t_ref, z_ref, rg):
    rows = pl.ds(pl.multiple_of(rg * 8, 8), 8)
    urow = (rows, pl.ds(pl.multiple_of(rg * 8 + 128, 8), 8))
    sigma = 1.0 / 256.0
    tau = 1.0 / 128.0

    def store(u, half, nt, a0, a1):
        u_ref[u, urow[half], _lanes(nt)] = _pack(a0, a1)

    acc = {}
    for d in range(16):
        wa = [[None, None], [None, None]]
        wb = [[None, None], [None, None]]
        for dt in range(2):
            if d > 0:
                lo, hi = _unpack(w_ref[2 * d - 1, rows, _lanes(dt)])
                wa[0][dt], wa[1][dt] = V(lo), V(hi)
            lo, hi = _unpack(w_ref[2 * d, rows, _lanes(dt)])
            wb[0][dt], wb[1][dt] = V(lo), V(hi)
        for p in range(2):
            for dt in range(2):
                for name, val in (("a", wa[p][dt]), ("b", wb[p][dt])):
                    key = (p, dt, name, d % 2)
                    acc[key] = _add(acc.get(key), val)
            zp = (_sub(wa[p][0], wb[p][1]), _add(wb[p][0], wa[p][1]))
            zm = (_add(wa[p][0], wb[p][1]), _sub(wb[p][0], wa[p][1]))
            for j, z in enumerate((zp, zm)):
                for comp in range(2):
                    z_ref[j, (p * 16 + d) * 2 + comp] = z[comp].times(sigma)
    for m, u in ((0, UNIT0), (32, UNIT32)):
        for dt in range(2):
            for half, name in enumerate(("a", "b")):
                vals = []
                for p in range(2):
                    ev, od = acc[p, dt, name, 0], acc[p, dt, name, 1]
                    v = _add(ev, od) if m == 0 else _sub(ev, od)
                    vals.append(v.times(tau * LHS_SIGN[u, half] * COL_SIGN[u, dt]))
                store(u, half, dt, vals[0], vals[1])

    for j, pm in enumerate((1, -1)):
        for p in range(2):
            for n2 in range(8):
                z = [C(V(z_ref[j, (p * 16 + d) * 2]), V(z_ref[j, (p * 16 + d) * 2 + 1])) for d in (n2, n2 + 8)]
                a = fft8(z + [None] * 6, 1)
                for k1 in range(8):
                    t = a[k1].mul_w(n2 * k1, 64)
                    assert (t.r.s, t.i.s) == WT_S1[k1, n2]
                    t_ref[p, (k1 * 8 + n2) * 2] = t.r.a
                    t_ref[p, (k1 * 8 + n2) * 2 + 1] = t.i.a
        for k1 in range(8):
            need = [k2 for k2 in range(8) if (k1 + 8 * k2) not in (0, 32)]
            outs = []
            for p in range(2):
                xs = [C(V(t_ref[p, (k1 * 8 + n2) * 2], WT_S1[k1, n2][0]),
                        V(t_ref[p, (k1 * 8 + n2) * 2 + 1], WT_S1[k1, n2][1])) for n2 in range(8)]
                outs.append(fft8(xs, 1, need))
            for k2 in need:
                m = k1 + 8 * k2
                for u, half, nt, (cr, ci) in _weight_forms(m, pm):
                    want = LHS_SIGN[u, half] * COL_SIGN[u, nt]
                    store(u, half, nt, _combo(outs[0][k2], cr, ci, want), _combo(outs[1][k2], cr, ci, want))


class View:
    def __init__(self, pool, base):
        self.pool = pool
        self.base = base

    def __getitem__(self, idx):
        h, i = idx
        return pltpu.bitcast(self.pool[self.base + h * 128 + i], f32)

    def __setitem__(self, idx, val):
        h, i = idx
        self.pool[self.base + h * 128 + i] = pltpu.bitcast(val, u32)


class XView:
    def __init__(self, pool, base, mg):
        self.pool, self.base, self.mg = pool, base, mg

    def index(self, u, g, c):
        return self.base + (u * self.mg + g) * 4 + c

    def store(self, u, g, c, val):
        self.pool[self.index(u, g, c)] = val

    def load(self, u, zero=None):
        rows = []
        for g in range(self.mg):
            row = []
            for c in range(4):
                idx = self.index(u, g, c)
                if zero is not None and g == 0 and c == 0:
                    idx = idx + zero
                row.append(self.pool[idx])
            rows.append(jnp.concatenate(row, axis=1))
        return jnp.concatenate(rows, axis=0)


_TW = (0, 42, 40, 42, 32, 42, 40, 42)
COST_F1 = tuple(73 + t for t in _TW)
COST_I1 = tuple(57 + t for t in _TW)
COST_F2, COST_I2, COST_ACT = 153, 53, 85
FWD_S1, _ = _fft64_signs(-1)
INV_S1, _INV_OUT = _fft64_signs(1, in_sign=Y_SIGN)
INV_S2 = {m: (v.r.s, v.i.s) for m, v in _INV_OUT.items()}
CLASSES = ((1, 7), (2, 6), (3, 5), (4, 0))


def _class_units(cls):
    ks = [k for k in range(1, 32) if k % 8 in cls or (-k) % 8 in cls]
    ks.sort(key=lambda k: (0 if k % 8 == cls[0] else 1, k))
    out = [("pair", k) for k in ks]
    if 0 in cls:
        out += [("real", 0), ("real", 32)]
    return out


def fwd_p1(load, t_ref, h, n2, ct, pc):
    xs = []
    for n1 in range(8):
        lo, hi = load(h, 8 * n1 + n2, ct, pc if n1 == 0 else None)
        xs.append(C(V(lo), V(hi)))
    a = fft8(xs, -1)
    for k1 in range(8):
        t = a[k1].mul_w(-n2 * k1, 64)
        assert (t.r.s, t.i.s) == FWD_S1[k1, n2]
        t_ref[h, (k1 * 8 + n2) * 2] = t.r.a
        t_ref[h, (k1 * 8 + n2) * 2 + 1] = t.i.a


def fwd_p2(t_ref, x_ref, g, ct, k1, pc):
    outs = []
    for h in range(2):
        xs = [C(V(t_ref[h, (k1 * 8 + n2) * 2], FWD_S1[k1, n2][0]),
                V(t_ref[h, (k1 * 8 + n2) * 2 + 1], FWD_S1[k1, n2][1])) for n2 in range(8)]
        if h == 0:
            xs[0].r.a = pc.here(xs[0].r.a)
        outs.append(fft8(xs, -1))
    for k2 in range(8):
        m = k1 + 8 * k2
        f0 = _lhs_forms(m, outs[0][k2])
        f1 = _lhs_forms(m, outs[1][k2])
        for i, ((u, half, v0), (_, _, v1)) in enumerate(zip(f0, f1)):
            assert v0.s == v1.s == LHS_SIGN[u, half]
            x_ref.store(u, g, 2 * half + ct, _pack(v0.a, v1.a))
    return COST_F2


def inv_p1(y_ref, t_ref, g, h, n2, pc):
    rows = pl.ds(g * 16 + 8 * h, 8)
    ysg = Y_SIGN
    xs = []
    for n1 in range(8):
        m = 8 * n1 + n2
        xs.append(C(V(y_ref[2 * m, rows, :], ysg.get((m, 0), 1)),
                    V(y_ref[2 * m + 1, rows, :], ysg.get((m, 1), 1))))
    xs[0].r.a = pc.here(xs[0].r.a)
    a = fft8(xs, 1)
    for k1 in range(8):
        t = a[k1].mul_w(n2 * k1, 64)
        assert (t.r.s, t.i.s) == INV_S1[k1, n2]
        t_ref[h, (k1 * 8 + n2) * 2] = t.r.a
        t_ref[h, (k1 * 8 + n2) * 2 + 1] = t.i.a


def inv_p2(t_ref, r_ref, h, k1, pc):
    xs = [C(V(t_ref[h, (k1 * 8 + n2) * 2], INV_S1[k1, n2][0]),
            V(t_ref[h, (k1 * 8 + n2) * 2 + 1], INV_S1[k1, n2][1])) for n2 in range(8)]
    xs[0].r.a = pc.here(xs[0].r.a)
    b = fft8(xs, 1, range(S // 8))
    for k2 in range(S // 8):
        assert (b[k2].r.s, b[k2].i.s) == INV_S2[k1 + 8 * k2]
        r_ref[h, (k1 * 6 + k2) * 2] = b[k2].r.a
        r_ref[h, (k1 * 6 + k2) * 2 + 1] = b[k2].i.a
    return COST_I2


def _act(r_ref, h, k1, k2, dt, first, pc):
    a = r_ref[h, (k1 * 6 + k2) * 2 + dt]
    if first:
        a = pc.here(a)
    return _gelu_half(V(a, INV_S2[k1 + 8 * k2][dt]))


def act_conv1(r_ref, zh_ref, tau0, q, pc):
    h, k1, part = q // 8, 2 * ((q % 8) // 2), q % 2
    first = True
    for k2 in range(3 * part, 3 * part + 3):
        for dt in range(2):
            ev = _act(r_ref, h, k1, k2, dt, first, pc)
            od = _act(r_ref, h, k1 + 1, k2, dt, False, pc)
            first = False
            zh_ref[tau0 + (k1 // 2 + 4 * k2), h, 0, :, _lanes(dt)] = pc.due(ev)
            zh_ref[tau0 + (k1 // 2 + 4 * k2), h, 1, :, _lanes(dt)] = pc.due(od)
    return COST_ACT


def act_conv2(r_ref, f_ref, tau0, q, pc):
    k1, part = q // 2, q % 2
    first = True
    for k2 in range(3 * part, 3 * part + 3):
        for dt in range(2):
            oa = _act(r_ref, 0, k1, k2, dt, first, pc)
            ob = _act(r_ref, 1, k1, k2, dt, False, pc)
            first = False
            f_ref[tau0 + (k1 + 8 * k2), :, _lanes(dt)] = pc.due(_pack(oa, ob))
    return COST_ACT


def inverse_tail(t_ref, r_ref, act, pc, pairs_in_time):
    P = functools.partial
    out = []
    if pairs_in_time:
        for h in range(2):
            for kp in range(4):
                out += [(P(inv_p2, t_ref, r_ref, h, 2 * kp + j, pc), COST_I2) for j in range(2)]
                out += [(P(act, h * 8 + kp * 2 + j, pc), COST_ACT) for j in range(2)]
    else:
        for k1 in range(8):
            out += [(P(inv_p2, t_ref, r_ref, h, k1, pc), COST_I2) for h in range(2)]
            out += [(P(act, k1 * 2 + j, pc), COST_ACT) for j in range(2)]
    return out


def _mm(x_ref, u_ref, j, pc=None):
    opaque = pc is not None and pc.unit % OPQ_EVERY == 0
    a = x_ref.load(j, pc.zero if opaque else None)
    if pc is not None:
        a = pc.gate(a)
    a = pltpu.bitcast(a, bf16)
    w = pltpu.bitcast(u_ref[j], bf16)
    return jnp.dot(a, w, preferred_element_type=f32)


def _tokens(y):
    m = y.shape[0]
    return [y[8 * r:8 * r + 8, 128 * n:128 * n + 128] for n in range(2) for r in range(m // 8)]


def matmul_stream(x_ref, u_ref, y_ref, pc=None):
    def tiles(y, u):
        return [V(y[:, :128], COL_SIGN[u, 0]), V(y[:, 128:], COL_SIGN[u, 1])]

    for cls in CLASSES:
        for kind, k in _class_units(cls):
            if kind == "pair":
                j = (k - 1) * 3
                y1 = _mm(x_ref, u_ref, j, pc)
                k1 = tiles(y1, j)
                yield _tokens(y1)
                y2 = _mm(x_ref, u_ref, j + 1, pc)
                k2 = tiles(y2, j + 1)
                for nt, m in ((0, k), (1, 64 - k)):
                    yi = k1[nt] + k2[nt]
                    assert (yi.s if nt == 0 else -yi.s) == Y_SIGN[m, 1]
                    y_ref[2 * m + 1] = yi.a
                yield _tokens(y2)
                y3 = _mm(x_ref, u_ref, j + 2, pc)
                k3 = tiles(y3, j + 2)
                for nt, m in ((0, k), (1, 64 - k)):
                    yr = k1[nt] - k3[nt]
                    assert yr.s == Y_SIGN[m, 0]
                    y_ref[2 * m] = yr.a
                yield _tokens(y3)
            else:
                y = _mm(x_ref, u_ref, UNIT0 if k == 0 else UNIT32, pc)
                y_ref[2 * k] = y[:, :128]
                y_ref[2 * k + 1] = y[:, 128:]
                yield _tokens(y)


def run_step(mm, pieces, costs, pc, ntok, lead, lag=None, due=None):
    total = float(sum(costs))
    lag = LAG if lag is None else lag
    tokens = []
    marks = []
    c = 0.0
    for piece, cost in zip(pieces, costs):
        pc.tok = None
        pc.tok2 = marks[-lag] if lag and len(marks) >= lag else None
        if c >= lead:
            want = min(int((c - lead) / (total - lead) * ntok), ntok - 1)
            ahead = min(want + AHEAD * (ntok // NUNITS), ntok - 1)
            while ahead >= len(tokens):
                tokens += next(mm)
            pc.tok = tokens[want]
        pc.outs = []
        piece()
        marks.append(pc.last)
        for i, v in enumerate(pc.outs):
            q = pc.unit + (DUE if due is None else due) + i // 4
            if q < NUNITS:
                pc.pending.append((q, v))
        c += cost
    pc.tok = pc.tok2 = None
    for _ in mm:
        pass


def _make_kernel(T):
    T1, T2 = T // 2, T // 4
    L1 = (T1 + 16) // SEG
    L2 = L1 // 2
    assert L1 * SEG == T1 + 16 and L1 % 2 == 0
    NB1 = -(-L1 // S)
    NB2 = -(-L2 // S)
    XPAD = 8
    XB = T1 + 16
    XROWS = XPAD + 2 * XB + 64
    MG = 3
    M = 16 * MG
    NC1 = -(-NB1 // MG)
    NC2 = -(-NB2 // MG)
    ZH = (NB2 - 1) * S + N
    ZDUMP = ZH
    TB = 56
    NCH = -(-L2 // TB)
    FROWS = max(NB2 * S, NCH * TB)
    FDUMP = FROWS
    last_valid = T2 - (SEG - 1) * L2
    XPART = (0, 304, 592)

    def x_rows(e, part):
        def start(e, part):
            if e >= SEG:
                return T1
            return max(L1 * e + XPART[part] - (8 if part == 0 else 0), 0) // 8 * 8
        if part + 1 < len(XPART):
            return start(e, part), start(e, part + 1)
        return start(e, part), start(e + 1, 0)

    def kernel(x_hbm, w1_hbm, w2_hbm, g_ref, wf_ref, wg_ref, wo_ref, o_hbm,
               xs0, xs1, w_ref, u_ref, pool, y_ref, zh_ref, f_ref, fe_ref, ge_ref,
               st_ref, sem_w, sem_x, sem_o):
        xs = (xs0, xs1)
        x_ref = XView(pool, 0, MG)
        tf = [[View(pool, NUNITS * MG * 4 + (g * 2 + ct) * 256) for ct in range(2)] for g in range(MG)]
        ti = [View(pool, NUNITS * MG * 4 + MG * 512 + g * 256) for g in range(MG)]
        tr = [View(pool, NUNITS * MG * 4 + MG * 768 + g * 256) for g in range(MG)]
        xh = x_hbm.bitcast(u32)
        w1w = w1_hbm.bitcast(u32)
        w2w = w2_hbm.bitcast(u32)

        def w1_copy(q):
            rows = pl.ds(32 * q, 32)
            return pltpu.make_async_copy(w1w.at[:, rows, :], w_ref.at[0, :, rows, :], sem_w.at[q])

        w2_copy = pltpu.make_async_copy(w2w, w_ref.at[1], sem_w.at[4])

        def x_copies(part):
            cps = []
            for b in range(2):
                for e in range(SEG):
                    lo, hi = x_rows(e, part)
                    for ct in range(2):
                        cps.append(pltpu.make_async_copy(
                            xh.at[b, pl.ds(lo, hi - lo), _lanes(ct)],
                            xs[ct].at[pl.ds(XPAD + b * XB + lo, hi - lo), :],
                            sem_x.at[part]))
            return cps

        w1_copy(0).start()
        w1_copy(1).start()

        z8 = jnp.zeros((8, 128), u32)
        for ct in range(2):
            xs[ct][pl.ds(0, 8), :] = z8
            for r in range(XPAD + T1, XPAD + XB, 8):
                xs[ct][pl.ds(r, 8), :] = z8
            for r in range(XPAD + XB + T1, XROWS, 8):
                xs[ct][pl.ds(r, 8), :] = z8

        def zero_zh(i, c):
            for h in range(2):
                for comp in range(2):
                    zh_ref[ZH - 1 - i, h, comp] = jnp.zeros((8, 256), f32)
            return c
        lax.fori_loop(0, ZH - 8 - L2, zero_zh, 0)

        zf = jnp.zeros((M, 128), f32)
        for m in range(0, 64, 4):
            y_ref[2 * m] = zf
            y_ref[2 * m + 1] = zf
        for g in range(MG):
            for h in range(2):
                for k1 in range(8):
                    for n2 in (1, 2, 3, 5, 6, 7):
                        for comp in range(2):
                            ti[g][h, (k1 * 8 + n2) * 2 + comp] = jnp.zeros((8, 128), f32)

        gg = g_ref[...].reshape(16, 256)
        ge_all = jnp.dot(gg, wg_ref[...], preferred_element_type=f32)
        ge_ref[...] = ge_all

        def transform(slot, hook=None):
            def body(rg, c):
                if hook is not None:
                    hook(rg)
                weight_transform(w_ref.at[slot], u_ref, tf[0][0], tf[0][1], rg)
                return c
            lax.fori_loop(0, 16, body, 0)

        def w1_hook(rg):
            for q in range(4):
                @pl.when(rg == 4 * q)
                def _(q=q):
                    w1_copy(q).wait()
                    if q + 2 < 4:
                        w1_copy(q + 2).start()
                    if q >= 1:
                        for cp in x_copies(q - 1):
                            cp.start()

        def conv(nchunk, nblk, make_load, act, pairs_in_time, out_index, wait_input=None):
            def loads(c):
                return [make_load(jnp.minimum(c * MG + g, nblk - 1)) for g in range(MG)]

            def P(fn, *a):
                return functools.partial(fn, *a)

            def f1(ld, pc):
                return [(P(fwd_p1, ld[g], tf[g][ct], h, n2, ct, pc), COST_F1[n2])
                        for g in range(MG) for ct in range(2) for h in range(2) for n2 in range(8)]

            def f2(cls, pc):
                return [(P(fwd_p2, tf[g][ct], x_ref, g, ct, k1, pc), COST_F2)
                        for g in range(MG) for ct in range(2) for k1 in cls]

            def i1(cls, pc):
                return [(P(inv_p1, y_ref, ti[g], g, h, n2, pc), COST_I1[n2])
                        for g in range(MG) for h in range(2) for n2 in cls]

            def i2(c, pc):
                out = []
                for g in range(MG):
                    out += inverse_tail(ti[g], tr[g], P(act, tr[g], out_index(c, g)), pc, pairs_in_time)
                return out

            idle = Pacer(None)
            if wait_input is not None:
                wait_input(0)
            with scope("pro"):
                for piece, _ in f1(loads(0), idle):
                    piece()
                for piece, _ in f2(CLASSES[0], idle):
                    piece()

            def step(c, cc):
                if wait_input is not None:
                    wait_input(c + 1)
                pc = Pacer(c < 0, lax.shift_right_arithmetic(c, 20))
                nxt = f1(loads(jnp.minimum(c + 1, nchunk - 1)), pc)
                half = len(nxt) // 2
                seq = (f2(CLASSES[1], pc) + f2(CLASSES[2], pc) + f2(CLASSES[3], pc)
                       + i1(CLASSES[3], pc) + i2(c - 1, pc)
                       + nxt[:half] + i1(CLASSES[0], pc) + nxt[half:]
                       + i1(CLASSES[1], pc) + f2(CLASSES[0], pc) + i1(CLASSES[2], pc))
                run_step(matmul_stream(x_ref, u_ref, y_ref, pc), [q[0] for q in seq], [q[1] for q in seq],
                         pc, NUNITS * (M // 4), LEAD)
                return cc
            with scope("steps"):
                lax.fori_loop(0, nchunk, step, 0)

            with scope("epi"):
                for piece, _ in i1(CLASSES[3], idle) + i2(nchunk - 1, idle):
                    piece()

        with scope("wt1"):
            transform(0, w1_hook)

        def wait_x0(c):
            if isinstance(c, int):
                for cp in x_copies(0):
                    cp.wait()
                return
            for part, first in ((1, 2), (2, 4)):
                @pl.when(c == first)
                def _(part=part):
                    for cp in x_copies(part):
                        cp.wait()

            @pl.when(c == 2)
            def _():
                w2_copy.start()

        def load1(blk):
            base = blk * S

            def load(h, n, ct, pc):
                w = xs[ct][pl.ds(base + n + h * L1, 8, stride=2 * L1), :]
                if pc is not None:
                    w = pc.here(w)
                return _unpack(w)
            return load

        def act1(rb, tau0, q, pc):
            return act_conv1(rb, zh_ref, tau0, q, pc)

        def out1(c, g):
            if isinstance(c, int):
                return 8 + (c * MG + g) * (S // 2)
            return jnp.where(c >= 0, 8 + (c * MG + g) * (S // 2), ZDUMP + g * (S // 2))

        conv(NC1, NB1, load1, act1, True, out1, wait_x0)

        row = lax.broadcasted_iota(i32, (8, 256), 0)
        for h in range(2):
            for comp in range(2):
                for t in range(last_valid, NB1 * S // 2):
                    zh_ref[8 + t, h, comp] = jnp.where(row == SEG - 1, 0.0, zh_ref[8 + t, h, comp])
                for j in range(8):
                    v = pltpu.roll(zh_ref[8 + L2 - 8 + j, h, comp], 1, axis=0)
                    zh_ref[j, h, comp] = jnp.where(row == 0, 0.0, v)
                for j in range(8):
                    v = pltpu.roll(zh_ref[8 + j, h, comp], SEG - 1, axis=0)
                    zh_ref[8 + L2 + j, h, comp] = jnp.where(row == SEG - 1, 0.0, v)

        w2_copy.wait()
        with scope("wt2"):
            transform(1)

        def load2(blk):
            def load(h, n, ct, pc):
                lo = zh_ref[blk * S + n, h, 0, :, _lanes(ct)]
                hi = zh_ref[blk * S + n, h, 1, :, _lanes(ct)]
                if pc is not None:
                    lo = pc.here(lo)
                return lo, hi
            return load

        def act2(rb, tau0, q, pc):
            return act_conv2(rb, f_ref, tau0, q, pc)

        def out2(c, g):
            if isinstance(c, int):
                return min(c * MG + g, NB2 - 1) * S
            return jnp.where(c >= 0, jnp.minimum(c * MG + g, NB2 - 1) * S, FDUMP + g * S)

        conv(NC2, NB2, load2, act2, False, out2)

        never = jnp.max(jnp.abs(ge_all)) < 0.0
        order = [(b, e) for b in range(2) for e in range(SEG)]

        def out_copy(half, q, t0, nvalid):
            b, e = order[q]
            r0 = (b * T2 + e * L2) * 8 + t0 * 8
            return pltpu.make_async_copy(st_ref.at[half, q, pl.ds(0, nvalid * 8), :],
                                         o_hbm.at[pl.ds(r0, nvalid * 8), :],
                                         sem_o.at[half])

        def width(e):
            lim = L2 if e < SEG - 1 else last_valid
            return lim - (NCH - 1) * TB

        def joint_chunk(ch, half, full, never):
            pc = Pacer(never)
            t0 = ch * TB
            fl = pltpu.bitcast(f_ref[pl.ds(t0, TB)].reshape(TB * 8, 256), bf16)
            fe = jnp.dot(fl, wf_ref[...], preferred_element_type=f32)
            fe_ref[...] = fe
            prev = [fe[8 * r:8 * r + 8, 128 * n:128 * n + 128] for n in range(2) for r in range(2 * TB)]
            prev = prev[len(prev) // 2:]
            for q, (b, e) in enumerate(order):
                ge = ge_ref[pl.ds(8 * b, 8), :]
                r = 4 * (e & 3) + 2 * b + (e >> 2)
                js = []
                for t in range(TB):
                    row = jnp.broadcast_to(fe_ref[pl.ds(16 * t + r, 1), :], (8, 256))
                    tok = prev[(t * len(prev)) // TB]
                    gt = jnp.concatenate([pc.tie(ge[:, :128], tok), pc.tie(ge[:, 128:], tok)], axis=1)
                    js.append(jnp.tanh(row + gt))
                jl = jnp.concatenate(js, axis=0).astype(bf16)
                y = jnp.dot(jl, wo_ref[...], preferred_element_type=f32)
                prev = [y[8 * rr:8 * rr + 8, 128 * n:128 * n + 128] for n in range(2) for rr in range(TB)]
                st_ref[half, q] = y.astype(bf16)
                out_copy(half, q, t0, TB if full else width(e)).start()

        def wait_chunk(half, full):
            for q, (b, e) in enumerate(order):
                out_copy(half, q, 0, TB if full else width(e)).wait()

        def joint_body(ch, c):
            half = ch % 2

            @pl.when(ch >= 2)
            def _():
                wait_chunk(half, True)
            joint_chunk(ch, half, True, ch < 0)
            return c
        with scope("joint"):
            lax.fori_loop(0, NCH - 1, joint_body, 0)
            last_half = (NCH - 1) % 2
            wait_chunk(last_half, True)
            joint_chunk(NCH - 1, last_half, False, never)
            wait_chunk(1 - last_half, True)
            wait_chunk(last_half, False)

    scratch = [
        pltpu.VMEM((XROWS, 128), u32), pltpu.VMEM((XROWS, 128), u32),
        pltpu.VMEM((2, 31, 128, 256), u32),
        pltpu.VMEM((NUNITS, 256, 256), u32),
        pltpu.VMEM((NUNITS * MG * 4 + MG * 1024, 8, 128), u32),
        pltpu.VMEM((128, M, 128), f32),
        pltpu.VMEM((ZH + MG * S // 2, 2, 2, 8, 256), f32),
        pltpu.VMEM((FROWS + MG * S, 8, 256), u32),
        pltpu.VMEM((TB * 16, 256), f32),
        pltpu.VMEM((16, 256), f32),
        pltpu.VMEM((2, 2 * SEG, TB * 8, 256), bf16),
        pltpu.SemaphoreType.DMA((5,)),
        pltpu.SemaphoreType.DMA((3,)),
        pltpu.SemaphoreType.DMA((2,)),
    ]
    return kernel, scratch


LEAD = 0
LAG = 0
AHEAD = 3
OPQ_EVERY = 1
DUE = 2
DUE_EVERY = 1000


def _call(x, w1, w2, g, w_f, w_g, w_o, interpret=False):
    B, T, D = x.shape
    kernel, scratch = _make_kernel(T)
    T2 = T // 4
    any_spec = pl.BlockSpec(memory_space=pl.ANY)
    vmem = pl.BlockSpec(memory_space=pltpu.VMEM)
    out = pl.pallas_call(
        kernel,
        out_shape=jax.ShapeDtypeStruct((B * T2 * 8, D), bf16),
        in_specs=[any_spec, any_spec, any_spec, vmem, vmem, vmem, vmem],
        out_specs=any_spec,
        scratch_shapes=scratch,
        compiler_params=pltpu.CompilerParams(vmem_limit_bytes=126 * 2**20),
        interpret=interpret,
        name="conv_stem_rnnt_joint",
    )(x, w1, w2, g, w_f, w_g, w_o)
    return out.reshape(B, T2, 8, D)


@jax.jit
def pallas_standalone__seq2seq_rnn_t_joint__speech_kernel(x, w1, w2, g, w_f, w_g, w_o):
    return _call(x, w1, w2, g, w_f, w_g, w_o)
```

```python
import functools
import math

import jax
import jax.numpy as jnp
import numpy as np
from jax import lax
from jax.experimental import pallas as pl
from jax.experimental.pallas import tpu as pltpu

f32, u32, bf16, i32 = jnp.float32, jnp.uint32, jnp.bfloat16, jnp.int32

PROFILE_SCOPES = False


class _NoScope:
    def __enter__(self):
        return self

    def __exit__(self, *a):
        return False


def scope(name):
    return jax.named_scope(name) if PROFILE_SCOPES else _NoScope()

N = 64
S = 48
SEG = 8


class V:
    __slots__ = ("a", "s")

    def __init__(self, a, s=1):
        self.a = a
        self.s = s

    def __neg__(self):
        return V(self.a, -self.s)

    def __add__(self, o):
        if self.s == o.s:
            return V(self.a + o.a, self.s)
        if self.s > 0:
            return V(self.a - o.a, 1)
        return V(o.a - self.a, 1)

    def __sub__(self, o):
        return self + (-o)

    def scale(self, c):
        if c == 1.0:
            return self
        if c == -1.0:
            return -self
        return V(self.a * np.float32(abs(c)), self.s * (1 if c > 0 else -1))

    def times(self, c):
        return self.a * np.float32(self.s * c)

    def signed(self, s):
        return self.a if self.s * s > 0 else -self.a


class C:
    __slots__ = ("r", "i")

    def __init__(self, r, i):
        self.r = r
        self.i = i

    def __add__(self, o):
        return C(self.r + o.r, self.i + o.i)

    def __sub__(self, o):
        return C(self.r - o.r, self.i - o.i)

    def __neg__(self):
        return C(-self.r, -self.i)

    def mul_w(self, num, den):
        num %= den
        if num == 0:
            return self
        if 4 * num == den:
            return C(-self.i, self.r)
        if 2 * num == den:
            return -self
        if 4 * num == 3 * den:
            return C(self.i, -self.r)
        if (8 * num) % den == 0:
            o = (8 * num) // den
            h = math.sqrt(0.5)
            sc = 1 if o in (1, 7) else -1
            ss = 1 if o in (1, 3) else -1
            r, m = self.r, self.i
            re = (r if sc > 0 else -r) - (m if ss > 0 else -m)
            im = (r if ss > 0 else -r) + (m if sc > 0 else -m)
            return C(re.scale(h), im.scale(h))
        c = math.cos(2 * math.pi * num / den)
        s = math.sin(2 * math.pi * num / den)
        return C(self.r.scale(c) - self.i.scale(s), self.r.scale(s) + self.i.scale(c))


def _add(a, b):
    if a is None:
        return b
    if b is None:
        return a
    return a + b


def _sub(a, b):
    if b is None:
        return a
    if a is None:
        return -b
    return a - b


def fft8(x, sgn, need=tuple(range(8))):
    def rot(a, num, den):
        return None if a is None else a.mul_w(sgn * num, den)

    need = set(need)
    a0, a1 = _add(x[0], x[4]), _sub(x[0], x[4])
    a2, a3 = _add(x[2], x[6]), rot(_sub(x[2], x[6]), 1, 4)
    a4, a5 = _add(x[1], x[5]), _sub(x[1], x[5])
    a6, a7 = _add(x[3], x[7]), rot(_sub(x[3], x[7]), 1, 4)
    out = {}
    if need & {0, 4}:
        b0, b4 = _add(a0, a2), _add(a4, a6)
        if 0 in need:
            out[0] = _add(b0, b4)
        if 4 in need:
            out[4] = _sub(b0, b4)
    if need & {2, 6}:
        b2, b6 = _sub(a0, a2), rot(_sub(a4, a6), 1, 4)
        if 2 in need:
            out[2] = _add(b2, b6)
        if 6 in need:
            out[6] = _sub(b2, b6)
    if need & {1, 5}:
        b1, b5 = _add(a1, a3), rot(_add(a5, a7), 1, 8)
        if 1 in need:
            out[1] = _add(b1, b5)
        if 5 in need:
            out[5] = _sub(b1, b5)
    if need & {3, 7}:
        b3, b7 = _sub(a1, a3), rot(_sub(a5, a7), 3, 8)
        if 3 in need:
            out[3] = _add(b3, b7)
        if 7 in need:
            out[7] = _sub(b3, b7)
    return out


class _Sym:
    def __add__(self, o):
        return self

    __sub__ = __mul__ = __add__

    def __neg__(self):
        return self


def _fft64_signs(sgn, present=tuple(range(64)), in_sign=None):
    d = _Sym()
    in_sign = in_sign or {}
    x = [C(V(d, in_sign.get((n, 0), 1)), V(d, in_sign.get((n, 1), 1))) if n in present else None
         for n in range(64)]
    t = {}
    for n2 in range(8):
        a = fft8([x[8 * n1 + n2] for n1 in range(8)], sgn)
        for k1 in range(8):
            t[k1, n2] = a[k1].mul_w(sgn * n2 * k1, 64)
    s1 = {key: (v.r.s, v.i.s) for key, v in t.items()}
    s2 = {}
    for k1 in range(8):
        b = fft8([t[k1, n2] for n2 in range(8)], sgn)
        for k2 in range(8):
            s2[k1 + 8 * k2] = b[k2]
    return s1, s2


def _unit(k, j):
    return (k - 1) * 3 + j


UNIT0, UNIT32 = 93, 94
NUNITS = 95


def _lhs_forms(m, z):
    if m in (0, 32):
        u = UNIT0 if m == 0 else UNIT32
        return [(u, 0, z.r), (u, 1, z.i)]
    if m < 32:
        return [(_unit(m, 0), 0, z.r + z.i), (_unit(m, 1), 0, z.r), (_unit(m, 2), 0, z.i)]
    k = 64 - m
    return [(_unit(k, 0), 1, z.r - z.i), (_unit(k, 1), 1, z.r), (_unit(k, 2), 1, z.i)]


def _lhs_signs():
    _, s2 = _fft64_signs(-1)
    sg = {}
    for m in range(64):
        for u, h, v in _lhs_forms(m, s2[m]):
            sg[u, h] = v.s
    return sg


LHS_SIGN = _lhs_signs()


def _weight_forms(m, pm):
    if m < 32:
        nt = 0 if pm > 0 else 1
        return [(_unit(m, 0), 1, nt, (1, 0)), (_unit(m, 1), 1, nt, (-1, 1)), (_unit(m, 2), 1, nt, (-1, -1))]
    k = 64 - m
    nt = 1 if pm > 0 else 0
    return [(_unit(k, 0), 0, nt, (1, 0)), (_unit(k, 1), 0, nt, (-1, -1)), (_unit(k, 2), 0, nt, (1, -1))]


def _weight_plan():
    s1, s2 = _fft64_signs(1, present=range(16))
    forms = {}
    for pm in (1, -1):
        for m in range(1, 64):
            if m == 32:
                continue
            for u, half, nt, (cr, ci) in _weight_forms(m, pm):
                forms[u, half, nt] = (cr * s2[m].r.s, ci * s2[m].i.s)
    col = {}
    for u in range(93):
        for nt in range(2):
            def negs(sig):
                n = 0
                for half in range(2):
                    cr, ci = forms[u, half, nt]
                    w = sig * LHS_SIGN[u, half]
                    n += (w * cr <= 0 and w * ci <= 0)
                return n
            col[u, nt] = 1 if negs(1) <= negs(-1) else -1
    for u in (UNIT0, UNIT32):
        col[u, 0] = col[u, 1] = 1
    return s1, s2, col


WT_S1, WT_S2, COL_SIGN = _weight_plan()


def _recombine(k1, k2, k3, k):
    out = {}
    for nt in range(2):
        yr = k1[nt] - k3[nt]
        yi = k1[nt] + k2[nt]
        if nt == 0:
            out[k, 0], out[k, 1] = yr, yi
        else:
            out[64 - k, 0], out[64 - k, 1] = yr, -yi
    return out


def _y_signs():
    d = _Sym()
    sg = {}
    for k in range(1, 32):
        ks = [[V(d, COL_SIGN[_unit(k, j), nt]) for nt in range(2)] for j in range(3)]
        for key, v in _recombine(ks[0], ks[1], ks[2], k).items():
            sg[key] = v.s
    for m, u in ((0, UNIT0), (32, UNIT32)):
        sg[m, 0], sg[m, 1] = COL_SIGN[u, 0], COL_SIGN[u, 1]
    return sg


Y_SIGN = _y_signs()


def _unpack(w):
    lo = pltpu.unpack_elementwise(w, index=0, packed_dtype=bf16, unpacked_dtype=f32)
    hi = pltpu.unpack_elementwise(w, index=1, packed_dtype=bf16, unpacked_dtype=f32)
    return lo, hi


def _pack(lo, hi):
    return pltpu.pack_elementwise([lo, hi], packed_dtype=bf16)


_GC1 = 2.0 * math.sqrt(2.0 / math.pi)
_GC2 = 8.0 * 0.044715 * math.sqrt(2.0 / math.pi)


def _gelu_half(v):
    a = v.a
    p = (a * a) * np.float32(_GC2) + np.float32(_GC1)
    t = jnp.tanh(p * a)
    return a * t + a if v.s > 0 else a * t - a


def _lanes(t):
    return pl.ds(128 * t, 128)


class Pacer:
    def __init__(self, never, zero=None):
        self.never = never
        self.tok = None
        self.tok2 = None
        self.last = None
        self.outs = []
        self.zero = zero
        self.pending = []
        self.unit = 0

    def gate(self, a):
        vals = [v for q, v in self.pending if q <= self.unit]
        self.pending = [(q, v) for q, v in self.pending if q > self.unit]
        self.unit += 1
        if not vals:
            return a
        m, k = a.shape
        tiles = [[a[8 * r:8 * r + 8, 128 * c:128 * c + 128] for c in range(k // 128)] for r in range(m // 8)]
        flat = [(r, c) for r in range(m // 8) for c in range(k // 128)]
        for i, v in enumerate(vals):
            r, c = flat[i % len(flat)]
            tiles[r][c] = self.tie(tiles[r][c], v)
        return jnp.concatenate([jnp.concatenate(row, axis=1) for row in tiles], axis=0)

    def here(self, x):
        tok, self.tok = self.tok, None
        tok2, self.tok2 = self.tok2, None
        return self.tie(self.tie(x, tok), tok2)

    def mark(self, x, nth=None):
        self.last = x
        if self.never is not None and nth is not None and nth % DUE_EVERY == DUE_EVERY - 1:
            self.outs.append(x)
        return x

    def due(self, x):
        if self.never is not None:
            self.outs.append(x)
        return x

    def tie(self, x, tok):
        if tok is None:
            return x
        if tok.dtype != x.dtype:
            tok = pltpu.bitcast(tok, x.dtype)
        return jnp.where(self.never, tok, x)


def _combo(f, cr, ci, want):
    if ci == 0:
        return f.r.signed(want * cr)
    v = (f.r if cr > 0 else -f.r) + (f.i if ci > 0 else -f.i)
    if v.s * want > 0:
        return v.a
    if f.r.s * cr != f.i.s * ci:
        return ((-f.r) if cr > 0 else f.r).__add__((-f.i) if ci > 0 else f.i).a
    return -v.a


def weight_transform(w_ref, u_ref, t_ref, z_ref, rg):
    rows = pl.ds(pl.multiple_of(rg * 8, 8), 8)
    urow = (rows, pl.ds(pl.multiple_of(rg * 8 + 128, 8), 8))
    sigma = 1.0 / 256.0
    tau = 1.0 / 128.0

    def store(u, half, nt, a0, a1):
        u_ref[u, urow[half], _lanes(nt)] = _pack(a0, a1)

    acc = {}
    for d in range(16):
        wa = [[None, None], [None, None]]
        wb = [[None, None], [None, None]]
        for dt in range(2):
            if d > 0:
                lo, hi = _unpack(w_ref[2 * d - 1, rows, _lanes(dt)])
                wa[0][dt], wa[1][dt] = V(lo), V(hi)
            lo, hi = _unpack(w_ref[2 * d, rows, _lanes(dt)])
            wb[0][dt], wb[1][dt] = V(lo), V(hi)
        for p in range(2):
            for dt in range(2):
                for name, val in (("a", wa[p][dt]), ("b", wb[p][dt])):
                    key = (p, dt, name, d % 2)
                    acc[key] = _add(acc.get(key), val)
            zp = (_sub(wa[p][0], wb[p][1]), _add(wb[p][0], wa[p][1]))
            zm = (_add(wa[p][0], wb[p][1]), _sub(wb[p][0], wa[p][1]))
            for j, z in enumerate((zp, zm)):
                for comp in range(2):
                    z_ref[j, (p * 16 + d) * 2 + comp] = z[comp].times(sigma)
    for m, u in ((0, UNIT0), (32, UNIT32)):
        for dt in range(2):
            for half, name in enumerate(("a", "b")):
                vals = []
                for p in range(2):
                    ev, od = acc[p, dt, name, 0], acc[p, dt, name, 1]
                    v = _add(ev, od) if m == 0 else _sub(ev, od)
                    vals.append(v.times(tau * LHS_SIGN[u, half] * COL_SIGN[u, dt]))
                store(u, half, dt, vals[0], vals[1])

    for j, pm in enumerate((1, -1)):
        for p in range(2):
            for n2 in range(8):
                z = [C(V(z_ref[j, (p * 16 + d) * 2]), V(z_ref[j, (p * 16 + d) * 2 + 1])) for d in (n2, n2 + 8)]
                a = fft8(z + [None] * 6, 1)
                for k1 in range(8):
                    t = a[k1].mul_w(n2 * k1, 64)
                    assert (t.r.s, t.i.s) == WT_S1[k1, n2]
                    t_ref[p, (k1 * 8 + n2) * 2] = t.r.a
                    t_ref[p, (k1 * 8 + n2) * 2 + 1] = t.i.a
        for k1 in range(8):
            need = [k2 for k2 in range(8) if (k1 + 8 * k2) not in (0, 32)]
            outs = []
            for p in range(2):
                xs = [C(V(t_ref[p, (k1 * 8 + n2) * 2], WT_S1[k1, n2][0]),
                        V(t_ref[p, (k1 * 8 + n2) * 2 + 1], WT_S1[k1, n2][1])) for n2 in range(8)]
                outs.append(fft8(xs, 1, need))
            for k2 in need:
                m = k1 + 8 * k2
                for u, half, nt, (cr, ci) in _weight_forms(m, pm):
                    want = LHS_SIGN[u, half] * COL_SIGN[u, nt]
                    store(u, half, nt, _combo(outs[0][k2], cr, ci, want), _combo(outs[1][k2], cr, ci, want))


class View:
    def __init__(self, pool, base):
        self.pool = pool
        self.base = base

    def __getitem__(self, idx):
        h, i = idx
        return pltpu.bitcast(self.pool[self.base + h * 128 + i], f32)

    def __setitem__(self, idx, val):
        h, i = idx
        self.pool[self.base + h * 128 + i] = pltpu.bitcast(val, u32)


class XView:
    def __init__(self, pool, base, mg):
        self.pool, self.base, self.mg = pool, base, mg

    def index(self, u, g, c):
        return self.base + (u * self.mg + g) * 4 + c

    def store(self, u, g, c, val):
        self.pool[self.index(u, g, c)] = val

    def load(self, u, zero=None, mg=None):
        rows = []
        for g in range(self.mg if mg is None else mg):
            row = []
            for c in range(4):
                idx = self.index(u, g, c)
                if zero is not None and g == 0 and c == 0:
                    idx = idx + zero
                row.append(self.pool[idx])
            rows.append(jnp.concatenate(row, axis=1))
        return jnp.concatenate(rows, axis=0)


_TW = (0, 42, 40, 42, 32, 42, 40, 42)
COST_F1 = tuple(73 + t for t in _TW)
COST_I1 = tuple(57 + t for t in _TW)
COST_F2, COST_I2, COST_ACT = 153, 53, 85
FWD_S1, _ = _fft64_signs(-1)
INV_S1, _INV_OUT = _fft64_signs(1, in_sign=Y_SIGN)
INV_S2 = {m: (v.r.s, v.i.s) for m, v in _INV_OUT.items()}
CLASSES = ((1, 7), (2, 6), (3, 5), (4, 0))


def _class_units(cls):
    ks = [k for k in range(1, 32) if k % 8 in cls or (-k) % 8 in cls]
    ks.sort(key=lambda k: (0 if k % 8 == cls[0] else 1, k))
    out = [("pair", k) for k in ks]
    if 0 in cls:
        out += [("real", 0), ("real", 32)]
    return out


def fwd_p1(load, t_ref, h, n2, ct, pc):
    xs = []
    for n1 in range(8):
        lo, hi = load(h, 8 * n1 + n2, ct, pc if n1 == 0 else None)
        xs.append(C(V(lo), V(hi)))
    a = fft8(xs, -1)
    for k1 in range(8):
        t = a[k1].mul_w(-n2 * k1, 64)
        assert (t.r.s, t.i.s) == FWD_S1[k1, n2]
        t_ref[h, (k1 * 8 + n2) * 2] = t.r.a
        t_ref[h, (k1 * 8 + n2) * 2 + 1] = t.i.a


def fwd_p2(t_ref, x_ref, g, ct, k1, pc):
    outs = []
    for h in range(2):
        xs = [C(V(t_ref[h, (k1 * 8 + n2) * 2], FWD_S1[k1, n2][0]),
                V(t_ref[h, (k1 * 8 + n2) * 2 + 1], FWD_S1[k1, n2][1])) for n2 in range(8)]
        if h == 0:
            xs[0].r.a = pc.here(xs[0].r.a)
        outs.append(fft8(xs, -1))
    for k2 in range(8):
        m = k1 + 8 * k2
        f0 = _lhs_forms(m, outs[0][k2])
        f1 = _lhs_forms(m, outs[1][k2])
        for i, ((u, half, v0), (_, _, v1)) in enumerate(zip(f0, f1)):
            assert v0.s == v1.s == LHS_SIGN[u, half]
            x_ref.store(u, g, 2 * half + ct, _pack(v0.a, v1.a))
    return COST_F2


def inv_p1(y_ref, t_ref, g, h, n2, pc):
    rows = pl.ds(g * 16 + 8 * h, 8)
    ysg = Y_SIGN
    xs = []
    for n1 in range(8):
        m = 8 * n1 + n2
        xs.append(C(V(y_ref[2 * m, rows, :], ysg.get((m, 0), 1)),
                    V(y_ref[2 * m + 1, rows, :], ysg.get((m, 1), 1))))
    xs[0].r.a = pc.here(xs[0].r.a)
    a = fft8(xs, 1)
    for k1 in range(8):
        t = a[k1].mul_w(n2 * k1, 64)
        assert (t.r.s, t.i.s) == INV_S1[k1, n2]
        t_ref[h, (k1 * 8 + n2) * 2] = t.r.a
        t_ref[h, (k1 * 8 + n2) * 2 + 1] = t.i.a


def inv_p2(t_ref, r_ref, h, k1, pc):
    xs = [C(V(t_ref[h, (k1 * 8 + n2) * 2], INV_S1[k1, n2][0]),
            V(t_ref[h, (k1 * 8 + n2) * 2 + 1], INV_S1[k1, n2][1])) for n2 in range(8)]
    xs[0].r.a = pc.here(xs[0].r.a)
    b = fft8(xs, 1, range(S // 8))
    for k2 in range(S // 8):
        assert (b[k2].r.s, b[k2].i.s) == INV_S2[k1 + 8 * k2]
        r_ref[h, (k1 * 6 + k2) * 2] = b[k2].r.a
        r_ref[h, (k1 * 6 + k2) * 2 + 1] = b[k2].i.a
    return COST_I2


def _act(r_ref, h, k1, k2, dt, first, pc):
    a = r_ref[h, (k1 * 6 + k2) * 2 + dt]
    if first:
        a = pc.here(a)
    return _gelu_half(V(a, INV_S2[k1 + 8 * k2][dt]))


def act_conv1(r_ref, zh_ref, tau0, q, pc):
    h, k1, part = q // 8, 2 * ((q % 8) // 2), q % 2
    first = True
    for k2 in range(3 * part, 3 * part + 3):
        for dt in range(2):
            ev = _act(r_ref, h, k1, k2, dt, first, pc)
            od = _act(r_ref, h, k1 + 1, k2, dt, False, pc)
            first = False
            zh_ref[tau0 + (k1 // 2 + 4 * k2), h, 0, :, _lanes(dt)] = pc.due(ev)
            zh_ref[tau0 + (k1 // 2 + 4 * k2), h, 1, :, _lanes(dt)] = pc.due(od)
    return COST_ACT


def act_conv2(r_ref, f_ref, tau0, q, pc):
    k1, part = q // 2, q % 2
    first = True
    for k2 in range(3 * part, 3 * part + 3):
        for dt in range(2):
            oa = _act(r_ref, 0, k1, k2, dt, first, pc)
            ob = _act(r_ref, 1, k1, k2, dt, False, pc)
            first = False
            f_ref[tau0 + (k1 + 8 * k2), :, _lanes(dt)] = pc.due(_pack(oa, ob))
    return COST_ACT


def inverse_tail(t_ref, r_ref, act, pc, pairs_in_time):
    P = functools.partial
    out = []
    if pairs_in_time:
        for h in range(2):
            for kp in range(4):
                out += [(P(inv_p2, t_ref, r_ref, h, 2 * kp + j, pc), COST_I2) for j in range(2)]
                out += [(P(act, h * 8 + kp * 2 + j, pc), COST_ACT) for j in range(2)]
    else:
        for k1 in range(8):
            out += [(P(inv_p2, t_ref, r_ref, h, k1, pc), COST_I2) for h in range(2)]
            out += [(P(act, k1 * 2 + j, pc), COST_ACT) for j in range(2)]
    return out


def _mm(x_ref, u_ref, j, pc=None, mg=None):
    opaque = pc is not None and pc.unit % OPQ_EVERY == 0
    a = x_ref.load(j, pc.zero if opaque else None, mg)
    if pc is not None:
        a = pc.gate(a)
    a = pltpu.bitcast(a, bf16)
    w = pltpu.bitcast(u_ref[j], bf16)
    return jnp.dot(a, w, preferred_element_type=f32)


def _tokens(y):
    m = y.shape[0]
    return [y[8 * r:8 * r + 8, 128 * n:128 * n + 128] for n in range(2) for r in range(m // 8)]


def matmul_stream(x_ref, u_ref, y_ref, pc=None, mg=None):
    def tiles(y, u):
        return [V(y[:, :128], COL_SIGN[u, 0]), V(y[:, 128:], COL_SIGN[u, 1])]

    if mg is not None:
        y_ref = y_ref.at[:, pl.ds(0, 16 * mg), :]
    for cls in CLASSES:
        for kind, k in _class_units(cls):
            if kind == "pair":
                j = (k - 1) * 3
                y1 = _mm(x_ref, u_ref, j, pc, mg)
                k1 = tiles(y1, j)
                yield _tokens(y1)
                y2 = _mm(x_ref, u_ref, j + 1, pc, mg)
                k2 = tiles(y2, j + 1)
                for nt, m in ((0, k), (1, 64 - k)):
                    yi = k1[nt] + k2[nt]
                    assert (yi.s if nt == 0 else -yi.s) == Y_SIGN[m, 1]
                    y_ref[2 * m + 1] = yi.a
                yield _tokens(y2)
                y3 = _mm(x_ref, u_ref, j + 2, pc, mg)
                k3 = tiles(y3, j + 2)
                for nt, m in ((0, k), (1, 64 - k)):
                    yr = k1[nt] - k3[nt]
                    assert yr.s == Y_SIGN[m, 0]
                    y_ref[2 * m] = yr.a
                yield _tokens(y3)
            else:
                y = _mm(x_ref, u_ref, UNIT0 if k == 0 else UNIT32, pc, mg)
                y_ref[2 * k] = y[:, :128]
                y_ref[2 * k + 1] = y[:, 128:]
                yield _tokens(y)


def run_step(mm, pieces, costs, pc, ntok, lead, lag=None, due=None):
    total = float(sum(costs))
    lag = LAG if lag is None else lag
    tokens = []
    marks = []
    c = 0.0
    for piece, cost in zip(pieces, costs):
        pc.tok = None
        pc.tok2 = marks[-lag] if lag and len(marks) >= lag else None
        if c >= lead:
            want = min(int((c - lead) / (total - lead) * ntok), ntok - 1)
            ahead = min(want + AHEAD * (ntok // NUNITS), ntok - 1)
            while ahead >= len(tokens):
                tokens += next(mm)
            pc.tok = tokens[want]
        pc.outs = []
        piece()
        marks.append(pc.last)
        for i, v in enumerate(pc.outs):
            q = pc.unit + (DUE if due is None else due) + i // 4
            if q < NUNITS:
                pc.pending.append((q, v))
        c += cost
    pc.tok = pc.tok2 = None
    for _ in mm:
        pass


def _make_kernel(T):
    T1, T2 = T // 2, T // 4
    L1 = (T1 + 16) // SEG
    L2 = L1 // 2
    assert L1 * SEG == T1 + 16 and L1 % 2 == 0
    NB1 = -(-L1 // S)
    NB2 = -(-L2 // S)
    XPAD = 8
    XB = T1 + 16
    XROWS = XPAD + 2 * XB + 64
    MG = 3
    M = 16 * MG
    NC1 = -(-NB1 // MG)
    NC2 = -(-NB2 // MG)
    ZH = (NB2 - 1) * S + N
    ZDUMP = ZH
    TB = 56
    NCH = -(-L2 // TB)
    FROWS = max(NB2 * S, NCH * TB)
    FDUMP = FROWS
    last_valid = T2 - (SEG - 1) * L2
    XPART = (0, 304, 592)

    def x_rows(e, part):
        def start(e, part):
            if e >= SEG:
                return T1
            return max(L1 * e + XPART[part] - (8 if part == 0 else 0), 0) // 8 * 8
        if part + 1 < len(XPART):
            return start(e, part), start(e, part + 1)
        return start(e, part), start(e + 1, 0)

    def kernel(x_hbm, w1_hbm, w2_hbm, g_ref, wf_ref, wg_ref, wo_ref, o_hbm,
               xs0, xs1, w_ref, u_ref, pool, y_ref, zh_ref, f_ref, fe_ref, ge_ref,
               st_ref, sem_w, sem_x, sem_o):
        xs = (xs0, xs1)
        x_ref = XView(pool, 0, MG)
        tf = [[View(pool, NUNITS * MG * 4 + (g * 2 + ct) * 256) for ct in range(2)] for g in range(MG)]
        ti = [View(pool, NUNITS * MG * 4 + MG * 512 + g * 256) for g in range(MG)]
        tr = [View(pool, NUNITS * MG * 4 + MG * 768 + g * 256) for g in range(MG)]
        xh = x_hbm.bitcast(u32)
        w1w = w1_hbm.bitcast(u32)
        w2w = w2_hbm.bitcast(u32)

        def w1_copy(q):
            rows = pl.ds(32 * q, 32)
            return pltpu.make_async_copy(w1w.at[:, rows, :], w_ref.at[0, :, rows, :], sem_w.at[q])

        w2_copy = pltpu.make_async_copy(w2w, w_ref.at[1], sem_w.at[4])

        def x_copies(part):
            cps = []
            for b in range(2):
                for e in range(SEG):
                    lo, hi = x_rows(e, part)
                    for ct in range(2):
                        cps.append(pltpu.make_async_copy(
                            xh.at[b, pl.ds(lo, hi - lo), _lanes(ct)],
                            xs[ct].at[pl.ds(XPAD + b * XB + lo, hi - lo), :],
                            sem_x.at[part]))
            return cps

        w1_copy(0).start()
        w1_copy(1).start()

        z8 = jnp.zeros((8, 128), u32)
        for ct in range(2):
            xs[ct][pl.ds(0, 8), :] = z8
            for r in range(XPAD + T1, XPAD + XB, 8):
                xs[ct][pl.ds(r, 8), :] = z8
            for r in range(XPAD + XB + T1, XROWS, 8):
                xs[ct][pl.ds(r, 8), :] = z8

        def zero_zh(i, c):
            for h in range(2):
                for comp in range(2):
                    zh_ref[ZH - 1 - i, h, comp] = jnp.zeros((8, 256), f32)
            return c
        lax.fori_loop(0, ZH - 8 - L2, zero_zh, 0)

        zf = jnp.zeros((M, 128), f32)
        for m in range(0, 64, 4):
            y_ref[2 * m] = zf
            y_ref[2 * m + 1] = zf
        for g in range(MG):
            for h in range(2):
                for k1 in range(8):
                    for n2 in (1, 2, 3, 5, 6, 7):
                        for comp in range(2):
                            ti[g][h, (k1 * 8 + n2) * 2 + comp] = jnp.zeros((8, 128), f32)

        gg = g_ref[...].reshape(16, 256)
        ge_all = jnp.dot(gg, wg_ref[...], preferred_element_type=f32)
        ge_ref[...] = ge_all
        never = jnp.max(jnp.abs(ge_all)) < 0.0

        def transform(slot, hook=None):
            def body(rg, c):
                if hook is not None:
                    hook(rg)
                weight_transform(w_ref.at[slot], u_ref, tf[0][0], tf[0][1], rg)
                return c
            lax.fori_loop(0, 16, body, 0)

        def w1_hook(rg):
            for q in range(4):
                @pl.when(rg == 4 * q)
                def _(q=q):
                    w1_copy(q).wait()
                    if q + 2 < 4:
                        w1_copy(q + 2).start()
                    if q >= 1:
                        for cp in x_copies(q - 1):
                            cp.start()

        def conv(nchunk, nblk, make_load, act, pairs_in_time, out_index, wait_input=None):
            def loads(c):
                return [make_load(jnp.minimum(c * MG + g, nblk - 1)) for g in range(MG)]

            def P(fn, *a):
                return functools.partial(fn, *a)

            def f1(ld, pc):
                return [(P(fwd_p1, ld[g], tf[g][ct], h, n2, ct, pc), COST_F1[n2])
                        for g in range(MG) for ct in range(2) for h in range(2) for n2 in range(8)]

            def f2(cls, pc, mg=MG):
                return [(P(fwd_p2, tf[g][ct], x_ref, g, ct, k1, pc), COST_F2)
                        for g in range(mg) for ct in range(2) for k1 in cls]

            def i1(cls, pc, mg=MG):
                return [(P(inv_p1, y_ref, ti[g], g, h, n2, pc), COST_I1[n2])
                        for g in range(mg) for h in range(2) for n2 in cls]

            def i2(c, pc, mg=MG):
                out = []
                for g in range(mg):
                    out += inverse_tail(ti[g], tr[g], P(act, tr[g], out_index(c, g)), pc, pairs_in_time)
                return out

            idle = Pacer(None)
            if wait_input is not None:
                wait_input(0)
            with scope("pro"):
                for piece, _ in f1(loads(0), idle):
                    piece()
                for piece, _ in f2(CLASSES[0], idle):
                    piece()

            def step(c, cc):
                if wait_input is not None:
                    wait_input(c + 1)
                pc = Pacer(c < 0, lax.shift_right_arithmetic(c, 20))
                nxt = f1(loads(jnp.minimum(c + 1, nchunk - 1)), pc)
                half = len(nxt) // 2
                seq = (f2(CLASSES[1], pc) + f2(CLASSES[2], pc) + f2(CLASSES[3], pc)
                       + i1(CLASSES[3], pc) + i2(c - 1, pc)
                       + nxt[:half] + i1(CLASSES[0], pc) + nxt[half:]
                       + i1(CLASSES[1], pc) + f2(CLASSES[0], pc) + i1(CLASSES[2], pc))
                run_step(matmul_stream(x_ref, u_ref, y_ref, pc), [q[0] for q in seq], [q[1] for q in seq],
                         pc, NUNITS * (M // 4), LEAD)
                return cc

            def short_step(c, never, zero, mg):
                pc = Pacer(never, zero)
                seq = (f2(CLASSES[1], pc, mg) + f2(CLASSES[2], pc, mg) + f2(CLASSES[3], pc, mg)
                       + i1(CLASSES[3], pc) + i2(c - 1, pc)
                       + i1(CLASSES[0], pc, mg) + i1(CLASSES[1], pc, mg) + i1(CLASSES[2], pc, mg))
                run_step(matmul_stream(x_ref, u_ref, y_ref, pc, mg), [q[0] for q in seq],
                         [q[1] for q in seq], pc, NUNITS * 4 * mg, LEAD)

            tail = nblk - (nchunk - 1) * MG
            with scope("steps"):
                lax.fori_loop(0, nchunk if tail == MG else nchunk - 1, step, 0)
                if tail < MG:
                    short_step(nchunk - 1, never, never.astype(i32), tail)

            with scope("epi"):
                for piece, _ in i1(CLASSES[3], idle, tail) + i2(nchunk - 1, idle, tail):
                    piece()

        with scope("wt1"):
            transform(0, w1_hook)

        def x_wait(part):
            rows = sum(4 * (x_rows(e, part)[1] - x_rows(e, part)[0]) for e in range(SEG))
            buf = xs0.at[pl.ds(0, rows), :]
            pltpu.make_async_copy(buf, buf, sem_x.at[part]).wait()

        def wait_x0(c):
            if isinstance(c, int):
                x_wait(0)
                return
            for part, first in ((1, 2), (2, 4)):
                @pl.when(c == first)
                def _(part=part):
                    x_wait(part)

            @pl.when(c == 2)
            def _():
                w2_copy.start()

        def load1(blk):
            base = blk * S

            def load(h, n, ct, pc):
                w = xs[ct][pl.ds(base + n + h * L1, 8, stride=2 * L1), :]
                if pc is not None:
                    w = pc.here(w)
                return _unpack(w)
            return load

        def act1(rb, tau0, q, pc):
            return act_conv1(rb, zh_ref, tau0, q, pc)

        def out1(c, g):
            if isinstance(c, int):
                return 8 + (c * MG + g) * (S // 2)
            return jnp.where(c >= 0, 8 + (c * MG + g) * (S // 2), ZDUMP + g * (S // 2))

        conv(NC1, NB1, load1, act1, True, out1, wait_x0)

        row = lax.broadcasted_iota(i32, (8, 256), 0)
        for h in range(2):
            for comp in range(2):
                for t in range(last_valid, NB1 * S // 2):
                    zh_ref[8 + t, h, comp] = jnp.where(row == SEG - 1, 0.0, zh_ref[8 + t, h, comp])
                for j in range(8):
                    v = pltpu.roll(zh_ref[8 + L2 - 8 + j, h, comp], 1, axis=0)
                    zh_ref[j, h, comp] = jnp.where(row == 0, 0.0, v)
                for j in range(8):
                    v = pltpu.roll(zh_ref[8 + j, h, comp], SEG - 1, axis=0)
                    zh_ref[8 + L2 + j, h, comp] = jnp.where(row == SEG - 1, 0.0, v)

        w2_copy.wait()
        with scope("wt2"):
            transform(1)

        def load2(blk):
            def load(h, n, ct, pc):
                lo = zh_ref[blk * S + n, h, 0, :, _lanes(ct)]
                hi = zh_ref[blk * S + n, h, 1, :, _lanes(ct)]
                if pc is not None:
                    lo = pc.here(lo)
                return lo, hi
            return load

        def act2(rb, tau0, q, pc):
            return act_conv2(rb, f_ref, tau0, q, pc)

        def out2(c, g):
            if isinstance(c, int):
                return min(c * MG + g, NB2 - 1) * S
            return jnp.where(c >= 0, jnp.minimum(c * MG + g, NB2 - 1) * S, FDUMP + g * S)

        conv(NC2, NB2, load2, act2, False, out2)

        order = [(b, e) for b in range(2) for e in range(SEG)]

        def out_copy(half, q, t0, nvalid):
            b, e = order[q]
            r0 = (b * T2 + e * L2) * 8 + t0 * 8
            return pltpu.make_async_copy(st_ref.at[half, q, pl.ds(0, nvalid * 8), :],
                                         o_hbm.at[pl.ds(r0, nvalid * 8), :],
                                         sem_o.at[half])

        def width(e):
            lim = L2 if e < SEG - 1 else last_valid
            return lim - (NCH - 1) * TB

        def joint_chunk(ch, half, full, never):
            pc = Pacer(never)
            t0 = ch * TB
            fl = pltpu.bitcast(f_ref[pl.ds(t0, TB)].reshape(TB * 8, 256), bf16)
            fe = jnp.dot(fl, wf_ref[...], preferred_element_type=f32)
            fe_ref[...] = fe
            prev = [fe[8 * r:8 * r + 8, 128 * n:128 * n + 128] for n in range(2) for r in range(2 * TB)]
            prev = prev[len(prev) // 2:]
            for q, (b, e) in enumerate(order):
                ge = ge_ref[pl.ds(8 * b, 8), :]
                r = 4 * (e & 3) + 2 * b + (e >> 2)
                js = []
                for t in range(TB):
                    row = jnp.broadcast_to(fe_ref[pl.ds(16 * t + r, 1), :], (8, 256))
                    tok = prev[(t * len(prev)) // TB]
                    gt = jnp.concatenate([pc.tie(ge[:, :128], tok), pc.tie(ge[:, 128:], tok)], axis=1)
                    js.append(jnp.tanh(row + gt))
                jl = jnp.concatenate(js, axis=0).astype(bf16)
                y = jnp.dot(jl, wo_ref[...], preferred_element_type=f32)
                prev = [y[8 * rr:8 * rr + 8, 128 * n:128 * n + 128] for n in range(2) for rr in range(TB)]
                st_ref[half, q] = y.astype(bf16)
                out_copy(half, q, t0, TB if full else width(e)).start()

        def wait_chunk(half, full):
            if full:
                pltpu.make_async_copy(st_ref.at[half], st_ref.at[half], sem_o.at[half]).wait()
                return
            for q, (b, e) in enumerate(order):
                out_copy(half, q, 0, width(e)).wait()

        def joint_body(ch, c):
            half = ch % 2

            @pl.when(ch >= 2)
            def _():
                wait_chunk(half, True)
            joint_chunk(ch, half, True, ch < 0)
            return c
        with scope("joint"):
            lax.fori_loop(0, NCH - 1, joint_body, 0)
            last_half = (NCH - 1) % 2
            wait_chunk(last_half, True)
            joint_chunk(NCH - 1, last_half, False, never)
            wait_chunk(1 - last_half, True)
            wait_chunk(last_half, False)

    scratch = [
        pltpu.VMEM((XROWS, 128), u32), pltpu.VMEM((XROWS, 128), u32),
        pltpu.VMEM((2, 31, 128, 256), u32),
        pltpu.VMEM((NUNITS, 256, 256), u32),
        pltpu.VMEM((NUNITS * MG * 4 + MG * 1024, 8, 128), u32),
        pltpu.VMEM((128, M, 128), f32),
        pltpu.VMEM((ZH + MG * S // 2, 2, 2, 8, 256), f32),
        pltpu.VMEM((FROWS + MG * S, 8, 256), u32),
        pltpu.VMEM((TB * 16, 256), f32),
        pltpu.VMEM((16, 256), f32),
        pltpu.VMEM((2, 2 * SEG, TB * 8, 256), bf16),
        pltpu.SemaphoreType.DMA((5,)),
        pltpu.SemaphoreType.DMA((3,)),
        pltpu.SemaphoreType.DMA((2,)),
    ]
    return kernel, scratch


LEAD = 0
LAG = 0
AHEAD = 3
OPQ_EVERY = 1
DUE = 2
DUE_EVERY = 1000


def _call(x, w1, w2, g, w_f, w_g, w_o, interpret=False):
    B, T, D = x.shape
    kernel, scratch = _make_kernel(T)
    T2 = T // 4
    any_spec = pl.BlockSpec(memory_space=pl.ANY)
    vmem = pl.BlockSpec(memory_space=pltpu.VMEM)
    out = pl.pallas_call(
        kernel,
        out_shape=jax.ShapeDtypeStruct((B * T2 * 8, D), bf16),
        in_specs=[any_spec, any_spec, any_spec, vmem, vmem, vmem, vmem],
        out_specs=any_spec,
        scratch_shapes=scratch,
        compiler_params=pltpu.CompilerParams(vmem_limit_bytes=126 * 2**20),
        interpret=interpret,
        name="conv_stem_rnnt_joint",
    )(x, w1, w2, g, w_f, w_g, w_o)
    return out.reshape(B, T2, 8, D)


@jax.jit
def pallas_standalone__seq2seq_rnn_t_joint__speech_kernel(x, w1, w2, g, w_f, w_g, w_o):
    return _call(x, w1, w2, g, w_f, w_g, w_o)
```

```python
import functools
import math

import jax
import jax.numpy as jnp
import numpy as np
from jax import lax
from jax.experimental import pallas as pl
from jax.experimental.pallas import tpu as pltpu

f32, u32, bf16, i32 = jnp.float32, jnp.uint32, jnp.bfloat16, jnp.int32

PROFILE_SCOPES = False


class _NoScope:
    def __enter__(self):
        return self

    def __exit__(self, *a):
        return False


def scope(name):
    return jax.named_scope(name) if PROFILE_SCOPES else _NoScope()

N = 64
S = 48
SEG = 8


class V:
    __slots__ = ("a", "s")

    def __init__(self, a, s=1):
        self.a = a
        self.s = s

    def __neg__(self):
        return V(self.a, -self.s)

    def __add__(self, o):
        if self.s == o.s:
            return V(self.a + o.a, self.s)
        if self.s > 0:
            return V(self.a - o.a, 1)
        return V(o.a - self.a, 1)

    def __sub__(self, o):
        return self + (-o)

    def scale(self, c):
        if c == 1.0:
            return self
        if c == -1.0:
            return -self
        return V(self.a * np.float32(abs(c)), self.s * (1 if c > 0 else -1))

    def times(self, c):
        return self.a * np.float32(self.s * c)

    def signed(self, s):
        return self.a if self.s * s > 0 else -self.a


class C:
    __slots__ = ("r", "i")

    def __init__(self, r, i):
        self.r = r
        self.i = i

    def __add__(self, o):
        return C(self.r + o.r, self.i + o.i)

    def __sub__(self, o):
        return C(self.r - o.r, self.i - o.i)

    def __neg__(self):
        return C(-self.r, -self.i)

    def mul_w(self, num, den):
        num %= den
        if num == 0:
            return self
        if 4 * num == den:
            return C(-self.i, self.r)
        if 2 * num == den:
            return -self
        if 4 * num == 3 * den:
            return C(self.i, -self.r)
        if (8 * num) % den == 0:
            o = (8 * num) // den
            h = math.sqrt(0.5)
            sc = 1 if o in (1, 7) else -1
            ss = 1 if o in (1, 3) else -1
            r, m = self.r, self.i
            re = (r if sc > 0 else -r) - (m if ss > 0 else -m)
            im = (r if ss > 0 else -r) + (m if sc > 0 else -m)
            return C(re.scale(h), im.scale(h))
        c = math.cos(2 * math.pi * num / den)
        s = math.sin(2 * math.pi * num / den)
        return C(self.r.scale(c) - self.i.scale(s), self.r.scale(s) + self.i.scale(c))


def _add(a, b):
    if a is None:
        return b
    if b is None:
        return a
    return a + b


def _sub(a, b):
    if b is None:
        return a
    if a is None:
        return -b
    return a - b


def fft8(x, sgn, need=tuple(range(8))):
    def rot(a, num, den):
        return None if a is None else a.mul_w(sgn * num, den)

    need = set(need)
    a0, a1 = _add(x[0], x[4]), _sub(x[0], x[4])
    a2, a3 = _add(x[2], x[6]), rot(_sub(x[2], x[6]), 1, 4)
    a4, a5 = _add(x[1], x[5]), _sub(x[1], x[5])
    a6, a7 = _add(x[3], x[7]), rot(_sub(x[3], x[7]), 1, 4)
    out = {}
    if need & {0, 4}:
        b0, b4 = _add(a0, a2), _add(a4, a6)
        if 0 in need:
            out[0] = _add(b0, b4)
        if 4 in need:
            out[4] = _sub(b0, b4)
    if need & {2, 6}:
        b2, b6 = _sub(a0, a2), rot(_sub(a4, a6), 1, 4)
        if 2 in need:
            out[2] = _add(b2, b6)
        if 6 in need:
            out[6] = _sub(b2, b6)
    if need & {1, 5}:
        b1, b5 = _add(a1, a3), rot(_add(a5, a7), 1, 8)
        if 1 in need:
            out[1] = _add(b1, b5)
        if 5 in need:
            out[5] = _sub(b1, b5)
    if need & {3, 7}:
        b3, b7 = _sub(a1, a3), rot(_sub(a5, a7), 3, 8)
        if 3 in need:
            out[3] = _add(b3, b7)
        if 7 in need:
            out[7] = _sub(b3, b7)
    return out


class _Sym:
    def __add__(self, o):
        return self

    __sub__ = __mul__ = __add__

    def __neg__(self):
        return self


def _fft64_signs(sgn, present=tuple(range(64)), in_sign=None):
    d = _Sym()
    in_sign = in_sign or {}
    x = [C(V(d, in_sign.get((n, 0), 1)), V(d, in_sign.get((n, 1), 1))) if n in present else None
         for n in range(64)]
    t = {}
    for n2 in range(8):
        a = fft8([x[8 * n1 + n2] for n1 in range(8)], sgn)
        for k1 in range(8):
            t[k1, n2] = a[k1].mul_w(sgn * n2 * k1, 64)
    s1 = {key: (v.r.s, v.i.s) for key, v in t.items()}
    s2 = {}
    for k1 in range(8):
        b = fft8([t[k1, n2] for n2 in range(8)], sgn)
        for k2 in range(8):
            s2[k1 + 8 * k2] = b[k2]
    return s1, s2


def _unit(k, j):
    return (k - 1) * 3 + j


UNIT0, UNIT32 = 93, 94
NUNITS = 95


def _lhs_forms(m, z):
    if m in (0, 32):
        u = UNIT0 if m == 0 else UNIT32
        return [(u, 0, z.r), (u, 1, z.i)]
    if m < 32:
        return [(_unit(m, 0), 0, z.r + z.i), (_unit(m, 1), 0, z.r), (_unit(m, 2), 0, z.i)]
    k = 64 - m
    return [(_unit(k, 0), 1, z.r - z.i), (_unit(k, 1), 1, z.r), (_unit(k, 2), 1, z.i)]


def _lhs_signs():
    _, s2 = _fft64_signs(-1)
    sg = {}
    for m in range(64):
        for u, h, v in _lhs_forms(m, s2[m]):
            sg[u, h] = v.s
    return sg


LHS_SIGN = _lhs_signs()


def _weight_forms(m, pm):
    if m < 32:
        nt = 0 if pm > 0 else 1
        return [(_unit(m, 0), 1, nt, (1, 0)), (_unit(m, 1), 1, nt, (-1, 1)), (_unit(m, 2), 1, nt, (-1, -1))]
    k = 64 - m
    nt = 1 if pm > 0 else 0
    return [(_unit(k, 0), 0, nt, (1, 0)), (_unit(k, 1), 0, nt, (-1, -1)), (_unit(k, 2), 0, nt, (1, -1))]


def _weight_plan():
    s1, s2 = _fft64_signs(1, present=range(16))
    forms = {}
    for pm in (1, -1):
        for m in range(1, 64):
            if m == 32:
                continue
            for u, half, nt, (cr, ci) in _weight_forms(m, pm):
                forms[u, half, nt] = (cr * s2[m].r.s, ci * s2[m].i.s)
    col = {}
    for u in range(93):
        for nt in range(2):
            def negs(sig):
                n = 0
                for half in range(2):
                    cr, ci = forms[u, half, nt]
                    w = sig * LHS_SIGN[u, half]
                    n += (w * cr <= 0 and w * ci <= 0)
                return n
            col[u, nt] = 1 if negs(1) <= negs(-1) else -1
    for u in (UNIT0, UNIT32):
        col[u, 0] = col[u, 1] = 1
    return s1, s2, col


WT_S1, WT_S2, COL_SIGN = _weight_plan()


def _recombine(k1, k2, k3, k):
    out = {}
    for nt in range(2):
        yr = k1[nt] - k3[nt]
        yi = k1[nt] + k2[nt]
        if nt == 0:
            out[k, 0], out[k, 1] = yr, yi
        else:
            out[64 - k, 0], out[64 - k, 1] = yr, -yi
    return out


def _y_signs():
    d = _Sym()
    sg = {}
    for k in range(1, 32):
        ks = [[V(d, COL_SIGN[_unit(k, j), nt]) for nt in range(2)] for j in range(3)]
        for key, v in _recombine(ks[0], ks[1], ks[2], k).items():
            sg[key] = v.s
    for m, u in ((0, UNIT0), (32, UNIT32)):
        sg[m, 0], sg[m, 1] = COL_SIGN[u, 0], COL_SIGN[u, 1]
    return sg


Y_SIGN = _y_signs()


def _unpack(w):
    lo = pltpu.unpack_elementwise(w, index=0, packed_dtype=bf16, unpacked_dtype=f32)
    hi = pltpu.unpack_elementwise(w, index=1, packed_dtype=bf16, unpacked_dtype=f32)
    return lo, hi


def _pack(lo, hi):
    return pltpu.pack_elementwise([lo, hi], packed_dtype=bf16)


_GC1 = 2.0 * math.sqrt(2.0 / math.pi)
_GC2 = 8.0 * 0.044715 * math.sqrt(2.0 / math.pi)


def _gelu_half(v):
    a = v.a
    p = (a * a) * np.float32(_GC2) + np.float32(_GC1)
    t = jnp.tanh(p * a)
    return a * t + a if v.s > 0 else a * t - a


def _lanes(t):
    return pl.ds(128 * t, 128)


class Pacer:
    def __init__(self, never, zero=None):
        self.never = never
        self.tok = None
        self.tok2 = None
        self.last = None
        self.outs = []
        self.zero = zero
        self.pending = []
        self.unit = 0

    def gate(self, a, first=0):
        vals = [v for q, v in self.pending if q <= self.unit]
        self.pending = [(q, v) for q, v in self.pending if q > self.unit]
        self.unit += 1
        if not vals:
            return a
        m, k = a.shape
        tiles = [[a[8 * r:8 * r + 8, 128 * c:128 * c + 128] for c in range(k // 128)] for r in range(m // 8)]
        flat = [(r, c) for r in range(first, m // 8) for c in range(k // 128)]
        for i, v in enumerate(vals):
            r, c = flat[i % len(flat)]
            tiles[r][c] = self.tie(tiles[r][c], v)
        return jnp.concatenate([jnp.concatenate(row, axis=1) for row in tiles], axis=0)

    def here(self, x):
        tok, self.tok = self.tok, None
        tok2, self.tok2 = self.tok2, None
        return self.tie(self.tie(x, tok), tok2)

    def mark(self, x, nth=None):
        self.last = x
        if self.never is not None and nth is not None and nth % DUE_EVERY == DUE_EVERY - 1:
            self.outs.append(x)
        return x

    def due(self, x):
        if self.never is not None:
            self.outs.append(x)
        return x

    def tie(self, x, tok):
        if tok is None:
            return x
        if tok.dtype != x.dtype:
            tok = pltpu.bitcast(tok, x.dtype)
        return jnp.where(self.never, tok, x)


def _combo(f, cr, ci, want):
    if ci == 0:
        return f.r.signed(want * cr)
    v = (f.r if cr > 0 else -f.r) + (f.i if ci > 0 else -f.i)
    if v.s * want > 0:
        return v.a
    if f.r.s * cr != f.i.s * ci:
        return ((-f.r) if cr > 0 else f.r).__add__((-f.i) if ci > 0 else f.i).a
    return -v.a


UP = 260
WP = 132


class UView:
    def __init__(self, ref):
        self.ref = ref

    def load(self, u):
        cols = []
        for nt in range(2):
            base = (nt * 96 + u) * UP
            cols.append(jnp.concatenate([self.ref[pl.ds(base + 8 * r, 8), :] for r in range(32)], axis=0))
        return jnp.concatenate(cols, axis=1)

    def store(self, u, half, nt, rg, val):
        self.ref[pl.ds((nt * 96 + u) * UP + half * 128 + rg * 8, 8), :] = val


def _tap_matrix():
    import ml_dtypes
    sigma, tau = 1.0 / 256.0, 1.0 / 128.0
    g = np.zeros((2, 2, 96, 32, 2))
    d = np.arange(16)
    for tap in range(31):
        for dt in range(2):
            wa = np.zeros((16, 2))
            wb = np.zeros((16, 2))
            if tap % 2:
                wa[(tap + 1) // 2, dt] = 1.0
            else:
                wb[tap // 2, dt] = 1.0
            z0 = wa[:, 0] + 1j * wb[:, 0]
            z1 = wa[:, 1] + 1j * wb[:, 1]
            for pm, z in ((1, z0 + 1j * z1), (-1, z0 - 1j * z1)):
                for m in range(1, 64):
                    if m == 32:
                        continue
                    f = sigma * np.sum(z * np.exp(2j * np.pi * m * d / 64))
                    for u, half, nt, (cr, ci) in _weight_forms(m, pm):
                        g[nt, half, u, tap, dt] = (LHS_SIGN[u, half] * COL_SIGN[u, nt]
                                                   * (cr * f.real + ci * f.imag))
            for m, u in ((0, UNIT0), (32, UNIT32)):
                e = np.cos(np.pi * m * d / 32)
                for half, wv in enumerate((wa, wb)):
                    g[dt, half, u, tap, dt] = (LHS_SIGN[u, half] * COL_SIGN[u, dt]
                                               * tau * np.sum(e * wv[:, dt]))
    g = g.reshape(384, 32, 2)
    mat = np.zeros((384, 128))
    for v in range(4):
        dt, t0 = v // 2, 16 * (v % 2)
        for s_ in range(8):
            for par in range(2):
                mat[:, 16 * v + 2 * s_ + par] = g[:, t0 + 8 * par + s_, dt]
    hi = mat.astype(ml_dtypes.bfloat16)
    lo = (mat - hi.astype(np.float64)).astype(ml_dtypes.bfloat16)
    full = np.concatenate([hi[:, :64], lo[:, :64]], axis=1).view(np.uint16).astype(np.uint32)
    return full[0::2] | (full[1::2] << 16)


def tap_operand(ws, cpair):
    ev, od = [], []
    for dt in range(2):
        for t0 in (0, 16):
            wa = ws[dt][pl.ds(t0 * WP + cpair, 8, stride=WP), :]
            wb = ws[dt][pl.ds((t0 + 8) * WP + cpair, 8, stride=WP), :]
            alo, ahi = _unpack(wa)
            blo, bhi = _unpack(wb)
            ev.append(_pack(alo, blo))
            od.append(_pack(ahi, bhi))
    return jnp.concatenate(ev + ev, axis=0), jnp.concatenate(od + od, axis=0)


def tap_stream(g_view, ws, u2_ref, it0, n, pc):
    for q in range(n):
        it = it0 + q
        lhs = pltpu.bitcast(pc.gate(g_view(pc.zero), TAP_GATE), bf16)
        ops = []
        for j in range(2):
            ops += list(tap_operand(ws, 2 * it + j))
        rhs = pltpu.bitcast(jnp.concatenate(ops, axis=1), bf16)
        y = jnp.dot(lhs, rhs, preferred_element_type=f32)
        for r in range(48):
            nt, half, u0 = r // 24, (r // 12) % 2, (r % 12) * 8
            for j in range(2):
                val = _pack(y[8 * r:8 * r + 8, 256 * j:256 * j + 128],
                            y[8 * r:8 * r + 8, 256 * j + 128:256 * j + 256])
                u2_ref[pl.ds((nt * 96 + u0) * UP + half * 128 + 2 * it + j, 8, stride=UP), :] = val
        yield [y[8 * r:8 * r + 8, 128 * t:128 * t + 128] for r in range(48) for t in range(4)]


def weight_pieces(w_ref, u_ref, t_ref, z_ref, rg, pc):
    rows = pl.ds(pl.multiple_of(rg * 8, 8), 8)
    sigma = 1.0 / 256.0
    tau = 1.0 / 128.0
    acc = {}

    def store(u, half, nt, a0, a1):
        u_ref.store(u, half, nt, rg, pc.due(_pack(a0, a1)))

    def prep(d):
        wa = [[None, None], [None, None]]
        wb = [[None, None], [None, None]]
        for dt in range(2):
            w = w_ref[2 * d, rows, _lanes(dt)]
            if dt == 0:
                w = pc.here(w)
            lo, hi = _unpack(w)
            wb[0][dt], wb[1][dt] = V(lo), V(hi)
            if d > 0:
                lo, hi = _unpack(w_ref[2 * d - 1, rows, _lanes(dt)])
                wa[0][dt], wa[1][dt] = V(lo), V(hi)
        for p in range(2):
            for dt in range(2):
                for name, val in (("a", wa[p][dt]), ("b", wb[p][dt])):
                    key = (p, dt, name, d % 2)
                    acc[key] = _add(acc.get(key), val)
            zp = (_sub(wa[p][0], wb[p][1]), _add(wb[p][0], wa[p][1]))
            zm = (_add(wa[p][0], wb[p][1]), _sub(wb[p][0], wa[p][1]))
            for j, z in enumerate((zp, zm)):
                for comp in range(2):
                    z_ref[j, (p * 16 + d) * 2 + comp] = z[comp].times(sigma)

    def real_bins():
        for m, u in ((0, UNIT0), (32, UNIT32)):
            for dt in range(2):
                for half, name in enumerate(("a", "b")):
                    vals = []
                    for p in range(2):
                        ev, od = acc[p, dt, name, 0], acc[p, dt, name, 1]
                        v = _add(ev, od) if m == 0 else _sub(ev, od)
                        vals.append(v.times(tau * LHS_SIGN[u, half] * COL_SIGN[u, dt]))
                    store(u, half, dt, vals[0], vals[1])

    def pass1(j, p, n2):
        z = [C(V(z_ref[j, (p * 16 + d) * 2]), V(z_ref[j, (p * 16 + d) * 2 + 1])) for d in (n2, n2 + 8)]
        z[0].r.a = pc.here(z[0].r.a)
        a = fft8(z + [None] * 6, 1)
        for k1 in range(8):
            t = a[k1].mul_w(n2 * k1, 64)
            assert (t.r.s, t.i.s) == WT_S1[k1, n2]
            t_ref[p, (k1 * 8 + n2) * 2] = t.r.a
            t_ref[p, (k1 * 8 + n2) * 2 + 1] = t.i.a

    def pass2(pm, k1):
        need = [k2 for k2 in range(8) if (k1 + 8 * k2) not in (0, 32)]
        outs = []
        for p in range(2):
            xs = [C(V(t_ref[p, (k1 * 8 + n2) * 2], WT_S1[k1, n2][0]),
                    V(t_ref[p, (k1 * 8 + n2) * 2 + 1], WT_S1[k1, n2][1])) for n2 in range(8)]
            if p == 0:
                xs[0].r.a = pc.here(xs[0].r.a)
            outs.append(fft8(xs, 1, need))
        for k2 in need:
            m = k1 + 8 * k2
            for u, half, nt, (cr, ci) in _weight_forms(m, pm):
                want = LHS_SIGN[u, half] * COL_SIGN[u, nt]
                store(u, half, nt, _combo(outs[0][k2], cr, ci, want), _combo(outs[1][k2], cr, ci, want))

    P = functools.partial
    out = [(P(prep, d), 40) for d in range(16)] + [(real_bins, 40)]
    for j, pm in enumerate((1, -1)):
        out += [(P(pass1, j, p, n2), 21 + _TW[n2]) for p in range(2) for n2 in range(8)]
        out += [(P(pass2, pm, k1), 193) for k1 in range(8)]
    return out


class View:
    def __init__(self, pool, base):
        self.pool = pool
        self.base = base

    def __getitem__(self, idx):
        h, i = idx
        return pltpu.bitcast(self.pool[self.base + h * 128 + i], f32)

    def __setitem__(self, idx, val):
        h, i = idx
        self.pool[self.base + h * 128 + i] = pltpu.bitcast(val, u32)


class XView:
    def __init__(self, pool, base, mg):
        self.pool, self.base, self.mg = pool, base, mg

    def index(self, u, g, c):
        return self.base + (u * self.mg + g) * 4 + c

    def store(self, u, g, c, val):
        self.pool[self.index(u, g, c)] = val

    def load(self, u, zero=None, mg=None):
        rows = []
        for g in range(self.mg if mg is None else mg):
            row = []
            for c in range(4):
                idx = self.index(u, g, c)
                if zero is not None and g == 0 and c == 0:
                    idx = idx + zero
                row.append(self.pool[idx])
            rows.append(jnp.concatenate(row, axis=1))
        return jnp.concatenate(rows, axis=0)


_TW = (0, 42, 40, 42, 32, 42, 40, 42)
COST_F1 = tuple(73 + t for t in _TW)
COST_I1 = tuple(57 + t for t in _TW)
COST_F2, COST_I2, COST_ACT = 153, 53, 85
FWD_S1, _ = _fft64_signs(-1)
INV_S1, _INV_OUT = _fft64_signs(1, in_sign=Y_SIGN)
INV_S2 = {m: (v.r.s, v.i.s) for m, v in _INV_OUT.items()}
CLASSES = ((1, 7), (2, 6), (3, 5), (4, 0))


def _class_units(cls):
    ks = [k for k in range(1, 32) if k % 8 in cls or (-k) % 8 in cls]
    ks.sort(key=lambda k: (0 if k % 8 == cls[0] else 1, k))
    out = [("pair", k) for k in ks]
    if 0 in cls:
        out += [("real", 0), ("real", 32)]
    return out


def fwd_p1(load, t_ref, h, n2, ct, pc):
    xs = []
    for n1 in range(8):
        lo, hi = load(h, 8 * n1 + n2, ct, pc if n1 == 0 else None)
        xs.append(C(V(lo), V(hi)))
    a = fft8(xs, -1)
    for k1 in range(8):
        t = a[k1].mul_w(-n2 * k1, 64)
        assert (t.r.s, t.i.s) == FWD_S1[k1, n2]
        t_ref[h, (k1 * 8 + n2) * 2] = t.r.a
        t_ref[h, (k1 * 8 + n2) * 2 + 1] = t.i.a


def fwd_p2(t_ref, x_ref, g, ct, k1, pc):
    outs = []
    for h in range(2):
        xs = [C(V(t_ref[h, (k1 * 8 + n2) * 2], FWD_S1[k1, n2][0]),
                V(t_ref[h, (k1 * 8 + n2) * 2 + 1], FWD_S1[k1, n2][1])) for n2 in range(8)]
        if h == 0:
            xs[0].r.a = pc.here(xs[0].r.a)
        outs.append(fft8(xs, -1))
    for k2 in range(8):
        m = k1 + 8 * k2
        f0 = _lhs_forms(m, outs[0][k2])
        f1 = _lhs_forms(m, outs[1][k2])
        for i, ((u, half, v0), (_, _, v1)) in enumerate(zip(f0, f1)):
            assert v0.s == v1.s == LHS_SIGN[u, half]
            x_ref.store(u, g, 2 * half + ct, _pack(v0.a, v1.a))
    return COST_F2


def inv_p1(y_ref, t_ref, g, h, n2, pc):
    rows = pl.ds(g * 16 + 8 * h, 8)
    ysg = Y_SIGN
    xs = []
    for n1 in range(8):
        m = 8 * n1 + n2
        xs.append(C(V(y_ref[2 * m, rows, :], ysg.get((m, 0), 1)),
                    V(y_ref[2 * m + 1, rows, :], ysg.get((m, 1), 1))))
    xs[0].r.a = pc.here(xs[0].r.a)
    a = fft8(xs, 1)
    for k1 in range(8):
        t = a[k1].mul_w(n2 * k1, 64)
        assert (t.r.s, t.i.s) == INV_S1[k1, n2]
        t_ref[h, (k1 * 8 + n2) * 2] = t.r.a
        t_ref[h, (k1 * 8 + n2) * 2 + 1] = t.i.a


def inv_p2(t_ref, r_ref, h, k1, pc):
    xs = [C(V(t_ref[h, (k1 * 8 + n2) * 2], INV_S1[k1, n2][0]),
            V(t_ref[h, (k1 * 8 + n2) * 2 + 1], INV_S1[k1, n2][1])) for n2 in range(8)]
    xs[0].r.a = pc.here(xs[0].r.a)
    b = fft8(xs, 1, range(S // 8))
    for k2 in range(S // 8):
        assert (b[k2].r.s, b[k2].i.s) == INV_S2[k1 + 8 * k2]
        r_ref[h, (k1 * 6 + k2) * 2] = b[k2].r.a
        r_ref[h, (k1 * 6 + k2) * 2 + 1] = b[k2].i.a
    return COST_I2


def _act(r_ref, h, k1, k2, dt, first, pc):
    a = r_ref[h, (k1 * 6 + k2) * 2 + dt]
    if first:
        a = pc.here(a)
    return _gelu_half(V(a, INV_S2[k1 + 8 * k2][dt]))


def act_conv1(r_ref, zh_ref, tau0, q, pc):
    h, k1, part = q // 8, 2 * ((q % 8) // 2), q % 2
    first = True
    for k2 in range(3 * part, 3 * part + 3):
        for dt in range(2):
            ev = _act(r_ref, h, k1, k2, dt, first, pc)
            od = _act(r_ref, h, k1 + 1, k2, dt, False, pc)
            first = False
            zh_ref[tau0 + (k1 // 2 + 4 * k2), h, 0, :, _lanes(dt)] = pc.due(ev)
            zh_ref[tau0 + (k1 // 2 + 4 * k2), h, 1, :, _lanes(dt)] = pc.due(od)
    return COST_ACT


def act_conv2(r_ref, f_ref, tau0, q, pc):
    k1, part = q // 2, q % 2
    first = True
    for k2 in range(3 * part, 3 * part + 3):
        for dt in range(2):
            oa = _act(r_ref, 0, k1, k2, dt, first, pc)
            ob = _act(r_ref, 1, k1, k2, dt, False, pc)
            first = False
            f_ref[tau0 + (k1 + 8 * k2), :, _lanes(dt)] = pc.due(_pack(oa, ob))
    return COST_ACT


def inverse_tail(t_ref, r_ref, act, pc, pairs_in_time):
    P = functools.partial
    out = []
    if pairs_in_time:
        for h in range(2):
            for kp in range(4):
                out += [(P(inv_p2, t_ref, r_ref, h, 2 * kp + j, pc), COST_I2) for j in range(2)]
                out += [(P(act, h * 8 + kp * 2 + j, pc), COST_ACT) for j in range(2)]
    else:
        for k1 in range(8):
            out += [(P(inv_p2, t_ref, r_ref, h, k1, pc), COST_I2) for h in range(2)]
            out += [(P(act, k1 * 2 + j, pc), COST_ACT) for j in range(2)]
    return out


def _mm(x_ref, u_ref, j, pc=None, mg=None):
    opaque = pc is not None and pc.unit % OPQ_EVERY == 0
    a = x_ref.load(j, pc.zero if opaque else None, mg)
    if pc is not None:
        a = pc.gate(a)
    a = pltpu.bitcast(a, bf16)
    w = pltpu.bitcast(u_ref.load(j), bf16)
    return jnp.dot(a, w, preferred_element_type=f32)


def _tokens(y):
    m = y.shape[0]
    return [y[8 * r:8 * r + 8, 128 * n:128 * n + 128] for n in range(2) for r in range(m // 8)]


def matmul_stream(x_ref, u_ref, y_ref, pc=None, mg=None):
    def tiles(y, u):
        return [V(y[:, :128], COL_SIGN[u, 0]), V(y[:, 128:], COL_SIGN[u, 1])]

    if mg is not None:
        y_ref = y_ref.at[:, pl.ds(0, 16 * mg), :]
    for cls in CLASSES:
        for kind, k in _class_units(cls):
            if kind == "pair":
                j = (k - 1) * 3
                y1 = _mm(x_ref, u_ref, j, pc, mg)
                k1 = tiles(y1, j)
                yield _tokens(y1)
                y2 = _mm(x_ref, u_ref, j + 1, pc, mg)
                k2 = tiles(y2, j + 1)
                for nt, m in ((0, k), (1, 64 - k)):
                    yi = k1[nt] + k2[nt]
                    assert (yi.s if nt == 0 else -yi.s) == Y_SIGN[m, 1]
                    y_ref[2 * m + 1] = yi.a
                yield _tokens(y2)
                y3 = _mm(x_ref, u_ref, j + 2, pc, mg)
                k3 = tiles(y3, j + 2)
                for nt, m in ((0, k), (1, 64 - k)):
                    yr = k1[nt] - k3[nt]
                    assert yr.s == Y_SIGN[m, 0]
                    y_ref[2 * m] = yr.a
                yield _tokens(y3)
            else:
                y = _mm(x_ref, u_ref, UNIT0 if k == 0 else UNIT32, pc, mg)
                y_ref[2 * k] = y[:, :128]
                y_ref[2 * k + 1] = y[:, 128:]
                yield _tokens(y)


def run_step(mm, pieces, costs, pc, ntok, lead, lag=None, due=None, nunits=NUNITS):
    total = float(sum(costs))
    lag = LAG if lag is None else lag
    tokens = []
    marks = []
    c = 0.0
    for piece, cost in zip(pieces, costs):
        pc.tok = None
        pc.tok2 = marks[-lag] if lag and len(marks) >= lag else None
        if c >= lead:
            want = min(int((c - lead) / (total - lead) * ntok), ntok - 1)
            ahead = min(want + (AHEAD * ntok) // max(nunits, NUNITS), ntok - 1)
            while ahead >= len(tokens):
                tokens += next(mm)
            pc.tok = tokens[want]
        pc.outs = []
        piece()
        marks.append(pc.last)
        for i, v in enumerate(pc.outs):
            q = pc.unit + (DUE if due is None else due) + i // 4
            if q < nunits:
                pc.pending.append((q, v))
        c += cost
    pc.tok = pc.tok2 = None
    for _ in mm:
        pass


def _make_kernel(T):
    T1, T2 = T // 2, T // 4
    L1 = (T1 + 16) // SEG
    L2 = L1 // 2
    assert L1 * SEG == T1 + 16 and L1 % 2 == 0
    NB1 = -(-L1 // S)
    NB2 = -(-L2 // S)
    XPAD = 8
    XB = T1 + 16
    XROWS = XPAD + 2 * XB + 64
    MG = 3
    M = 16 * MG
    NC1 = -(-NB1 // MG)
    NC2 = -(-NB2 // MG)
    ZH = (NB2 - 1) * S + N
    ZDUMP = ZH
    TB = 56
    NCH = -(-L2 // TB)
    FROWS = max(NB2 * S, NCH * TB)
    FDUMP = FROWS
    last_valid = T2 - (SEG - 1) * L2
    XPART = (0, 304, 592)

    def x_rows(e, part):
        def start(e, part):
            if e >= SEG:
                return T1
            return max(L1 * e + XPART[part] - (8 if part == 0 else 0), 0) // 8 * 8
        if part + 1 < len(XPART):
            return start(e, part), start(e, part + 1)
        return start(e, part), start(e + 1, 0)

    def kernel(x_hbm, w1_hbm, w2_hbm, g_ref, wf_ref, wg_ref, wo_ref, gm_ref, o_hbm,
               xs0, xs1, w_ref, ws0, ws1, u1_ref, u2_ref, pool, y_ref, zh_ref, f_ref, fe_ref, ge_ref,
               st_ref, sem_w, sem_x, sem_o):
        xs = (xs0, xs1)
        x_ref = XView(pool, 0, MG)
        tf = [[View(pool, NUNITS * MG * 4 + (g * 2 + ct) * 256) for ct in range(2)] for g in range(MG)]
        ti = [View(pool, NUNITS * MG * 4 + MG * 512 + g * 256) for g in range(MG)]
        tr = [View(pool, NUNITS * MG * 4 + MG * 768 + g * 256) for g in range(MG)]
        xh = x_hbm.bitcast(u32)
        w1w = w1_hbm.bitcast(u32)
        w2w = w2_hbm.bitcast(u32)

        W1PART = (0, 32, 64, 96, 128)
        W2PART = (0, 32, 128)

        def w1_copy(q):
            rows = pl.ds(W1PART[q], W1PART[q + 1] - W1PART[q])
            return pltpu.make_async_copy(w1w.at[:, rows, :], w_ref.at[:, rows, :], sem_w.at[q])

        ws = (ws0, ws1)

        def w2_copies(part):
            lo, n = W2PART[part], W2PART[part + 1] - W2PART[part]
            return [pltpu.make_async_copy(w2w.at[i, pl.ds(lo, n), _lanes(dt)],
                                          ws[dt].at[pl.ds(WP * i + lo, n), :], sem_w.at[4 + part])
                    for i in range(31) for dt in range(2)]

        def w2_wait(part):
            buf = ws0.at[pl.ds(0, 31 * (W2PART[part + 1] - W2PART[part])), :]
            for _ in range(2):
                pltpu.make_async_copy(buf, buf, sem_w.at[4 + part]).wait()

        def x_copies(part):
            cps = []
            for b in range(2):
                for e in range(SEG):
                    lo, hi = x_rows(e, part)
                    for ct in range(2):
                        cps.append(pltpu.make_async_copy(
                            xh.at[b, pl.ds(lo, hi - lo), _lanes(ct)],
                            xs[ct].at[pl.ds(XPAD + b * XB + lo, hi - lo), :],
                            sem_x.at[part]))
            return cps

        w1_copy(0).start()
        for cp in w2_copies(0):
            cp.start()
        w1_copy(1).start()
        for cp in w2_copies(1):
            cp.start()
        for dt in range(2):
            for r in range(31 * WP, 31 * WP + 128, 8):
                ws[dt][pl.ds(r, 8), :] = jnp.zeros((8, 128), u32)
        gbase = NUNITS * MG * 4 + MG * 1024
        for r in range(24):
            pool[gbase + r] = gm_ref[pl.ds(8 * r, 8), :]

        def g_view(zero):
            return jnp.concatenate([pool[gbase + r + (zero if r == TAP_OPQ else 0)] for r in range(24)], axis=0)

        z8 = jnp.zeros((8, 128), u32)
        for ct in range(2):
            xs[ct][pl.ds(0, 8), :] = z8
            for r in range(XPAD + T1, XPAD + XB, 8):
                xs[ct][pl.ds(r, 8), :] = z8
            for r in range(XPAD + XB + T1, XROWS, 8):
                xs[ct][pl.ds(r, 8), :] = z8

        def zero_zh(i, c):
            for h in range(2):
                for comp in range(2):
                    zh_ref[ZH - 1 - i, h, comp] = jnp.zeros((8, 256), f32)
            return c
        lax.fori_loop(0, ZH - 8 - L2, zero_zh, 0)

        zf = jnp.zeros((M, 128), f32)
        for m in range(0, 64, 4):
            y_ref[2 * m] = zf
            y_ref[2 * m + 1] = zf
        for g in range(MG):
            for h in range(2):
                for k1 in range(8):
                    for n2 in (1, 2, 3, 5, 6, 7):
                        for comp in range(2):
                            ti[g][h, (k1 * 8 + n2) * 2 + comp] = jnp.zeros((8, 128), f32)

        gg = g_ref[...].reshape(16, 256)
        ge_all = jnp.dot(gg, wg_ref[...], preferred_element_type=f32)
        ge_ref[...] = ge_all
        never = jnp.max(jnp.abs(ge_all)) < 0.0

        def transform(hook):
            def body(rg, c):
                hook(rg)
                pc = Pacer(rg < 0, lax.shift_right_arithmetic(rg, 20))
                seq = weight_pieces(w_ref, UView(u1_ref), tf[0][0], tf[0][1], rg, pc)
                run_step(tap_stream(g_view, ws, u2_ref, 4 * rg, 4, pc), [q[0] for q in seq],
                         [q[1] for q in seq], pc, 4 * 192, LEAD, nunits=4)
                return c
            lax.fori_loop(0, 16, body, 0)

        def w1_hook(rg):
            for q in range(4):
                @pl.when(rg == 4 * q)
                def _(q=q):
                    w1_copy(q).wait()
                    if q == 1:
                        w2_wait(1)
                    if q + 2 < 4:
                        w1_copy(q + 2).start()
                    if q >= 1:
                        for cp in x_copies(q - 1):
                            cp.start()

        def conv(nchunk, nblk, u_ref, make_load, act, pairs_in_time, out_index, wait_input=None):
            def loads(c):
                return [make_load(jnp.minimum(c * MG + g, nblk - 1)) for g in range(MG)]

            def P(fn, *a):
                return functools.partial(fn, *a)

            def f1(ld, pc):
                return [(P(fwd_p1, ld[g], tf[g][ct], h, n2, ct, pc), COST_F1[n2])
                        for g in range(MG) for ct in range(2) for h in range(2) for n2 in range(8)]

            def f2(cls, pc, mg=MG):
                return [(P(fwd_p2, tf[g][ct], x_ref, g, ct, k1, pc), COST_F2)
                        for g in range(mg) for ct in range(2) for k1 in cls]

            def i1(cls, pc, mg=MG):
                return [(P(inv_p1, y_ref, ti[g], g, h, n2, pc), COST_I1[n2])
                        for g in range(mg) for h in range(2) for n2 in cls]

            def i2(c, pc, mg=MG):
                out = []
                for g in range(mg):
                    out += inverse_tail(ti[g], tr[g], P(act, tr[g], out_index(c, g)), pc, pairs_in_time)
                return out

            idle = Pacer(None)
            if wait_input is not None:
                wait_input(0)
            with scope("pro"):
                for piece, _ in f1(loads(0), idle):
                    piece()
                for piece, _ in f2(CLASSES[0], idle):
                    piece()

            def step(c, cc):
                if wait_input is not None:
                    wait_input(c + 1)
                pc = Pacer(c < 0, lax.shift_right_arithmetic(c, 20))
                nxt = f1(loads(jnp.minimum(c + 1, nchunk - 1)), pc)
                half = len(nxt) // 2
                seq = (f2(CLASSES[1], pc) + f2(CLASSES[2], pc) + f2(CLASSES[3], pc)
                       + i1(CLASSES[3], pc) + i2(c - 1, pc)
                       + nxt[:half] + i1(CLASSES[0], pc) + nxt[half:]
                       + i1(CLASSES[1], pc) + f2(CLASSES[0], pc) + i1(CLASSES[2], pc))
                run_step(matmul_stream(x_ref, u_ref, y_ref, pc), [q[0] for q in seq], [q[1] for q in seq],
                         pc, NUNITS * (M // 4), LEAD)
                return cc

            def short_step(c, never, zero, mg):
                pc = Pacer(never, zero)
                seq = (f2(CLASSES[1], pc, mg) + f2(CLASSES[2], pc, mg) + f2(CLASSES[3], pc, mg)
                       + i1(CLASSES[3], pc) + i2(c - 1, pc)
                       + i1(CLASSES[0], pc, mg) + i1(CLASSES[1], pc, mg) + i1(CLASSES[2], pc, mg))
                run_step(matmul_stream(x_ref, u_ref, y_ref, pc, mg), [q[0] for q in seq],
                         [q[1] for q in seq], pc, NUNITS * 4 * mg, LEAD)

            tail = nblk - (nchunk - 1) * MG
            with scope("steps"):
                lax.fori_loop(0, nchunk if tail == MG else nchunk - 1, step, 0)
                if tail < MG:
                    short_step(nchunk - 1, never, never.astype(i32), tail)

            with scope("epi"):
                for piece, _ in i1(CLASSES[3], idle, tail) + i2(nchunk - 1, idle, tail):
                    piece()

        with scope("wt1"):
            w2_wait(0)
            transform(w1_hook)

        def x_wait(part):
            rows = sum(4 * (x_rows(e, part)[1] - x_rows(e, part)[0]) for e in range(SEG))
            buf = xs0.at[pl.ds(0, rows), :]
            pltpu.make_async_copy(buf, buf, sem_x.at[part]).wait()

        def wait_x0(c):
            if isinstance(c, int):
                x_wait(0)
                return
            for part, first in ((1, 2), (2, 4)):
                @pl.when(c == first)
                def _(part=part):
                    x_wait(part)

        def load1(blk):
            base = blk * S

            def load(h, n, ct, pc):
                w = xs[ct][pl.ds(base + n + h * L1, 8, stride=2 * L1), :]
                if pc is not None:
                    w = pc.here(w)
                return _unpack(w)
            return load

        def act1(rb, tau0, q, pc):
            return act_conv1(rb, zh_ref, tau0, q, pc)

        def out1(c, g):
            if isinstance(c, int):
                return 8 + (c * MG + g) * (S // 2)
            return jnp.where(c >= 0, 8 + (c * MG + g) * (S // 2), ZDUMP)

        conv(NC1, NB1, UView(u1_ref), load1, act1, True, out1, wait_x0)

        row = lax.broadcasted_iota(i32, (8, 256), 0)
        for h in range(2):
            for comp in range(2):
                for t in range(last_valid, NB1 * S // 2):
                    zh_ref[8 + t, h, comp] = jnp.where(row == SEG - 1, 0.0, zh_ref[8 + t, h, comp])
                for j in range(8):
                    v = pltpu.roll(zh_ref[8 + L2 - 8 + j, h, comp], 1, axis=0)
                    zh_ref[j, h, comp] = jnp.where(row == 0, 0.0, v)
                for j in range(8):
                    v = pltpu.roll(zh_ref[8 + j, h, comp], SEG - 1, axis=0)
                    zh_ref[8 + L2 + j, h, comp] = jnp.where(row == SEG - 1, 0.0, v)


        def load2(blk):
            def load(h, n, ct, pc):
                lo = zh_ref[blk * S + n, h, 0, :, _lanes(ct)]
                hi = zh_ref[blk * S + n, h, 1, :, _lanes(ct)]
                if pc is not None:
                    lo = pc.here(lo)
                return lo, hi
            return load

        def act2(rb, tau0, q, pc):
            return act_conv2(rb, f_ref, tau0, q, pc)

        def out2(c, g):
            if isinstance(c, int):
                return min(c * MG + g, NB2 - 1) * S
            return jnp.where(c >= 0, jnp.minimum(c * MG + g, NB2 - 1) * S, FDUMP)

        conv(NC2, NB2, UView(u2_ref), load2, act2, False, out2)

        order = [(b, e) for b in range(2) for e in range(SEG)]

        def out_copy(half, q, t0, nvalid):
            b, e = order[q]
            r0 = (b * T2 + e * L2) * 8 + t0 * 8
            return pltpu.make_async_copy(st_ref.at[half, q, pl.ds(0, nvalid * 8), :],
                                         o_hbm.at[pl.ds(r0, nvalid * 8), :],
                                         sem_o.at[half])

        def width(e):
            lim = L2 if e < SEG - 1 else last_valid
            return lim - (NCH - 1) * TB

        def joint_chunk(ch, half, full, never):
            pc = Pacer(never)
            t0 = ch * TB
            fl = pltpu.bitcast(f_ref[pl.ds(t0, TB)].reshape(TB * 8, 256), bf16)
            fe = jnp.dot(fl, wf_ref[...], preferred_element_type=f32)
            fe_ref[...] = fe
            prev = [fe[8 * r:8 * r + 8, 128 * n:128 * n + 128] for n in range(2) for r in range(2 * TB)]
            prev = prev[len(prev) // 2:]
            for q, (b, e) in enumerate(order):
                ge = ge_ref[pl.ds(8 * b, 8), :]
                r = 4 * (e & 3) + 2 * b + (e >> 2)
                js = []
                for t in range(TB):
                    row = jnp.broadcast_to(fe_ref[pl.ds(16 * t + r, 1), :], (8, 256))
                    tok = prev[(t * len(prev)) // TB]
                    gt = jnp.concatenate([pc.tie(ge[:, :128], tok), pc.tie(ge[:, 128:], tok)], axis=1)
                    js.append(jnp.tanh(row + gt))
                jl = jnp.concatenate(js, axis=0).astype(bf16)
                y = jnp.dot(jl, wo_ref[...], preferred_element_type=f32)
                prev = [y[8 * rr:8 * rr + 8, 128 * n:128 * n + 128] for n in range(2) for rr in range(TB)]
                st_ref[half, q] = y.astype(bf16)
                out_copy(half, q, t0, TB if full else width(e)).start()

        def wait_chunk(half, full):
            if full:
                pltpu.make_async_copy(st_ref.at[half], st_ref.at[half], sem_o.at[half]).wait()
                return
            for q, (b, e) in enumerate(order):
                out_copy(half, q, 0, width(e)).wait()

        def joint_body(ch, c):
            half = ch % 2

            @pl.when(ch >= 2)
            def _():
                wait_chunk(half, True)
            joint_chunk(ch, half, True, ch < 0)
            return c
        with scope("joint"):
            lax.fori_loop(0, NCH - 1, joint_body, 0)
            last_half = (NCH - 1) % 2
            wait_chunk(last_half, True)
            joint_chunk(NCH - 1, last_half, False, never)
            wait_chunk(1 - last_half, True)
            wait_chunk(last_half, False)

    scratch = [
        pltpu.VMEM((XROWS, 128), u32), pltpu.VMEM((XROWS, 128), u32),
        pltpu.VMEM((31, 128, 256), u32),
        pltpu.VMEM((32 * WP + 8, 128), u32), pltpu.VMEM((32 * WP + 8, 128), u32),
        pltpu.VMEM((2 * 96 * UP, 128), u32), pltpu.VMEM((2 * 96 * UP, 128), u32),
        pltpu.VMEM((NUNITS * MG * 4 + MG * 1024 + 24, 8, 128), u32),
        pltpu.VMEM((128, M, 128), f32),
        pltpu.VMEM((ZH + S // 2, 2, 2, 8, 256), f32),
        pltpu.VMEM((FROWS + S, 8, 256), u32),
        pltpu.VMEM((TB * 16, 256), f32),
        pltpu.VMEM((16, 256), f32),
        pltpu.VMEM((2, 2 * SEG, TB * 8, 256), bf16),
        pltpu.SemaphoreType.DMA((6,)),
        pltpu.SemaphoreType.DMA((3,)),
        pltpu.SemaphoreType.DMA((2,)),
    ]
    return kernel, scratch


TAP_MATRIX = _tap_matrix()
TAP_OPQ = 23
TAP_GATE = 20
LEAD = 0
LAG = 0
AHEAD = 2
OPQ_EVERY = 1
DUE = 0
DUE_EVERY = 1000


def _call(x, w1, w2, g, w_f, w_g, w_o, interpret=False):
    B, T, D = x.shape
    kernel, scratch = _make_kernel(T)
    T2 = T // 4
    any_spec = pl.BlockSpec(memory_space=pl.ANY)
    vmem = pl.BlockSpec(memory_space=pltpu.VMEM)
    out = pl.pallas_call(
        kernel,
        out_shape=jax.ShapeDtypeStruct((B * T2 * 8, D), bf16),
        in_specs=[any_spec, any_spec, any_spec, vmem, vmem, vmem, vmem, vmem],
        out_specs=any_spec,
        scratch_shapes=scratch,
        compiler_params=pltpu.CompilerParams(vmem_limit_bytes=126 * 2**20),
        interpret=interpret,
        name="conv_stem_rnnt_joint",
    )(x, w1, w2, g, w_f, w_g, w_o, TAP_MATRIX)
    return out.reshape(B, T2, 8, D)


@jax.jit
def pallas_standalone__seq2seq_rnn_t_joint__speech_kernel(x, w1, w2, g, w_f, w_g, w_o):
    return _call(x, w1, w2, g, w_f, w_g, w_o)
```

```python
import functools
import math

import jax
import jax.numpy as jnp
import numpy as np
from jax import lax
from jax.experimental import pallas as pl
from jax.experimental.pallas import tpu as pltpu

f32, u32, bf16, i32 = jnp.float32, jnp.uint32, jnp.bfloat16, jnp.int32

PROFILE_SCOPES = False


class _NoScope:
    def __enter__(self):
        return self

    def __exit__(self, *a):
        return False


def scope(name):
    return jax.named_scope(name) if PROFILE_SCOPES else _NoScope()

N = 64
S = 48
SEG = 8


class V:
    __slots__ = ("a", "s")

    def __init__(self, a, s=1):
        self.a = a
        self.s = s

    def __neg__(self):
        return V(self.a, -self.s)

    def __add__(self, o):
        if self.s == o.s:
            return V(self.a + o.a, self.s)
        if self.s > 0:
            return V(self.a - o.a, 1)
        return V(o.a - self.a, 1)

    def __sub__(self, o):
        return self + (-o)

    def scale(self, c):
        if c == 1.0:
            return self
        if c == -1.0:
            return -self
        return V(self.a * np.float32(abs(c)), self.s * (1 if c > 0 else -1))

    def times(self, c):
        return self.a * np.float32(self.s * c)

    def signed(self, s):
        return self.a if self.s * s > 0 else -self.a


class C:
    __slots__ = ("r", "i")

    def __init__(self, r, i):
        self.r = r
        self.i = i

    def __add__(self, o):
        return C(self.r + o.r, self.i + o.i)

    def __sub__(self, o):
        return C(self.r - o.r, self.i - o.i)

    def __neg__(self):
        return C(-self.r, -self.i)

    def mul_w(self, num, den):
        num %= den
        if num == 0:
            return self
        if 4 * num == den:
            return C(-self.i, self.r)
        if 2 * num == den:
            return -self
        if 4 * num == 3 * den:
            return C(self.i, -self.r)
        if (8 * num) % den == 0:
            o = (8 * num) // den
            h = math.sqrt(0.5)
            sc = 1 if o in (1, 7) else -1
            ss = 1 if o in (1, 3) else -1
            r, m = self.r, self.i
            re = (r if sc > 0 else -r) - (m if ss > 0 else -m)
            im = (r if ss > 0 else -r) + (m if sc > 0 else -m)
            return C(re.scale(h), im.scale(h))
        c = math.cos(2 * math.pi * num / den)
        s = math.sin(2 * math.pi * num / den)
        return C(self.r.scale(c) - self.i.scale(s), self.r.scale(s) + self.i.scale(c))


def _add(a, b):
    if a is None:
        return b
    if b is None:
        return a
    return a + b


def _sub(a, b):
    if b is None:
        return a
    if a is None:
        return -b
    return a - b


def fft8(x, sgn, need=tuple(range(8))):
    def rot(a, num, den):
        return None if a is None else a.mul_w(sgn * num, den)

    need = set(need)
    a0, a1 = _add(x[0], x[4]), _sub(x[0], x[4])
    a2, a3 = _add(x[2], x[6]), rot(_sub(x[2], x[6]), 1, 4)
    a4, a5 = _add(x[1], x[5]), _sub(x[1], x[5])
    a6, a7 = _add(x[3], x[7]), rot(_sub(x[3], x[7]), 1, 4)
    out = {}
    if need & {0, 4}:
        b0, b4 = _add(a0, a2), _add(a4, a6)
        if 0 in need:
            out[0] = _add(b0, b4)
        if 4 in need:
            out[4] = _sub(b0, b4)
    if need & {2, 6}:
        b2, b6 = _sub(a0, a2), rot(_sub(a4, a6), 1, 4)
        if 2 in need:
            out[2] = _add(b2, b6)
        if 6 in need:
            out[6] = _sub(b2, b6)
    if need & {1, 5}:
        b1, b5 = _add(a1, a3), rot(_add(a5, a7), 1, 8)
        if 1 in need:
            out[1] = _add(b1, b5)
        if 5 in need:
            out[5] = _sub(b1, b5)
    if need & {3, 7}:
        b3, b7 = _sub(a1, a3), rot(_sub(a5, a7), 3, 8)
        if 3 in need:
            out[3] = _add(b3, b7)
        if 7 in need:
            out[7] = _sub(b3, b7)
    return out


class _Sym:
    def __add__(self, o):
        return self

    __sub__ = __mul__ = __add__

    def __neg__(self):
        return self


def _fft64_signs(sgn, present=tuple(range(64)), in_sign=None):
    d = _Sym()
    in_sign = in_sign or {}
    x = [C(V(d, in_sign.get((n, 0), 1)), V(d, in_sign.get((n, 1), 1))) if n in present else None
         for n in range(64)]
    t = {}
    for n2 in range(8):
        a = fft8([x[8 * n1 + n2] for n1 in range(8)], sgn)
        for k1 in range(8):
            t[k1, n2] = a[k1].mul_w(sgn * n2 * k1, 64)
    s1 = {key: (v.r.s, v.i.s) for key, v in t.items()}
    s2 = {}
    for k1 in range(8):
        b = fft8([t[k1, n2] for n2 in range(8)], sgn)
        for k2 in range(8):
            s2[k1 + 8 * k2] = b[k2]
    return s1, s2


def _unit(k, j):
    return (k - 1) * 3 + j


UNIT0, UNIT32 = 93, 94
NUNITS = 95


def _lhs_forms(m, z):
    if m in (0, 32):
        u = UNIT0 if m == 0 else UNIT32
        return [(u, 0, z.r), (u, 1, z.i)]
    if m < 32:
        return [(_unit(m, 0), 0, z.r + z.i), (_unit(m, 1), 0, z.r), (_unit(m, 2), 0, z.i)]
    k = 64 - m
    return [(_unit(k, 0), 1, z.r - z.i), (_unit(k, 1), 1, z.r), (_unit(k, 2), 1, z.i)]


def _lhs_signs():
    _, s2 = _fft64_signs(-1)
    sg = {}
    for m in range(64):
        for u, h, v in _lhs_forms(m, s2[m]):
            sg[u, h] = v.s
    return sg


LHS_SIGN = _lhs_signs()


def _weight_forms(m, pm):
    if m < 32:
        nt = 0 if pm > 0 else 1
        return [(_unit(m, 0), 1, nt, (1, 0)), (_unit(m, 1), 1, nt, (-1, 1)), (_unit(m, 2), 1, nt, (-1, -1))]
    k = 64 - m
    nt = 1 if pm > 0 else 0
    return [(_unit(k, 0), 0, nt, (1, 0)), (_unit(k, 1), 0, nt, (-1, -1)), (_unit(k, 2), 0, nt, (1, -1))]


def _weight_plan():
    s1, s2 = _fft64_signs(1, present=range(16))
    forms = {}
    for pm in (1, -1):
        for m in range(1, 64):
            if m == 32:
                continue
            for u, half, nt, (cr, ci) in _weight_forms(m, pm):
                forms[u, half, nt] = (cr * s2[m].r.s, ci * s2[m].i.s)
    col = {}
    for u in range(93):
        for nt in range(2):
            def negs(sig):
                n = 0
                for half in range(2):
                    cr, ci = forms[u, half, nt]
                    w = sig * LHS_SIGN[u, half]
                    n += (w * cr <= 0 and w * ci <= 0)
                return n
            col[u, nt] = 1 if negs(1) <= negs(-1) else -1
    for u in (UNIT0, UNIT32):
        col[u, 0] = col[u, 1] = 1
    return s1, s2, col


WT_S1, WT_S2, COL_SIGN = _weight_plan()


def _recombine(k1, k2, k3, k):
    out = {}
    for nt in range(2):
        yr = k1[nt] - k3[nt]
        yi = k1[nt] + k2[nt]
        if nt == 0:
            out[k, 0], out[k, 1] = yr, yi
        else:
            out[64 - k, 0], out[64 - k, 1] = yr, -yi
    return out


def _y_signs():
    d = _Sym()
    sg = {}
    for k in range(1, 32):
        ks = [[V(d, COL_SIGN[_unit(k, j), nt]) for nt in range(2)] for j in range(3)]
        for key, v in _recombine(ks[0], ks[1], ks[2], k).items():
            sg[key] = v.s
    for m, u in ((0, UNIT0), (32, UNIT32)):
        sg[m, 0], sg[m, 1] = COL_SIGN[u, 0], COL_SIGN[u, 1]
    return sg


Y_SIGN = _y_signs()


def _unpack(w):
    lo = pltpu.unpack_elementwise(w, index=0, packed_dtype=bf16, unpacked_dtype=f32)
    hi = pltpu.unpack_elementwise(w, index=1, packed_dtype=bf16, unpacked_dtype=f32)
    return lo, hi


def _pack(lo, hi):
    return pltpu.pack_elementwise([lo, hi], packed_dtype=bf16)


_GC1 = 2.0 * math.sqrt(2.0 / math.pi)
_GC2 = 8.0 * 0.044715 * math.sqrt(2.0 / math.pi)


def _gelu_half(v):
    a = v.a
    p = (a * a) * np.float32(_GC2) + np.float32(_GC1)
    t = jnp.tanh(p * a)
    return a * t + a if v.s > 0 else a * t - a


def _lanes(t):
    return pl.ds(128 * t, 128)


class Pacer:
    def __init__(self, never, zero=None):
        self.never = never
        self.tok = None
        self.tok2 = None
        self.last = None
        self.outs = []
        self.zero = zero
        self.pending = []
        self.unit = 0

    def gate(self, a, first=0):
        vals = [v for q, v in self.pending if q <= self.unit]
        self.pending = [(q, v) for q, v in self.pending if q > self.unit]
        self.unit += 1
        if not vals:
            return a
        m, k = a.shape
        tiles = [[a[8 * r:8 * r + 8, 128 * c:128 * c + 128] for c in range(k // 128)] for r in range(m // 8)]
        flat = [(r, c) for r in range(first, m // 8) for c in range(k // 128)]
        for i, v in enumerate(vals):
            r, c = flat[i % len(flat)]
            tiles[r][c] = self.tie(tiles[r][c], v)
        return jnp.concatenate([jnp.concatenate(row, axis=1) for row in tiles], axis=0)

    def here(self, x):
        tok, self.tok = self.tok, None
        tok2, self.tok2 = self.tok2, None
        return self.tie(self.tie(x, tok), tok2)

    def mark(self, x, nth=None):
        self.last = x
        if self.never is not None and nth is not None and nth % DUE_EVERY == DUE_EVERY - 1:
            self.outs.append(x)
        return x

    def due(self, x):
        if self.never is not None:
            self.outs.append(x)
        return x

    def tie(self, x, tok):
        if tok is None:
            return x
        if tok.dtype != x.dtype:
            tok = pltpu.bitcast(tok, x.dtype)
        return jnp.where(self.never, tok, x)


def _combo(f, cr, ci, want):
    if ci == 0:
        return f.r.signed(want * cr)
    v = (f.r if cr > 0 else -f.r) + (f.i if ci > 0 else -f.i)
    if v.s * want > 0:
        return v.a
    if f.r.s * cr != f.i.s * ci:
        return ((-f.r) if cr > 0 else f.r).__add__((-f.i) if ci > 0 else f.i).a
    return -v.a


UP = 260
WP = 132


class UView:
    def __init__(self, ref):
        self.ref = ref

    def load(self, u):
        cols = []
        for nt in range(2):
            base = (nt * 96 + u) * UP
            cols.append(jnp.concatenate([self.ref[pl.ds(base + 8 * r, 8), :] for r in range(32)], axis=0))
        return jnp.concatenate(cols, axis=1)

    def store(self, u, half, nt, rg, val):
        self.ref[pl.ds((nt * 96 + u) * UP + half * 128 + rg * 8, 8), :] = val


def _tap_matrix():
    import ml_dtypes
    sigma, tau = 1.0 / 256.0, 1.0 / 128.0
    g = np.zeros((2, 2, 96, 32, 2))
    d = np.arange(16)
    for tap in range(31):
        for dt in range(2):
            wa = np.zeros((16, 2))
            wb = np.zeros((16, 2))
            if tap % 2:
                wa[(tap + 1) // 2, dt] = 1.0
            else:
                wb[tap // 2, dt] = 1.0
            z0 = wa[:, 0] + 1j * wb[:, 0]
            z1 = wa[:, 1] + 1j * wb[:, 1]
            for pm, z in ((1, z0 + 1j * z1), (-1, z0 - 1j * z1)):
                for m in range(1, 64):
                    if m == 32:
                        continue
                    f = sigma * np.sum(z * np.exp(2j * np.pi * m * d / 64))
                    for u, half, nt, (cr, ci) in _weight_forms(m, pm):
                        g[nt, half, u, tap, dt] = (LHS_SIGN[u, half] * COL_SIGN[u, nt]
                                                   * (cr * f.real + ci * f.imag))
            for m, u in ((0, UNIT0), (32, UNIT32)):
                e = np.cos(np.pi * m * d / 32)
                for half, wv in enumerate((wa, wb)):
                    g[dt, half, u, tap, dt] = (LHS_SIGN[u, half] * COL_SIGN[u, dt]
                                               * tau * np.sum(e * wv[:, dt]))
    g = g.reshape(384, 32, 2)
    mat = np.zeros((384, 128))
    for v in range(4):
        dt, t0 = v // 2, 16 * (v % 2)
        for s_ in range(8):
            for par in range(2):
                mat[:, 16 * v + 2 * s_ + par] = g[:, t0 + 8 * par + s_, dt]
    hi = mat.astype(ml_dtypes.bfloat16)
    lo = (mat - hi.astype(np.float64)).astype(ml_dtypes.bfloat16)
    full = np.concatenate([hi[:, :64], lo[:, :64]], axis=1).view(np.uint16).astype(np.uint32)
    return full[0::2] | (full[1::2] << 16)


def tap_operand(ws, cpair):
    ev, od = [], []
    for dt in range(2):
        for t0 in (0, 16):
            wa = ws[dt][pl.ds(t0 * WP + cpair, 8, stride=WP), :]
            wb = ws[dt][pl.ds((t0 + 8) * WP + cpair, 8, stride=WP), :]
            alo, ahi = _unpack(wa)
            blo, bhi = _unpack(wb)
            ev.append(_pack(alo, blo))
            od.append(_pack(ahi, bhi))
    return jnp.concatenate(ev + ev, axis=0), jnp.concatenate(od + od, axis=0)


def tap_stream(g_view, ws, u2_ref, it0, n, pc):
    for q in range(n):
        it = it0 + q
        lhs = pltpu.bitcast(pc.gate(g_view(pc.zero), TAP_GATE), bf16)
        ops = []
        for j in range(2):
            ops += list(tap_operand(ws, 2 * it + j))
        rhs = pltpu.bitcast(jnp.concatenate(ops, axis=1), bf16)
        y = jnp.dot(lhs, rhs, preferred_element_type=f32)
        for r in range(48):
            nt, half, u0 = r // 24, (r // 12) % 2, (r % 12) * 8
            for j in range(2):
                val = _pack(y[8 * r:8 * r + 8, 256 * j:256 * j + 128],
                            y[8 * r:8 * r + 8, 256 * j + 128:256 * j + 256])
                u2_ref[pl.ds((nt * 96 + u0) * UP + half * 128 + 2 * it + j, 8, stride=UP), :] = val
        yield [y[8 * r:8 * r + 8, 128 * t:128 * t + 128] for r in range(48) for t in range(4)]


def weight_pieces(w_ref, u_ref, t_ref, z_ref, rg, pc):
    rows = pl.ds(pl.multiple_of(rg * 8, 8), 8)
    sigma = 1.0 / 256.0
    tau = 1.0 / 128.0
    acc = {}

    def store(u, half, nt, a0, a1):
        u_ref.store(u, half, nt, rg, pc.due(_pack(a0, a1)))

    def prep(d):
        wa = [[None, None], [None, None]]
        wb = [[None, None], [None, None]]
        for dt in range(2):
            w = w_ref[2 * d, rows, _lanes(dt)]
            if dt == 0:
                w = pc.here(w)
            lo, hi = _unpack(w)
            wb[0][dt], wb[1][dt] = V(lo), V(hi)
            if d > 0:
                lo, hi = _unpack(w_ref[2 * d - 1, rows, _lanes(dt)])
                wa[0][dt], wa[1][dt] = V(lo), V(hi)
        for p in range(2):
            for dt in range(2):
                for name, val in (("a", wa[p][dt]), ("b", wb[p][dt])):
                    key = (p, dt, name, d % 2)
                    acc[key] = _add(acc.get(key), val)
            zp = (_sub(wa[p][0], wb[p][1]), _add(wb[p][0], wa[p][1]))
            zm = (_add(wa[p][0], wb[p][1]), _sub(wb[p][0], wa[p][1]))
            for j, z in enumerate((zp, zm)):
                for comp in range(2):
                    z_ref[j, (p * 16 + d) * 2 + comp] = z[comp].times(sigma)

    def real_bins():
        for m, u in ((0, UNIT0), (32, UNIT32)):
            for dt in range(2):
                for half, name in enumerate(("a", "b")):
                    vals = []
                    for p in range(2):
                        ev, od = acc[p, dt, name, 0], acc[p, dt, name, 1]
                        v = _add(ev, od) if m == 0 else _sub(ev, od)
                        vals.append(v.times(tau * LHS_SIGN[u, half] * COL_SIGN[u, dt]))
                    store(u, half, dt, vals[0], vals[1])

    def pass1(j, p, n2):
        z = [C(V(z_ref[j, (p * 16 + d) * 2]), V(z_ref[j, (p * 16 + d) * 2 + 1])) for d in (n2, n2 + 8)]
        z[0].r.a = pc.here(z[0].r.a)
        a = fft8(z + [None] * 6, 1)
        for k1 in range(8):
            t = a[k1].mul_w(n2 * k1, 64)
            assert (t.r.s, t.i.s) == WT_S1[k1, n2]
            t_ref[p, (k1 * 8 + n2) * 2] = t.r.a
            t_ref[p, (k1 * 8 + n2) * 2 + 1] = t.i.a

    def pass2(pm, k1):
        need = [k2 for k2 in range(8) if (k1 + 8 * k2) not in (0, 32)]
        outs = []
        for p in range(2):
            xs = [C(V(t_ref[p, (k1 * 8 + n2) * 2], WT_S1[k1, n2][0]),
                    V(t_ref[p, (k1 * 8 + n2) * 2 + 1], WT_S1[k1, n2][1])) for n2 in range(8)]
            if p == 0:
                xs[0].r.a = pc.here(xs[0].r.a)
            outs.append(fft8(xs, 1, need))
        for k2 in need:
            m = k1 + 8 * k2
            for u, half, nt, (cr, ci) in _weight_forms(m, pm):
                want = LHS_SIGN[u, half] * COL_SIGN[u, nt]
                store(u, half, nt, _combo(outs[0][k2], cr, ci, want), _combo(outs[1][k2], cr, ci, want))

    P = functools.partial
    out = [(P(prep, d), 40) for d in range(16)] + [(real_bins, 40)]
    for j, pm in enumerate((1, -1)):
        out += [(P(pass1, j, p, n2), 21 + _TW[n2]) for p in range(2) for n2 in range(8)]
        out += [(P(pass2, pm, k1), 193) for k1 in range(8)]
    return out


class View:
    def __init__(self, pool, base):
        self.pool = pool
        self.base = base

    def __getitem__(self, idx):
        h, i = idx
        return pltpu.bitcast(self.pool[self.base + h * 128 + i], f32)

    def __setitem__(self, idx, val):
        h, i = idx
        self.pool[self.base + h * 128 + i] = pltpu.bitcast(val, u32)


class XView:
    def __init__(self, pool, base, mg):
        self.pool, self.base, self.mg = pool, base, mg

    def index(self, u, g, c):
        return self.base + (u * self.mg + g) * 4 + c

    def store(self, u, g, c, val):
        self.pool[self.index(u, g, c)] = val

    def load(self, u, zero=None, mg=None):
        rows = []
        for g in range(self.mg if mg is None else mg):
            row = []
            for c in range(4):
                idx = self.index(u, g, c)
                if zero is not None and g == 0 and c == 0:
                    idx = idx + zero
                row.append(self.pool[idx])
            rows.append(jnp.concatenate(row, axis=1))
        return jnp.concatenate(rows, axis=0)


_TW = (0, 42, 40, 42, 32, 42, 40, 42)
COST_F1 = tuple(73 + t for t in _TW)
COST_I1 = tuple(57 + t for t in _TW)
COST_F2, COST_I2, COST_ACT = 153, 53, 85
FWD_S1, _ = _fft64_signs(-1)
INV_S1, _INV_OUT = _fft64_signs(1, in_sign=Y_SIGN)
INV_S2 = {m: (v.r.s, v.i.s) for m, v in _INV_OUT.items()}
CLASSES = ((1, 7), (2, 6), (3, 5), (4, 0))


def _class_units(cls):
    ks = [k for k in range(1, 32) if k % 8 in cls or (-k) % 8 in cls]
    ks.sort(key=lambda k: (0 if k % 8 == cls[0] else 1, k))
    out = [("pair", k) for k in ks]
    if 0 in cls:
        out += [("real", 0), ("real", 32)]
    return out


def fwd_p1(load, t_ref, h, n2, ct, pc):
    xs = []
    for n1 in range(8):
        lo, hi = load(h, 8 * n1 + n2, ct, pc if n1 == 0 else None)
        xs.append(C(V(lo), V(hi)))
    a = fft8(xs, -1)
    for k1 in range(8):
        t = a[k1].mul_w(-n2 * k1, 64)
        assert (t.r.s, t.i.s) == FWD_S1[k1, n2]
        t_ref[h, (k1 * 8 + n2) * 2] = t.r.a
        t_ref[h, (k1 * 8 + n2) * 2 + 1] = t.i.a


def fwd_p2(t_ref, x_ref, g, ct, k1, pc):
    outs = []
    for h in range(2):
        xs = [C(V(t_ref[h, (k1 * 8 + n2) * 2], FWD_S1[k1, n2][0]),
                V(t_ref[h, (k1 * 8 + n2) * 2 + 1], FWD_S1[k1, n2][1])) for n2 in range(8)]
        if h == 0:
            xs[0].r.a = pc.here(xs[0].r.a)
        outs.append(fft8(xs, -1))
    for k2 in range(8):
        m = k1 + 8 * k2
        f0 = _lhs_forms(m, outs[0][k2])
        f1 = _lhs_forms(m, outs[1][k2])
        for i, ((u, half, v0), (_, _, v1)) in enumerate(zip(f0, f1)):
            assert v0.s == v1.s == LHS_SIGN[u, half]
            x_ref.store(u, g, 2 * half + ct, _pack(v0.a, v1.a))
    return COST_F2


def inv_p1(y_ref, t_ref, g, h, n2, pc):
    rows = pl.ds(g * 16 + 8 * h, 8)
    ysg = Y_SIGN
    xs = []
    for n1 in range(8):
        m = 8 * n1 + n2
        xs.append(C(V(y_ref[2 * m, rows, :], ysg.get((m, 0), 1)),
                    V(y_ref[2 * m + 1, rows, :], ysg.get((m, 1), 1))))
    xs[0].r.a = pc.here(xs[0].r.a)
    a = fft8(xs, 1)
    for k1 in range(8):
        t = a[k1].mul_w(n2 * k1, 64)
        assert (t.r.s, t.i.s) == INV_S1[k1, n2]
        t_ref[h, (k1 * 8 + n2) * 2] = t.r.a
        t_ref[h, (k1 * 8 + n2) * 2 + 1] = t.i.a


def inv_p2(t_ref, r_ref, h, k1, pc):
    xs = [C(V(t_ref[h, (k1 * 8 + n2) * 2], INV_S1[k1, n2][0]),
            V(t_ref[h, (k1 * 8 + n2) * 2 + 1], INV_S1[k1, n2][1])) for n2 in range(8)]
    xs[0].r.a = pc.here(xs[0].r.a)
    b = fft8(xs, 1, range(S // 8))
    for k2 in range(S // 8):
        assert (b[k2].r.s, b[k2].i.s) == INV_S2[k1 + 8 * k2]
        r_ref[h, (k1 * 6 + k2) * 2] = b[k2].r.a
        r_ref[h, (k1 * 6 + k2) * 2 + 1] = b[k2].i.a
    return COST_I2


def _act(r_ref, h, k1, k2, dt, first, pc):
    a = r_ref[h, (k1 * 6 + k2) * 2 + dt]
    if first:
        a = pc.here(a)
    return _gelu_half(V(a, INV_S2[k1 + 8 * k2][dt]))


def act_conv1(r_ref, zh_ref, tau0, q, pc):
    h, k1, part = q // 8, 2 * ((q % 8) // 2), q % 2
    first = True
    for k2 in range(3 * part, 3 * part + 3):
        for dt in range(2):
            ev = _act(r_ref, h, k1, k2, dt, first, pc)
            od = _act(r_ref, h, k1 + 1, k2, dt, False, pc)
            first = False
            zh_ref[tau0 + (k1 // 2 + 4 * k2), h, 0, :, _lanes(dt)] = pc.due(ev)
            zh_ref[tau0 + (k1 // 2 + 4 * k2), h, 1, :, _lanes(dt)] = pc.due(od)
    return COST_ACT


def act_conv2(r_ref, f_ref, tau0, q, pc):
    k1, part = q // 2, q % 2
    first = True
    for k2 in range(3 * part, 3 * part + 3):
        for dt in range(2):
            oa = _act(r_ref, 0, k1, k2, dt, first, pc)
            ob = _act(r_ref, 1, k1, k2, dt, False, pc)
            first = False
            f_ref[tau0 + (k1 + 8 * k2), :, _lanes(dt)] = pc.due(_pack(oa, ob))
    return COST_ACT


def inverse_tail(t_ref, r_ref, act, pc, pairs_in_time):
    P = functools.partial
    out = []
    if pairs_in_time:
        for h in range(2):
            for kp in range(4):
                out += [(P(inv_p2, t_ref, r_ref, h, 2 * kp + j, pc), COST_I2) for j in range(2)]
                out += [(P(act, h * 8 + kp * 2 + j, pc), COST_ACT) for j in range(2)]
    else:
        for k1 in range(8):
            out += [(P(inv_p2, t_ref, r_ref, h, k1, pc), COST_I2) for h in range(2)]
            out += [(P(act, k1 * 2 + j, pc), COST_ACT) for j in range(2)]
    return out


def _mm(x_ref, u_ref, j, pc=None, mg=None):
    opaque = pc is not None and pc.unit % OPQ_EVERY == 0
    a = x_ref.load(j, pc.zero if opaque else None, mg)
    if pc is not None:
        a = pc.gate(a)
    a = pltpu.bitcast(a, bf16)
    w = pltpu.bitcast(u_ref.load(j), bf16)
    return jnp.dot(a, w, preferred_element_type=f32)


def _tokens(y):
    m = y.shape[0]
    return [y[8 * r:8 * r + 8, 128 * n:128 * n + 128] for n in range(2) for r in range(m // 8)]


def matmul_stream(x_ref, u_ref, y_ref, pc=None, mg=None):
    def tiles(y, u):
        return [V(y[:, :128], COL_SIGN[u, 0]), V(y[:, 128:], COL_SIGN[u, 1])]

    if mg is not None:
        y_ref = y_ref.at[:, pl.ds(0, 16 * mg), :]
    for cls in CLASSES:
        for kind, k in _class_units(cls):
            if kind == "pair":
                j = (k - 1) * 3
                y1 = _mm(x_ref, u_ref, j, pc, mg)
                k1 = tiles(y1, j)
                yield _tokens(y1)
                y2 = _mm(x_ref, u_ref, j + 1, pc, mg)
                k2 = tiles(y2, j + 1)
                for nt, m in ((0, k), (1, 64 - k)):
                    yi = k1[nt] + k2[nt]
                    assert (yi.s if nt == 0 else -yi.s) == Y_SIGN[m, 1]
                    y_ref[2 * m + 1] = yi.a
                yield _tokens(y2)
                y3 = _mm(x_ref, u_ref, j + 2, pc, mg)
                k3 = tiles(y3, j + 2)
                for nt, m in ((0, k), (1, 64 - k)):
                    yr = k1[nt] - k3[nt]
                    assert yr.s == Y_SIGN[m, 0]
                    y_ref[2 * m] = yr.a
                yield _tokens(y3)
            else:
                y = _mm(x_ref, u_ref, UNIT0 if k == 0 else UNIT32, pc, mg)
                y_ref[2 * k] = y[:, :128]
                y_ref[2 * k + 1] = y[:, 128:]
                yield _tokens(y)


def run_step(mm, pieces, costs, pc, ntok, lead, lag=None, due=None, nunits=NUNITS):
    total = float(sum(costs))
    lag = LAG if lag is None else lag
    tokens = []
    marks = []
    c = 0.0
    for piece, cost in zip(pieces, costs):
        pc.tok = None
        pc.tok2 = marks[-lag] if lag and len(marks) >= lag else None
        if c >= lead:
            want = min(int((c - lead) / (total - lead) * ntok), ntok - 1)
            ahead = min(want + (AHEAD * ntok) // max(nunits, NUNITS), ntok - 1)
            while ahead >= len(tokens):
                tokens += next(mm)
            pc.tok = tokens[want]
        pc.outs = []
        piece()
        marks.append(pc.last)
        for i, v in enumerate(pc.outs):
            q = pc.unit + (DUE if due is None else due) + i // 4
            if q < nunits:
                pc.pending.append((q, v))
        c += cost
    pc.tok = pc.tok2 = None
    for _ in mm:
        pass


def _make_kernel(T):
    T1, T2 = T // 2, T // 4
    L1 = (T1 + 16) // SEG
    L2 = L1 // 2
    assert L1 * SEG == T1 + 16 and L1 % 2 == 0
    NB1 = -(-L1 // S)
    NB2 = -(-L2 // S)
    XPAD = 8
    XB = T1 + 16
    XROWS = XPAD + 2 * XB + 64
    MG = 3
    M = 16 * MG
    NC1 = -(-NB1 // MG)
    NC2 = -(-NB2 // MG)
    ZH = (NB2 - 1) * S + N
    ZDUMP = ZH
    TB = 56
    NCH = -(-L2 // TB)
    FROWS = max(NB2 * S, NCH * TB)
    FDUMP = FROWS
    last_valid = T2 - (SEG - 1) * L2
    XPART = (0, 304, 592)

    def x_rows(e, part):
        def start(e, part):
            if e >= SEG:
                return T1
            return max(L1 * e + XPART[part] - (8 if part == 0 else 0), 0) // 8 * 8
        if part + 1 < len(XPART):
            return start(e, part), start(e, part + 1)
        return start(e, part), start(e + 1, 0)

    def kernel(x_hbm, w1_hbm, w2_hbm, g_ref, wf_ref, wg_ref, wo_ref, gm_ref, o_hbm,
               xs0, xs1, w_ref, ws0, ws1, u1_ref, u2_ref, pool, y_ref, zh_ref, f_ref, fe_ref, ge_ref,
               st_ref, sem_w, sem_x, sem_o):
        xs = (xs0, xs1)
        x_ref = XView(pool, 0, MG)
        tf = [[View(pool, NUNITS * MG * 4 + (g * 2 + ct) * 256) for ct in range(2)] for g in range(MG)]
        ti = [View(pool, NUNITS * MG * 4 + MG * 512 + g * 256) for g in range(MG)]
        tr = [View(pool, NUNITS * MG * 4 + MG * 768 + g * 256) for g in range(MG)]
        xh = x_hbm.bitcast(u32)
        w1w = w1_hbm.bitcast(u32)
        w2w = w2_hbm.bitcast(u32)

        W1PART = (0, 16, 32, 64, 96, 128)
        W2PART = (0, 16, 32, 128)

        def w1_copy(q):
            rows = pl.ds(W1PART[q], W1PART[q + 1] - W1PART[q])
            return pltpu.make_async_copy(w1w.at[:, rows, :], w_ref.at[:, rows, :], sem_w.at[q % 4])

        ws = (ws0, ws1)

        def w2_copies(part):
            lo, n = W2PART[part], W2PART[part + 1] - W2PART[part]
            return [pltpu.make_async_copy(w2w.at[i, pl.ds(lo, n), _lanes(dt)],
                                          ws[dt].at[pl.ds(WP * i + lo, n), :], sem_w.at[4 + part % 2])
                    for i in range(31) for dt in range(2)]

        def w2_wait(part):
            buf = ws0.at[pl.ds(0, 31 * (W2PART[part + 1] - W2PART[part])), :]
            for _ in range(2):
                pltpu.make_async_copy(buf, buf, sem_w.at[4 + part % 2]).wait()

        def x_copies(part):
            cps = []
            for b in range(2):
                for e in range(SEG):
                    lo, hi = x_rows(e, part)
                    for ct in range(2):
                        cps.append(pltpu.make_async_copy(
                            xh.at[b, pl.ds(lo, hi - lo), _lanes(ct)],
                            xs[ct].at[pl.ds(XPAD + b * XB + lo, hi - lo), :],
                            sem_x.at[part]))
            return cps

        w1_copy(0).start()
        for cp in w2_copies(0):
            cp.start()
        w1_copy(1).start()
        for cp in w2_copies(1):
            cp.start()
        w1_copy(2).start()
        for dt in range(2):
            for r in range(31 * WP, 31 * WP + 128, 8):
                ws[dt][pl.ds(r, 8), :] = jnp.zeros((8, 128), u32)
        gbase = NUNITS * MG * 4 + MG * 1024
        for r in range(24):
            pool[gbase + r] = gm_ref[pl.ds(8 * r, 8), :]

        def g_view(zero):
            return jnp.concatenate([pool[gbase + r + (zero if r == TAP_OPQ else 0)] for r in range(24)], axis=0)

        z8 = jnp.zeros((8, 128), u32)
        for ct in range(2):
            xs[ct][pl.ds(0, 8), :] = z8
            for r in range(XPAD + T1, XPAD + XB, 8):
                xs[ct][pl.ds(r, 8), :] = z8
            for r in range(XPAD + XB + T1, XROWS, 8):
                xs[ct][pl.ds(r, 8), :] = z8

        def zero_zh(i, c):
            for h in range(2):
                for comp in range(2):
                    zh_ref[ZH - 1 - i, h, comp] = jnp.zeros((8, 256), f32)
            return c
        lax.fori_loop(0, ZH - 8 - L2, zero_zh, 0)

        zf = jnp.zeros((M, 128), f32)
        for m in range(0, 64, 4):
            y_ref[2 * m] = zf
            y_ref[2 * m + 1] = zf
        for g in range(MG):
            for h in range(2):
                for k1 in range(8):
                    for n2 in (1, 2, 3, 5, 6, 7):
                        for comp in range(2):
                            ti[g][h, (k1 * 8 + n2) * 2 + comp] = jnp.zeros((8, 128), f32)

        gg = g_ref[...].reshape(16, 256)
        ge_all = jnp.dot(gg, wg_ref[...], preferred_element_type=f32)
        ge_ref[...] = ge_all
        never = jnp.max(jnp.abs(ge_all)) < 0.0

        def transform(hook):
            def body(i, c):
                for j in range(WT_UNROLL):
                    hook(i * WT_UNROLL + j)
                pc = Pacer(i < 0, lax.shift_right_arithmetic(i, 20))
                seq = []
                for j in range(WT_UNROLL):
                    seq += weight_pieces(w_ref, UView(u1_ref), tf[j][0], tf[j][1], i * WT_UNROLL + j, pc)
                n = 4 * WT_UNROLL
                run_step(tap_stream(g_view, ws, u2_ref, n * i, n, pc), [q[0] for q in seq],
                         [q[1] for q in seq], pc, n * 192, LEAD, nunits=n)
                return c
            lax.fori_loop(0, 16 // WT_UNROLL, body, 0)

        def w1_hook(rg):
            for q in range(len(W1PART) - 1):
                @pl.when(rg * 8 == W1PART[q])
                def _(q=q):
                    w1_copy(q).wait()
                    if q < len(W2PART) - 1:
                        w2_wait(q)
                    if q == 0:
                        for cp in w2_copies(2):
                            cp.start()
                    if q + 3 < len(W1PART) - 1:
                        w1_copy(q + 3).start()
                    if q >= 2:
                        for cp in x_copies(q - 2):
                            cp.start()

        def conv(nchunk, nblk, u_ref, make_load, act, pairs_in_time, out_index, wait_input=None):
            def loads(c):
                return [make_load(jnp.minimum(c * MG + g, nblk - 1)) for g in range(MG)]

            def P(fn, *a):
                return functools.partial(fn, *a)

            def f1(ld, pc):
                return [(P(fwd_p1, ld[g], tf[g][ct], h, n2, ct, pc), COST_F1[n2])
                        for g in range(MG) for ct in range(2) for h in range(2) for n2 in range(8)]

            def f2(cls, pc, mg=MG):
                return [(P(fwd_p2, tf[g][ct], x_ref, g, ct, k1, pc), COST_F2)
                        for g in range(mg) for ct in range(2) for k1 in cls]

            def i1(cls, pc, mg=MG):
                return [(P(inv_p1, y_ref, ti[g], g, h, n2, pc), COST_I1[n2])
                        for g in range(mg) for h in range(2) for n2 in cls]

            def i2(c, pc, mg=MG):
                out = []
                for g in range(mg):
                    out += inverse_tail(ti[g], tr[g], P(act, tr[g], out_index(c, g)), pc, pairs_in_time)
                return out

            idle = Pacer(None)
            if wait_input is not None:
                wait_input(0)
            with scope("pro"):
                for piece, _ in f1(loads(0), idle):
                    piece()
                for piece, _ in f2(CLASSES[0], idle):
                    piece()

            def step(c, cc):
                if wait_input is not None:
                    wait_input(c + 1)
                pc = Pacer(c < 0, lax.shift_right_arithmetic(c, 20))
                nxt = f1(loads(jnp.minimum(c + 1, nchunk - 1)), pc)
                half = len(nxt) // 2
                seq = (f2(CLASSES[1], pc) + f2(CLASSES[2], pc) + f2(CLASSES[3], pc)
                       + i1(CLASSES[3], pc) + i2(c - 1, pc)
                       + nxt[:half] + i1(CLASSES[0], pc) + nxt[half:]
                       + i1(CLASSES[1], pc) + f2(CLASSES[0], pc) + i1(CLASSES[2], pc))
                run_step(matmul_stream(x_ref, u_ref, y_ref, pc), [q[0] for q in seq], [q[1] for q in seq],
                         pc, NUNITS * (M // 4), LEAD)
                return cc

            def short_step(c, never, zero, mg):
                pc = Pacer(never, zero)
                seq = (f2(CLASSES[1], pc, mg) + f2(CLASSES[2], pc, mg) + f2(CLASSES[3], pc, mg)
                       + i1(CLASSES[3], pc) + i2(c - 1, pc)
                       + i1(CLASSES[0], pc, mg) + i1(CLASSES[1], pc, mg) + i1(CLASSES[2], pc, mg))
                run_step(matmul_stream(x_ref, u_ref, y_ref, pc, mg), [q[0] for q in seq],
                         [q[1] for q in seq], pc, NUNITS * 4 * mg, LEAD)

            tail = nblk - (nchunk - 1) * MG
            with scope("steps"):
                lax.fori_loop(0, nchunk if tail == MG else nchunk - 1, step, 0)
                if tail < MG:
                    short_step(nchunk - 1, never, never.astype(i32), tail)

            with scope("epi"):
                for piece, _ in i1(CLASSES[3], idle, tail) + i2(nchunk - 1, idle, tail):
                    piece()

        with scope("wt1"):
            transform(w1_hook)

        def x_wait(part):
            rows = sum(4 * (x_rows(e, part)[1] - x_rows(e, part)[0]) for e in range(SEG))
            buf = xs0.at[pl.ds(0, rows), :]
            pltpu.make_async_copy(buf, buf, sem_x.at[part]).wait()

        def wait_x0(c):
            if isinstance(c, int):
                x_wait(0)
                return
            for part, first in ((1, 2), (2, 4)):
                @pl.when(c == first)
                def _(part=part):
                    x_wait(part)

        def load1(blk):
            base = blk * S

            def load(h, n, ct, pc):
                w = xs[ct][pl.ds(base + n + h * L1, 8, stride=2 * L1), :]
                if pc is not None:
                    w = pc.here(w)
                return _unpack(w)
            return load

        def act1(rb, tau0, q, pc):
            return act_conv1(rb, zh_ref, tau0, q, pc)

        def out1(c, g):
            if isinstance(c, int):
                return 8 + (c * MG + g) * (S // 2)
            return jnp.where(c >= 0, 8 + (c * MG + g) * (S // 2), ZDUMP)

        conv(NC1, NB1, UView(u1_ref), load1, act1, True, out1, wait_x0)

        row = lax.broadcasted_iota(i32, (8, 256), 0)
        for h in range(2):
            for comp in range(2):
                for t in range(last_valid, NB1 * S // 2):
                    zh_ref[8 + t, h, comp] = jnp.where(row == SEG - 1, 0.0, zh_ref[8 + t, h, comp])
                for j in range(8):
                    v = pltpu.roll(zh_ref[8 + L2 - 8 + j, h, comp], 1, axis=0)
                    zh_ref[j, h, comp] = jnp.where(row == 0, 0.0, v)
                for j in range(8):
                    v = pltpu.roll(zh_ref[8 + j, h, comp], SEG - 1, axis=0)
                    zh_ref[8 + L2 + j, h, comp] = jnp.where(row == SEG - 1, 0.0, v)


        def load2(blk):
            def load(h, n, ct, pc):
                lo = zh_ref[blk * S + n, h, 0, :, _lanes(ct)]
                hi = zh_ref[blk * S + n, h, 1, :, _lanes(ct)]
                if pc is not None:
                    lo = pc.here(lo)
                return lo, hi
            return load

        def act2(rb, tau0, q, pc):
            return act_conv2(rb, f_ref, tau0, q, pc)

        def out2(c, g):
            if isinstance(c, int):
                return min(c * MG + g, NB2 - 1) * S
            return jnp.where(c >= 0, jnp.minimum(c * MG + g, NB2 - 1) * S, FDUMP)

        conv(NC2, NB2, UView(u2_ref), load2, act2, False, out2)

        order = [(b, e) for b in range(2) for e in range(SEG)]

        def out_copy(half, q, t0, nvalid):
            b, e = order[q]
            r0 = (b * T2 + e * L2) * 8 + t0 * 8
            return pltpu.make_async_copy(st_ref.at[half, q, pl.ds(0, nvalid * 8), :],
                                         o_hbm.at[pl.ds(r0, nvalid * 8), :],
                                         sem_o.at[half])

        def width(e):
            lim = L2 if e < SEG - 1 else last_valid
            return lim - (NCH - 1) * TB

        def joint_chunk(ch, half, full, never):
            pc = Pacer(never)
            t0 = ch * TB
            fl = pltpu.bitcast(f_ref[pl.ds(t0, TB)].reshape(TB * 8, 256), bf16)
            fe = jnp.dot(fl, wf_ref[...], preferred_element_type=f32)
            fe_ref[...] = fe
            prev = [fe[8 * r:8 * r + 8, 128 * n:128 * n + 128] for n in range(2) for r in range(2 * TB)]
            prev = prev[len(prev) // 2:]
            for q, (b, e) in enumerate(order):
                ge = ge_ref[pl.ds(8 * b, 8), :]
                r = 4 * (e & 3) + 2 * b + (e >> 2)
                js = []
                for t in range(TB):
                    row = jnp.broadcast_to(fe_ref[pl.ds(16 * t + r, 1), :], (8, 256))
                    tok = prev[(t * len(prev)) // TB]
                    gt = jnp.concatenate([pc.tie(ge[:, :128], tok), pc.tie(ge[:, 128:], tok)], axis=1)
                    js.append(jnp.tanh(row + gt))
                jl = jnp.concatenate(js, axis=0).astype(bf16)
                y = jnp.dot(jl, wo_ref[...], preferred_element_type=f32)
                prev = [y[8 * rr:8 * rr + 8, 128 * n:128 * n + 128] for n in range(2) for rr in range(TB)]
                st_ref[half, q] = y.astype(bf16)
                out_copy(half, q, t0, TB if full else width(e)).start()

        def wait_chunk(half, full):
            if full:
                pltpu.make_async_copy(st_ref.at[half], st_ref.at[half], sem_o.at[half]).wait()
                return
            for q, (b, e) in enumerate(order):
                out_copy(half, q, 0, width(e)).wait()

        def joint_body(ch, c):
            half = ch % 2

            @pl.when(ch >= 2)
            def _():
                wait_chunk(half, True)
            joint_chunk(ch, half, True, ch < 0)
            return c
        with scope("joint"):
            lax.fori_loop(0, NCH - 1, joint_body, 0)
            last_half = (NCH - 1) % 2
            wait_chunk(last_half, True)
            joint_chunk(NCH - 1, last_half, False, never)
            wait_chunk(1 - last_half, True)
            wait_chunk(last_half, False)

    scratch = [
        pltpu.VMEM((XROWS, 128), u32), pltpu.VMEM((XROWS, 128), u32),
        pltpu.VMEM((31, 128, 256), u32),
        pltpu.VMEM((32 * WP + 8, 128), u32), pltpu.VMEM((32 * WP + 8, 128), u32),
        pltpu.VMEM((2 * 96 * UP, 128), u32), pltpu.VMEM((2 * 96 * UP, 128), u32),
        pltpu.VMEM((NUNITS * MG * 4 + MG * 1024 + 24, 8, 128), u32),
        pltpu.VMEM((128, M, 128), f32),
        pltpu.VMEM((ZH + S // 2, 2, 2, 8, 256), f32),
        pltpu.VMEM((FROWS + S, 8, 256), u32),
        pltpu.VMEM((TB * 16, 256), f32),
        pltpu.VMEM((16, 256), f32),
        pltpu.VMEM((2, 2 * SEG, TB * 8, 256), bf16),
        pltpu.SemaphoreType.DMA((6,)),
        pltpu.SemaphoreType.DMA((3,)),
        pltpu.SemaphoreType.DMA((2,)),
    ]
    return kernel, scratch


TAP_MATRIX = _tap_matrix()
WT_UNROLL = 2
TAP_OPQ = 23
TAP_GATE = 20
LEAD = 0
LAG = 0
AHEAD = 2
OPQ_EVERY = 1
DUE = 0
DUE_EVERY = 1000


def _call(x, w1, w2, g, w_f, w_g, w_o, interpret=False):
    B, T, D = x.shape
    kernel, scratch = _make_kernel(T)
    T2 = T // 4
    any_spec = pl.BlockSpec(memory_space=pl.ANY)
    vmem = pl.BlockSpec(memory_space=pltpu.VMEM)
    out = pl.pallas_call(
        kernel,
        out_shape=jax.ShapeDtypeStruct((B * T2 * 8, D), bf16),
        in_specs=[any_spec, any_spec, any_spec, vmem, vmem, vmem, vmem, vmem],
        out_specs=any_spec,
        scratch_shapes=scratch,
        compiler_params=pltpu.CompilerParams(vmem_limit_bytes=126 * 2**20),
        interpret=interpret,
        name="conv_stem_rnnt_joint",
    )(x, w1, w2, g, w_f, w_g, w_o, TAP_MATRIX)
    return out.reshape(B, T2, 8, D)


@jax.jit
def pallas_standalone__seq2seq_rnn_t_joint__speech_kernel(x, w1, w2, g, w_f, w_g, w_o):
    return _call(x, w1, w2, g, w_f, w_g, w_o)
```

```python
import functools
import math

import jax
import jax.numpy as jnp
import numpy as np
from jax import lax
from jax.experimental import pallas as pl
from jax.experimental.pallas import tpu as pltpu

f32, u32, bf16, i32 = jnp.float32, jnp.uint32, jnp.bfloat16, jnp.int32

PROFILE_SCOPES = False


class _NoScope:
    def __enter__(self):
        return self

    def __exit__(self, *a):
        return False


def scope(name):
    return jax.named_scope(name) if PROFILE_SCOPES else _NoScope()

N = 64
S = 48
SEG = 8


class V:
    __slots__ = ("a", "s")

    def __init__(self, a, s=1):
        self.a = a
        self.s = s

    def __neg__(self):
        return V(self.a, -self.s)

    def __add__(self, o):
        if self.s == o.s:
            return V(self.a + o.a, self.s)
        if self.s > 0:
            return V(self.a - o.a, 1)
        return V(o.a - self.a, 1)

    def __sub__(self, o):
        return self + (-o)

    def scale(self, c):
        if c == 1.0:
            return self
        if c == -1.0:
            return -self
        return V(self.a * np.float32(abs(c)), self.s * (1 if c > 0 else -1))

    def times(self, c):
        return self.a * np.float32(self.s * c)

    def signed(self, s):
        return self.a if self.s * s > 0 else -self.a


class C:
    __slots__ = ("r", "i")

    def __init__(self, r, i):
        self.r = r
        self.i = i

    def __add__(self, o):
        return C(self.r + o.r, self.i + o.i)

    def __sub__(self, o):
        return C(self.r - o.r, self.i - o.i)

    def __neg__(self):
        return C(-self.r, -self.i)

    def mul_w(self, num, den):
        num %= den
        if num == 0:
            return self
        if 4 * num == den:
            return C(-self.i, self.r)
        if 2 * num == den:
            return -self
        if 4 * num == 3 * den:
            return C(self.i, -self.r)
        if (8 * num) % den == 0:
            o = (8 * num) // den
            h = math.sqrt(0.5)
            sc = 1 if o in (1, 7) else -1
            ss = 1 if o in (1, 3) else -1
            r, m = self.r, self.i
            re = (r if sc > 0 else -r) - (m if ss > 0 else -m)
            im = (r if ss > 0 else -r) + (m if sc > 0 else -m)
            return C(re.scale(h), im.scale(h))
        c = math.cos(2 * math.pi * num / den)
        s = math.sin(2 * math.pi * num / den)
        return C(self.r.scale(c) - self.i.scale(s), self.r.scale(s) + self.i.scale(c))


def _add(a, b):
    if a is None:
        return b
    if b is None:
        return a
    return a + b


def _sub(a, b):
    if b is None:
        return a
    if a is None:
        return -b
    return a - b


def fft8(x, sgn, need=tuple(range(8))):
    def rot(a, num, den):
        return None if a is None else a.mul_w(sgn * num, den)

    need = set(need)
    a0, a1 = _add(x[0], x[4]), _sub(x[0], x[4])
    a2, a3 = _add(x[2], x[6]), rot(_sub(x[2], x[6]), 1, 4)
    a4, a5 = _add(x[1], x[5]), _sub(x[1], x[5])
    a6, a7 = _add(x[3], x[7]), rot(_sub(x[3], x[7]), 1, 4)
    out = {}
    if need & {0, 4}:
        b0, b4 = _add(a0, a2), _add(a4, a6)
        if 0 in need:
            out[0] = _add(b0, b4)
        if 4 in need:
            out[4] = _sub(b0, b4)
    if need & {2, 6}:
        b2, b6 = _sub(a0, a2), rot(_sub(a4, a6), 1, 4)
        if 2 in need:
            out[2] = _add(b2, b6)
        if 6 in need:
            out[6] = _sub(b2, b6)
    if need & {1, 5}:
        b1, b5 = _add(a1, a3), rot(_add(a5, a7), 1, 8)
        if 1 in need:
            out[1] = _add(b1, b5)
        if 5 in need:
            out[5] = _sub(b1, b5)
    if need & {3, 7}:
        b3, b7 = _sub(a1, a3), rot(_sub(a5, a7), 3, 8)
        if 3 in need:
            out[3] = _add(b3, b7)
        if 7 in need:
            out[7] = _sub(b3, b7)
    return out


class _Sym:
    def __add__(self, o):
        return self

    __sub__ = __mul__ = __add__

    def __neg__(self):
        return self


def _fft64_signs(sgn, present=tuple(range(64)), in_sign=None):
    d = _Sym()
    in_sign = in_sign or {}
    x = [C(V(d, in_sign.get((n, 0), 1)), V(d, in_sign.get((n, 1), 1))) if n in present else None
         for n in range(64)]
    t = {}
    for n2 in range(8):
        a = fft8([x[8 * n1 + n2] for n1 in range(8)], sgn)
        for k1 in range(8):
            t[k1, n2] = a[k1].mul_w(sgn * n2 * k1, 64)
    s1 = {key: (v.r.s, v.i.s) for key, v in t.items()}
    s2 = {}
    for k1 in range(8):
        b = fft8([t[k1, n2] for n2 in range(8)], sgn)
        for k2 in range(8):
            s2[k1 + 8 * k2] = b[k2]
    return s1, s2


def _unit(k, j):
    return (k - 1) * 3 + j


UNIT0, UNIT32 = 93, 94
NUNITS = 95


def _lhs_forms(m, z):
    if m in (0, 32):
        u = UNIT0 if m == 0 else UNIT32
        return [(u, 0, z.r), (u, 1, z.i)]
    if m < 32:
        return [(_unit(m, 0), 0, z.r + z.i), (_unit(m, 1), 0, z.r), (_unit(m, 2), 0, z.i)]
    k = 64 - m
    return [(_unit(k, 0), 1, z.r - z.i), (_unit(k, 1), 1, z.r), (_unit(k, 2), 1, z.i)]


def _lhs_signs():
    _, s2 = _fft64_signs(-1)
    sg = {}
    for m in range(64):
        for u, h, v in _lhs_forms(m, s2[m]):
            sg[u, h] = v.s
    return sg


LHS_SIGN = _lhs_signs()


def _weight_forms(m, pm):
    if m < 32:
        nt = 0 if pm > 0 else 1
        return [(_unit(m, 0), 1, nt, (1, 0)), (_unit(m, 1), 1, nt, (-1, 1)), (_unit(m, 2), 1, nt, (-1, -1))]
    k = 64 - m
    nt = 1 if pm > 0 else 0
    return [(_unit(k, 0), 0, nt, (1, 0)), (_unit(k, 1), 0, nt, (-1, -1)), (_unit(k, 2), 0, nt, (1, -1))]


def _weight_plan():
    s1, s2 = _fft64_signs(1, present=range(16))
    forms = {}
    for pm in (1, -1):
        for m in range(1, 64):
            if m == 32:
                continue
            for u, half, nt, (cr, ci) in _weight_forms(m, pm):
                forms[u, half, nt] = (cr * s2[m].r.s, ci * s2[m].i.s)
    col = {}
    for u in range(93):
        for nt in range(2):
            def negs(sig):
                n = 0
                for half in range(2):
                    cr, ci = forms[u, half, nt]
                    w = sig * LHS_SIGN[u, half]
                    n += (w * cr <= 0 and w * ci <= 0)
                return n
            col[u, nt] = 1 if negs(1) <= negs(-1) else -1
    for u in (UNIT0, UNIT32):
        col[u, 0] = col[u, 1] = 1
    return s1, s2, col


WT_S1, WT_S2, COL_SIGN = _weight_plan()


def _recombine(k1, k2, k3, k):
    out = {}
    for nt in range(2):
        yr = k1[nt] - k3[nt]
        yi = k1[nt] + k2[nt]
        if nt == 0:
            out[k, 0], out[k, 1] = yr, yi
        else:
            out[64 - k, 0], out[64 - k, 1] = yr, -yi
    return out


def _y_signs():
    d = _Sym()
    sg = {}
    for k in range(1, 32):
        ks = [[V(d, COL_SIGN[_unit(k, j), nt]) for nt in range(2)] for j in range(3)]
        for key, v in _recombine(ks[0], ks[1], ks[2], k).items():
            sg[key] = v.s
    for m, u in ((0, UNIT0), (32, UNIT32)):
        sg[m, 0], sg[m, 1] = COL_SIGN[u, 0], COL_SIGN[u, 1]
    return sg


Y_SIGN = _y_signs()


def _unpack(w):
    lo = pltpu.unpack_elementwise(w, index=0, packed_dtype=bf16, unpacked_dtype=f32)
    hi = pltpu.unpack_elementwise(w, index=1, packed_dtype=bf16, unpacked_dtype=f32)
    return lo, hi


def _pack(lo, hi):
    return pltpu.pack_elementwise([lo, hi], packed_dtype=bf16)


_GC1 = 2.0 * math.sqrt(2.0 / math.pi)
_GC2 = 8.0 * 0.044715 * math.sqrt(2.0 / math.pi)


def _gelu_half(v):
    a = v.a
    p = (a * a) * np.float32(_GC2) + np.float32(_GC1)
    t = jnp.tanh(p * a)
    return a * t + a if v.s > 0 else a * t - a


def _lanes(t):
    return pl.ds(128 * t, 128)


class Pacer:
    def __init__(self, never, zero=None):
        self.never = never
        self.tok = None
        self.tok2 = None
        self.last = None
        self.outs = []
        self.zero = zero
        self.pending = []
        self.unit = 0

    def gate(self, a, first=0):
        vals = [v for q, v in self.pending if q <= self.unit]
        self.pending = [(q, v) for q, v in self.pending if q > self.unit]
        self.unit += 1
        if not vals:
            return a
        m, k = a.shape
        tiles = [[a[8 * r:8 * r + 8, 128 * c:128 * c + 128] for c in range(k // 128)] for r in range(m // 8)]
        flat = [(r, c) for r in range(first, m // 8) for c in range(k // 128)]
        for i, v in enumerate(vals):
            r, c = flat[i % len(flat)]
            tiles[r][c] = self.tie(tiles[r][c], v)
        return jnp.concatenate([jnp.concatenate(row, axis=1) for row in tiles], axis=0)

    def here(self, x):
        tok, self.tok = self.tok, None
        tok2, self.tok2 = self.tok2, None
        return self.tie(self.tie(x, tok), tok2)

    def mark(self, x, nth=None):
        self.last = x
        if self.never is not None and nth is not None and nth % DUE_EVERY == DUE_EVERY - 1:
            self.outs.append(x)
        return x

    def due(self, x):
        if self.never is not None:
            self.outs.append(x)
        return x

    def tie(self, x, tok):
        if tok is None:
            return x
        if tok.dtype != x.dtype:
            tok = pltpu.bitcast(tok, x.dtype)
        return jnp.where(self.never, tok, x)


def _combo(f, cr, ci, want):
    if ci == 0:
        return f.r.signed(want * cr)
    v = (f.r if cr > 0 else -f.r) + (f.i if ci > 0 else -f.i)
    if v.s * want > 0:
        return v.a
    if f.r.s * cr != f.i.s * ci:
        return ((-f.r) if cr > 0 else f.r).__add__((-f.i) if ci > 0 else f.i).a
    return -v.a


UP = 260
WP = 132


class UView:
    def __init__(self, ref):
        self.ref = ref

    def load(self, u):
        return jnp.concatenate([self.ref[pl.ds((nt * 96 + u) * UP, 256), :] for nt in range(2)], axis=1)

    def store(self, u, half, nt, rg, val):
        self.ref[pl.ds((nt * 96 + u) * UP + half * 128 + rg * 8, 8), :] = val


def _tap_matrix():
    import ml_dtypes
    sigma, tau = 1.0 / 256.0, 1.0 / 128.0
    g = np.zeros((2, 2, 96, 32, 2))
    d = np.arange(16)
    for tap in range(31):
        for dt in range(2):
            wa = np.zeros((16, 2))
            wb = np.zeros((16, 2))
            if tap % 2:
                wa[(tap + 1) // 2, dt] = 1.0
            else:
                wb[tap // 2, dt] = 1.0
            z0 = wa[:, 0] + 1j * wb[:, 0]
            z1 = wa[:, 1] + 1j * wb[:, 1]
            for pm, z in ((1, z0 + 1j * z1), (-1, z0 - 1j * z1)):
                for m in range(1, 64):
                    if m == 32:
                        continue
                    f = sigma * np.sum(z * np.exp(2j * np.pi * m * d / 64))
                    for u, half, nt, (cr, ci) in _weight_forms(m, pm):
                        g[nt, half, u, tap, dt] = (LHS_SIGN[u, half] * COL_SIGN[u, nt]
                                                   * (cr * f.real + ci * f.imag))
            for m, u in ((0, UNIT0), (32, UNIT32)):
                e = np.cos(np.pi * m * d / 32)
                for half, wv in enumerate((wa, wb)):
                    g[dt, half, u, tap, dt] = (LHS_SIGN[u, half] * COL_SIGN[u, dt]
                                               * tau * np.sum(e * wv[:, dt]))
    g = g.reshape(384, 32, 2)
    mat = np.zeros((384, 128))
    for v in range(4):
        dt, t0 = v // 2, 16 * (v % 2)
        for s_ in range(8):
            for par in range(2):
                mat[:, 16 * v + 2 * s_ + par] = g[:, t0 + 8 * par + s_, dt]
    hi = mat.astype(ml_dtypes.bfloat16)
    lo = (mat - hi.astype(np.float64)).astype(ml_dtypes.bfloat16)
    full = np.concatenate([hi[:, :64], lo[:, :64]], axis=1).view(np.uint16).astype(np.uint32)
    return full[0::2] | (full[1::2] << 16)


def tap_operand(ws, cpair):
    ev, od = [], []
    for dt in range(2):
        for t0 in (0, 16):
            wa = ws[dt][pl.ds(t0 * WP + cpair, 8, stride=WP), :]
            wb = ws[dt][pl.ds((t0 + 8) * WP + cpair, 8, stride=WP), :]
            alo, ahi = _unpack(wa)
            blo, bhi = _unpack(wb)
            ev.append(_pack(alo, blo))
            od.append(_pack(ahi, bhi))
    return jnp.concatenate(ev + ev, axis=0), jnp.concatenate(od + od, axis=0)


def tap_stream(g_view, ws, u2_ref, it0, n, pc):
    for q in range(n):
        it = it0 + q
        lhs = pltpu.bitcast(pc.gate(g_view(pc.zero), TAP_GATE), bf16)
        ops = []
        for j in range(2):
            ops += list(tap_operand(ws, 2 * it + j))
        rhs = pltpu.bitcast(jnp.concatenate(ops, axis=1), bf16)
        y = jnp.dot(lhs, rhs, preferred_element_type=f32)
        for r in range(48):
            nt, half, u0 = r // 24, (r // 12) % 2, (r % 12) * 8
            for j in range(2):
                val = _pack(y[8 * r:8 * r + 8, 256 * j:256 * j + 128],
                            y[8 * r:8 * r + 8, 256 * j + 128:256 * j + 256])
                u2_ref[pl.ds((nt * 96 + u0) * UP + half * 128 + 2 * it + j, 8, stride=UP), :] = val
        yield [y[8 * r:8 * r + 8, 128 * t:128 * t + 128] for r in range(48) for t in range(4)]


def weight_pieces(w_ref, u_ref, t_ref, z_ref, rg, pc):
    rows = pl.ds(pl.multiple_of(rg * 8, 8), 8)
    sigma = 1.0 / 256.0
    tau = 1.0 / 128.0
    acc = {}

    def store(u, half, nt, a0, a1):
        u_ref.store(u, half, nt, rg, pc.due(_pack(a0, a1)))

    def prep(d):
        wa = [[None, None], [None, None]]
        wb = [[None, None], [None, None]]
        for dt in range(2):
            w = w_ref[2 * d, rows, _lanes(dt)]
            if dt == 0:
                w = pc.here(w)
            lo, hi = _unpack(w)
            wb[0][dt], wb[1][dt] = V(lo), V(hi)
            if d > 0:
                lo, hi = _unpack(w_ref[2 * d - 1, rows, _lanes(dt)])
                wa[0][dt], wa[1][dt] = V(lo), V(hi)
        for p in range(2):
            for dt in range(2):
                for name, val in (("a", wa[p][dt]), ("b", wb[p][dt])):
                    key = (p, dt, name, d % 2)
                    acc[key] = _add(acc.get(key), val)
            zp = (_sub(wa[p][0], wb[p][1]), _add(wb[p][0], wa[p][1]))
            zm = (_add(wa[p][0], wb[p][1]), _sub(wb[p][0], wa[p][1]))
            for j, z in enumerate((zp, zm)):
                for comp in range(2):
                    z_ref[j, (p * 16 + d) * 2 + comp] = z[comp].times(sigma)

    def real_bins():
        for m, u in ((0, UNIT0), (32, UNIT32)):
            for dt in range(2):
                for half, name in enumerate(("a", "b")):
                    vals = []
                    for p in range(2):
                        ev, od = acc[p, dt, name, 0], acc[p, dt, name, 1]
                        v = _add(ev, od) if m == 0 else _sub(ev, od)
                        vals.append(v.times(tau * LHS_SIGN[u, half] * COL_SIGN[u, dt]))
                    store(u, half, dt, vals[0], vals[1])

    def pass1(j, p, n2):
        z = [C(V(z_ref[j, (p * 16 + d) * 2]), V(z_ref[j, (p * 16 + d) * 2 + 1])) for d in (n2, n2 + 8)]
        z[0].r.a = pc.here(z[0].r.a)
        a = fft8(z + [None] * 6, 1)
        for k1 in range(8):
            t = a[k1].mul_w(n2 * k1, 64)
            assert (t.r.s, t.i.s) == WT_S1[k1, n2]
            t_ref[p, (k1 * 8 + n2) * 2] = t.r.a
            t_ref[p, (k1 * 8 + n2) * 2 + 1] = t.i.a

    def pass2(pm, k1):
        need = [k2 for k2 in range(8) if (k1 + 8 * k2) not in (0, 32)]
        outs = []
        for p in range(2):
            xs = [C(V(t_ref[p, (k1 * 8 + n2) * 2], WT_S1[k1, n2][0]),
                    V(t_ref[p, (k1 * 8 + n2) * 2 + 1], WT_S1[k1, n2][1])) for n2 in range(8)]
            if p == 0:
                xs[0].r.a = pc.here(xs[0].r.a)
            outs.append(fft8(xs, 1, need))
        for k2 in need:
            m = k1 + 8 * k2
            for u, half, nt, (cr, ci) in _weight_forms(m, pm):
                want = LHS_SIGN[u, half] * COL_SIGN[u, nt]
                store(u, half, nt, _combo(outs[0][k2], cr, ci, want), _combo(outs[1][k2], cr, ci, want))

    P = functools.partial
    out = [(P(prep, d), 40) for d in range(16)] + [(real_bins, 40)]
    for j, pm in enumerate((1, -1)):
        out += [(P(pass1, j, p, n2), 21 + _TW[n2]) for p in range(2) for n2 in range(8)]
        out += [(P(pass2, pm, k1), 193) for k1 in range(8)]
    return out


class View:
    def __init__(self, pool, base):
        self.pool = pool
        self.base = base

    def __getitem__(self, idx):
        h, i = idx
        return pltpu.bitcast(self.pool[self.base + h * 128 + i], f32)

    def __setitem__(self, idx, val):
        h, i = idx
        self.pool[self.base + h * 128 + i] = pltpu.bitcast(val, u32)


class XView:
    def __init__(self, pool, base, mg):
        self.pool, self.base, self.mg = pool, base, mg

    def index(self, u, g, c):
        return self.base + (u * self.mg + g) * 4 + c

    def store(self, u, g, c, val):
        self.pool[self.index(u, g, c)] = val

    def load(self, u, zero=None, mg=None):
        rows = []
        for g in range(self.mg if mg is None else mg):
            row = []
            for c in range(4):
                idx = self.index(u, g, c)
                if zero is not None and g == 0 and c == 0:
                    idx = idx + zero
                row.append(self.pool[idx])
            rows.append(jnp.concatenate(row, axis=1))
        return jnp.concatenate(rows, axis=0)


_TW = (0, 42, 40, 42, 32, 42, 40, 42)
COST_F1 = tuple(73 + t for t in _TW)
COST_I1 = tuple(57 + t for t in _TW)
COST_F2, COST_I2, COST_ACT = 153, 53, 85
FWD_S1, _ = _fft64_signs(-1)
INV_S1, _INV_OUT = _fft64_signs(1, in_sign=Y_SIGN)
INV_S2 = {m: (v.r.s, v.i.s) for m, v in _INV_OUT.items()}
CLASSES = ((1, 7), (2, 6), (3, 5), (4, 0))


def _class_units(cls):
    ks = [k for k in range(1, 32) if k % 8 in cls or (-k) % 8 in cls]
    ks.sort(key=lambda k: (0 if k % 8 == cls[0] else 1, k))
    out = [("pair", k) for k in ks]
    if 0 in cls:
        out += [("real", 0), ("real", 32)]
    return out


def fwd_p1(load, t_ref, h, n2, ct, pc):
    xs = []
    for n1 in range(8):
        lo, hi = load(h, 8 * n1 + n2, ct, pc if n1 == 0 else None)
        xs.append(C(V(lo), V(hi)))
    a = fft8(xs, -1)
    for k1 in range(8):
        t = a[k1].mul_w(-n2 * k1, 64)
        assert (t.r.s, t.i.s) == FWD_S1[k1, n2]
        t_ref[h, (k1 * 8 + n2) * 2] = t.r.a
        t_ref[h, (k1 * 8 + n2) * 2 + 1] = t.i.a


def fwd_p2(t_ref, x_ref, g, ct, k1, pc):
    outs = []
    for h in range(2):
        xs = [C(V(t_ref[h, (k1 * 8 + n2) * 2], FWD_S1[k1, n2][0]),
                V(t_ref[h, (k1 * 8 + n2) * 2 + 1], FWD_S1[k1, n2][1])) for n2 in range(8)]
        if h == 0:
            xs[0].r.a = pc.here(xs[0].r.a)
        outs.append(fft8(xs, -1))
    for k2 in range(8):
        m = k1 + 8 * k2
        f0 = _lhs_forms(m, outs[0][k2])
        f1 = _lhs_forms(m, outs[1][k2])
        for i, ((u, half, v0), (_, _, v1)) in enumerate(zip(f0, f1)):
            assert v0.s == v1.s == LHS_SIGN[u, half]
            x_ref.store(u, g, 2 * half + ct, _pack(v0.a, v1.a))
    return COST_F2


def inv_p1(y_ref, t_ref, g, h, n2, pc):
    rows = pl.ds(g * 16 + 8 * h, 8)
    ysg = Y_SIGN
    xs = []
    for n1 in range(8):
        m = 8 * n1 + n2
        xs.append(C(V(y_ref[2 * m, rows, :], ysg.get((m, 0), 1)),
                    V(y_ref[2 * m + 1, rows, :], ysg.get((m, 1), 1))))
    xs[0].r.a = pc.here(xs[0].r.a)
    a = fft8(xs, 1)
    for k1 in range(8):
        t = a[k1].mul_w(n2 * k1, 64)
        assert (t.r.s, t.i.s) == INV_S1[k1, n2]
        t_ref[h, (k1 * 8 + n2) * 2] = t.r.a
        t_ref[h, (k1 * 8 + n2) * 2 + 1] = t.i.a


def inv_p2(t_ref, r_ref, h, k1, pc):
    xs = [C(V(t_ref[h, (k1 * 8 + n2) * 2], INV_S1[k1, n2][0]),
            V(t_ref[h, (k1 * 8 + n2) * 2 + 1], INV_S1[k1, n2][1])) for n2 in range(8)]
    xs[0].r.a = pc.here(xs[0].r.a)
    b = fft8(xs, 1, range(S // 8))
    for k2 in range(S // 8):
        assert (b[k2].r.s, b[k2].i.s) == INV_S2[k1 + 8 * k2]
        r_ref[h, (k1 * 6 + k2) * 2] = b[k2].r.a
        r_ref[h, (k1 * 6 + k2) * 2 + 1] = b[k2].i.a
    return COST_I2


def _act(r_ref, h, k1, k2, dt, first, pc):
    a = r_ref[h, (k1 * 6 + k2) * 2 + dt]
    if first:
        a = pc.here(a)
    return _gelu_half(V(a, INV_S2[k1 + 8 * k2][dt]))


def act_conv1(r_ref, zh_ref, tau0, q, pc):
    h, k1, part = q // 8, 2 * ((q % 8) // 2), q % 2
    first = True
    for k2 in range(3 * part, 3 * part + 3):
        for dt in range(2):
            ev = _act(r_ref, h, k1, k2, dt, first, pc)
            od = _act(r_ref, h, k1 + 1, k2, dt, False, pc)
            first = False
            zh_ref[tau0 + (k1 // 2 + 4 * k2), h, 0, :, _lanes(dt)] = pc.due(ev)
            zh_ref[tau0 + (k1 // 2 + 4 * k2), h, 1, :, _lanes(dt)] = pc.due(od)
    return COST_ACT


def act_conv2(r_ref, f_ref, tau0, q, pc):
    k1, part = q // 2, q % 2
    first = True
    for k2 in range(3 * part, 3 * part + 3):
        for dt in range(2):
            oa = _act(r_ref, 0, k1, k2, dt, first, pc)
            ob = _act(r_ref, 1, k1, k2, dt, False, pc)
            first = False
            f_ref[tau0 + (k1 + 8 * k2), :, _lanes(dt)] = pc.due(_pack(oa, ob))
    return COST_ACT


def inverse_tail(t_ref, r_ref, act, pc, pairs_in_time):
    P = functools.partial
    out = []
    if pairs_in_time:
        for h in range(2):
            for kp in range(4):
                out += [(P(inv_p2, t_ref, r_ref, h, 2 * kp + j, pc), COST_I2) for j in range(2)]
                out += [(P(act, h * 8 + kp * 2 + j, pc), COST_ACT) for j in range(2)]
    else:
        for k1 in range(8):
            out += [(P(inv_p2, t_ref, r_ref, h, k1, pc), COST_I2) for h in range(2)]
            out += [(P(act, k1 * 2 + j, pc), COST_ACT) for j in range(2)]
    return out


def _mm(x_ref, u_ref, j, pc=None, mg=None):
    opaque = pc is not None and pc.unit % OPQ_EVERY == 0
    a = x_ref.load(j, pc.zero if opaque else None, mg)
    if pc is not None:
        a = pc.gate(a)
    a = pltpu.bitcast(a, bf16)
    w = pltpu.bitcast(u_ref.load(j), bf16)
    return jnp.dot(a, w, preferred_element_type=f32)


def _tokens(y):
    m = y.shape[0]
    return [y[8 * r:8 * r + 8, 128 * n:128 * n + 128] for n in range(2) for r in range(m // 8)]


def matmul_stream(x_ref, u_ref, y_ref, pc=None, mg=None):
    def tiles(y, u):
        return [V(y[:, :128], COL_SIGN[u, 0]), V(y[:, 128:], COL_SIGN[u, 1])]

    if mg is not None:
        y_ref = y_ref.at[:, pl.ds(0, 16 * mg), :]
    for cls in CLASSES:
        for kind, k in _class_units(cls):
            if kind == "pair":
                j = (k - 1) * 3
                y1 = _mm(x_ref, u_ref, j, pc, mg)
                k1 = tiles(y1, j)
                yield _tokens(y1)
                y2 = _mm(x_ref, u_ref, j + 1, pc, mg)
                k2 = tiles(y2, j + 1)
                for nt, m in ((0, k), (1, 64 - k)):
                    yi = k1[nt] + k2[nt]
                    assert (yi.s if nt == 0 else -yi.s) == Y_SIGN[m, 1]
                    y_ref[2 * m + 1] = yi.a
                yield _tokens(y2)
                y3 = _mm(x_ref, u_ref, j + 2, pc, mg)
                k3 = tiles(y3, j + 2)
                for nt, m in ((0, k), (1, 64 - k)):
                    yr = k1[nt] - k3[nt]
                    assert yr.s == Y_SIGN[m, 0]
                    y_ref[2 * m] = yr.a
                yield _tokens(y3)
            else:
                y = _mm(x_ref, u_ref, UNIT0 if k == 0 else UNIT32, pc, mg)
                y_ref[2 * k] = y[:, :128]
                y_ref[2 * k + 1] = y[:, 128:]
                yield _tokens(y)


def run_step(mm, pieces, costs, pc, ntok, lead, lag=None, due=None, nunits=NUNITS):
    total = float(sum(costs))
    lag = LAG if lag is None else lag
    tokens = []
    marks = []
    c = 0.0
    for piece, cost in zip(pieces, costs):
        pc.tok = None
        pc.tok2 = marks[-lag] if lag and len(marks) >= lag else None
        if c >= lead:
            want = min(int((c - lead) / (total - lead) * ntok), ntok - 1)
            ahead = min(want + (AHEAD * ntok) // max(nunits, NUNITS), ntok - 1)
            while ahead >= len(tokens):
                tokens += next(mm)
            pc.tok = tokens[want]
        pc.outs = []
        piece()
        marks.append(pc.last)
        for i, v in enumerate(pc.outs):
            q = pc.unit + (DUE if due is None else due) + i // 4
            if q < nunits:
                pc.pending.append((q, v))
        c += cost
    pc.tok = pc.tok2 = None
    for _ in mm:
        pass


def _make_kernel(T):
    T1, T2 = T // 2, T // 4
    L1 = (T1 + 16) // SEG
    L2 = L1 // 2
    assert L1 * SEG == T1 + 16 and L1 % 2 == 0
    NB1 = -(-L1 // S)
    NB2 = -(-L2 // S)
    XPAD = 8
    XB = T1 + 16
    XROWS = XPAD + 2 * XB + 64
    MG = 3
    M = 16 * MG
    NC1 = -(-NB1 // MG)
    NC2 = -(-NB2 // MG)
    ZH = (NB2 - 1) * S + N
    ZDUMP = ZH
    TB = 56
    NCH = -(-L2 // TB)
    FROWS = max(NB2 * S, NCH * TB)
    FDUMP = FROWS
    last_valid = T2 - (SEG - 1) * L2
    XPART = (0, 304, 592)

    def x_rows(e, part):
        def start(e, part):
            if e >= SEG:
                return T1
            return max(L1 * e + XPART[part] - (8 if part == 0 else 0), 0) // 8 * 8
        if part + 1 < len(XPART):
            return start(e, part), start(e, part + 1)
        return start(e, part), start(e + 1, 0)

    def kernel(x_hbm, w1_hbm, w2_hbm, g_ref, wf_ref, wg_ref, wo_ref, gm_ref, o_hbm,
               xs0, xs1, w_ref, ws0, ws1, u1_ref, u2_ref, pool, y_ref, zh_ref, f_ref, fe_ref, ge_ref,
               st_ref, sem_w, sem_x, sem_o):
        xs = (xs0, xs1)
        x_ref = XView(pool, 0, MG)
        tf = [[View(pool, NUNITS * MG * 4 + (g * 2 + ct) * 256) for ct in range(2)] for g in range(MG)]
        ti = [View(pool, NUNITS * MG * 4 + MG * 512 + g * 256) for g in range(MG)]
        tr = [View(pool, NUNITS * MG * 4 + MG * 768 + g * 256) for g in range(MG)]
        xh = x_hbm.bitcast(u32)
        w1w = w1_hbm.bitcast(u32)
        w2w = w2_hbm.bitcast(u32)

        W1PART = (0, 16, 32, 64, 96, 128)
        W2PART = (0, 16, 32, 128)

        def w1_copy(q):
            rows = pl.ds(W1PART[q], W1PART[q + 1] - W1PART[q])
            return pltpu.make_async_copy(w1w.at[:, rows, :], w_ref.at[:, rows, :], sem_w.at[q % 4])

        ws = (ws0, ws1)

        def w2_copies(part):
            lo, n = W2PART[part], W2PART[part + 1] - W2PART[part]
            return [pltpu.make_async_copy(w2w.at[i, pl.ds(lo, n), _lanes(dt)],
                                          ws[dt].at[pl.ds(WP * i + lo, n), :], sem_w.at[4 + part % 2])
                    for i in range(31) for dt in range(2)]

        def w2_wait(part):
            buf = ws0.at[pl.ds(0, 31 * (W2PART[part + 1] - W2PART[part])), :]
            for _ in range(2):
                pltpu.make_async_copy(buf, buf, sem_w.at[4 + part % 2]).wait()

        def x_copies(part):
            cps = []
            for b in range(2):
                for e in range(SEG):
                    lo, hi = x_rows(e, part)
                    for ct in range(2):
                        cps.append(pltpu.make_async_copy(
                            xh.at[b, pl.ds(lo, hi - lo), _lanes(ct)],
                            xs[ct].at[pl.ds(XPAD + b * XB + lo, hi - lo), :],
                            sem_x.at[part]))
            return cps

        w1_copy(0).start()
        for cp in w2_copies(0):
            cp.start()
        w1_copy(1).start()
        for cp in w2_copies(1):
            cp.start()
        w1_copy(2).start()
        for dt in range(2):
            for r in range(31 * WP, 31 * WP + 128, 8):
                ws[dt][pl.ds(r, 8), :] = jnp.zeros((8, 128), u32)
        gbase = NUNITS * MG * 4 + MG * 1024
        for r in range(24):
            pool[gbase + r] = gm_ref[pl.ds(8 * r, 8), :]

        def g_view(zero):
            return jnp.concatenate([pool[gbase + r + (zero if r == TAP_OPQ else 0)] for r in range(24)], axis=0)

        z8 = jnp.zeros((8, 128), u32)
        for ct in range(2):
            xs[ct][pl.ds(0, 8), :] = z8
            for r in range(XPAD + T1, XPAD + XB, 8):
                xs[ct][pl.ds(r, 8), :] = z8
            for r in range(XPAD + XB + T1, XROWS, 8):
                xs[ct][pl.ds(r, 8), :] = z8

        def zero_zh(i, c):
            for h in range(2):
                for comp in range(2):
                    zh_ref[ZH - 1 - i, h, comp] = jnp.zeros((8, 256), f32)
            return c
        lax.fori_loop(0, ZH - 8 - L2, zero_zh, 0)

        zf = jnp.zeros((M, 128), f32)
        for m in range(0, 64, 4):
            y_ref[2 * m] = zf
            y_ref[2 * m + 1] = zf
        for g in range(MG):
            for h in range(2):
                for k1 in range(8):
                    for n2 in (1, 2, 3, 5, 6, 7):
                        for comp in range(2):
                            ti[g][h, (k1 * 8 + n2) * 2 + comp] = jnp.zeros((8, 128), f32)

        gg = g_ref[...].reshape(16, 256)
        ge_all = jnp.dot(gg, wg_ref[...], preferred_element_type=f32)
        ge_ref[...] = ge_all
        never = jnp.max(jnp.abs(ge_all)) < 0.0

        def transform(hook):
            def body(i, c):
                for j in range(WT_UNROLL):
                    hook(i * WT_UNROLL + j)
                pc = Pacer(i < 0, lax.shift_right_arithmetic(i, 20))
                seq = []
                for j in range(WT_UNROLL):
                    seq += weight_pieces(w_ref, UView(u1_ref), tf[j][0], tf[j][1], i * WT_UNROLL + j, pc)
                n = 4 * WT_UNROLL
                run_step(tap_stream(g_view, ws, u2_ref, n * i, n, pc), [q[0] for q in seq],
                         [q[1] for q in seq], pc, n * 192, LEAD, nunits=n)
                return c
            lax.fori_loop(0, 16 // WT_UNROLL, body, 0)

        def w1_hook(rg):
            for q in range(len(W1PART) - 1):
                @pl.when(rg * 8 == W1PART[q])
                def _(q=q):
                    w1_copy(q).wait()
                    if q < len(W2PART) - 1:
                        w2_wait(q)
                    if q == 0:
                        for cp in w2_copies(2):
                            cp.start()
                    if q + 3 < len(W1PART) - 1:
                        w1_copy(q + 3).start()
                    if q >= 2:
                        for cp in x_copies(q - 2):
                            cp.start()

        def conv(nchunk, nblk, u_ref, make_load, act, pairs_in_time, out_index, wait_input=None):
            def loads(c):
                return [make_load(jnp.minimum(c * MG + g, nblk - 1)) for g in range(MG)]

            def P(fn, *a):
                return functools.partial(fn, *a)

            def f1(ld, pc):
                return [(P(fwd_p1, ld[g], tf[g][ct], h, n2, ct, pc), COST_F1[n2])
                        for g in range(MG) for ct in range(2) for h in range(2) for n2 in range(8)]

            def f2(cls, pc, mg=MG):
                return [(P(fwd_p2, tf[g][ct], x_ref, g, ct, k1, pc), COST_F2)
                        for g in range(mg) for ct in range(2) for k1 in cls]

            def i1(cls, pc, mg=MG):
                return [(P(inv_p1, y_ref, ti[g], g, h, n2, pc), COST_I1[n2])
                        for g in range(mg) for h in range(2) for n2 in cls]

            def i2(c, pc, mg=MG):
                out = []
                for g in range(mg):
                    out += inverse_tail(ti[g], tr[g], P(act, tr[g], out_index(c, g)), pc, pairs_in_time)
                return out

            idle = Pacer(None)
            if wait_input is not None:
                wait_input(0)
            with scope("pro"):
                for piece, _ in f1(loads(0), idle):
                    piece()
                for piece, _ in f2(CLASSES[0], idle):
                    piece()

            def step(c, cc):
                if wait_input is not None:
                    wait_input(c + 1)
                pc = Pacer(c < 0, lax.shift_right_arithmetic(c, 20))
                nxt = f1(loads(jnp.minimum(c + 1, nchunk - 1)), pc)
                half = len(nxt) // 2
                seq = (f2(CLASSES[1], pc) + f2(CLASSES[2], pc) + f2(CLASSES[3], pc)
                       + i1(CLASSES[3], pc) + i2(c - 1, pc)
                       + nxt[:half] + i1(CLASSES[0], pc) + nxt[half:]
                       + i1(CLASSES[1], pc) + f2(CLASSES[0], pc) + i1(CLASSES[2], pc))
                run_step(matmul_stream(x_ref, u_ref, y_ref, pc), [q[0] for q in seq], [q[1] for q in seq],
                         pc, NUNITS * (M // 4), LEAD)
                return cc

            def short_step(c, never, zero, mg):
                pc = Pacer(never, zero)
                seq = (f2(CLASSES[1], pc, mg) + f2(CLASSES[2], pc, mg) + f2(CLASSES[3], pc, mg)
                       + i1(CLASSES[3], pc) + i2(c - 1, pc)
                       + i1(CLASSES[0], pc, mg) + i1(CLASSES[1], pc, mg) + i1(CLASSES[2], pc, mg))
                run_step(matmul_stream(x_ref, u_ref, y_ref, pc, mg), [q[0] for q in seq],
                         [q[1] for q in seq], pc, NUNITS * 4 * mg, LEAD)

            tail = nblk - (nchunk - 1) * MG
            with scope("steps"):
                lax.fori_loop(0, nchunk if tail == MG else nchunk - 1, step, 0)
                if tail < MG:
                    short_step(nchunk - 1, never, never.astype(i32), tail)

            with scope("epi"):
                for piece, _ in i1(CLASSES[3], idle, tail) + i2(nchunk - 1, idle, tail):
                    piece()

        with scope("wt1"):
            transform(w1_hook)

        def x_wait(part):
            rows = sum(4 * (x_rows(e, part)[1] - x_rows(e, part)[0]) for e in range(SEG))
            buf = xs0.at[pl.ds(0, rows), :]
            pltpu.make_async_copy(buf, buf, sem_x.at[part]).wait()

        def wait_x0(c):
            if isinstance(c, int):
                x_wait(0)
                return
            for part, first in ((1, 2), (2, 4)):
                @pl.when(c == first)
                def _(part=part):
                    x_wait(part)

        def load1(blk):
            base = blk * S

            def load(h, n, ct, pc):
                w = xs[ct][pl.ds(base + n + h * L1, 8, stride=2 * L1), :]
                if pc is not None:
                    w = pc.here(w)
                return _unpack(w)
            return load

        def act1(rb, tau0, q, pc):
            return act_conv1(rb, zh_ref, tau0, q, pc)

        def out1(c, g):
            if isinstance(c, int):
                return 8 + (c * MG + g) * (S // 2)
            return jnp.where(c >= 0, 8 + (c * MG + g) * (S // 2), ZDUMP)

        conv(NC1, NB1, UView(u1_ref), load1, act1, True, out1, wait_x0)

        row = lax.broadcasted_iota(i32, (8, 256), 0)
        for h in range(2):
            for comp in range(2):
                for t in range(last_valid, NB1 * S // 2):
                    zh_ref[8 + t, h, comp] = jnp.where(row == SEG - 1, 0.0, zh_ref[8 + t, h, comp])
                for j in range(8):
                    v = pltpu.roll(zh_ref[8 + L2 - 8 + j, h, comp], 1, axis=0)
                    zh_ref[j, h, comp] = jnp.where(row == 0, 0.0, v)
                for j in range(8):
                    v = pltpu.roll(zh_ref[8 + j, h, comp], SEG - 1, axis=0)
                    zh_ref[8 + L2 + j, h, comp] = jnp.where(row == SEG - 1, 0.0, v)


        def load2(blk):
            def load(h, n, ct, pc):
                lo = zh_ref[blk * S + n, h, 0, :, _lanes(ct)]
                hi = zh_ref[blk * S + n, h, 1, :, _lanes(ct)]
                if pc is not None:
                    lo = pc.here(lo)
                return lo, hi
            return load

        def act2(rb, tau0, q, pc):
            return act_conv2(rb, f_ref, tau0, q, pc)

        def out2(c, g):
            if isinstance(c, int):
                return min(c * MG + g, NB2 - 1) * S
            return jnp.where(c >= 0, jnp.minimum(c * MG + g, NB2 - 1) * S, FDUMP)

        conv(NC2, NB2, UView(u2_ref), load2, act2, False, out2)

        order = [(b, e) for b in range(2) for e in range(SEG)]

        def out_copy(half, q, t0, nvalid):
            b, e = order[q]
            r0 = (b * T2 + e * L2) * 8 + t0 * 8
            return pltpu.make_async_copy(st_ref.at[half, q, pl.ds(0, nvalid * 8), :],
                                         o_hbm.at[pl.ds(r0, nvalid * 8), :],
                                         sem_o.at[half])

        def width(e):
            lim = L2 if e < SEG - 1 else last_valid
            return lim - (NCH - 1) * TB

        def joint_chunk(ch, half, full, never):
            pc = Pacer(never)
            t0 = ch * TB
            fl = pltpu.bitcast(f_ref[pl.ds(t0, TB)].reshape(TB * 8, 256), bf16)
            fe = jnp.dot(fl, wf_ref[...], preferred_element_type=f32)
            fe_ref[...] = fe
            prev = [fe[8 * r:8 * r + 8, 128 * n:128 * n + 128] for n in range(2) for r in range(2 * TB)]
            prev = prev[len(prev) // 2:]
            for q, (b, e) in enumerate(order):
                ge = ge_ref[pl.ds(8 * b, 8), :]
                r = 4 * (e & 3) + 2 * b + (e >> 2)
                js = []
                for t in range(TB):
                    row = jnp.broadcast_to(fe_ref[pl.ds(16 * t + r, 1), :], (8, 256))
                    tok = prev[(t * len(prev)) // TB]
                    gt = jnp.concatenate([pc.tie(ge[:, :128], tok), pc.tie(ge[:, 128:], tok)], axis=1)
                    js.append(jnp.tanh(row + gt))
                jl = jnp.concatenate(js, axis=0).astype(bf16)
                y = jnp.dot(jl, wo_ref[...], preferred_element_type=f32)
                prev = [y[8 * rr:8 * rr + 8, 128 * n:128 * n + 128] for n in range(2) for rr in range(TB)]
                st_ref[half, q] = y.astype(bf16)
                out_copy(half, q, t0, TB if full else width(e)).start()

        def wait_chunk(half, full):
            if full:
                pltpu.make_async_copy(st_ref.at[half], st_ref.at[half], sem_o.at[half]).wait()
                return
            for q, (b, e) in enumerate(order):
                out_copy(half, q, 0, width(e)).wait()

        def joint_body(ch, c):
            half = ch % 2

            @pl.when(ch >= 2)
            def _():
                wait_chunk(half, True)
            joint_chunk(ch, half, True, ch < 0)
            return c
        with scope("joint"):
            lax.fori_loop(0, NCH - 1, joint_body, 0)
            last_half = (NCH - 1) % 2
            wait_chunk(last_half, True)
            joint_chunk(NCH - 1, last_half, False, never)
            wait_chunk(1 - last_half, True)
            wait_chunk(last_half, False)

    scratch = [
        pltpu.VMEM((XROWS, 128), u32), pltpu.VMEM((XROWS, 128), u32),
        pltpu.VMEM((31, 128, 256), u32),
        pltpu.VMEM((32 * WP + 8, 128), u32), pltpu.VMEM((32 * WP + 8, 128), u32),
        pltpu.VMEM((2 * 96 * UP, 128), u32), pltpu.VMEM((2 * 96 * UP, 128), u32),
        pltpu.VMEM((NUNITS * MG * 4 + MG * 1024 + 24, 8, 128), u32),
        pltpu.VMEM((128, M, 128), f32),
        pltpu.VMEM((ZH + S // 2, 2, 2, 8, 256), f32),
        pltpu.VMEM((FROWS + S, 8, 256), u32),
        pltpu.VMEM((TB * 16, 256), f32),
        pltpu.VMEM((16, 256), f32),
        pltpu.VMEM((2, 2 * SEG, TB * 8, 256), bf16),
        pltpu.SemaphoreType.DMA((6,)),
        pltpu.SemaphoreType.DMA((3,)),
        pltpu.SemaphoreType.DMA((2,)),
    ]
    return kernel, scratch


TAP_MATRIX = _tap_matrix()
WT_UNROLL = 2
TAP_OPQ = 23
TAP_GATE = 20
LEAD = 0
LAG = 0
AHEAD = 2
OPQ_EVERY = 1
DUE = 0
DUE_EVERY = 1000


def _call(x, w1, w2, g, w_f, w_g, w_o, interpret=False):
    B, T, D = x.shape
    kernel, scratch = _make_kernel(T)
    T2 = T // 4
    any_spec = pl.BlockSpec(memory_space=pl.ANY)
    vmem = pl.BlockSpec(memory_space=pltpu.VMEM)
    out = pl.pallas_call(
        kernel,
        out_shape=jax.ShapeDtypeStruct((B * T2 * 8, D), bf16),
        in_specs=[any_spec, any_spec, any_spec, vmem, vmem, vmem, vmem, vmem],
        out_specs=any_spec,
        scratch_shapes=scratch,
        compiler_params=pltpu.CompilerParams(vmem_limit_bytes=126 * 2**20),
        interpret=interpret,
        name="conv_stem_rnnt_joint",
    )(x, w1, w2, g, w_f, w_g, w_o, TAP_MATRIX)
    return out.reshape(B, T2, 8, D)


@jax.jit
def pallas_standalone__seq2seq_rnn_t_joint__speech_kernel(x, w1, w2, g, w_f, w_g, w_o):
    return _call(x, w1, w2, g, w_f, w_g, w_o)
```

```python
import functools
import math

import jax
import jax.numpy as jnp
import numpy as np
from jax import lax
from jax.experimental import pallas as pl
from jax.experimental.pallas import tpu as pltpu

f32, u32, bf16, i32 = jnp.float32, jnp.uint32, jnp.bfloat16, jnp.int32

PROFILE_SCOPES = False


class _NoScope:
    def __enter__(self):
        return self

    def __exit__(self, *a):
        return False


def scope(name):
    return jax.named_scope(name) if PROFILE_SCOPES else _NoScope()

N = 64
S = 48
SEG = 8


class V:
    __slots__ = ("a", "s")

    def __init__(self, a, s=1):
        self.a = a
        self.s = s

    def __neg__(self):
        return V(self.a, -self.s)

    def __add__(self, o):
        if self.s == o.s:
            return V(self.a + o.a, self.s)
        if self.s > 0:
            return V(self.a - o.a, 1)
        return V(o.a - self.a, 1)

    def __sub__(self, o):
        return self + (-o)

    def scale(self, c):
        if c == 1.0:
            return self
        if c == -1.0:
            return -self
        return V(self.a * np.float32(abs(c)), self.s * (1 if c > 0 else -1))

    def times(self, c):
        return self.a * np.float32(self.s * c)

    def signed(self, s):
        return self.a if self.s * s > 0 else -self.a


class C:
    __slots__ = ("r", "i")

    def __init__(self, r, i):
        self.r = r
        self.i = i

    def __add__(self, o):
        return C(self.r + o.r, self.i + o.i)

    def __sub__(self, o):
        return C(self.r - o.r, self.i - o.i)

    def __neg__(self):
        return C(-self.r, -self.i)

    def mul_w(self, num, den):
        num %= den
        if num == 0:
            return self
        if 4 * num == den:
            return C(-self.i, self.r)
        if 2 * num == den:
            return -self
        if 4 * num == 3 * den:
            return C(self.i, -self.r)
        if (8 * num) % den == 0:
            o = (8 * num) // den
            h = math.sqrt(0.5)
            sc = 1 if o in (1, 7) else -1
            ss = 1 if o in (1, 3) else -1
            r, m = self.r, self.i
            re = (r if sc > 0 else -r) - (m if ss > 0 else -m)
            im = (r if ss > 0 else -r) + (m if sc > 0 else -m)
            return C(re.scale(h), im.scale(h))
        c = math.cos(2 * math.pi * num / den)
        s = math.sin(2 * math.pi * num / den)
        return C(self.r.scale(c) - self.i.scale(s), self.r.scale(s) + self.i.scale(c))


def _add(a, b):
    if a is None:
        return b
    if b is None:
        return a
    return a + b


def _sub(a, b):
    if b is None:
        return a
    if a is None:
        return -b
    return a - b


def fft8(x, sgn, need=tuple(range(8))):
    def rot(a, num, den):
        return None if a is None else a.mul_w(sgn * num, den)

    need = set(need)
    a0, a1 = _add(x[0], x[4]), _sub(x[0], x[4])
    a2, a3 = _add(x[2], x[6]), rot(_sub(x[2], x[6]), 1, 4)
    a4, a5 = _add(x[1], x[5]), _sub(x[1], x[5])
    a6, a7 = _add(x[3], x[7]), rot(_sub(x[3], x[7]), 1, 4)
    out = {}
    if need & {0, 4}:
        b0, b4 = _add(a0, a2), _add(a4, a6)
        if 0 in need:
            out[0] = _add(b0, b4)
        if 4 in need:
            out[4] = _sub(b0, b4)
    if need & {2, 6}:
        b2, b6 = _sub(a0, a2), rot(_sub(a4, a6), 1, 4)
        if 2 in need:
            out[2] = _add(b2, b6)
        if 6 in need:
            out[6] = _sub(b2, b6)
    if need & {1, 5}:
        b1, b5 = _add(a1, a3), rot(_add(a5, a7), 1, 8)
        if 1 in need:
            out[1] = _add(b1, b5)
        if 5 in need:
            out[5] = _sub(b1, b5)
    if need & {3, 7}:
        b3, b7 = _sub(a1, a3), rot(_sub(a5, a7), 3, 8)
        if 3 in need:
            out[3] = _add(b3, b7)
        if 7 in need:
            out[7] = _sub(b3, b7)
    return out


class _Sym:
    def __add__(self, o):
        return self

    __sub__ = __mul__ = __add__

    def __neg__(self):
        return self


def _fft64_signs(sgn, present=tuple(range(64)), in_sign=None):
    d = _Sym()
    in_sign = in_sign or {}
    x = [C(V(d, in_sign.get((n, 0), 1)), V(d, in_sign.get((n, 1), 1))) if n in present else None
         for n in range(64)]
    t = {}
    for n2 in range(8):
        a = fft8([x[8 * n1 + n2] for n1 in range(8)], sgn)
        for k1 in range(8):
            t[k1, n2] = a[k1].mul_w(sgn * n2 * k1, 64)
    s1 = {key: (v.r.s, v.i.s) for key, v in t.items()}
    s2 = {}
    for k1 in range(8):
        b = fft8([t[k1, n2] for n2 in range(8)], sgn)
        for k2 in range(8):
            s2[k1 + 8 * k2] = b[k2]
    return s1, s2


def _unit(k, j):
    return (k - 1) * 3 + j


UNIT0, UNIT32 = 93, 94
NUNITS = 95


def _lhs_forms(m, z):
    if m in (0, 32):
        u = UNIT0 if m == 0 else UNIT32
        return [(u, 0, z.r), (u, 1, z.i)]
    if m < 32:
        return [(_unit(m, 0), 0, z.r + z.i), (_unit(m, 1), 0, z.r), (_unit(m, 2), 0, z.i)]
    k = 64 - m
    return [(_unit(k, 0), 1, z.r - z.i), (_unit(k, 1), 1, z.r), (_unit(k, 2), 1, z.i)]


def _lhs_signs():
    _, s2 = _fft64_signs(-1)
    sg = {}
    for m in range(64):
        for u, h, v in _lhs_forms(m, s2[m]):
            sg[u, h] = v.s
    return sg


LHS_SIGN = _lhs_signs()


def _weight_forms(m, pm):
    if m < 32:
        nt = 0 if pm > 0 else 1
        return [(_unit(m, 0), 1, nt, (1, 0)), (_unit(m, 1), 1, nt, (-1, 1)), (_unit(m, 2), 1, nt, (-1, -1))]
    k = 64 - m
    nt = 1 if pm > 0 else 0
    return [(_unit(k, 0), 0, nt, (1, 0)), (_unit(k, 1), 0, nt, (-1, -1)), (_unit(k, 2), 0, nt, (1, -1))]


def _weight_plan():
    s1, s2 = _fft64_signs(1, present=range(16))
    forms = {}
    for pm in (1, -1):
        for m in range(1, 64):
            if m == 32:
                continue
            for u, half, nt, (cr, ci) in _weight_forms(m, pm):
                forms[u, half, nt] = (cr * s2[m].r.s, ci * s2[m].i.s)
    col = {}
    for u in range(93):
        for nt in range(2):
            def negs(sig):
                n = 0
                for half in range(2):
                    cr, ci = forms[u, half, nt]
                    w = sig * LHS_SIGN[u, half]
                    n += (w * cr <= 0 and w * ci <= 0)
                return n
            col[u, nt] = 1 if negs(1) <= negs(-1) else -1
    for u in (UNIT0, UNIT32):
        col[u, 0] = col[u, 1] = 1
    return s1, s2, col


WT_S1, WT_S2, COL_SIGN = _weight_plan()


def _recombine(k1, k2, k3, k):
    out = {}
    for nt in range(2):
        yr = k1[nt] - k3[nt]
        yi = k1[nt] + k2[nt]
        if nt == 0:
            out[k, 0], out[k, 1] = yr, yi
        else:
            out[64 - k, 0], out[64 - k, 1] = yr, -yi
    return out


def _y_signs():
    d = _Sym()
    sg = {}
    for k in range(1, 32):
        ks = [[V(d, COL_SIGN[_unit(k, j), nt]) for nt in range(2)] for j in range(3)]
        for key, v in _recombine(ks[0], ks[1], ks[2], k).items():
            sg[key] = v.s
    for m, u in ((0, UNIT0), (32, UNIT32)):
        sg[m, 0], sg[m, 1] = COL_SIGN[u, 0], COL_SIGN[u, 1]
    return sg


Y_SIGN = _y_signs()


def _unpack(w):
    lo = pltpu.unpack_elementwise(w, index=0, packed_dtype=bf16, unpacked_dtype=f32)
    hi = pltpu.unpack_elementwise(w, index=1, packed_dtype=bf16, unpacked_dtype=f32)
    return lo, hi


def _pack(lo, hi):
    return pltpu.pack_elementwise([lo, hi], packed_dtype=bf16)


_GC1 = 2.0 * math.sqrt(2.0 / math.pi)
_GC2 = 8.0 * 0.044715 * math.sqrt(2.0 / math.pi)


def _gelu_half(v):
    a = v.a
    p = (a * a) * np.float32(_GC2) + np.float32(_GC1)
    t = jnp.tanh(p * a)
    return a * t + a if v.s > 0 else a * t - a


def _lanes(t):
    return pl.ds(128 * t, 128)


class Pacer:
    def __init__(self, never, zero=None):
        self.never = never
        self.tok = None
        self.tok2 = None
        self.last = None
        self.outs = []
        self.zero = zero
        self.pending = []
        self.unit = 0

    def gate(self, a, first=0):
        vals = [v for q, v in self.pending if q <= self.unit]
        self.pending = [(q, v) for q, v in self.pending if q > self.unit]
        self.unit += 1
        if not vals:
            return a
        m, k = a.shape
        tiles = [[a[8 * r:8 * r + 8, 128 * c:128 * c + 128] for c in range(k // 128)] for r in range(m // 8)]
        flat = [(r, c) for r in range(first, m // 8) for c in range(k // 128)]
        for i, v in enumerate(vals):
            r, c = flat[i % len(flat)]
            tiles[r][c] = self.tie(tiles[r][c], v)
        return jnp.concatenate([jnp.concatenate(row, axis=1) for row in tiles], axis=0)

    def here(self, x):
        tok, self.tok = self.tok, None
        tok2, self.tok2 = self.tok2, None
        return self.tie(self.tie(x, tok), tok2)

    def mark(self, x, nth=None):
        self.last = x
        if self.never is not None and nth is not None and nth % DUE_EVERY == DUE_EVERY - 1:
            self.outs.append(x)
        return x

    def due(self, x):
        if self.never is not None:
            self.outs.append(x)
        return x

    def tie(self, x, tok):
        if tok is None:
            return x
        if tok.dtype != x.dtype:
            tok = pltpu.bitcast(tok, x.dtype)
        return jnp.where(self.never, tok, x)


def _combo(f, cr, ci, want):
    if ci == 0:
        return f.r.signed(want * cr)
    v = (f.r if cr > 0 else -f.r) + (f.i if ci > 0 else -f.i)
    if v.s * want > 0:
        return v.a
    if f.r.s * cr != f.i.s * ci:
        return ((-f.r) if cr > 0 else f.r).__add__((-f.i) if ci > 0 else f.i).a
    return -v.a


UP = 260
WP = 132


class UView:
    def __init__(self, ref):
        self.ref = ref

    def load(self, u):
        return jnp.concatenate([self.ref[pl.ds((nt * 96 + u) * UP, 256), :] for nt in range(2)], axis=1)

    def store(self, u, half, nt, rg, val):
        self.ref[pl.ds((nt * 96 + u) * UP + half * 128 + rg * 8, 8), :] = val


def _tap_matrix():
    import ml_dtypes
    sigma, tau = 1.0 / 256.0, 1.0 / 128.0
    g = np.zeros((2, 2, 96, 32, 2))
    d = np.arange(16)
    for tap in range(31):
        for dt in range(2):
            wa = np.zeros((16, 2))
            wb = np.zeros((16, 2))
            if tap % 2:
                wa[(tap + 1) // 2, dt] = 1.0
            else:
                wb[tap // 2, dt] = 1.0
            z0 = wa[:, 0] + 1j * wb[:, 0]
            z1 = wa[:, 1] + 1j * wb[:, 1]
            for pm, z in ((1, z0 + 1j * z1), (-1, z0 - 1j * z1)):
                for m in range(1, 64):
                    if m == 32:
                        continue
                    f = sigma * np.sum(z * np.exp(2j * np.pi * m * d / 64))
                    for u, half, nt, (cr, ci) in _weight_forms(m, pm):
                        g[nt, half, u, tap, dt] = (LHS_SIGN[u, half] * COL_SIGN[u, nt]
                                                   * (cr * f.real + ci * f.imag))
            for m, u in ((0, UNIT0), (32, UNIT32)):
                e = np.cos(np.pi * m * d / 32)
                for half, wv in enumerate((wa, wb)):
                    g[dt, half, u, tap, dt] = (LHS_SIGN[u, half] * COL_SIGN[u, dt]
                                               * tau * np.sum(e * wv[:, dt]))
    g = g.reshape(384, 32, 2)
    mat = np.zeros((384, 128))
    for v in range(4):
        dt, t0 = v // 2, 16 * (v % 2)
        for s_ in range(8):
            for par in range(2):
                mat[:, 16 * v + 2 * s_ + par] = g[:, t0 + 8 * par + s_, dt]
    hi = mat.astype(ml_dtypes.bfloat16)
    lo = (mat - hi.astype(np.float64)).astype(ml_dtypes.bfloat16)
    full = np.concatenate([hi[:, :64], lo[:, :64]], axis=1).view(np.uint16).astype(np.uint32)
    return full[0::2] | (full[1::2] << 16)


def tap_operand(ws, cpair):
    ev, od = [], []
    for dt in range(2):
        for t0 in (0, 16):
            wa = ws[dt][pl.ds(t0 * WP + cpair, 8, stride=WP), :]
            wb = ws[dt][pl.ds((t0 + 8) * WP + cpair, 8, stride=WP), :]
            alo, ahi = _unpack(wa)
            blo, bhi = _unpack(wb)
            ev.append(_pack(alo, blo))
            od.append(_pack(ahi, bhi))
    return jnp.concatenate(ev + ev, axis=0), jnp.concatenate(od + od, axis=0)


def tap_stream(g_view, ws, u2_ref, it0, n, pc):
    for q in range(n):
        it = it0 + q
        lhs = pltpu.bitcast(pc.gate(g_view(pc.zero), TAP_GATE), bf16)
        ops = []
        for j in range(2):
            ops += list(tap_operand(ws, 2 * it + j))
        rhs = pltpu.bitcast(jnp.concatenate(ops, axis=1), bf16)
        y = jnp.dot(lhs, rhs, preferred_element_type=f32)
        for r in range(48):
            nt, half, u0 = r // 24, (r // 12) % 2, (r % 12) * 8
            for j in range(2):
                val = _pack(y[8 * r:8 * r + 8, 256 * j:256 * j + 128],
                            y[8 * r:8 * r + 8, 256 * j + 128:256 * j + 256])
                u2_ref[pl.ds((nt * 96 + u0) * UP + half * 128 + 2 * it + j, 8, stride=UP), :] = val
        yield [y[8 * r:8 * r + 8, 128 * t:128 * t + 128] for r in range(48) for t in range(4)]


def weight_pieces(w_ref, u_ref, t_ref, z_ref, rg, pc):
    rows = pl.ds(pl.multiple_of(rg * 8, 8), 8)
    sigma = 1.0 / 256.0
    tau = 1.0 / 128.0
    acc = {}

    def store(u, half, nt, a0, a1):
        u_ref.store(u, half, nt, rg, pc.due(_pack(a0, a1)))

    def prep(d):
        wa = [[None, None], [None, None]]
        wb = [[None, None], [None, None]]
        for dt in range(2):
            w = w_ref[2 * d, rows, _lanes(dt)]
            if dt == 0:
                w = pc.here(w)
            lo, hi = _unpack(w)
            wb[0][dt], wb[1][dt] = V(lo), V(hi)
            if d > 0:
                lo, hi = _unpack(w_ref[2 * d - 1, rows, _lanes(dt)])
                wa[0][dt], wa[1][dt] = V(lo), V(hi)
        for p in range(2):
            for dt in range(2):
                for name, val in (("a", wa[p][dt]), ("b", wb[p][dt])):
                    key = (p, dt, name, d % 2)
                    acc[key] = _add(acc.get(key), val)
            zp = (_sub(wa[p][0], wb[p][1]), _add(wb[p][0], wa[p][1]))
            zm = (_add(wa[p][0], wb[p][1]), _sub(wb[p][0], wa[p][1]))
            for j, z in enumerate((zp, zm)):
                for comp in range(2):
                    z_ref[j, (p * 16 + d) * 2 + comp] = z[comp].times(sigma)

    def real_bins():
        for m, u in ((0, UNIT0), (32, UNIT32)):
            for dt in range(2):
                for half, name in enumerate(("a", "b")):
                    vals = []
                    for p in range(2):
                        ev, od = acc[p, dt, name, 0], acc[p, dt, name, 1]
                        v = _add(ev, od) if m == 0 else _sub(ev, od)
                        vals.append(v.times(tau * LHS_SIGN[u, half] * COL_SIGN[u, dt]))
                    store(u, half, dt, vals[0], vals[1])

    def pass1(j, p, n2):
        z = [C(V(z_ref[j, (p * 16 + d) * 2]), V(z_ref[j, (p * 16 + d) * 2 + 1])) for d in (n2, n2 + 8)]
        z[0].r.a = pc.here(z[0].r.a)
        a = fft8(z + [None] * 6, 1)
        for k1 in range(8):
            t = a[k1].mul_w(n2 * k1, 64)
            assert (t.r.s, t.i.s) == WT_S1[k1, n2]
            t_ref[p, (k1 * 8 + n2) * 2] = t.r.a
            t_ref[p, (k1 * 8 + n2) * 2 + 1] = t.i.a

    def pass2(pm, k1):
        need = [k2 for k2 in range(8) if (k1 + 8 * k2) not in (0, 32)]
        outs = []
        for p in range(2):
            xs = [C(V(t_ref[p, (k1 * 8 + n2) * 2], WT_S1[k1, n2][0]),
                    V(t_ref[p, (k1 * 8 + n2) * 2 + 1], WT_S1[k1, n2][1])) for n2 in range(8)]
            if p == 0:
                xs[0].r.a = pc.here(xs[0].r.a)
            outs.append(fft8(xs, 1, need))
        for k2 in need:
            m = k1 + 8 * k2
            for u, half, nt, (cr, ci) in _weight_forms(m, pm):
                want = LHS_SIGN[u, half] * COL_SIGN[u, nt]
                store(u, half, nt, _combo(outs[0][k2], cr, ci, want), _combo(outs[1][k2], cr, ci, want))

    P = functools.partial
    out = [(P(prep, d), 40) for d in range(16)] + [(real_bins, 40)]
    for j, pm in enumerate((1, -1)):
        out += [(P(pass1, j, p, n2), 21 + _TW[n2]) for p in range(2) for n2 in range(8)]
        out += [(P(pass2, pm, k1), 193) for k1 in range(8)]
    return out


class View:
    def __init__(self, pool, base):
        self.pool = pool
        self.base = base

    def __getitem__(self, idx):
        h, i = idx
        return pltpu.bitcast(self.pool[self.base + h * 128 + i], f32)

    def __setitem__(self, idx, val):
        h, i = idx
        self.pool[self.base + h * 128 + i] = pltpu.bitcast(val, u32)


class XView:
    def __init__(self, pool, base, mg):
        self.pool, self.base, self.mg = pool, base, mg

    def index(self, u, g, c):
        return self.base + (u * self.mg + g) * 4 + c

    def store(self, u, g, c, val):
        self.pool[self.index(u, g, c)] = val

    def load(self, u, zero=None, mg=None):
        rows = []
        for g in range(self.mg if mg is None else mg):
            row = []
            for c in range(4):
                idx = self.index(u, g, c)
                if zero is not None and g == 0 and c == 0:
                    idx = idx + zero
                row.append(self.pool[idx])
            rows.append(jnp.concatenate(row, axis=1))
        return jnp.concatenate(rows, axis=0)


_TW = (0, 42, 40, 42, 32, 42, 40, 42)
COST_F1 = tuple(73 + t for t in _TW)
COST_I1 = tuple(57 + t for t in _TW)
COST_F2, COST_I2, COST_ACT = 153, 53, 85
FWD_S1, _ = _fft64_signs(-1)
INV_S1, _INV_OUT = _fft64_signs(1, in_sign=Y_SIGN)
INV_S2 = {m: (v.r.s, v.i.s) for m, v in _INV_OUT.items()}
CLASSES = ((1, 7), (2, 6), (3, 5), (4, 0))


def _class_units(cls):
    ks = [k for k in range(1, 32) if k % 8 in cls or (-k) % 8 in cls]
    ks.sort(key=lambda k: (0 if k % 8 == cls[0] else 1, k))
    out = [("pair", k) for k in ks]
    if 0 in cls:
        out += [("real", 0), ("real", 32)]
    return out


def fwd_p1(load, t_ref, h, n2, ct, pc):
    xs = []
    for n1 in range(8):
        lo, hi = load(h, 8 * n1 + n2, ct, pc if n1 == 0 else None)
        xs.append(C(V(lo), V(hi)))
    a = fft8(xs, -1)
    for k1 in range(8):
        t = a[k1].mul_w(-n2 * k1, 64)
        assert (t.r.s, t.i.s) == FWD_S1[k1, n2]
        t_ref[h, (k1 * 8 + n2) * 2] = t.r.a
        t_ref[h, (k1 * 8 + n2) * 2 + 1] = t.i.a


def fwd_p2(t_ref, x_ref, g, ct, k1, pc):
    outs = []
    for h in range(2):
        xs = [C(V(t_ref[h, (k1 * 8 + n2) * 2], FWD_S1[k1, n2][0]),
                V(t_ref[h, (k1 * 8 + n2) * 2 + 1], FWD_S1[k1, n2][1])) for n2 in range(8)]
        if h == 0:
            xs[0].r.a = pc.here(xs[0].r.a)
        outs.append(fft8(xs, -1))
    for k2 in range(8):
        m = k1 + 8 * k2
        f0 = _lhs_forms(m, outs[0][k2])
        f1 = _lhs_forms(m, outs[1][k2])
        for i, ((u, half, v0), (_, _, v1)) in enumerate(zip(f0, f1)):
            assert v0.s == v1.s == LHS_SIGN[u, half]
            x_ref.store(u, g, 2 * half + ct, _pack(v0.a, v1.a))
    return COST_F2


def inv_p1(y_ref, t_ref, g, h, n2, pc):
    rows = pl.ds(g * 16 + 8 * h, 8)
    ysg = Y_SIGN
    xs = []
    for n1 in range(8):
        m = 8 * n1 + n2
        xs.append(C(V(y_ref[2 * m, rows, :], ysg.get((m, 0), 1)),
                    V(y_ref[2 * m + 1, rows, :], ysg.get((m, 1), 1))))
    xs[0].r.a = pc.here(xs[0].r.a)
    a = fft8(xs, 1)
    for k1 in range(8):
        t = a[k1].mul_w(n2 * k1, 64)
        assert (t.r.s, t.i.s) == INV_S1[k1, n2]
        t_ref[h, (k1 * 8 + n2) * 2] = t.r.a
        t_ref[h, (k1 * 8 + n2) * 2 + 1] = t.i.a


def inv_p2(t_ref, r_ref, h, k1, pc):
    xs = [C(V(t_ref[h, (k1 * 8 + n2) * 2], INV_S1[k1, n2][0]),
            V(t_ref[h, (k1 * 8 + n2) * 2 + 1], INV_S1[k1, n2][1])) for n2 in range(8)]
    xs[0].r.a = pc.here(xs[0].r.a)
    b = fft8(xs, 1, range(S // 8))
    for k2 in range(S // 8):
        assert (b[k2].r.s, b[k2].i.s) == INV_S2[k1 + 8 * k2]
        r_ref[h, (k1 * 6 + k2) * 2] = b[k2].r.a
        r_ref[h, (k1 * 6 + k2) * 2 + 1] = b[k2].i.a
    return COST_I2


def _act(r_ref, h, k1, k2, dt, first, pc):
    a = r_ref[h, (k1 * 6 + k2) * 2 + dt]
    if first:
        a = pc.here(a)
    return _gelu_half(V(a, INV_S2[k1 + 8 * k2][dt]))


def act_conv1(r_ref, zh_ref, tau0, q, pc):
    h, k1, part = q // 8, 2 * ((q % 8) // 2), q % 2
    first = True
    for k2 in range(3 * part, 3 * part + 3):
        for dt in range(2):
            ev = _act(r_ref, h, k1, k2, dt, first, pc)
            od = _act(r_ref, h, k1 + 1, k2, dt, False, pc)
            first = False
            zh_ref[tau0 + (k1 // 2 + 4 * k2), h, 0, :, _lanes(dt)] = pc.due(ev)
            zh_ref[tau0 + (k1 // 2 + 4 * k2), h, 1, :, _lanes(dt)] = pc.due(od)
    return COST_ACT


def act_conv2(r_ref, f_ref, tau0, q, pc):
    k1, part = q // 2, q % 2
    first = True
    for k2 in range(3 * part, 3 * part + 3):
        for dt in range(2):
            oa = _act(r_ref, 0, k1, k2, dt, first, pc)
            ob = _act(r_ref, 1, k1, k2, dt, False, pc)
            first = False
            f_ref[tau0 + (k1 + 8 * k2), :, _lanes(dt)] = pc.due(_pack(oa, ob))
    return COST_ACT


def inverse_tail(t_ref, r_ref, act, pc, pairs_in_time):
    P = functools.partial
    out = []
    if pairs_in_time:
        for h in range(2):
            for kp in range(4):
                out += [(P(inv_p2, t_ref, r_ref, h, 2 * kp + j, pc), COST_I2) for j in range(2)]
                out += [(P(act, h * 8 + kp * 2 + j, pc), COST_ACT) for j in range(2)]
    else:
        for k1 in range(8):
            out += [(P(inv_p2, t_ref, r_ref, h, k1, pc), COST_I2) for h in range(2)]
            out += [(P(act, k1 * 2 + j, pc), COST_ACT) for j in range(2)]
    return out


def _mm(x_ref, u_ref, j, pc=None, mg=None):
    opaque = pc is not None and pc.unit % OPQ_EVERY == 0
    a = x_ref.load(j, pc.zero if opaque else None, mg)
    if pc is not None:
        a = pc.gate(a)
    a = pltpu.bitcast(a, bf16)
    w = pltpu.bitcast(u_ref.load(j), bf16)
    return jnp.dot(a, w, preferred_element_type=f32)


def _tokens(y):
    m = y.shape[0]
    return [y[8 * r:8 * r + 8, 128 * n:128 * n + 128] for n in range(2) for r in range(m // 8)]


def matmul_stream(x_ref, u_ref, y_ref, pc=None, mg=None):
    def tiles(y, u):
        return [V(y[:, :128], COL_SIGN[u, 0]), V(y[:, 128:], COL_SIGN[u, 1])]

    if mg is not None:
        y_ref = y_ref.at[:, pl.ds(0, 16 * mg), :]
    for cls in CLASSES:
        for kind, k in _class_units(cls):
            if kind == "pair":
                j = (k - 1) * 3
                y1 = _mm(x_ref, u_ref, j, pc, mg)
                k1 = tiles(y1, j)
                yield _tokens(y1)
                y2 = _mm(x_ref, u_ref, j + 1, pc, mg)
                k2 = tiles(y2, j + 1)
                for nt, m in ((0, k), (1, 64 - k)):
                    yi = k1[nt] + k2[nt]
                    assert (yi.s if nt == 0 else -yi.s) == Y_SIGN[m, 1]
                    y_ref[2 * m + 1] = yi.a
                yield _tokens(y2)
                y3 = _mm(x_ref, u_ref, j + 2, pc, mg)
                k3 = tiles(y3, j + 2)
                for nt, m in ((0, k), (1, 64 - k)):
                    yr = k1[nt] - k3[nt]
                    assert yr.s == Y_SIGN[m, 0]
                    y_ref[2 * m] = yr.a
                yield _tokens(y3)
            else:
                y = _mm(x_ref, u_ref, UNIT0 if k == 0 else UNIT32, pc, mg)
                y_ref[2 * k] = y[:, :128]
                y_ref[2 * k + 1] = y[:, 128:]
                yield _tokens(y)


def run_step(mm, pieces, costs, pc, ntok, lead, lag=None, due=None, nunits=NUNITS):
    total = float(sum(costs))
    lag = LAG if lag is None else lag
    tokens = []
    marks = []
    c = 0.0
    for piece, cost in zip(pieces, costs):
        pc.tok = None
        pc.tok2 = marks[-lag] if lag and len(marks) >= lag else None
        if c >= lead:
            want = min(int((c - lead) / (total - lead) * ntok), ntok - 1)
            ahead = min(want + (AHEAD * ntok) // max(nunits, NUNITS), ntok - 1)
            while ahead >= len(tokens):
                tokens += next(mm)
            pc.tok = tokens[want]
        pc.outs = []
        piece()
        marks.append(pc.last)
        for i, v in enumerate(pc.outs):
            q = pc.unit + (DUE if due is None else due) + i // 4
            if q < nunits:
                pc.pending.append((q, v))
        c += cost
    pc.tok = pc.tok2 = None
    for _ in mm:
        pass


def _make_kernel(T):
    T1, T2 = T // 2, T // 4
    L1 = (T1 + 16) // SEG
    L2 = L1 // 2
    assert L1 * SEG == T1 + 16 and L1 % 2 == 0
    NB1 = -(-L1 // S)
    NB2 = -(-L2 // S)
    XPAD = 8
    XB = T1 + 16
    XROWS = XPAD + 2 * XB + 64
    MG = 3
    M = 16 * MG
    NC1 = -(-NB1 // MG)
    NC2 = -(-NB2 // MG)
    ZH = (NB2 - 1) * S + N
    ZDUMP = ZH
    TB = 56
    NCH = -(-L2 // TB)
    FROWS = max(NB2 * S, NCH * TB)
    FDUMP = FROWS
    last_valid = T2 - (SEG - 1) * L2
    XCUT = (24, 304, 592, 848)
    X_NEEDED = ((1, 0), (2, 2), (3, 4))

    def x_rows(e, part):
        def cut(e, i):
            return min((L1 * e + XCUT[i]) // 8 * 8, T1)
        if part == 0:
            out = [(cut(e, 3), cut(e + 1, 0) if e + 1 < SEG else T1)]
            return out + ([(0, cut(0, 0))] if e == 0 else [])
        return [(cut(e, part - 1), cut(e, part))]

    def kernel(x_hbm, w1_hbm, w2_hbm, g_ref, wf_ref, wg_ref, wo_ref, gm_ref, o_hbm,
               xs0, xs1, w_ref, ws0, ws1, u1_ref, u2_ref, pool, y_ref, zh_ref, f_ref, fe_ref, ge_ref,
               st_ref, sem_w, sem_x, sem_o):
        xs = (xs0, xs1)
        x_ref = XView(pool, 0, MG)
        tf = [[View(pool, NUNITS * MG * 4 + (g * 2 + ct) * 256) for ct in range(2)] for g in range(MG)]
        ti = [View(pool, NUNITS * MG * 4 + MG * 512 + g * 256) for g in range(MG)]
        tr = [View(pool, NUNITS * MG * 4 + MG * 768 + g * 224) for g in range(MG)]
        xh = x_hbm.bitcast(u32)
        w1w = w1_hbm.bitcast(u32)
        w2w = w2_hbm.bitcast(u32)

        W1PART = (0, 16, 32, 64, 96, 128)
        W2PART = (0, 16, 32, 128)

        def w1_copy(q):
            rows = pl.ds(W1PART[q], W1PART[q + 1] - W1PART[q])
            return pltpu.make_async_copy(w1w.at[:, rows, :], w_ref.at[:, rows, :], sem_w.at[q % 4])

        ws = (ws0, ws1)

        def w2_copies(part):
            lo, n = W2PART[part], W2PART[part + 1] - W2PART[part]
            return [pltpu.make_async_copy(w2w.at[i, pl.ds(lo, n), _lanes(dt)],
                                          ws[dt].at[pl.ds(WP * i + lo, n), :], sem_w.at[4 + part % 2])
                    for i in range(31) for dt in range(2)]

        def w2_wait(part):
            buf = ws0.at[pl.ds(0, 31 * (W2PART[part + 1] - W2PART[part])), :]
            for _ in range(2):
                pltpu.make_async_copy(buf, buf, sem_w.at[4 + part % 2]).wait()

        def x_copies(part):
            cps = []
            for b in range(2):
                for e in range(SEG):
                    for lo, hi in x_rows(e, part):
                        for ct in range(2):
                            cps.append(pltpu.make_async_copy(
                                xh.at[b, pl.ds(lo, hi - lo), _lanes(ct)],
                                xs[ct].at[pl.ds(XPAD + b * XB + lo, hi - lo), :],
                                sem_x.at[part % 3]))
            return cps

        w1_copy(0).start()
        for cp in w2_copies(0):
            cp.start()
        w1_copy(1).start()
        for cp in w2_copies(1):
            cp.start()
        w1_copy(2).start()
        for dt in range(2):
            for r in range(31 * WP, 31 * WP + 128, 8):
                ws[dt][pl.ds(r, 8), :] = jnp.zeros((8, 128), u32)
        gbase = NUNITS * MG * 4 + MG * 992
        for r in range(24):
            pool[gbase + r] = gm_ref[pl.ds(8 * r, 8), :]

        def g_view(zero):
            return jnp.concatenate([pool[gbase + r + (zero if r == TAP_OPQ else 0)] for r in range(24)], axis=0)

        z8 = jnp.zeros((8, 128), u32)
        for ct in range(2):
            xs[ct][pl.ds(0, 8), :] = z8
            for r in range(XPAD + T1, XPAD + XB, 8):
                xs[ct][pl.ds(r, 8), :] = z8
            for r in range(XPAD + XB + T1, XROWS, 8):
                xs[ct][pl.ds(r, 8), :] = z8

        def zero_zh(i, c):
            for h in range(2):
                for comp in range(2):
                    zh_ref[ZH - 1 - i, h, comp] = jnp.zeros((8, 256), f32)
            return c
        lax.fori_loop(0, ZH - 8 - L2, zero_zh, 0)

        zf = jnp.zeros((M, 128), f32)
        for m in range(0, 64, 4):
            y_ref[2 * m] = zf
            y_ref[2 * m + 1] = zf
        for g in range(MG):
            for h in range(2):
                for k1 in range(8):
                    for n2 in (1, 2, 3, 5, 6, 7):
                        for comp in range(2):
                            ti[g][h, (k1 * 8 + n2) * 2 + comp] = jnp.zeros((8, 128), f32)

        gg = g_ref[...].reshape(16, 256)
        ge_all = jnp.dot(gg, wg_ref[...], preferred_element_type=f32)
        ge_ref[...] = ge_all
        never = jnp.max(jnp.abs(ge_all)) < 0.0

        def transform(hook):
            def body(i, c):
                for j in range(WT_UNROLL):
                    hook(i * WT_UNROLL + j)
                pc = Pacer(i < 0, lax.shift_right_arithmetic(i, 20))
                seq = []
                for j in range(WT_UNROLL):
                    seq += weight_pieces(w_ref, UView(u1_ref), tf[j][0], tf[j][1], i * WT_UNROLL + j, pc)
                n = 4 * WT_UNROLL
                run_step(tap_stream(g_view, ws, u2_ref, n * i, n, pc), [q[0] for q in seq],
                         [q[1] for q in seq], pc, n * 192, LEAD, nunits=n)
                return c
            lax.fori_loop(0, 16 // WT_UNROLL, body, 0)

        def w1_hook(rg):
            for q in range(len(W1PART) - 1):
                @pl.when(rg * 8 == W1PART[q])
                def _(q=q):
                    w1_copy(q).wait()
                    if q < len(W2PART) - 1:
                        w2_wait(q)
                    if q == 0:
                        for cp in w2_copies(2):
                            cp.start()
                    if q + 3 < len(W1PART) - 1:
                        w1_copy(q + 3).start()
                    if q >= 2:
                        for cp in x_copies(q - 2):
                            cp.start()

        P = functools.partial

        def f1(ld, pc):
            return [(P(fwd_p1, ld[g], tf[g][ct], h, n2, ct, pc), COST_F1[n2])
                    for g in range(len(ld)) for ct in range(2) for h in range(2) for n2 in range(8)]

        def f2(cls, pc, mg=MG):
            return [(P(fwd_p2, tf[g][ct], x_ref, g, ct, k1, pc), COST_F2)
                    for g in range(mg) for ct in range(2) for k1 in cls]

        def i1(cls, pc, mg=MG):
            return [(P(inv_p1, y_ref, ti[g], g, h, n2, pc), COST_I1[n2])
                    for g in range(mg) for h in range(2) for n2 in cls]

        def i2(act, pairs_in_time, outs, pc):
            out = []
            for g, o in enumerate(outs):
                out += inverse_tail(ti[g], tr[g], P(act, tr[g], o), pc, pairs_in_time)
            return out

        def step(pc, u_view, mg, loads, act, pairs_in_time, outs):
            nxt = f1(loads, pc)
            half = len(nxt) // 2
            seq = (f2(CLASSES[1], pc, mg) + f2(CLASSES[2], pc, mg) + f2(CLASSES[3], pc, mg)
                   + i1(CLASSES[3], pc, len(outs)) + i2(act, pairs_in_time, outs, pc)
                   + nxt[:half] + i1(CLASSES[0], pc, mg) + nxt[half:]
                   + i1(CLASSES[1], pc, mg) + f2(CLASSES[0], pc, len(loads)) + i1(CLASSES[2], pc, mg))
            run_step(matmul_stream(x_ref, u_view, y_ref, pc, None if mg == MG else mg),
                     [q[0] for q in seq], [q[1] for q in seq], pc, NUNITS * 4 * mg, LEAD)

        def pacer(c):
            return Pacer(c < 0, lax.shift_right_arithmetic(c, 20))

        idle = Pacer(None)
        u1, u2 = UView(u1_ref), UView(u2_ref)

        def x_wait(part):
            rows = sum(4 * (hi - lo) for e in range(SEG) for lo, hi in x_rows(e, part))
            buf = xs0.at[pl.ds(0, rows), :]
            pltpu.make_async_copy(buf, buf, sem_x.at[part % 3]).wait()

        def load1(blk):
            base = blk * S

            def load(h, n, ct, pc):
                w = xs[ct][pl.ds(base + n + h * L1, 8, stride=2 * L1), :]
                if pc is not None:
                    w = pc.here(w)
                return _unpack(w)
            return load

        def load2(blk):
            def load(h, n, ct, pc):
                lo = zh_ref[blk * S + n, h, 0, :, _lanes(ct)]
                hi = zh_ref[blk * S + n, h, 1, :, _lanes(ct)]
                if pc is not None:
                    lo = pc.here(lo)
                return lo, hi
            return load

        def act1(rb, tau0, q, pc):
            return act_conv1(rb, zh_ref, tau0, q, pc)

        def act2(rb, tau0, q, pc):
            return act_conv2(rb, f_ref, tau0, q, pc)

        def loads1(chunk):
            return [load1(chunk * MG + g) for g in range(MG)]

        def loads2(chunk):
            return [load2(jnp.minimum(chunk * MG + g, NB2 - 1)) for g in range(MG)]

        def outs1(chunk):
            return [8 + (chunk * MG + g) * (S // 2) for g in range(MG)]

        def outs2(chunk, n=MG):
            return [(chunk * MG + g) * S for g in range(n)]

        with scope("wt1"):
            transform(w1_hook)

        x_wait(0)
        for cp in x_copies(3):
            cp.start()
        with scope("pro"):
            for piece, _ in f1(loads1(NC1 - 1), idle) + f2(CLASSES[0], idle):
                piece()

        def conv1_step(c, cc):
            for part, first in X_NEEDED:
                @pl.when(c == first)
                def _(part=part):
                    x_wait(part)
            prev = jnp.where(c == 1, NC1 - 1, c - 2)
            outs = [jnp.where(c >= 1, o, ZDUMP) for o in outs1(prev)]
            step(pacer(c), u1, MG, loads1(c), act1, True, outs)
            return cc
        with scope("steps"):
            lax.fori_loop(0, NC1 - 1, conv1_step, 0)

        row = lax.broadcasted_iota(i32, (8, 256), 0)
        for h in range(2):
            for comp in range(2):
                for t in range(last_valid, NB1 * S // 2):
                    zh_ref[8 + t, h, comp] = jnp.where(row == SEG - 1, 0.0, zh_ref[8 + t, h, comp])
                for j in range(8):
                    v = pltpu.roll(zh_ref[8 + L2 - 8 + j, h, comp], 1, axis=0)
                    zh_ref[j, h, comp] = jnp.where(row == 0, 0.0, v)
                for j in range(8):
                    v = pltpu.roll(zh_ref[8 + j, h, comp], SEG - 1, axis=0)
                    zh_ref[8 + L2 + j, h, comp] = jnp.where(row == SEG - 1, 0.0, v)

        fixed = Pacer(never, never.astype(i32))
        with scope("steps"):
            step(fixed, u1, MG, loads2(0), act1, True, outs1(NC1 - 3))
        fixed = Pacer(never, never.astype(i32))
        with scope("steps"):
            step(fixed, u2, MG, loads2(1), act1, True, outs1(NC1 - 2))

        def conv2_step(c, cc):
            step(pacer(c), u2, MG, loads2(c + 1), act2, False, outs2(c - 1))
            return cc
        tail = NB2 - (NC2 - 1) * MG
        with scope("steps"):
            lax.fori_loop(1, NC2 - 1, conv2_step, 0)
            step(Pacer(never, never.astype(i32)), u2, tail, [], act2, False, outs2(NC2 - 2))
        with scope("epi"):
            for piece, _ in i1(CLASSES[3], idle, tail) + i2(act2, False, outs2(NC2 - 1, tail), idle):
                piece()

        order = [(b, e) for b in range(2) for e in range(SEG)]

        def out_copy(half, q, t0, nvalid):
            b, e = order[q]
            r0 = (b * T2 + e * L2) * 8 + t0 * 8
            return pltpu.make_async_copy(st_ref.at[half, q, pl.ds(0, nvalid * 8), :],
                                         o_hbm.at[pl.ds(r0, nvalid * 8), :],
                                         sem_o.at[half])

        def width(e):
            lim = L2 if e < SEG - 1 else last_valid
            return lim - (NCH - 1) * TB

        def joint_chunk(ch, half, full, never):
            pc = Pacer(never)
            t0 = ch * TB
            fl = pltpu.bitcast(f_ref[pl.ds(t0, TB)].reshape(TB * 8, 256), bf16)
            fe = jnp.dot(fl, wf_ref[...], preferred_element_type=f32)
            fe_ref[...] = fe
            prev = [fe[8 * r:8 * r + 8, 128 * n:128 * n + 128] for n in range(2) for r in range(2 * TB)]
            prev = prev[len(prev) // 2:]
            for q, (b, e) in enumerate(order):
                ge = ge_ref[pl.ds(8 * b, 8), :]
                r = 4 * (e & 3) + 2 * b + (e >> 2)
                js = []
                for t in range(TB):
                    row = jnp.broadcast_to(fe_ref[pl.ds(16 * t + r, 1), :], (8, 256))
                    tok = prev[(t * len(prev)) // TB]
                    gt = jnp.concatenate([pc.tie(ge[:, :128], tok), pc.tie(ge[:, 128:], tok)], axis=1)
                    js.append(jnp.tanh(row + gt))
                jl = jnp.concatenate(js, axis=0).astype(bf16)
                y = jnp.dot(jl, wo_ref[...], preferred_element_type=f32)
                prev = [y[8 * rr:8 * rr + 8, 128 * n:128 * n + 128] for n in range(2) for rr in range(TB)]
                st_ref[half, q] = y.astype(bf16)
                out_copy(half, q, t0, TB if full else width(e)).start()

        def wait_chunk(half, full):
            if full:
                pltpu.make_async_copy(st_ref.at[half], st_ref.at[half], sem_o.at[half]).wait()
                return
            for q, (b, e) in enumerate(order):
                out_copy(half, q, 0, width(e)).wait()

        def joint_body(ch, c):
            half = ch % 2

            @pl.when(ch >= 2)
            def _():
                wait_chunk(half, True)
            joint_chunk(ch, half, True, ch < 0)
            return c
        with scope("joint"):
            lax.fori_loop(0, NCH - 1, joint_body, 0)
            last_half = (NCH - 1) % 2
            wait_chunk(last_half, True)
            joint_chunk(NCH - 1, last_half, False, never)
            wait_chunk(1 - last_half, True)
            wait_chunk(last_half, False)

    scratch = [
        pltpu.VMEM((XROWS, 128), u32), pltpu.VMEM((XROWS, 128), u32),
        pltpu.VMEM((31, 128, 256), u32),
        pltpu.VMEM((32 * WP + 8, 128), u32), pltpu.VMEM((32 * WP + 8, 128), u32),
        pltpu.VMEM((2 * 96 * UP, 128), u32), pltpu.VMEM((2 * 96 * UP, 128), u32),
        pltpu.VMEM((NUNITS * MG * 4 + MG * 992 + 24, 8, 128), u32),
        pltpu.VMEM((128, M, 128), f32),
        pltpu.VMEM((ZH + S // 2, 2, 2, 8, 256), f32),
        pltpu.VMEM((FROWS + S, 8, 256), u32),
        pltpu.VMEM((TB * 16, 256), f32),
        pltpu.VMEM((16, 256), f32),
        pltpu.VMEM((2, 2 * SEG, TB * 8, 256), bf16),
        pltpu.SemaphoreType.DMA((6,)),
        pltpu.SemaphoreType.DMA((3,)),
        pltpu.SemaphoreType.DMA((2,)),
    ]
    return kernel, scratch


TAP_MATRIX = _tap_matrix()
WT_UNROLL = 2
TAP_OPQ = 23
TAP_GATE = 20
LEAD = 0
LAG = 0
AHEAD = 2
OPQ_EVERY = 1
DUE = 0
DUE_EVERY = 1000


def _call(x, w1, w2, g, w_f, w_g, w_o, interpret=False):
    B, T, D = x.shape
    kernel, scratch = _make_kernel(T)
    T2 = T // 4
    any_spec = pl.BlockSpec(memory_space=pl.ANY)
    vmem = pl.BlockSpec(memory_space=pltpu.VMEM)
    out = pl.pallas_call(
        kernel,
        out_shape=jax.ShapeDtypeStruct((B * T2 * 8, D), bf16),
        in_specs=[any_spec, any_spec, any_spec, vmem, vmem, vmem, vmem, vmem],
        out_specs=any_spec,
        scratch_shapes=scratch,
        compiler_params=pltpu.CompilerParams(vmem_limit_bytes=127 * 2**20),
        interpret=interpret,
        name="conv_stem_rnnt_joint",
    )(x, w1, w2, g, w_f, w_g, w_o, TAP_MATRIX)
    return out.reshape(B, T2, 8, D)


@jax.jit
def pallas_standalone__seq2seq_rnn_t_joint__speech_kernel(x, w1, w2, g, w_f, w_g, w_o):
    return _call(x, w1, w2, g, w_f, w_g, w_o)
```

```python
import functools
import math

import jax
import jax.numpy as jnp
import numpy as np
from jax import lax
from jax.experimental import pallas as pl
from jax.experimental.pallas import tpu as pltpu

f32, u32, bf16, i32 = jnp.float32, jnp.uint32, jnp.bfloat16, jnp.int32

PROFILE_SCOPES = False


class _NoScope:
    def __enter__(self):
        return self

    def __exit__(self, *a):
        return False


def scope(name):
    return jax.named_scope(name) if PROFILE_SCOPES else _NoScope()

N = 64
S = 48
SEG = 8


class V:
    __slots__ = ("a", "s")

    def __init__(self, a, s=1):
        self.a = a
        self.s = s

    def __neg__(self):
        return V(self.a, -self.s)

    def __add__(self, o):
        if self.s == o.s:
            return V(self.a + o.a, self.s)
        if self.s > 0:
            return V(self.a - o.a, 1)
        return V(o.a - self.a, 1)

    def __sub__(self, o):
        return self + (-o)

    def scale(self, c):
        if c == 1.0:
            return self
        if c == -1.0:
            return -self
        return V(self.a * np.float32(abs(c)), self.s * (1 if c > 0 else -1))

    def times(self, c):
        return self.a * np.float32(self.s * c)

    def signed(self, s):
        return self.a if self.s * s > 0 else -self.a


class C:
    __slots__ = ("r", "i")

    def __init__(self, r, i):
        self.r = r
        self.i = i

    def __add__(self, o):
        return C(self.r + o.r, self.i + o.i)

    def __sub__(self, o):
        return C(self.r - o.r, self.i - o.i)

    def __neg__(self):
        return C(-self.r, -self.i)

    def mul_w(self, num, den):
        num %= den
        if num == 0:
            return self
        if 4 * num == den:
            return C(-self.i, self.r)
        if 2 * num == den:
            return -self
        if 4 * num == 3 * den:
            return C(self.i, -self.r)
        if (8 * num) % den == 0:
            o = (8 * num) // den
            h = math.sqrt(0.5)
            sc = 1 if o in (1, 7) else -1
            ss = 1 if o in (1, 3) else -1
            r, m = self.r, self.i
            re = (r if sc > 0 else -r) - (m if ss > 0 else -m)
            im = (r if ss > 0 else -r) + (m if sc > 0 else -m)
            return C(re.scale(h), im.scale(h))
        c = math.cos(2 * math.pi * num / den)
        s = math.sin(2 * math.pi * num / den)
        return C(self.r.scale(c) - self.i.scale(s), self.r.scale(s) + self.i.scale(c))


def _add(a, b):
    if a is None:
        return b
    if b is None:
        return a
    return a + b


def _sub(a, b):
    if b is None:
        return a
    if a is None:
        return -b
    return a - b


def fft8(x, sgn, need=tuple(range(8))):
    def rot(a, num, den):
        return None if a is None else a.mul_w(sgn * num, den)

    need = set(need)
    a0, a1 = _add(x[0], x[4]), _sub(x[0], x[4])
    a2, a3 = _add(x[2], x[6]), rot(_sub(x[2], x[6]), 1, 4)
    a4, a5 = _add(x[1], x[5]), _sub(x[1], x[5])
    a6, a7 = _add(x[3], x[7]), rot(_sub(x[3], x[7]), 1, 4)
    out = {}
    if need & {0, 4}:
        b0, b4 = _add(a0, a2), _add(a4, a6)
        if 0 in need:
            out[0] = _add(b0, b4)
        if 4 in need:
            out[4] = _sub(b0, b4)
    if need & {2, 6}:
        b2, b6 = _sub(a0, a2), rot(_sub(a4, a6), 1, 4)
        if 2 in need:
            out[2] = _add(b2, b6)
        if 6 in need:
            out[6] = _sub(b2, b6)
    if need & {1, 5}:
        b1, b5 = _add(a1, a3), rot(_add(a5, a7), 1, 8)
        if 1 in need:
            out[1] = _add(b1, b5)
        if 5 in need:
            out[5] = _sub(b1, b5)
    if need & {3, 7}:
        b3, b7 = _sub(a1, a3), rot(_sub(a5, a7), 3, 8)
        if 3 in need:
            out[3] = _add(b3, b7)
        if 7 in need:
            out[7] = _sub(b3, b7)
    return out


class _Sym:
    def __add__(self, o):
        return self

    __sub__ = __mul__ = __add__

    def __neg__(self):
        return self


def _fft64_signs(sgn, present=tuple(range(64)), in_sign=None):
    d = _Sym()
    in_sign = in_sign or {}
    x = [C(V(d, in_sign.get((n, 0), 1)), V(d, in_sign.get((n, 1), 1))) if n in present else None
         for n in range(64)]
    t = {}
    for n2 in range(8):
        a = fft8([x[8 * n1 + n2] for n1 in range(8)], sgn)
        for k1 in range(8):
            t[k1, n2] = a[k1].mul_w(sgn * n2 * k1, 64)
    s1 = {key: (v.r.s, v.i.s) for key, v in t.items()}
    s2 = {}
    for k1 in range(8):
        b = fft8([t[k1, n2] for n2 in range(8)], sgn)
        for k2 in range(8):
            s2[k1 + 8 * k2] = b[k2]
    return s1, s2


def _unit(k, j):
    return (k - 1) * 3 + j


UNIT0, UNIT32 = 93, 94
NUNITS = 95


def _lhs_forms(m, z):
    if m in (0, 32):
        u = UNIT0 if m == 0 else UNIT32
        return [(u, 0, z.r), (u, 1, z.i)]
    if m < 32:
        return [(_unit(m, 0), 0, z.r + z.i), (_unit(m, 1), 0, z.r), (_unit(m, 2), 0, z.i)]
    k = 64 - m
    return [(_unit(k, 0), 1, z.r - z.i), (_unit(k, 1), 1, z.r), (_unit(k, 2), 1, z.i)]


def _lhs_signs():
    _, s2 = _fft64_signs(-1)
    sg = {}
    for m in range(64):
        for u, h, v in _lhs_forms(m, s2[m]):
            sg[u, h] = v.s
    return sg


LHS_SIGN = _lhs_signs()


def _weight_forms(m, pm):
    if m < 32:
        nt = 0 if pm > 0 else 1
        return [(_unit(m, 0), 1, nt, (1, 0)), (_unit(m, 1), 1, nt, (-1, 1)), (_unit(m, 2), 1, nt, (-1, -1))]
    k = 64 - m
    nt = 1 if pm > 0 else 0
    return [(_unit(k, 0), 0, nt, (1, 0)), (_unit(k, 1), 0, nt, (-1, -1)), (_unit(k, 2), 0, nt, (1, -1))]


def _weight_plan():
    s1, s2 = _fft64_signs(1, present=range(16))
    forms = {}
    for pm in (1, -1):
        for m in range(1, 64):
            if m == 32:
                continue
            for u, half, nt, (cr, ci) in _weight_forms(m, pm):
                forms[u, half, nt] = (cr * s2[m].r.s, ci * s2[m].i.s)
    col = {}
    for u in range(93):
        for nt in range(2):
            def negs(sig):
                n = 0
                for half in range(2):
                    cr, ci = forms[u, half, nt]
                    w = sig * LHS_SIGN[u, half]
                    n += (w * cr <= 0 and w * ci <= 0)
                return n
            col[u, nt] = 1 if negs(1) <= negs(-1) else -1
    for u in (UNIT0, UNIT32):
        col[u, 0] = col[u, 1] = 1
    return s1, s2, col


WT_S1, WT_S2, COL_SIGN = _weight_plan()


def _recombine(k1, k2, k3, k):
    out = {}
    for nt in range(2):
        yr = k1[nt] - k3[nt]
        yi = k1[nt] + k2[nt]
        if nt == 0:
            out[k, 0], out[k, 1] = yr, yi
        else:
            out[64 - k, 0], out[64 - k, 1] = yr, -yi
    return out


def _y_signs():
    d = _Sym()
    sg = {}
    for k in range(1, 32):
        ks = [[V(d, COL_SIGN[_unit(k, j), nt]) for nt in range(2)] for j in range(3)]
        for key, v in _recombine(ks[0], ks[1], ks[2], k).items():
            sg[key] = v.s
    for m, u in ((0, UNIT0), (32, UNIT32)):
        sg[m, 0], sg[m, 1] = COL_SIGN[u, 0], COL_SIGN[u, 1]
    return sg


Y_SIGN = _y_signs()


def _unpack(w):
    lo = pltpu.unpack_elementwise(w, index=0, packed_dtype=bf16, unpacked_dtype=f32)
    hi = pltpu.unpack_elementwise(w, index=1, packed_dtype=bf16, unpacked_dtype=f32)
    return lo, hi


def _pack(lo, hi):
    return pltpu.pack_elementwise([lo, hi], packed_dtype=bf16)


_GC1 = 2.0 * math.sqrt(2.0 / math.pi)
_GC2 = 8.0 * 0.044715 * math.sqrt(2.0 / math.pi)


def _gelu_half(v):
    a = v.a
    p = (a * a) * np.float32(_GC2) + np.float32(_GC1)
    t = jnp.tanh(p * a)
    return a * t + a if v.s > 0 else a * t - a


def _lanes(t):
    return pl.ds(128 * t, 128)


class Pacer:
    def __init__(self, never, zero=None):
        self.never = never
        self.tok = None
        self.tok2 = None
        self.last = None
        self.outs = []
        self.zero = zero
        self.pending = []
        self.unit = 0

    def gate(self, a, first=0):
        vals = [v for q, v in self.pending if q <= self.unit]
        self.pending = [(q, v) for q, v in self.pending if q > self.unit]
        self.unit += 1
        if not vals:
            return a
        m, k = a.shape
        tiles = [[a[8 * r:8 * r + 8, 128 * c:128 * c + 128] for c in range(k // 128)] for r in range(m // 8)]
        flat = [(r, c) for r in range(first, m // 8) for c in range(k // 128)]
        for i, v in enumerate(vals):
            r, c = flat[i % len(flat)]
            tiles[r][c] = self.tie(tiles[r][c], v)
        return jnp.concatenate([jnp.concatenate(row, axis=1) for row in tiles], axis=0)

    def here(self, x):
        tok, self.tok = self.tok, None
        tok2, self.tok2 = self.tok2, None
        return self.tie(self.tie(x, tok), tok2)

    def mark(self, x, nth=None):
        self.last = x
        if self.never is not None and nth is not None and nth % DUE_EVERY == DUE_EVERY - 1:
            self.outs.append(x)
        return x

    def due(self, x):
        if self.never is not None:
            self.outs.append(x)
        return x

    def tie(self, x, tok):
        if tok is None:
            return x
        if tok.dtype != x.dtype:
            tok = pltpu.bitcast(tok, x.dtype)
        return jnp.where(self.never, tok, x)


def _combo(f, cr, ci, want):
    if ci == 0:
        return f.r.signed(want * cr)
    v = (f.r if cr > 0 else -f.r) + (f.i if ci > 0 else -f.i)
    if v.s * want > 0:
        return v.a
    if f.r.s * cr != f.i.s * ci:
        return ((-f.r) if cr > 0 else f.r).__add__((-f.i) if ci > 0 else f.i).a
    return -v.a


UP = 260
WP = 132


class UView:
    def __init__(self, ref):
        self.ref = ref

    def load(self, u):
        return jnp.concatenate([self.ref[pl.ds((nt * 96 + u) * UP, 256), :] for nt in range(2)], axis=1)

    def store(self, u, half, nt, rg, val):
        self.ref[pl.ds((nt * 96 + u) * UP + half * 128 + rg * 8, 8), :] = val


def _tap_matrix():
    import ml_dtypes
    sigma, tau = 1.0 / 256.0, 1.0 / 128.0
    g = np.zeros((2, 2, 96, 32, 2))
    d = np.arange(16)
    for tap in range(31):
        for dt in range(2):
            wa = np.zeros((16, 2))
            wb = np.zeros((16, 2))
            if tap % 2:
                wa[(tap + 1) // 2, dt] = 1.0
            else:
                wb[tap // 2, dt] = 1.0
            z0 = wa[:, 0] + 1j * wb[:, 0]
            z1 = wa[:, 1] + 1j * wb[:, 1]
            for pm, z in ((1, z0 + 1j * z1), (-1, z0 - 1j * z1)):
                for m in range(1, 64):
                    if m == 32:
                        continue
                    f = sigma * np.sum(z * np.exp(2j * np.pi * m * d / 64))
                    for u, half, nt, (cr, ci) in _weight_forms(m, pm):
                        g[nt, half, u, tap, dt] = (LHS_SIGN[u, half] * COL_SIGN[u, nt]
                                                   * (cr * f.real + ci * f.imag))
            for m, u in ((0, UNIT0), (32, UNIT32)):
                e = np.cos(np.pi * m * d / 32)
                for half, wv in enumerate((wa, wb)):
                    g[dt, half, u, tap, dt] = (LHS_SIGN[u, half] * COL_SIGN[u, dt]
                                               * tau * np.sum(e * wv[:, dt]))
    g = g.reshape(384, 32, 2)
    mat = np.zeros((384, 128))
    for v in range(4):
        dt, t0 = v // 2, 16 * (v % 2)
        for s_ in range(8):
            for par in range(2):
                mat[:, 16 * v + 2 * s_ + par] = g[:, t0 + 8 * par + s_, dt]
    hi = mat.astype(ml_dtypes.bfloat16)
    lo = (mat - hi.astype(np.float64)).astype(ml_dtypes.bfloat16)
    full = np.concatenate([hi[:, :64], lo[:, :64]], axis=1).view(np.uint16).astype(np.uint32)
    return full[0::2] | (full[1::2] << 16)


def tap_operand(ws, cpair):
    ev, od = [], []
    for dt in range(2):
        for t0 in (0, 16):
            wa = ws[dt][pl.ds(t0 * WP + cpair, 8, stride=WP), :]
            wb = ws[dt][pl.ds((t0 + 8) * WP + cpair, 8, stride=WP), :]
            alo, ahi = _unpack(wa)
            blo, bhi = _unpack(wb)
            ev.append(_pack(alo, blo))
            od.append(_pack(ahi, bhi))
    return jnp.concatenate(ev + ev, axis=0), jnp.concatenate(od + od, axis=0)


def tap_stream(g_view, ws, u2_ref, it0, n, pc):
    for q in range(n):
        it = it0 + q
        lhs = pltpu.bitcast(pc.gate(g_view(pc.zero), TAP_GATE), bf16)
        ops = []
        for j in range(2):
            ops += list(tap_operand(ws, 2 * it + j))
        rhs = pltpu.bitcast(jnp.concatenate(ops, axis=1), bf16)
        y = jnp.dot(lhs, rhs, preferred_element_type=f32)
        for r in range(48):
            nt, half, u0 = r // 24, (r // 12) % 2, (r % 12) * 8
            for j in range(2):
                val = _pack(y[8 * r:8 * r + 8, 256 * j:256 * j + 128],
                            y[8 * r:8 * r + 8, 256 * j + 128:256 * j + 256])
                u2_ref[pl.ds((nt * 96 + u0) * UP + half * 128 + 2 * it + j, 8, stride=UP), :] = val
        yield [y[8 * r:8 * r + 8, 128 * t:128 * t + 128] for r in range(48) for t in range(4)]


def weight_pieces(w_ref, u_ref, t_ref, z_ref, rg, pc):
    rows = pl.ds(pl.multiple_of(rg * 8, 8), 8)
    sigma = 1.0 / 256.0
    tau = 1.0 / 128.0
    acc = {}

    def store(u, half, nt, a0, a1):
        u_ref.store(u, half, nt, rg, pc.due(_pack(a0, a1)))

    def prep(d):
        wa = [[None, None], [None, None]]
        wb = [[None, None], [None, None]]
        for dt in range(2):
            w = w_ref[2 * d, rows, _lanes(dt)]
            if dt == 0:
                w = pc.here(w)
            lo, hi = _unpack(w)
            wb[0][dt], wb[1][dt] = V(lo), V(hi)
            if d > 0:
                lo, hi = _unpack(w_ref[2 * d - 1, rows, _lanes(dt)])
                wa[0][dt], wa[1][dt] = V(lo), V(hi)
        for p in range(2):
            for dt in range(2):
                for name, val in (("a", wa[p][dt]), ("b", wb[p][dt])):
                    key = (p, dt, name, d % 2)
                    acc[key] = _add(acc.get(key), val)
            zp = (_sub(wa[p][0], wb[p][1]), _add(wb[p][0], wa[p][1]))
            zm = (_add(wa[p][0], wb[p][1]), _sub(wb[p][0], wa[p][1]))
            for j, z in enumerate((zp, zm)):
                for comp in range(2):
                    z_ref[j, (p * 16 + d) * 2 + comp] = z[comp].times(sigma)

    def real_bins():
        for m, u in ((0, UNIT0), (32, UNIT32)):
            for dt in range(2):
                for half, name in enumerate(("a", "b")):
                    vals = []
                    for p in range(2):
                        ev, od = acc[p, dt, name, 0], acc[p, dt, name, 1]
                        v = _add(ev, od) if m == 0 else _sub(ev, od)
                        vals.append(v.times(tau * LHS_SIGN[u, half] * COL_SIGN[u, dt]))
                    store(u, half, dt, vals[0], vals[1])

    def pass1(j, p, n2):
        z = [C(V(z_ref[j, (p * 16 + d) * 2]), V(z_ref[j, (p * 16 + d) * 2 + 1])) for d in (n2, n2 + 8)]
        z[0].r.a = pc.here(z[0].r.a)
        a = fft8(z + [None] * 6, 1)
        for k1 in range(8):
            t = a[k1].mul_w(n2 * k1, 64)
            assert (t.r.s, t.i.s) == WT_S1[k1, n2]
            t_ref[p, (k1 * 8 + n2) * 2] = t.r.a
            t_ref[p, (k1 * 8 + n2) * 2 + 1] = t.i.a

    def pass2(pm, k1):
        need = [k2 for k2 in range(8) if (k1 + 8 * k2) not in (0, 32)]
        outs = []
        for p in range(2):
            xs = [C(V(t_ref[p, (k1 * 8 + n2) * 2], WT_S1[k1, n2][0]),
                    V(t_ref[p, (k1 * 8 + n2) * 2 + 1], WT_S1[k1, n2][1])) for n2 in range(8)]
            if p == 0:
                xs[0].r.a = pc.here(xs[0].r.a)
            outs.append(fft8(xs, 1, need))
        for k2 in need:
            m = k1 + 8 * k2
            for u, half, nt, (cr, ci) in _weight_forms(m, pm):
                want = LHS_SIGN[u, half] * COL_SIGN[u, nt]
                store(u, half, nt, _combo(outs[0][k2], cr, ci, want), _combo(outs[1][k2], cr, ci, want))

    P = functools.partial
    out = [(P(prep, d), 40) for d in range(16)] + [(real_bins, 40)]
    for j, pm in enumerate((1, -1)):
        out += [(P(pass1, j, p, n2), 21 + _TW[n2]) for p in range(2) for n2 in range(8)]
        out += [(P(pass2, pm, k1), 193) for k1 in range(8)]
    return out


class View:
    def __init__(self, pool, base):
        self.pool = pool
        self.base = base

    def __getitem__(self, idx):
        h, i = idx
        return pltpu.bitcast(self.pool[self.base + h * 128 + i], f32)

    def __setitem__(self, idx, val):
        h, i = idx
        self.pool[self.base + h * 128 + i] = pltpu.bitcast(val, u32)


class XView:
    def __init__(self, pool, base, mg):
        self.pool, self.base, self.mg = pool, base, mg

    def index(self, u, g, c):
        return self.base + (u * self.mg + g) * 4 + c

    def store(self, u, g, c, val):
        self.pool[self.index(u, g, c)] = val

    def load(self, u, zero=None, mg=None):
        rows = []
        for g in range(self.mg if mg is None else mg):
            row = []
            for c in range(4):
                idx = self.index(u, g, c)
                if zero is not None and g == 0 and c == 0:
                    idx = idx + zero
                row.append(self.pool[idx])
            rows.append(jnp.concatenate(row, axis=1))
        return jnp.concatenate(rows, axis=0)


_TW = (0, 42, 40, 42, 32, 42, 40, 42)
COST_F1 = tuple(73 + t for t in _TW)
COST_I1 = tuple(57 + t for t in _TW)
COST_F2, COST_I2, COST_ACT = 153, 53, 85
FWD_S1, _ = _fft64_signs(-1)
INV_S1, _INV_OUT = _fft64_signs(1, in_sign=Y_SIGN)
INV_S2 = {m: (v.r.s, v.i.s) for m, v in _INV_OUT.items()}
CLASSES = ((1, 7), (2, 6), (3, 5), (4, 0))


def _class_units(cls):
    ks = [k for k in range(1, 32) if k % 8 in cls or (-k) % 8 in cls]
    ks.sort(key=lambda k: (0 if k % 8 == cls[0] else 1, k))
    out = [("pair", k) for k in ks]
    if 0 in cls:
        out += [("real", 0), ("real", 32)]
    return out


def fwd_p1(load, t_ref, h, n2, ct, pc):
    xs = []
    for n1 in range(8):
        lo, hi = load(h, 8 * n1 + n2, ct, pc if n1 == 0 else None)
        xs.append(C(V(lo), V(hi)))
    a = fft8(xs, -1)
    for k1 in range(8):
        t = a[k1].mul_w(-n2 * k1, 64)
        assert (t.r.s, t.i.s) == FWD_S1[k1, n2]
        t_ref[h, (k1 * 8 + n2) * 2] = t.r.a
        t_ref[h, (k1 * 8 + n2) * 2 + 1] = t.i.a


def fwd_p2(t_ref, x_ref, g, ct, k1, pc):
    outs = []
    for h in range(2):
        xs = [C(V(t_ref[h, (k1 * 8 + n2) * 2], FWD_S1[k1, n2][0]),
                V(t_ref[h, (k1 * 8 + n2) * 2 + 1], FWD_S1[k1, n2][1])) for n2 in range(8)]
        if h == 0:
            xs[0].r.a = pc.here(xs[0].r.a)
        outs.append(fft8(xs, -1))
    for k2 in range(8):
        m = k1 + 8 * k2
        f0 = _lhs_forms(m, outs[0][k2])
        f1 = _lhs_forms(m, outs[1][k2])
        for i, ((u, half, v0), (_, _, v1)) in enumerate(zip(f0, f1)):
            assert v0.s == v1.s == LHS_SIGN[u, half]
            x_ref.store(u, g, 2 * half + ct, _pack(v0.a, v1.a))
    return COST_F2


def inv_p1(y_ref, t_ref, g, h, n2, pc):
    rows = pl.ds(g * 16 + 8 * h, 8)
    ysg = Y_SIGN
    xs = []
    for n1 in range(8):
        m = 8 * n1 + n2
        xs.append(C(V(y_ref[2 * m, rows, :], ysg.get((m, 0), 1)),
                    V(y_ref[2 * m + 1, rows, :], ysg.get((m, 1), 1))))
    xs[0].r.a = pc.here(xs[0].r.a)
    a = fft8(xs, 1)
    for k1 in range(8):
        t = a[k1].mul_w(n2 * k1, 64)
        assert (t.r.s, t.i.s) == INV_S1[k1, n2]
        t_ref[h, (k1 * 8 + n2) * 2] = t.r.a
        t_ref[h, (k1 * 8 + n2) * 2 + 1] = t.i.a


def inv_p2(t_ref, r_ref, h, k1, pc):
    xs = [C(V(t_ref[h, (k1 * 8 + n2) * 2], INV_S1[k1, n2][0]),
            V(t_ref[h, (k1 * 8 + n2) * 2 + 1], INV_S1[k1, n2][1])) for n2 in range(8)]
    xs[0].r.a = pc.here(xs[0].r.a)
    b = fft8(xs, 1, range(S // 8))
    for k2 in range(S // 8):
        assert (b[k2].r.s, b[k2].i.s) == INV_S2[k1 + 8 * k2]
        r_ref[h, (k1 * 6 + k2) * 2] = b[k2].r.a
        r_ref[h, (k1 * 6 + k2) * 2 + 1] = b[k2].i.a
    return COST_I2


def _act(r_ref, h, k1, k2, dt, first, pc):
    a = r_ref[h, (k1 * 6 + k2) * 2 + dt]
    if first:
        a = pc.here(a)
    return _gelu_half(V(a, INV_S2[k1 + 8 * k2][dt]))


def act_conv1(r_ref, zh_ref, tau0, q, pc):
    h, k1, part = q // 8, 2 * ((q % 8) // 2), q % 2
    first = True
    for k2 in range(3 * part, 3 * part + 3):
        for dt in range(2):
            ev = _act(r_ref, h, k1, k2, dt, first, pc)
            od = _act(r_ref, h, k1 + 1, k2, dt, False, pc)
            first = False
            zh_ref[tau0 + (k1 // 2 + 4 * k2), h, 0, :, _lanes(dt)] = pc.due(ev)
            zh_ref[tau0 + (k1 // 2 + 4 * k2), h, 1, :, _lanes(dt)] = pc.due(od)
    return COST_ACT


def act_conv2(r_ref, f_ref, tau0, q, pc):
    k1, part = q // 2, q % 2
    first = True
    for k2 in range(3 * part, 3 * part + 3):
        for dt in range(2):
            oa = _act(r_ref, 0, k1, k2, dt, first, pc)
            ob = _act(r_ref, 1, k1, k2, dt, False, pc)
            first = False
            f_ref[tau0 + (k1 + 8 * k2), :, _lanes(dt)] = pc.due(_pack(oa, ob))
    return COST_ACT


def inverse_tail(t_ref, r_ref, act, pc, pairs_in_time):
    P = functools.partial
    out = []
    if pairs_in_time:
        for h in range(2):
            for kp in range(4):
                out += [(P(inv_p2, t_ref, r_ref, h, 2 * kp + j, pc), COST_I2) for j in range(2)]
                out += [(P(act, h * 8 + kp * 2 + j, pc), COST_ACT) for j in range(2)]
    else:
        for k1 in range(8):
            out += [(P(inv_p2, t_ref, r_ref, h, k1, pc), COST_I2) for h in range(2)]
            out += [(P(act, k1 * 2 + j, pc), COST_ACT) for j in range(2)]
    return out


def _mm(x_ref, u_ref, j, pc=None, mg=None):
    opaque = pc is not None and pc.unit % OPQ_EVERY == 0
    a = x_ref.load(j, pc.zero if opaque else None, mg)
    if pc is not None:
        a = pc.gate(a)
    a = pltpu.bitcast(a, bf16)
    w = pltpu.bitcast(u_ref.load(j), bf16)
    return jnp.dot(a, w, preferred_element_type=f32)


def _tokens(y):
    m = y.shape[0]
    return [y[8 * r:8 * r + 8, 128 * n:128 * n + 128] for n in range(2) for r in range(m // 8)]


def matmul_stream(x_ref, u_ref, y_ref, pc=None, mg=None):
    def tiles(y, u):
        return [V(y[:, :128], COL_SIGN[u, 0]), V(y[:, 128:], COL_SIGN[u, 1])]

    if mg is not None:
        y_ref = y_ref.at[:, pl.ds(0, 16 * mg), :]
    for cls in CLASSES:
        for kind, k in _class_units(cls):
            if kind == "pair":
                j = (k - 1) * 3
                y1 = _mm(x_ref, u_ref, j, pc, mg)
                k1 = tiles(y1, j)
                yield _tokens(y1)
                y2 = _mm(x_ref, u_ref, j + 1, pc, mg)
                k2 = tiles(y2, j + 1)
                for nt, m in ((0, k), (1, 64 - k)):
                    yi = k1[nt] + k2[nt]
                    assert (yi.s if nt == 0 else -yi.s) == Y_SIGN[m, 1]
                    y_ref[2 * m + 1] = yi.a
                yield _tokens(y2)
                y3 = _mm(x_ref, u_ref, j + 2, pc, mg)
                k3 = tiles(y3, j + 2)
                for nt, m in ((0, k), (1, 64 - k)):
                    yr = k1[nt] - k3[nt]
                    assert yr.s == Y_SIGN[m, 0]
                    y_ref[2 * m] = yr.a
                yield _tokens(y3)
            else:
                y = _mm(x_ref, u_ref, UNIT0 if k == 0 else UNIT32, pc, mg)
                y_ref[2 * k] = y[:, :128]
                y_ref[2 * k + 1] = y[:, 128:]
                yield _tokens(y)


def run_step(mm, pieces, costs, pc, ntok, lead, lag=None, due=None, nunits=NUNITS):
    total = float(sum(costs))
    lag = LAG if lag is None else lag
    tokens = []
    marks = []
    c = 0.0
    for piece, cost in zip(pieces, costs):
        pc.tok = None
        pc.tok2 = marks[-lag] if lag and len(marks) >= lag else None
        if c >= lead:
            want = min(int((c - lead) / (total - lead) * ntok), ntok - 1)
            ahead = min(want + (AHEAD * ntok) // max(nunits, NUNITS), ntok - 1)
            while ahead >= len(tokens):
                tokens += next(mm)
            pc.tok = tokens[want]
        pc.outs = []
        piece()
        marks.append(pc.last)
        for i, v in enumerate(pc.outs):
            q = pc.unit + (DUE if due is None else due) + i // 4
            if q < nunits:
                pc.pending.append((q, v))
        c += cost
    pc.tok = pc.tok2 = None
    for _ in mm:
        pass


def _make_kernel(T):
    T1, T2 = T // 2, T // 4
    L1 = (T1 + 16) // SEG
    L2 = L1 // 2
    assert L1 * SEG == T1 + 16 and L1 % 2 == 0
    NB1 = -(-L1 // S)
    NB2 = -(-L2 // S)
    XPAD = 8
    XB = T1 + 16
    XROWS = XPAD + 2 * XB + 64
    MG = 3
    M = 16 * MG
    NC1 = -(-NB1 // MG)
    NC2 = -(-NB2 // MG)
    ZH = (NB2 - 1) * S + N
    ZDUMP = ZH
    TB = 56
    NCH = -(-L2 // TB)
    FROWS = max(NB2 * S, NCH * TB)
    FDUMP = FROWS
    last_valid = T2 - (SEG - 1) * L2
    XCUT = (24, 304, 592, 848)
    X_NEEDED = ((1, 0), (2, 2), (3, 4))

    def x_rows(e, part):
        def cut(e, i):
            return min((L1 * e + XCUT[i]) // 8 * 8, T1)
        if part == 0:
            out = [(cut(e, 3), cut(e + 1, 0) if e + 1 < SEG else T1)]
            return out + ([(0, cut(0, 0))] if e == 0 else [])
        return [(cut(e, part - 1), cut(e, part))]

    def kernel(x_hbm, w1_hbm, w2_hbm, g_ref, wf_ref, wg_ref, wo_ref, gm_ref, o_hbm,
               xs0, xs1, w_ref, ws0, ws1, u1_ref, u2_ref, pool, y_ref, zh_ref, f_ref, fe_ref, ge_ref,
               st_ref, sem_w, sem_x, sem_o):
        xs = (xs0, xs1)
        x_ref = XView(pool, 0, MG)
        tf = [[View(pool, NUNITS * MG * 4 + (g * 2 + ct) * 256) for ct in range(2)] for g in range(MG)]
        ti = [View(pool, NUNITS * MG * 4 + MG * 512 + g * 256) for g in range(MG)]
        tr = [View(pool, NUNITS * MG * 4 + MG * 768 + g * 224) for g in range(MG)]
        xh = x_hbm.bitcast(u32)
        w1w = w1_hbm.bitcast(u32)
        w2w = w2_hbm.bitcast(u32)

        W1PART = (0, 16, 32, 64, 96, 128)
        W2PART = (0, 16, 32, 128)

        def w1_copy(q):
            rows = pl.ds(W1PART[q], W1PART[q + 1] - W1PART[q])
            return pltpu.make_async_copy(w1w.at[:, rows, :], w_ref.at[:, rows, :], sem_w.at[q % 4])

        ws = (ws0, ws1)

        def w2_copies(part):
            lo, n = W2PART[part], W2PART[part + 1] - W2PART[part]
            return [pltpu.make_async_copy(w2w.at[i, pl.ds(lo, n), _lanes(dt)],
                                          ws[dt].at[pl.ds(WP * i + lo, n), :], sem_w.at[4 + part % 2])
                    for i in range(31) for dt in range(2)]

        def w2_wait(part):
            buf = ws0.at[pl.ds(0, 31 * (W2PART[part + 1] - W2PART[part])), :]
            for _ in range(2):
                pltpu.make_async_copy(buf, buf, sem_w.at[4 + part % 2]).wait()

        def x_copies(part):
            cps = []
            for b in range(2):
                for e in range(SEG):
                    for lo, hi in x_rows(e, part):
                        for ct in range(2):
                            cps.append(pltpu.make_async_copy(
                                xh.at[b, pl.ds(lo, hi - lo), _lanes(ct)],
                                xs[ct].at[pl.ds(XPAD + b * XB + lo, hi - lo), :],
                                sem_x.at[part % 3]))
            return cps

        w1_copy(0).start()
        for cp in w2_copies(0):
            cp.start()
        w1_copy(1).start()
        for cp in w2_copies(1):
            cp.start()
        w1_copy(2).start()
        for dt in range(2):
            for r in range(31 * WP, 31 * WP + 128, 8):
                ws[dt][pl.ds(r, 8), :] = jnp.zeros((8, 128), u32)
        gbase = NUNITS * MG * 4 + MG * 992
        for r in range(24):
            pool[gbase + r] = gm_ref[pl.ds(8 * r, 8), :]

        def g_view(zero):
            return jnp.concatenate([pool[gbase + r + (zero if r == TAP_OPQ else 0)] for r in range(24)], axis=0)

        z8 = jnp.zeros((8, 128), u32)
        for ct in range(2):
            xs[ct][pl.ds(0, 8), :] = z8
            for r in range(XPAD + T1, XPAD + XB, 8):
                xs[ct][pl.ds(r, 8), :] = z8
            for r in range(XPAD + XB + T1, XROWS, 8):
                xs[ct][pl.ds(r, 8), :] = z8

        def zero_zh(i, c):
            for h in range(2):
                for comp in range(2):
                    zh_ref[ZH - 1 - i, h, comp] = jnp.zeros((8, 256), f32)
            return c
        lax.fori_loop(0, ZH - 8 - L2, zero_zh, 0)

        zf = jnp.zeros((M, 128), f32)
        for m in range(0, 64, 4):
            y_ref[2 * m] = zf
            y_ref[2 * m + 1] = zf
        for g in range(MG):
            for h in range(2):
                for k1 in range(8):
                    for n2 in (1, 2, 3, 5, 6, 7):
                        for comp in range(2):
                            ti[g][h, (k1 * 8 + n2) * 2 + comp] = jnp.zeros((8, 128), f32)

        gg = g_ref[...].reshape(16, 256)
        ge_all = jnp.dot(gg, wg_ref[...], preferred_element_type=f32)
        ge_ref[...] = ge_all
        never = jnp.max(jnp.abs(ge_all)) < 0.0
        one = 1 - never.astype(i32)

        def transform(hook):
            def body(i, c):
                for j in range(WT_UNROLL):
                    hook(i * WT_UNROLL + j)
                pc = Pacer(i < 0, lax.shift_right_arithmetic(i, 20))
                seq = []
                for j in range(WT_UNROLL):
                    seq += weight_pieces(w_ref, UView(u1_ref), tf[j][0], tf[j][1], i * WT_UNROLL + j, pc)
                n = 4 * WT_UNROLL
                run_step(tap_stream(g_view, ws, u2_ref, n * i, n, pc), [q[0] for q in seq],
                         [q[1] for q in seq], pc, n * 192, LEAD, nunits=n)
                return c
            lax.fori_loop(0, 16 // WT_UNROLL, body, 0)

        def w1_hook(rg):
            for q in range(len(W1PART) - 1):
                @pl.when(rg * 8 == W1PART[q])
                def _(q=q):
                    w1_copy(q).wait()
                    if q < len(W2PART) - 1:
                        w2_wait(q)
                    if q == 0:
                        for cp in w2_copies(2):
                            cp.start()
                    if q + 3 < len(W1PART) - 1:
                        w1_copy(q + 3).start()
                    if q >= 2:
                        for cp in x_copies(q - 2):
                            cp.start()

        P = functools.partial

        def f1(ld, pc):
            return [(P(fwd_p1, ld[g], tf[g][ct], h, n2, ct, pc), COST_F1[n2])
                    for g in range(len(ld)) for ct in range(2) for h in range(2) for n2 in range(8)]

        def f2(cls, pc, mg=MG):
            return [(P(fwd_p2, tf[g][ct], x_ref, g, ct, k1, pc), COST_F2)
                    for g in range(mg) for ct in range(2) for k1 in cls]

        def i1(cls, pc, mg=MG):
            return [(P(inv_p1, y_ref, ti[g], g, h, n2, pc), COST_I1[n2])
                    for g in range(mg) for h in range(2) for n2 in cls]

        def i2(act, pairs_in_time, outs, pc):
            out = []
            for g, o in enumerate(outs):
                out += inverse_tail(ti[g], tr[g], P(act, tr[g], o), pc, pairs_in_time)
            return out

        def step(pc, u_view, mg, loads, act, pairs_in_time, outs):
            nxt = f1(loads, pc)
            half = len(nxt) // 2
            seq = (f2(CLASSES[1], pc, mg) + f2(CLASSES[2], pc, mg) + f2(CLASSES[3], pc, mg)
                   + i1(CLASSES[3], pc, len(outs)) + i2(act, pairs_in_time, outs, pc)
                   + nxt[:half] + i1(CLASSES[0], pc, mg) + nxt[half:]
                   + i1(CLASSES[1], pc, mg) + f2(CLASSES[0], pc, len(loads)) + i1(CLASSES[2], pc, mg))
            run_step(matmul_stream(x_ref, u_view, y_ref, pc, None if mg == MG else mg),
                     [q[0] for q in seq], [q[1] for q in seq], pc, NUNITS * 4 * mg, LEAD)

        def pacer(c):
            return Pacer(c < 0, lax.shift_right_arithmetic(c, 20))

        idle = Pacer(None)
        u1, u2 = UView(u1_ref), UView(u2_ref)

        def x_wait(part):
            rows = sum(4 * (hi - lo) for e in range(SEG) for lo, hi in x_rows(e, part))
            buf = xs0.at[pl.ds(0, rows), :]
            pltpu.make_async_copy(buf, buf, sem_x.at[part % 3]).wait()

        def load1(blk):
            base = blk * S

            def load(h, n, ct, pc):
                w = xs[ct][pl.ds(base + n + h * L1, 8, stride=2 * L1), :]
                if pc is not None:
                    w = pc.here(w)
                return _unpack(w)
            return load

        def load2(blk):
            def load(h, n, ct, pc):
                lo = zh_ref[blk * S + n, h, 0, :, _lanes(ct)]
                hi = zh_ref[blk * S + n, h, 1, :, _lanes(ct)]
                if pc is not None:
                    lo = pc.here(lo)
                return lo, hi
            return load

        def act1(rb, tau0, q, pc):
            return act_conv1(rb, zh_ref, tau0, q, pc)

        def act2(rb, tau0, q, pc):
            return act_conv2(rb, f_ref, tau0, q, pc)

        def loads1(chunk):
            return [load1(chunk * MG + g) for g in range(MG)]

        def loads2(chunk):
            return [load2(jnp.minimum(chunk * MG + g, NB2 - 1)) for g in range(MG)]

        def outs1(chunk):
            return [8 + (chunk * MG + g) * (S // 2) for g in range(MG)]

        def outs2(chunk, n=MG):
            return [(chunk * MG + g) * S for g in range(n)]

        with scope("wt1"):
            transform(w1_hook)

        x_wait(0)
        for cp in x_copies(3):
            cp.start()
        with scope("pro"):
            for piece, _ in f1(loads1(NC1 - 1), idle) + f2(CLASSES[0], idle):
                piece()

        def conv1_step(c, cc):
            for part, first in X_NEEDED:
                @pl.when(c == first)
                def _(part=part):
                    x_wait(part)
            prev = jnp.where(c == 1, NC1 - 1, c - 2)
            outs = [jnp.where(c >= 1, o, ZDUMP) for o in outs1(prev)]
            step(pacer(c), u1, MG, loads1(c), act1, True, outs)
            return cc
        with scope("steps"):
            lax.fori_loop(0, NC1 - 1, conv1_step, 0)

        row = lax.broadcasted_iota(i32, (8, 256), 0)
        for h in range(2):
            for comp in range(2):
                for t in range(last_valid, NB1 * S // 2):
                    zh_ref[8 + t, h, comp] = jnp.where(row == SEG - 1, 0.0, zh_ref[8 + t, h, comp])
                for j in range(8):
                    v = pltpu.roll(zh_ref[8 + L2 - 8 + j, h, comp], 1, axis=0)
                    zh_ref[j, h, comp] = jnp.where(row == 0, 0.0, v)
                for j in range(8):
                    v = pltpu.roll(zh_ref[8 + j, h, comp], SEG - 1, axis=0)
                    zh_ref[8 + L2 + j, h, comp] = jnp.where(row == SEG - 1, 0.0, v)

        def hand_over_1(c, cc):
            step(pacer(c), u1, MG, loads2(0), act1, True, outs1(NC1 - 3))
            return cc

        def hand_over_2(c, cc):
            step(pacer(c), u2, MG, loads2(1), act1, True, outs1(NC1 - 2))
            return cc
        with scope("steps"):
            lax.fori_loop(0, one, hand_over_1, 0)
            lax.fori_loop(0, one, hand_over_2, 0)

        def conv2_step(c, cc):
            step(pacer(c), u2, MG, loads2(c + 1), act2, False, outs2(c - 1))
            return cc
        tail = NB2 - (NC2 - 1) * MG

        def last_step(c, cc):
            step(pacer(c), u2, tail, [], act2, False, outs2(NC2 - 2))
            return cc
        with scope("steps"):
            lax.fori_loop(1, NC2 - 1, conv2_step, 0)
            lax.fori_loop(0, one, last_step, 0)
        with scope("epi"):
            for piece, _ in i1(CLASSES[3], idle, tail) + i2(act2, False, outs2(NC2 - 1, tail), idle):
                piece()

        order = [(b, e) for b in range(2) for e in range(SEG)]

        def out_copy(half, q, t0, nvalid):
            b, e = order[q]
            r0 = (b * T2 + e * L2) * 8 + t0 * 8
            return pltpu.make_async_copy(st_ref.at[half, q, pl.ds(0, nvalid * 8), :],
                                         o_hbm.at[pl.ds(r0, nvalid * 8), :],
                                         sem_o.at[half])

        def width(e):
            lim = L2 if e < SEG - 1 else last_valid
            return lim - (NCH - 1) * TB

        def joint_chunk(ch, half, full, never):
            pc = Pacer(never)
            t0 = ch * TB
            fl = pltpu.bitcast(f_ref[pl.ds(t0, TB)].reshape(TB * 8, 256), bf16)
            fe = jnp.dot(fl, wf_ref[...], preferred_element_type=f32)
            fe_ref[...] = fe
            prev = [fe[8 * r:8 * r + 8, 128 * n:128 * n + 128] for n in range(2) for r in range(2 * TB)]
            prev = prev[len(prev) // 2:]
            for q, (b, e) in enumerate(order):
                ge = ge_ref[pl.ds(8 * b, 8), :]
                r = 4 * (e & 3) + 2 * b + (e >> 2)
                js = []
                for t in range(TB):
                    row = jnp.broadcast_to(fe_ref[pl.ds(16 * t + r, 1), :], (8, 256))
                    tok = prev[(t * len(prev)) // TB]
                    gt = jnp.concatenate([pc.tie(ge[:, :128], tok), pc.tie(ge[:, 128:], tok)], axis=1)
                    js.append(jnp.tanh(row + gt))
                jl = jnp.concatenate(js, axis=0).astype(bf16)
                y = jnp.dot(jl, wo_ref[...], preferred_element_type=f32)
                prev = [y[8 * rr:8 * rr + 8, 128 * n:128 * n + 128] for n in range(2) for rr in range(TB)]
                st_ref[half, q] = y.astype(bf16)
                out_copy(half, q, t0, TB if full else width(e)).start()

        def wait_chunk(half, full):
            if full:
                pltpu.make_async_copy(st_ref.at[half], st_ref.at[half], sem_o.at[half]).wait()
                return
            for q, (b, e) in enumerate(order):
                out_copy(half, q, 0, width(e)).wait()

        def joint_body(ch, c):
            half = ch % 2

            @pl.when(ch >= 2)
            def _():
                wait_chunk(half, True)
            joint_chunk(ch, half, True, ch < 0)
            return c
        with scope("joint"):
            lax.fori_loop(0, NCH - 1, joint_body, 0)
            last_half = (NCH - 1) % 2
            wait_chunk(last_half, True)
            joint_chunk(NCH - 1, last_half, False, never)
            wait_chunk(1 - last_half, True)
            wait_chunk(last_half, False)

    scratch = [
        pltpu.VMEM((XROWS, 128), u32), pltpu.VMEM((XROWS, 128), u32),
        pltpu.VMEM((31, 128, 256), u32),
        pltpu.VMEM((32 * WP + 8, 128), u32), pltpu.VMEM((32 * WP + 8, 128), u32),
        pltpu.VMEM((2 * 96 * UP, 128), u32), pltpu.VMEM((2 * 96 * UP, 128), u32),
        pltpu.VMEM((NUNITS * MG * 4 + MG * 992 + 24, 8, 128), u32),
        pltpu.VMEM((128, M, 128), f32),
        pltpu.VMEM((ZH + S // 2, 2, 2, 8, 256), f32),
        pltpu.VMEM((FROWS + S, 8, 256), u32),
        pltpu.VMEM((TB * 16, 256), f32),
        pltpu.VMEM((16, 256), f32),
        pltpu.VMEM((2, 2 * SEG, TB * 8, 256), bf16),
        pltpu.SemaphoreType.DMA((6,)),
        pltpu.SemaphoreType.DMA((3,)),
        pltpu.SemaphoreType.DMA((2,)),
    ]
    return kernel, scratch


TAP_MATRIX = _tap_matrix()
WT_UNROLL = 2
TAP_OPQ = 23
TAP_GATE = 20
LEAD = 0
LAG = 0
AHEAD = 2
OPQ_EVERY = 1
DUE = 0
DUE_EVERY = 1000


def _call(x, w1, w2, g, w_f, w_g, w_o, interpret=False):
    B, T, D = x.shape
    kernel, scratch = _make_kernel(T)
    T2 = T // 4
    any_spec = pl.BlockSpec(memory_space=pl.ANY)
    vmem = pl.BlockSpec(memory_space=pltpu.VMEM)
    out = pl.pallas_call(
        kernel,
        out_shape=jax.ShapeDtypeStruct((B * T2 * 8, D), bf16),
        in_specs=[any_spec, any_spec, any_spec, vmem, vmem, vmem, vmem, vmem],
        out_specs=any_spec,
        scratch_shapes=scratch,
        compiler_params=pltpu.CompilerParams(vmem_limit_bytes=127 * 2**20),
        interpret=interpret,
        name="conv_stem_rnnt_joint",
    )(x, w1, w2, g, w_f, w_g, w_o, TAP_MATRIX)
    return out.reshape(B, T2, 8, D)


@jax.jit
def pallas_standalone__seq2seq_rnn_t_joint__speech_kernel(x, w1, w2, g, w_f, w_g, w_o):
    return _call(x, w1, w2, g, w_f, w_g, w_o)
```

```python
import functools
import math

import jax
import jax.numpy as jnp
import numpy as np
from jax import lax
from jax.experimental import pallas as pl
from jax.experimental.pallas import tpu as pltpu

f32, u32, bf16, i32 = jnp.float32, jnp.uint32, jnp.bfloat16, jnp.int32

PROFILE_SCOPES = False


class _NoScope:
    def __enter__(self):
        return self

    def __exit__(self, *a):
        return False


def scope(name):
    return jax.named_scope(name) if PROFILE_SCOPES else _NoScope()

N = 64
S = 48
SEG = 8


class V:
    __slots__ = ("a", "s")

    def __init__(self, a, s=1):
        self.a = a
        self.s = s

    def __neg__(self):
        return V(self.a, -self.s)

    def __add__(self, o):
        if self.s == o.s:
            return V(self.a + o.a, self.s)
        if self.s > 0:
            return V(self.a - o.a, 1)
        return V(o.a - self.a, 1)

    def __sub__(self, o):
        return self + (-o)

    def scale(self, c):
        if c == 1.0:
            return self
        if c == -1.0:
            return -self
        return V(self.a * np.float32(abs(c)), self.s * (1 if c > 0 else -1))

    def times(self, c):
        return self.a * np.float32(self.s * c)

    def signed(self, s):
        return self.a if self.s * s > 0 else -self.a


class C:
    __slots__ = ("r", "i")

    def __init__(self, r, i):
        self.r = r
        self.i = i

    def __add__(self, o):
        return C(self.r + o.r, self.i + o.i)

    def __sub__(self, o):
        return C(self.r - o.r, self.i - o.i)

    def __neg__(self):
        return C(-self.r, -self.i)

    def mul_w(self, num, den):
        num %= den
        if num == 0:
            return self
        if 4 * num == den:
            return C(-self.i, self.r)
        if 2 * num == den:
            return -self
        if 4 * num == 3 * den:
            return C(self.i, -self.r)
        if (8 * num) % den == 0:
            o = (8 * num) // den
            h = math.sqrt(0.5)
            sc = 1 if o in (1, 7) else -1
            ss = 1 if o in (1, 3) else -1
            r, m = self.r, self.i
            re = (r if sc > 0 else -r) - (m if ss > 0 else -m)
            im = (r if ss > 0 else -r) + (m if sc > 0 else -m)
            return C(re.scale(h), im.scale(h))
        c = math.cos(2 * math.pi * num / den)
        s = math.sin(2 * math.pi * num / den)
        return C(self.r.scale(c) - self.i.scale(s), self.r.scale(s) + self.i.scale(c))


def _add(a, b):
    if a is None:
        return b
    if b is None:
        return a
    return a + b


def _sub(a, b):
    if b is None:
        return a
    if a is None:
        return -b
    return a - b


def fft8(x, sgn, need=tuple(range(8))):
    def rot(a, num, den):
        return None if a is None else a.mul_w(sgn * num, den)

    need = set(need)
    a0, a1 = _add(x[0], x[4]), _sub(x[0], x[4])
    a2, a3 = _add(x[2], x[6]), rot(_sub(x[2], x[6]), 1, 4)
    a4, a5 = _add(x[1], x[5]), _sub(x[1], x[5])
    a6, a7 = _add(x[3], x[7]), rot(_sub(x[3], x[7]), 1, 4)
    out = {}
    if need & {0, 4}:
        b0, b4 = _add(a0, a2), _add(a4, a6)
        if 0 in need:
            out[0] = _add(b0, b4)
        if 4 in need:
            out[4] = _sub(b0, b4)
    if need & {2, 6}:
        b2, b6 = _sub(a0, a2), rot(_sub(a4, a6), 1, 4)
        if 2 in need:
            out[2] = _add(b2, b6)
        if 6 in need:
            out[6] = _sub(b2, b6)
    if need & {1, 5}:
        b1, b5 = _add(a1, a3), rot(_add(a5, a7), 1, 8)
        if 1 in need:
            out[1] = _add(b1, b5)
        if 5 in need:
            out[5] = _sub(b1, b5)
    if need & {3, 7}:
        b3, b7 = _sub(a1, a3), rot(_sub(a5, a7), 3, 8)
        if 3 in need:
            out[3] = _add(b3, b7)
        if 7 in need:
            out[7] = _sub(b3, b7)
    return out


class _Sym:
    def __add__(self, o):
        return self

    __sub__ = __mul__ = __add__

    def __neg__(self):
        return self


def _fft64_signs(sgn, present=tuple(range(64)), in_sign=None):
    d = _Sym()
    in_sign = in_sign or {}
    x = [C(V(d, in_sign.get((n, 0), 1)), V(d, in_sign.get((n, 1), 1))) if n in present else None
         for n in range(64)]
    t = {}
    for n2 in range(8):
        a = fft8([x[8 * n1 + n2] for n1 in range(8)], sgn)
        for k1 in range(8):
            t[k1, n2] = a[k1].mul_w(sgn * n2 * k1, 64)
    s1 = {key: (v.r.s, v.i.s) for key, v in t.items()}
    s2 = {}
    for k1 in range(8):
        b = fft8([t[k1, n2] for n2 in range(8)], sgn)
        for k2 in range(8):
            s2[k1 + 8 * k2] = b[k2]
    return s1, s2


def _unit(k, j):
    return (k - 1) * 3 + j


UNIT0, UNIT32 = 93, 94
NUNITS = 95


def _lhs_forms(m, z):
    if m in (0, 32):
        u = UNIT0 if m == 0 else UNIT32
        return [(u, 0, z.r), (u, 1, z.i)]
    if m < 32:
        return [(_unit(m, 0), 0, z.r + z.i), (_unit(m, 1), 0, z.r), (_unit(m, 2), 0, z.i)]
    k = 64 - m
    return [(_unit(k, 0), 1, z.r - z.i), (_unit(k, 1), 1, z.r), (_unit(k, 2), 1, z.i)]


def _lhs_signs():
    _, s2 = _fft64_signs(-1)
    sg = {}
    for m in range(64):
        for u, h, v in _lhs_forms(m, s2[m]):
            sg[u, h] = v.s
    return sg


LHS_SIGN = _lhs_signs()


def _weight_forms(m, pm):
    if m < 32:
        nt = 0 if pm > 0 else 1
        return [(_unit(m, 0), 1, nt, (1, 0)), (_unit(m, 1), 1, nt, (-1, 1)), (_unit(m, 2), 1, nt, (-1, -1))]
    k = 64 - m
    nt = 1 if pm > 0 else 0
    return [(_unit(k, 0), 0, nt, (1, 0)), (_unit(k, 1), 0, nt, (-1, -1)), (_unit(k, 2), 0, nt, (1, -1))]


def _weight_plan():
    s1, s2 = _fft64_signs(1, present=range(16))
    forms = {}
    for pm in (1, -1):
        for m in range(1, 64):
            if m == 32:
                continue
            for u, half, nt, (cr, ci) in _weight_forms(m, pm):
                forms[u, half, nt] = (cr * s2[m].r.s, ci * s2[m].i.s)
    col = {}
    for u in range(93):
        for nt in range(2):
            def negs(sig):
                n = 0
                for half in range(2):
                    cr, ci = forms[u, half, nt]
                    w = sig * LHS_SIGN[u, half]
                    n += (w * cr <= 0 and w * ci <= 0)
                return n
            col[u, nt] = 1 if negs(1) <= negs(-1) else -1
    for u in (UNIT0, UNIT32):
        col[u, 0] = col[u, 1] = 1
    return s1, s2, col


WT_S1, WT_S2, COL_SIGN = _weight_plan()


def _recombine(k1, k2, k3, k):
    out = {}
    for nt in range(2):
        yr = k1[nt] - k3[nt]
        yi = k1[nt] + k2[nt]
        if nt == 0:
            out[k, 0], out[k, 1] = yr, yi
        else:
            out[64 - k, 0], out[64 - k, 1] = yr, -yi
    return out


def _y_signs():
    d = _Sym()
    sg = {}
    for k in range(1, 32):
        ks = [[V(d, COL_SIGN[_unit(k, j), nt]) for nt in range(2)] for j in range(3)]
        for key, v in _recombine(ks[0], ks[1], ks[2], k).items():
            sg[key] = v.s
    for m, u in ((0, UNIT0), (32, UNIT32)):
        sg[m, 0], sg[m, 1] = COL_SIGN[u, 0], COL_SIGN[u, 1]
    return sg


Y_SIGN = _y_signs()


def _unpack(w):
    lo = pltpu.unpack_elementwise(w, index=0, packed_dtype=bf16, unpacked_dtype=f32)
    hi = pltpu.unpack_elementwise(w, index=1, packed_dtype=bf16, unpacked_dtype=f32)
    return lo, hi


def _pack(lo, hi):
    return pltpu.pack_elementwise([lo, hi], packed_dtype=bf16)


_GC1 = 2.0 * math.sqrt(2.0 / math.pi)
_GC2 = 8.0 * 0.044715 * math.sqrt(2.0 / math.pi)


def _gelu_half(v):
    a = v.a
    p = (a * a) * np.float32(_GC2) + np.float32(_GC1)
    t = jnp.tanh(p * a)
    return a * t + a if v.s > 0 else a * t - a


def _lanes(t):
    return pl.ds(128 * t, 128)


class Pacer:
    def __init__(self, never, zero=None):
        self.never = never
        self.tok = None
        self.outs = []
        self.zero = zero
        self.pending = []
        self.unit = 0

    def gate(self, a, first=0):
        vals = [v for q, v in self.pending if q <= self.unit]
        self.pending = [(q, v) for q, v in self.pending if q > self.unit]
        self.unit += 1
        if not vals:
            return a
        m, k = a.shape
        tiles = [[a[8 * r:8 * r + 8, 128 * c:128 * c + 128] for c in range(k // 128)] for r in range(m // 8)]
        flat = [(r, c) for r in range(first, m // 8) for c in range(k // 128)]
        for i, v in enumerate(vals):
            r, c = flat[i % len(flat)]
            tiles[r][c] = self.tie(tiles[r][c], v)
        return jnp.concatenate([jnp.concatenate(row, axis=1) for row in tiles], axis=0)

    def here(self, x):
        tok, self.tok = self.tok, None
        return self.tie(x, tok)

    def due(self, x):
        if self.never is not None:
            self.outs.append(x)
        return x

    def tie(self, x, tok):
        if tok is None:
            return x
        if tok.dtype != x.dtype:
            tok = pltpu.bitcast(tok, x.dtype)
        return jnp.where(self.never, tok, x)


def _combo(f, cr, ci, want):
    if ci == 0:
        return f.r.signed(want * cr)
    v = (f.r if cr > 0 else -f.r) + (f.i if ci > 0 else -f.i)
    if v.s * want > 0:
        return v.a
    if f.r.s * cr != f.i.s * ci:
        return ((-f.r) if cr > 0 else f.r).__add__((-f.i) if ci > 0 else f.i).a
    return -v.a


UP = 260
WP = 132


class UView:
    def __init__(self, ref):
        self.ref = ref

    def load(self, u):
        return jnp.concatenate([self.ref[pl.ds((nt * 96 + u) * UP, 256), :] for nt in range(2)], axis=1)

    def store(self, u, half, nt, rg, val):
        self.ref[pl.ds((nt * 96 + u) * UP + half * 128 + rg * 8, 8), :] = val


def _tap_matrix():
    import ml_dtypes
    sigma, tau = 1.0 / 256.0, 1.0 / 128.0
    g = np.zeros((2, 2, 96, 32, 2))
    d = np.arange(16)
    for tap in range(31):
        for dt in range(2):
            wa = np.zeros((16, 2))
            wb = np.zeros((16, 2))
            if tap % 2:
                wa[(tap + 1) // 2, dt] = 1.0
            else:
                wb[tap // 2, dt] = 1.0
            z0 = wa[:, 0] + 1j * wb[:, 0]
            z1 = wa[:, 1] + 1j * wb[:, 1]
            for pm, z in ((1, z0 + 1j * z1), (-1, z0 - 1j * z1)):
                for m in range(1, 64):
                    if m == 32:
                        continue
                    f = sigma * np.sum(z * np.exp(2j * np.pi * m * d / 64))
                    for u, half, nt, (cr, ci) in _weight_forms(m, pm):
                        g[nt, half, u, tap, dt] = (LHS_SIGN[u, half] * COL_SIGN[u, nt]
                                                   * (cr * f.real + ci * f.imag))
            for m, u in ((0, UNIT0), (32, UNIT32)):
                e = np.cos(np.pi * m * d / 32)
                for half, wv in enumerate((wa, wb)):
                    g[dt, half, u, tap, dt] = (LHS_SIGN[u, half] * COL_SIGN[u, dt]
                                               * tau * np.sum(e * wv[:, dt]))
    g = g.reshape(384, 32, 2)
    mat = np.zeros((384, 128))
    for v in range(4):
        dt, t0 = v // 2, 16 * (v % 2)
        for s_ in range(8):
            for par in range(2):
                mat[:, 16 * v + 2 * s_ + par] = g[:, t0 + 8 * par + s_, dt]
    hi = mat.astype(ml_dtypes.bfloat16)
    lo = (mat - hi.astype(np.float64)).astype(ml_dtypes.bfloat16)
    full = np.concatenate([hi[:, :64], lo[:, :64]], axis=1).view(np.uint16).astype(np.uint32)
    return full[0::2] | (full[1::2] << 16)


def tap_operand(ws, cpair):
    ev, od = [], []
    for dt in range(2):
        for t0 in (0, 16):
            wa = ws[dt][pl.ds(t0 * WP + cpair, 8, stride=WP), :]
            wb = ws[dt][pl.ds((t0 + 8) * WP + cpair, 8, stride=WP), :]
            alo, ahi = _unpack(wa)
            blo, bhi = _unpack(wb)
            ev.append(_pack(alo, blo))
            od.append(_pack(ahi, bhi))
    return jnp.concatenate(ev + ev, axis=0), jnp.concatenate(od + od, axis=0)


def tap_stream(g_view, ws, u2_ref, it0, n, pc):
    for q in range(n):
        it = it0 + q
        lhs = pltpu.bitcast(pc.gate(g_view(pc.zero), TAP_GATE), bf16)
        ops = []
        for j in range(2):
            ops += list(tap_operand(ws, 2 * it + j))
        rhs = pltpu.bitcast(jnp.concatenate(ops, axis=1), bf16)
        y = jnp.dot(lhs, rhs, preferred_element_type=f32)
        for r in range(48):
            nt, half, u0 = r // 24, (r // 12) % 2, (r % 12) * 8
            for j in range(2):
                val = _pack(y[8 * r:8 * r + 8, 256 * j:256 * j + 128],
                            y[8 * r:8 * r + 8, 256 * j + 128:256 * j + 256])
                u2_ref[pl.ds((nt * 96 + u0) * UP + half * 128 + 2 * it + j, 8, stride=UP), :] = val
        yield [y[8 * r:8 * r + 8, 128 * t:128 * t + 128] for r in range(48) for t in range(4)]


def weight_pieces(w_ref, u_ref, t_ref, z_ref, rg, pc):
    rows = pl.ds(pl.multiple_of(rg * 8, 8), 8)
    sigma = 1.0 / 256.0
    tau = 1.0 / 128.0
    acc = {}

    def store(u, half, nt, a0, a1):
        u_ref.store(u, half, nt, rg, pc.due(_pack(a0, a1)))

    def prep(d):
        wa = [[None, None], [None, None]]
        wb = [[None, None], [None, None]]
        for dt in range(2):
            w = w_ref[2 * d, rows, _lanes(dt)]
            if dt == 0:
                w = pc.here(w)
            lo, hi = _unpack(w)
            wb[0][dt], wb[1][dt] = V(lo), V(hi)
            if d > 0:
                lo, hi = _unpack(w_ref[2 * d - 1, rows, _lanes(dt)])
                wa[0][dt], wa[1][dt] = V(lo), V(hi)
        for p in range(2):
            for dt in range(2):
                for name, val in (("a", wa[p][dt]), ("b", wb[p][dt])):
                    key = (p, dt, name, d % 2)
                    acc[key] = _add(acc.get(key), val)
            zp = (_sub(wa[p][0], wb[p][1]), _add(wb[p][0], wa[p][1]))
            zm = (_add(wa[p][0], wb[p][1]), _sub(wb[p][0], wa[p][1]))
            for j, z in enumerate((zp, zm)):
                for comp in range(2):
                    z_ref[j, (p * 16 + d) * 2 + comp] = z[comp].times(sigma)

    def real_bins():
        for m, u in ((0, UNIT0), (32, UNIT32)):
            for dt in range(2):
                for half, name in enumerate(("a", "b")):
                    vals = []
                    for p in range(2):
                        ev, od = acc[p, dt, name, 0], acc[p, dt, name, 1]
                        v = _add(ev, od) if m == 0 else _sub(ev, od)
                        vals.append(v.times(tau * LHS_SIGN[u, half] * COL_SIGN[u, dt]))
                    store(u, half, dt, vals[0], vals[1])

    def pass1(j, p, n2):
        z = [C(V(z_ref[j, (p * 16 + d) * 2]), V(z_ref[j, (p * 16 + d) * 2 + 1])) for d in (n2, n2 + 8)]
        z[0].r.a = pc.here(z[0].r.a)
        a = fft8(z + [None] * 6, 1)
        for k1 in range(8):
            t = a[k1].mul_w(n2 * k1, 64)
            assert (t.r.s, t.i.s) == WT_S1[k1, n2]
            t_ref[p, (k1 * 8 + n2) * 2] = t.r.a
            t_ref[p, (k1 * 8 + n2) * 2 + 1] = t.i.a

    def pass2(pm, k1):
        need = [k2 for k2 in range(8) if (k1 + 8 * k2) not in (0, 32)]
        outs = []
        for p in range(2):
            xs = [C(V(t_ref[p, (k1 * 8 + n2) * 2], WT_S1[k1, n2][0]),
                    V(t_ref[p, (k1 * 8 + n2) * 2 + 1], WT_S1[k1, n2][1])) for n2 in range(8)]
            if p == 0:
                xs[0].r.a = pc.here(xs[0].r.a)
            outs.append(fft8(xs, 1, need))
        for k2 in need:
            m = k1 + 8 * k2
            for u, half, nt, (cr, ci) in _weight_forms(m, pm):
                want = LHS_SIGN[u, half] * COL_SIGN[u, nt]
                store(u, half, nt, _combo(outs[0][k2], cr, ci, want), _combo(outs[1][k2], cr, ci, want))

    P = functools.partial
    out = [(P(prep, d), 40) for d in range(16)] + [(real_bins, 40)]
    for j, pm in enumerate((1, -1)):
        out += [(P(pass1, j, p, n2), 21 + _TW[n2]) for p in range(2) for n2 in range(8)]
        out += [(P(pass2, pm, k1), 193) for k1 in range(8)]
    return out


class View:
    def __init__(self, pool, base):
        self.pool = pool
        self.base = base

    def __getitem__(self, idx):
        h, i = idx
        return pltpu.bitcast(self.pool[self.base + h * 128 + i], f32)

    def __setitem__(self, idx, val):
        h, i = idx
        self.pool[self.base + h * 128 + i] = pltpu.bitcast(val, u32)


class XView:
    def __init__(self, pool, base, mg):
        self.pool, self.base, self.mg = pool, base, mg

    def index(self, u, g, c):
        return self.base + (u * self.mg + g) * 4 + c

    def store(self, u, g, c, val):
        self.pool[self.index(u, g, c)] = val

    def load(self, u, zero=None, mg=None):
        rows = []
        for g in range(self.mg if mg is None else mg):
            row = []
            for c in range(4):
                idx = self.index(u, g, c)
                if zero is not None and g == 0 and c == 0:
                    idx = idx + zero
                row.append(self.pool[idx])
            rows.append(jnp.concatenate(row, axis=1))
        return jnp.concatenate(rows, axis=0)


_TW = (0, 42, 40, 42, 32, 42, 40, 42)
COST_F1 = tuple(73 + t for t in _TW)
COST_I1 = tuple(57 + t for t in _TW)
COST_F2, COST_I2, COST_ACT = 153, 53, 85
FWD_S1, _ = _fft64_signs(-1)
INV_S1, _INV_OUT = _fft64_signs(1, in_sign=Y_SIGN)
INV_S2 = {m: (v.r.s, v.i.s) for m, v in _INV_OUT.items()}
CLASSES = ((1, 7), (2, 6), (3, 5), (4, 0))


def _class_units(cls):
    ks = [k for k in range(1, 32) if k % 8 in cls or (-k) % 8 in cls]
    ks.sort(key=lambda k: (0 if k % 8 == cls[0] else 1, k))
    out = [("pair", k) for k in ks]
    if 0 in cls:
        out += [("real", 0), ("real", 32)]
    return out


def fwd_p1(load, t_ref, h, n2, ct, pc):
    xs = []
    for n1 in range(8):
        lo, hi = load(h, 8 * n1 + n2, ct, pc if n1 == 0 else None)
        xs.append(C(V(lo), V(hi)))
    a = fft8(xs, -1)
    for k1 in range(8):
        t = a[k1].mul_w(-n2 * k1, 64)
        assert (t.r.s, t.i.s) == FWD_S1[k1, n2]
        t_ref[h, (k1 * 8 + n2) * 2] = t.r.a
        t_ref[h, (k1 * 8 + n2) * 2 + 1] = t.i.a


def fwd_p2(t_ref, x_ref, g, ct, k1, pc):
    outs = []
    for h in range(2):
        xs = [C(V(t_ref[h, (k1 * 8 + n2) * 2], FWD_S1[k1, n2][0]),
                V(t_ref[h, (k1 * 8 + n2) * 2 + 1], FWD_S1[k1, n2][1])) for n2 in range(8)]
        if h == 0:
            xs[0].r.a = pc.here(xs[0].r.a)
        outs.append(fft8(xs, -1))
    for k2 in range(8):
        m = k1 + 8 * k2
        f0 = _lhs_forms(m, outs[0][k2])
        f1 = _lhs_forms(m, outs[1][k2])
        for i, ((u, half, v0), (_, _, v1)) in enumerate(zip(f0, f1)):
            assert v0.s == v1.s == LHS_SIGN[u, half]
            x_ref.store(u, g, 2 * half + ct, _pack(v0.a, v1.a))
    return COST_F2


def inv_p1(y_ref, t_ref, g, h, n2, pc):
    rows = pl.ds(g * 16 + 8 * h, 8)
    ysg = Y_SIGN
    xs = []
    for n1 in range(8):
        m = 8 * n1 + n2
        xs.append(C(V(y_ref[2 * m, rows, :], ysg.get((m, 0), 1)),
                    V(y_ref[2 * m + 1, rows, :], ysg.get((m, 1), 1))))
    xs[0].r.a = pc.here(xs[0].r.a)
    a = fft8(xs, 1)
    for k1 in range(8):
        t = a[k1].mul_w(n2 * k1, 64)
        assert (t.r.s, t.i.s) == INV_S1[k1, n2]
        t_ref[h, (k1 * 8 + n2) * 2] = t.r.a
        t_ref[h, (k1 * 8 + n2) * 2 + 1] = t.i.a


def inv_p2(t_ref, r_ref, h, k1, pc):
    xs = [C(V(t_ref[h, (k1 * 8 + n2) * 2], INV_S1[k1, n2][0]),
            V(t_ref[h, (k1 * 8 + n2) * 2 + 1], INV_S1[k1, n2][1])) for n2 in range(8)]
    xs[0].r.a = pc.here(xs[0].r.a)
    b = fft8(xs, 1, range(S // 8))
    for k2 in range(S // 8):
        assert (b[k2].r.s, b[k2].i.s) == INV_S2[k1 + 8 * k2]
        r_ref[h, (k1 * 6 + k2) * 2] = b[k2].r.a
        r_ref[h, (k1 * 6 + k2) * 2 + 1] = b[k2].i.a
    return COST_I2


def _act(r_ref, h, k1, k2, dt, first, pc):
    a = r_ref[h, (k1 * 6 + k2) * 2 + dt]
    if first:
        a = pc.here(a)
    return _gelu_half(V(a, INV_S2[k1 + 8 * k2][dt]))


def act_conv1(r_ref, zh_ref, tau0, q, pc):
    h, k1, part = q // 8, 2 * ((q % 8) // 2), q % 2
    first = True
    for k2 in range(3 * part, 3 * part + 3):
        for dt in range(2):
            ev = _act(r_ref, h, k1, k2, dt, first, pc)
            od = _act(r_ref, h, k1 + 1, k2, dt, False, pc)
            first = False
            zh_ref[tau0 + (k1 // 2 + 4 * k2), h, 0, :, _lanes(dt)] = pc.due(ev)
            zh_ref[tau0 + (k1 // 2 + 4 * k2), h, 1, :, _lanes(dt)] = pc.due(od)
    return COST_ACT


def act_conv2(r_ref, f_ref, tau0, q, pc):
    k1, part = q // 2, q % 2
    first = True
    for k2 in range(3 * part, 3 * part + 3):
        for dt in range(2):
            oa = _act(r_ref, 0, k1, k2, dt, first, pc)
            ob = _act(r_ref, 1, k1, k2, dt, False, pc)
            first = False
            f_ref[tau0 + (k1 + 8 * k2), :, _lanes(dt)] = pc.due(_pack(oa, ob))
    return COST_ACT


def inverse_tail(t_ref, r_ref, act, pc, pairs_in_time):
    P = functools.partial
    out = []
    if pairs_in_time:
        for h in range(2):
            for kp in range(4):
                out += [(P(inv_p2, t_ref, r_ref, h, 2 * kp + j, pc), COST_I2) for j in range(2)]
                out += [(P(act, h * 8 + kp * 2 + j, pc), COST_ACT) for j in range(2)]
    else:
        for k1 in range(8):
            out += [(P(inv_p2, t_ref, r_ref, h, k1, pc), COST_I2) for h in range(2)]
            out += [(P(act, k1 * 2 + j, pc), COST_ACT) for j in range(2)]
    return out


def _mm(x_ref, u_ref, j, pc=None, mg=None):
    opaque = pc is not None and pc.unit % OPQ_EVERY == 0
    a = x_ref.load(j, pc.zero if opaque else None, mg)
    if pc is not None:
        a = pc.gate(a)
    a = pltpu.bitcast(a, bf16)
    w = pltpu.bitcast(u_ref.load(j), bf16)
    return jnp.dot(a, w, preferred_element_type=f32)


def _tokens(y):
    m = y.shape[0]
    return [y[8 * r:8 * r + 8, 128 * n:128 * n + 128] for n in range(2) for r in range(m // 8)]


def matmul_stream(x_ref, u_ref, y_ref, pc=None, mg=None):
    def tiles(y, u):
        return [V(y[:, :128], COL_SIGN[u, 0]), V(y[:, 128:], COL_SIGN[u, 1])]

    if mg is not None:
        y_ref = y_ref.at[:, pl.ds(0, 16 * mg), :]
    for cls in CLASSES:
        for kind, k in _class_units(cls):
            if kind == "pair":
                j = (k - 1) * 3
                y1 = _mm(x_ref, u_ref, j, pc, mg)
                k1 = tiles(y1, j)
                yield _tokens(y1)
                y2 = _mm(x_ref, u_ref, j + 1, pc, mg)
                k2 = tiles(y2, j + 1)
                for nt, m in ((0, k), (1, 64 - k)):
                    yi = k1[nt] + k2[nt]
                    assert (yi.s if nt == 0 else -yi.s) == Y_SIGN[m, 1]
                    y_ref[2 * m + 1] = yi.a
                yield _tokens(y2)
                y3 = _mm(x_ref, u_ref, j + 2, pc, mg)
                k3 = tiles(y3, j + 2)
                for nt, m in ((0, k), (1, 64 - k)):
                    yr = k1[nt] - k3[nt]
                    assert yr.s == Y_SIGN[m, 0]
                    y_ref[2 * m] = yr.a
                yield _tokens(y3)
            else:
                y = _mm(x_ref, u_ref, UNIT0 if k == 0 else UNIT32, pc, mg)
                y_ref[2 * k] = y[:, :128]
                y_ref[2 * k + 1] = y[:, 128:]
                yield _tokens(y)


def run_step(mm, pieces, costs, pc, ntok, lead, due=None, nunits=NUNITS):
    total = float(sum(costs))
    tokens = []
    c = 0.0
    for piece, cost in zip(pieces, costs):
        pc.tok = None
        if c >= lead:
            want = min(int((c - lead) / (total - lead) * ntok), ntok - 1)
            ahead = min(want + (AHEAD * ntok) // max(nunits, NUNITS), ntok - 1)
            while ahead >= len(tokens):
                tokens += next(mm)
            pc.tok = tokens[want]
        pc.outs = []
        piece()
        for i, v in enumerate(pc.outs):
            q = pc.unit + (DUE if due is None else due) + i // 4
            if q < nunits:
                pc.pending.append((q, v))
        c += cost
    pc.tok = None
    for _ in mm:
        pass


def _make_kernel(T):
    T1, T2 = T // 2, T // 4
    L1 = (T1 + 16) // SEG
    L2 = L1 // 2
    assert L1 * SEG == T1 + 16 and L1 % 2 == 0
    NB1 = -(-L1 // S)
    NB2 = -(-L2 // S)
    XPAD = 8
    XB = T1 + 16
    XROWS = XPAD + 2 * XB + 64
    MG = 3
    M = 16 * MG
    NC1 = -(-NB1 // MG)
    NC2 = -(-NB2 // MG)
    ZH = (NB2 - 1) * S + N
    ZDUMP = ZH
    TB = 56
    NCH = -(-L2 // TB)
    FROWS = max(NB2 * S, NCH * TB)
    FDUMP = FROWS
    last_valid = T2 - (SEG - 1) * L2
    XCUT = (24, 304, 592, 848)
    X_NEEDED = ((1, 0), (2, 2), (3, 4))

    def x_rows(e, part):
        def cut(e, i):
            return min((L1 * e + XCUT[i]) // 8 * 8, T1)
        if part == 0:
            out = [(cut(e, 3), cut(e + 1, 0) if e + 1 < SEG else T1)]
            return out + ([(0, cut(0, 0))] if e == 0 else [])
        return [(cut(e, part - 1), cut(e, part))]

    def kernel(x_hbm, w1_hbm, w2_hbm, g_ref, wf_ref, wg_ref, wo_ref, gm_ref, o_hbm,
               xs0, xs1, w_ref, ws0, ws1, u1_ref, u2_ref, pool, y_ref, zh_ref, f_ref, fe_ref, ge_ref,
               st_ref, sem_w, sem_x, sem_o):
        xs = (xs0, xs1)
        x_ref = XView(pool, 0, MG)
        tf = [[View(pool, NUNITS * MG * 4 + (g * 2 + ct) * 256) for ct in range(2)] for g in range(MG)]
        ti = [View(pool, NUNITS * MG * 4 + MG * 512 + g * 256) for g in range(MG)]
        tr = [View(pool, NUNITS * MG * 4 + MG * 768 + g * 224) for g in range(MG)]
        xh = x_hbm.bitcast(u32)
        w1w = w1_hbm.bitcast(u32)
        w2w = w2_hbm.bitcast(u32)

        W1PART = (0, 16, 32, 64, 96, 128)
        W2PART = (0, 16, 32, 128)

        def w1_copy(q):
            rows = pl.ds(W1PART[q], W1PART[q + 1] - W1PART[q])
            return pltpu.make_async_copy(w1w.at[:, rows, :], w_ref.at[:, rows, :], sem_w.at[q % 4])

        ws = (ws0, ws1)

        def w2_copies(part):
            lo, n = W2PART[part], W2PART[part + 1] - W2PART[part]
            return [pltpu.make_async_copy(w2w.at[i, pl.ds(lo, n), _lanes(dt)],
                                          ws[dt].at[pl.ds(WP * i + lo, n), :], sem_w.at[4 + part % 2])
                    for i in range(31) for dt in range(2)]

        def w2_wait(part):
            buf = xs0.at[pl.ds(0, 62 * (W2PART[part + 1] - W2PART[part])), :]
            pltpu.make_async_copy(buf, buf, sem_w.at[4 + part % 2]).wait()

        def x_copies(part):
            cps = []
            for b in range(2):
                for e in range(SEG):
                    for lo, hi in x_rows(e, part):
                        for ct in range(2):
                            cps.append(pltpu.make_async_copy(
                                xh.at[b, pl.ds(lo, hi - lo), _lanes(ct)],
                                xs[ct].at[pl.ds(XPAD + b * XB + lo, hi - lo), :],
                                sem_x.at[part % 3]))
            return cps

        w1_copy(0).start()
        for cp in w2_copies(0):
            cp.start()
        w1_copy(1).start()
        for cp in w2_copies(1):
            cp.start()
        w1_copy(2).start()
        for dt in range(2):
            for r in range(31 * WP, 31 * WP + 128, 8):
                ws[dt][pl.ds(r, 8), :] = jnp.zeros((8, 128), u32)
        gbase = NUNITS * MG * 4 + MG * 992
        for r in range(24):
            pool[gbase + r] = gm_ref[pl.ds(8 * r, 8), :]

        def g_view(zero):
            return jnp.concatenate([pool[gbase + r + (zero if r == TAP_OPQ else 0)] for r in range(24)], axis=0)

        z8 = jnp.zeros((8, 128), u32)
        for ct in range(2):
            xs[ct][pl.ds(0, 8), :] = z8
            for r in range(XPAD + T1, XPAD + XB, 8):
                xs[ct][pl.ds(r, 8), :] = z8
            for r in range(XPAD + XB + T1, XROWS, 8):
                xs[ct][pl.ds(r, 8), :] = z8

        def zero_zh(i, c):
            for h in range(2):
                for comp in range(2):
                    zh_ref[ZH - 1 - i, h, comp] = jnp.zeros((8, 256), f32)
            return c
        lax.fori_loop(0, ZH - 8 - L2, zero_zh, 0)

        zf = jnp.zeros((M, 128), f32)
        for m in range(0, 64, 4):
            y_ref[2 * m] = zf
            y_ref[2 * m + 1] = zf
        for g in range(MG):
            for h in range(2):
                for k1 in range(8):
                    for n2 in (1, 2, 3, 5, 6, 7):
                        for comp in range(2):
                            ti[g][h, (k1 * 8 + n2) * 2 + comp] = jnp.zeros((8, 128), f32)

        gg = g_ref[...].reshape(16, 256)
        ge_all = jnp.dot(gg, wg_ref[...], preferred_element_type=f32)
        ge_ref[...] = ge_all
        never = jnp.max(jnp.abs(ge_all)) < 0.0
        one = 1 - never.astype(i32)

        def transform(hook):
            def body(i, c):
                for j in range(WT_UNROLL):
                    hook(i * WT_UNROLL + j)
                pc = Pacer(i < 0, lax.shift_right_arithmetic(i, 20))
                seq = []
                for j in range(WT_UNROLL):
                    seq += weight_pieces(w_ref, UView(u1_ref), tf[j][0], tf[j][1], i * WT_UNROLL + j, pc)
                n = 4 * WT_UNROLL
                run_step(tap_stream(g_view, ws, u2_ref, n * i, n, pc), [q[0] for q in seq],
                         [q[1] for q in seq], pc, n * 192, LEAD, due=TAP_DUE, nunits=n)
                return c
            lax.fori_loop(0, 16 // WT_UNROLL, body, 0)

        def w1_hook(rg):
            for q in range(len(W1PART) - 1):
                @pl.when(rg * 8 == W1PART[q])
                def _(q=q):
                    w1_copy(q).wait()
                    if q < len(W2PART) - 1:
                        w2_wait(q)
                    if q == 0:
                        for cp in w2_copies(2):
                            cp.start()
                    if q + 3 < len(W1PART) - 1:
                        w1_copy(q + 3).start()
                    if q >= 2:
                        for cp in x_copies(q - 2):
                            cp.start()

        P = functools.partial

        def f1(ld, pc):
            return [(P(fwd_p1, ld[g], tf[g][ct], h, n2, ct, pc), COST_F1[n2])
                    for g in range(len(ld)) for ct in range(2) for h in range(2) for n2 in range(8)]

        def f2(cls, pc, mg=MG):
            return [(P(fwd_p2, tf[g][ct], x_ref, g, ct, k1, pc), COST_F2)
                    for g in range(mg) for ct in range(2) for k1 in cls]

        def i1(cls, pc, mg=MG):
            return [(P(inv_p1, y_ref, ti[g], g, h, n2, pc), COST_I1[n2])
                    for g in range(mg) for h in range(2) for n2 in cls]

        def i2(act, pairs_in_time, outs, pc):
            out = []
            for g, o in enumerate(outs):
                out += inverse_tail(ti[g], tr[g], P(act, tr[g], o), pc, pairs_in_time)
            return out

        def step(pc, u_view, mg, loads, act, pairs_in_time, outs):
            nxt = f1(loads, pc)
            half = len(nxt) // 2
            seq = (f2(CLASSES[1], pc, mg) + f2(CLASSES[2], pc, mg) + f2(CLASSES[3], pc, mg)
                   + i1(CLASSES[3], pc, len(outs)) + i2(act, pairs_in_time, outs, pc)
                   + nxt[:half] + i1(CLASSES[0], pc, mg) + nxt[half:]
                   + i1(CLASSES[1], pc, mg) + f2(CLASSES[0], pc, len(loads)) + i1(CLASSES[2], pc, mg))
            run_step(matmul_stream(x_ref, u_view, y_ref, pc, None if mg == MG else mg),
                     [q[0] for q in seq], [q[1] for q in seq], pc, NUNITS * 4 * mg, LEAD)

        def pacer(c):
            return Pacer(c < 0, lax.shift_right_arithmetic(c, 20))

        idle = Pacer(None)
        u1, u2 = UView(u1_ref), UView(u2_ref)

        def x_wait(part):
            rows = sum(4 * (hi - lo) for e in range(SEG) for lo, hi in x_rows(e, part))
            buf = xs0.at[pl.ds(0, rows), :]
            pltpu.make_async_copy(buf, buf, sem_x.at[part % 3]).wait()

        def load1(blk):
            base = blk * S

            def load(h, n, ct, pc):
                w = xs[ct][pl.ds(base + n + h * L1, 8, stride=2 * L1), :]
                if pc is not None:
                    w = pc.here(w)
                return _unpack(w)
            return load

        def load2(blk):
            def load(h, n, ct, pc):
                lo = zh_ref[blk * S + n, h, 0, :, _lanes(ct)]
                hi = zh_ref[blk * S + n, h, 1, :, _lanes(ct)]
                if pc is not None:
                    lo = pc.here(lo)
                return lo, hi
            return load

        def act1(rb, tau0, q, pc):
            return act_conv1(rb, zh_ref, tau0, q, pc)

        def act2(rb, tau0, q, pc):
            return act_conv2(rb, f_ref, tau0, q, pc)

        def loads1(chunk):
            return [load1(chunk * MG + g) for g in range(MG)]

        def loads2(chunk):
            return [load2(jnp.minimum(chunk * MG + g, NB2 - 1)) for g in range(MG)]

        def outs1(chunk):
            return [8 + (chunk * MG + g) * (S // 2) for g in range(MG)]

        def outs2(chunk, n=MG):
            return [(chunk * MG + g) * S for g in range(n)]

        with scope("wt1"):
            transform(w1_hook)

        x_wait(0)
        for cp in x_copies(3):
            cp.start()
        with scope("pro"):
            for piece, _ in f1(loads1(NC1 - 1), idle) + f2(CLASSES[0], idle):
                piece()

        def conv1_step(c, cc):
            for part, first in X_NEEDED:
                @pl.when(c == first)
                def _(part=part):
                    x_wait(part)
            prev = jnp.where(c == 1, NC1 - 1, c - 2)
            outs = [jnp.where(c >= 1, o, ZDUMP) for o in outs1(prev)]
            step(pacer(c), u1, MG, loads1(c), act1, True, outs)
            return cc
        with scope("steps"):
            lax.fori_loop(0, NC1 - 1, conv1_step, 0)

        row = lax.broadcasted_iota(i32, (8, 256), 0)
        for h in range(2):
            for comp in range(2):
                for t in range(last_valid, NB1 * S // 2):
                    zh_ref[8 + t, h, comp] = jnp.where(row == SEG - 1, 0.0, zh_ref[8 + t, h, comp])
                for j in range(8):
                    v = pltpu.roll(zh_ref[8 + L2 - 8 + j, h, comp], 1, axis=0)
                    zh_ref[j, h, comp] = jnp.where(row == 0, 0.0, v)
                for j in range(8):
                    v = pltpu.roll(zh_ref[8 + j, h, comp], SEG - 1, axis=0)
                    zh_ref[8 + L2 + j, h, comp] = jnp.where(row == SEG - 1, 0.0, v)

        def hand_over_1(c, cc):
            step(pacer(c), u1, MG, loads2(0), act1, True, outs1(NC1 - 3))
            return cc

        def hand_over_2(c, cc):
            step(pacer(c), u2, MG, loads2(1), act1, True, outs1(NC1 - 2))
            return cc
        with scope("steps"):
            lax.fori_loop(0, one, hand_over_1, 0)
            lax.fori_loop(0, one, hand_over_2, 0)

        def conv2_step(c, cc):
            step(pacer(c), u2, MG, loads2(c + 1), act2, False, outs2(c - 1))
            return cc
        tail = NB2 - (NC2 - 1) * MG

        def last_step(c, cc):
            step(pacer(c), u2, tail, [], act2, False, outs2(NC2 - 2))
            return cc
        with scope("steps"):
            lax.fori_loop(1, NC2 - 1, conv2_step, 0)
            lax.fori_loop(0, one, last_step, 0)
        with scope("epi"):
            for piece, _ in i1(CLASSES[3], idle, tail) + i2(act2, False, outs2(NC2 - 1, tail), idle):
                piece()

        order = [(b, e) for b in range(2) for e in range(SEG)]

        def out_copy(half, q, t0, nvalid):
            b, e = order[q]
            r0 = (b * T2 + e * L2) * 8 + t0 * 8
            return pltpu.make_async_copy(st_ref.at[half, q, pl.ds(0, nvalid * 8), :],
                                         o_hbm.at[pl.ds(r0, nvalid * 8), :],
                                         sem_o.at[half])

        def width(e):
            lim = L2 if e < SEG - 1 else last_valid
            return lim - (NCH - 1) * TB

        def joint_chunk(ch, half, full, never):
            pc = Pacer(never)
            t0 = ch * TB
            fl = pltpu.bitcast(f_ref[pl.ds(t0, TB)].reshape(TB * 8, 256), bf16)
            fe = jnp.dot(fl, wf_ref[...], preferred_element_type=f32)
            fe_ref[...] = fe
            prev = [fe[8 * r:8 * r + 8, 128 * n:128 * n + 128] for n in range(2) for r in range(2 * TB)]
            prev = prev[len(prev) // 2:]
            for q, (b, e) in enumerate(order):
                ge = ge_ref[pl.ds(8 * b, 8), :]
                r = 4 * (e & 3) + 2 * b + (e >> 2)
                js = []
                for t in range(TB):
                    row = jnp.broadcast_to(fe_ref[pl.ds(16 * t + r, 1), :], (8, 256))
                    tok = prev[(t * len(prev)) // TB]
                    gt = jnp.concatenate([pc.tie(ge[:, :128], tok), pc.tie(ge[:, 128:], tok)], axis=1)
                    js.append(jnp.tanh(row + gt))
                jl = jnp.concatenate(js, axis=0).astype(bf16)
                y = jnp.dot(jl, wo_ref[...], preferred_element_type=f32)
                prev = [y[8 * rr:8 * rr + 8, 128 * n:128 * n + 128] for n in range(2) for rr in range(TB)]
                st_ref[half, q] = y.astype(bf16)
                out_copy(half, q, t0, TB if full else width(e)).start()

        def wait_chunk(half, full):
            if full:
                pltpu.make_async_copy(st_ref.at[half], st_ref.at[half], sem_o.at[half]).wait()
                return
            for q, (b, e) in enumerate(order):
                out_copy(half, q, 0, width(e)).wait()

        def joint_body(ch, c):
            half = ch % 2

            @pl.when(ch >= 2)
            def _():
                wait_chunk(half, True)
            joint_chunk(ch, half, True, ch < 0)
            return c
        with scope("joint"):
            lax.fori_loop(0, NCH - 1, joint_body, 0)
            last_half = (NCH - 1) % 2
            wait_chunk(last_half, True)
            joint_chunk(NCH - 1, last_half, False, never)
            wait_chunk(1 - last_half, True)
            wait_chunk(last_half, False)

    scratch = [
        pltpu.VMEM((XROWS, 128), u32), pltpu.VMEM((XROWS, 128), u32),
        pltpu.VMEM((31, 128, 256), u32),
        pltpu.VMEM((32 * WP + 8, 128), u32), pltpu.VMEM((32 * WP + 8, 128), u32),
        pltpu.VMEM((2 * 96 * UP, 128), u32), pltpu.VMEM((2 * 96 * UP, 128), u32),
        pltpu.VMEM((NUNITS * MG * 4 + MG * 992 + 24, 8, 128), u32),
        pltpu.VMEM((128, M, 128), f32),
        pltpu.VMEM((ZH + S // 2, 2, 2, 8, 256), f32),
        pltpu.VMEM((FROWS + S, 8, 256), u32),
        pltpu.VMEM((TB * 16, 256), f32),
        pltpu.VMEM((16, 256), f32),
        pltpu.VMEM((2, 2 * SEG, TB * 8, 256), bf16),
        pltpu.SemaphoreType.DMA((6,)),
        pltpu.SemaphoreType.DMA((3,)),
        pltpu.SemaphoreType.DMA((2,)),
    ]
    return kernel, scratch


TAP_MATRIX = _tap_matrix()

WT_UNROLL = 2
TAP_DUE = 0
TAP_OPQ = 23
TAP_GATE = 20
LEAD = 0
AHEAD = 2
OPQ_EVERY = 1
DUE = 0


def _call(x, w1, w2, g, w_f, w_g, w_o, interpret=False):
    B, T, D = x.shape
    kernel, scratch = _make_kernel(T)
    T2 = T // 4
    any_spec = pl.BlockSpec(memory_space=pl.ANY)
    vmem = pl.BlockSpec(memory_space=pltpu.VMEM)
    out = pl.pallas_call(
        kernel,
        out_shape=jax.ShapeDtypeStruct((B * T2 * 8, D), bf16),
        in_specs=[any_spec, any_spec, any_spec, vmem, vmem, vmem, vmem, vmem],
        out_specs=any_spec,
        scratch_shapes=scratch,
        compiler_params=pltpu.CompilerParams(vmem_limit_bytes=127 * 2**20),
        interpret=interpret,
        name="conv_stem_rnnt_joint",
    )(x, w1, w2, g, w_f, w_g, w_o, TAP_MATRIX)
    return out.reshape(B, T2, 8, D)


@jax.jit
def pallas_standalone__seq2seq_rnn_t_joint__speech_kernel(x, w1, w2, g, w_f, w_g, w_o):
    return _call(x, w1, w2, g, w_f, w_g, w_o)
```
